```python
import jax
import jax.numpy as jnp

def _softmax(x, axis=-1):
    return jax.nn.softmax(x, axis=axis)

def _gelu(x):
    return jax.nn.gelu(x, approximate=True)

def _silu(x):
    return jax.nn.silu(x)

def _sigmoid(x):
    return jax.nn.sigmoid(x)

def _layernorm(x, axis=-1, eps=1e-05):
    m = jnp.mean(x, axis=axis, keepdims=True)
    v = jnp.var(x, axis=axis, keepdims=True)
    return (x - m) / jnp.sqrt(v + eps)

def _scatter_add(tgt, idx, src, axis=0):
    return tgt.at[idx].add(src)

def _segment_sum(src, seg, n):
    return jax.ops.segment_sum(src, seg, n)

class _Rng:

    def __init__(self, key):
        self._k = key

    def _next(self):
        self._k, sub = jax.random.split(self._k)
        return sub

    def normal(self, shape):
        return jax.random.normal(self._next(), shape, dtype=jnp.bfloat16)

    def randint(self, lo, hi, shape):
        return jax.random.randint(self._next(), shape, lo, hi, dtype=jnp.int32)

    def uniform(self, shape, lo=0.0, hi=1.0):
        return jax.random.uniform(self._next(), shape, jnp.bfloat16, lo, hi)

    def permutation(self, n):
        return jax.random.permutation(self._next(), n)
kernel_name = 'concat_heads__compressed_kv_cla__memory_aug_recurrent_mem_tr__prompt'

def setup_inputs():
    _rng = _Rng(jax.random.key(int.from_bytes(__import__("os").urandom(4), "little")))
    _w = lambda a: (lambda t: t.astype(jnp.bfloat16) if jnp.issubdtype(t.dtype, jnp.floating) else t)(jnp.asarray(a))

    def _A_setup():
        B, H, Sq, Sk, D, M = (1, 32, 2048, 2048, 128, 576)
        Dc = 4 * D
        return {'x': _w((lambda *s: _rng.normal(s) * 0.05)(B, Sq, M)), 'c_kv': _w((lambda *s: _rng.normal(s) * 0.05)(B, Sk, Dc)), 'w_q': _w((lambda *s: _rng.normal(s) * 0.05)(M, H, D) * M ** (-0.5)), 'w_uk': _w((lambda *s: _rng.normal(s) * 0.05)(Dc, H, D) * Dc ** (-0.5)), 'w_uv': _w((lambda *s: _rng.normal(s) * 0.05)(Dc, H, D) * Dc ** (-0.5)), 'w_o': _w((lambda *s: _rng.normal(s) * 0.05)(H, D, M) * (H * D) ** (-0.5))}
    _A_in = _A_setup()

    def _B_setup():
        B, S, Dm = (1, 2048, 576)
        H, Dh = (32, 128)
        M, seg = (8, 32)
        seg = min(seg, S)
        S = S // seg * seg
        return {'x': _w((lambda *s: _rng.normal(s) * 0.05)(B, S, Dm)), 'mem0': _w((lambda *s: _rng.normal(s) * 0.05)(B, M, Dm)), 'Wq': _w((lambda *s: _rng.normal(s) * 0.05)(Dm, H, Dh) * Dm ** (-0.5)), 'Wk': _w((lambda *s: _rng.normal(s) * 0.05)(Dm, H, Dh) * Dm ** (-0.5)), 'Wv': _w((lambda *s: _rng.normal(s) * 0.05)(Dm, H, Dh) * Dm ** (-0.5)), 'Wo': _w((lambda *s: _rng.normal(s) * 0.05)(H, Dh, Dm) * (H * Dh) ** (-0.5)), 'seg_len': seg}
    _B_in = _B_setup()
    return {'A_x': _A_in['x'], 'A_c_kv': _A_in['c_kv'], 'A_w_q': _A_in['w_q'], 'A_w_uk': _A_in['w_uk'], 'A_w_uv': _A_in['w_uv'], 'A_w_o': _A_in['w_o'], 'B_x': _B_in['x'], 'B_mem0': _B_in['mem0'], 'B_Wq': _B_in['Wq'], 'B_Wk': _B_in['Wk'], 'B_Wv': _B_in['Wv'], 'B_Wo': _B_in['Wo'], 'B_seg_len': _B_in['seg_len']}

def reference(A_x, A_c_kv, A_w_q, A_w_uk, A_w_uv, A_w_o, B_x, B_mem0, B_Wq, B_Wk, B_Wv, B_Wo, B_seg_len):

    def _A_ref(x, c_kv, w_q, w_uk, w_uv, w_o):
        B, Sq, M = (x.shape[0], x.shape[1], x.shape[2])
        Sk = c_kv.shape[1]
        H, D = (w_q.shape[1], w_q.shape[2])
        q = jnp.einsum('bqm,mhd->bhqd', x, w_q)
        k = jnp.einsum('bkc,chd->bhkd', c_kv, w_uk)
        v = jnp.einsum('bkc,chd->bhkd', c_kv, w_uv)
        scores = jnp.einsum('bhqd,bhkd->bhqk', q, k) * D ** (-0.5)
        off = Sk - Sq
        qi = jnp.arange(Sq)[:, None]
        kj = jnp.arange(Sk)[None, :]
        cmask = kj <= qi + off
        scores = jnp.where(cmask[None, None], scores, -1000000000.0)
        p = _softmax(scores, axis=-1)
        ctx = jnp.einsum('bhqk,bhkd->bhqd', p, v)
        return jnp.einsum('bhqd,hdm->bqm', ctx, w_o)

    def _B_ref(x, mem0, Wq, Wk, Wv, Wo, seg_len):
        B, S, Dm = x.shape
        H, Dh = (Wq.shape[1], Wq.shape[2])
        M = mem0.shape[1]
        scale = Dh ** (-0.5)
        n_seg = S // seg_len
        L = M + seg_len
        idx = jnp.arange(L)
        mask = (idx[:, None] < M) | (idx[:, None] >= idx[None, :])
        mem = mem0
        outs = []
        for s in range(n_seg):
            xs = x[:, s * seg_len:(s + 1) * seg_len, :].copy()
            h = jnp.concatenate([mem, xs], axis=1)
            q = jnp.einsum('btd,dhe->bhte', h, Wq)
            k = jnp.einsum('btd,dhe->bhte', h, Wk)
            v = jnp.einsum('btd,dhe->bhte', h, Wv)
            scores = jnp.einsum('bhqe,bhke->bhqk', q, k) * scale
            scores = jnp.where(mask[None, None], scores, -1000000000.0)
            p = _softmax(scores, axis=-1)
            o = jnp.einsum('bhqk,bhke->bhqe', p, v)
            o = jnp.einsum('bhte,hed->btd', o, Wo)
            mem = o[:, :M, :].copy()
            outs.append(o[:, M:, :])
        return jnp.concatenate(outs, axis=1)
    a = _A_ref(A_x, A_c_kv, A_w_q, A_w_uk, A_w_uv, A_w_o)
    b = _B_ref(B_x, B_mem0, B_Wq, B_Wk, B_Wv, B_Wo, B_seg_len)
    return jnp.concatenate([a, b], axis=-1)
```

```python
import jax
import jax.numpy as jnp
import jax.experimental.pallas as pl
import jax.experimental.pallas.tpu as pltpu

S = 2048
DM = 576
DC = 512
H = 32
D = 128
MEM = 8
SEG = 32
L = MEM + SEG
NSEG = S // SEG
HP = H // 2

LOG2E = 1.4426950408889634
QSCALE = D ** -0.5 * LOG2E
NEG = -1.0e9 * LOG2E

TQ = 128
RB = 512
HG = 4
G = H // HG
GW = HG * 3 * D
PRE = 512
T = 24
OUTER = 8

bf16 = jnp.bfloat16
f32 = jnp.float32
u32 = jnp.uint32
NT = (((1,), (1,)), ((), ()))

SEM_CKV = 0
SEM_XAT = 1
SEM_XBT = 2
SEM_MEM = 3
SEM_WOA = 4
SEM_WOB = 5
SEM_OUT = 6
SEM_W = 16
NSEM = SEM_W + 6 * 32


def _unpack(w32):
    return pltpu.bitcast(w32, bf16)


def _pack(x):
    return pltpu.bitcast(x, u32)


def _recip(l):
    r = pl.reciprocal(l, approx=True)
    return r * (2.0 - l * r)


def _eye():
    r = jax.lax.broadcasted_iota(jnp.int32, (D, D), 0)
    c = jax.lax.broadcasted_iota(jnp.int32, (D, D), 1)
    return jnp.where(r == c, 1.0, 0.0).astype(bf16)


def _kernel(xat_hbm, ckv_hbm, wqa_hbm, wuk_hbm, wuv_hbm, woa_hbm,
            xbt_hbm, mem0_hbm, wqb_hbm, wkb_hbm, wvb_hbm, wob_hbm,
            out_hbm,
            out_v, xb_v, wb_v, wob_v, lhs1_v, sem):

    def w_copy(w_hbm, dst, widx, par, hp):
        return pltpu.make_async_copy(w_hbm.bitcast(u32).at[:, par * HP + hp, :], dst.at[par, hp],
                                     sem.at[SEM_W + widx * 32 + par * HP + hp])

    def w_start(w_hbm, dst, widx):
        for hp in range(HP):
            for par in range(2):
                w_copy(w_hbm, dst, widx, par, hp).start()

    def w_combine(w_hbm, dst, widx, hp):
        w_copy(w_hbm, dst, widx, 0, hp).wait()
        w_copy(w_hbm, dst, widx, 1, hp).wait()
        a = dst[0, hp]
        b = dst[1, hp]
        ev = (a & u32(0xFFFF)) | (b << 16)
        od = (a >> 16) | (b & u32(0xFFFF0000))
        return ev, od

    def transpose_rows(src_t, dst, ncols):
        eye = _eye()
        for t in range(S // D):
            blk = src_t[:, t * D:(t + 1) * D]
            dst[t * D:(t + 1) * D, :] = jax.lax.dot_general(
                eye, blk, NT, preferred_element_type=f32).astype(bf16)

    def phase_a(ckv_v, xat_v, xa_v, wuk_v, wuv_v, wqa_v, woa_v, xbt_v, wobt_v, q_v, k_v, v_v):
        ckv_cp = pltpu.make_async_copy(ckv_hbm, ckv_v, sem.at[SEM_CKV])
        xat_cp = pltpu.make_async_copy(xat_hbm, xat_v, sem.at[SEM_XAT])
        woa_cp = pltpu.make_async_copy(woa_hbm.bitcast(u32), woa_v, sem.at[SEM_WOA])
        xbt_cp = pltpu.make_async_copy(xbt_hbm, xbt_v, sem.at[SEM_XBT])
        mem_cp = pltpu.make_async_copy(mem0_hbm, lhs1_v.at[0:MEM, :], sem.at[SEM_MEM])
        wob_cp = pltpu.make_async_copy(wob_hbm.bitcast(u32), wobt_v, sem.at[SEM_WOB])

        ckv_cp.start()
        w_start(wuk_hbm, wuk_v, 0)
        w_start(wuv_hbm, wuv_v, 1)
        xat_cp.start()
        w_start(wqa_hbm, wqa_v, 2)
        woa_cp.start()
        ckv_cp.wait()

        def project(lhs_v, w_hbm, w_v, widx, dst_v, scale):
            def body(hp, c):
                ev, od = w_combine(w_hbm, w_v, widx, hp)
                w = _unpack(jnp.concatenate([ev, od], axis=1))
                for rb in range(S // RB):
                    r = jnp.dot(lhs_v[rb * RB:(rb + 1) * RB, :], w, preferred_element_type=f32)
                    if scale is not None:
                        r = r * scale
                    r = r.astype(bf16)
                    rows = slice(rb * RB // 2, (rb + 1) * RB // 2)
                    dst_v[2 * hp, rows, :] = _pack(r[:, 0:D])
                    dst_v[2 * hp + 1, rows, :] = _pack(r[:, D:2 * D])
                return c
            jax.lax.fori_loop(0, HP, body, 0)

        project(ckv_v, wuk_hbm, wuk_v, 0, k_v, None)

        xbt_cp.start()
        mem_cp.start()
        wob_cp.start()
        w_start(wqb_hbm, wb_v.at[0], 3)
        w_start(wkb_hbm, wb_v.at[1], 4)
        w_start(wvb_hbm, wb_v.at[2], 5)

        project(ckv_v, wuv_hbm, wuv_v, 1, v_v, None)
        xat_cp.wait()
        transpose_rows(xat_v, xa_v, DM)
        project(xa_v, wqa_hbm, wqa_v, 2, q_v, QSCALE)

        row = jax.lax.broadcasted_iota(jnp.int32, (TQ, TQ), 0)
        col = jax.lax.broadcasted_iota(jnp.int32, (TQ, TQ), 1)
        tri = col <= row
        nb = S // TQ
        hq = TQ // 2

        def head(h, c):
            def qk(i):
                q = _unpack(q_v[h, i * hq:(i + 1) * hq, :])
                k = _unpack(k_v[h, 0:(i + 1) * hq, :])
                return jax.lax.dot_general(q, k, NT, preferred_element_type=f32)

            s_next = qk(nb - 1)
            for i in range(nb - 1, -1, -1):
                s = s_next
                if i > 0:
                    s_next = qk(i - 1)
                sd = jnp.where(tri, s[:, i * TQ:], NEG)
                s = jnp.concatenate([s[:, :i * TQ], sd], axis=1) if i > 0 else sd
                m = jnp.max(s, axis=1, keepdims=True)
                p = jnp.exp2(s - m)
                l = jnp.sum(p, axis=1, keepdims=True)
                v = _unpack(v_v[h, 0:(i + 1) * hq, :])
                o = jnp.dot(p.astype(bf16), v, preferred_element_type=f32)
                q_v[h, i * hq:(i + 1) * hq, :] = _pack((o * _recip(l)).astype(bf16))
            return c
        jax.lax.fori_loop(0, H, head, 0)

        woa_cp.wait()

        def oproj(rb, c):
            r0 = pl.multiple_of(rb * (RB // 2), RB // 2)
            ctx = _unpack(jnp.concatenate([q_v[h, pl.ds(r0, RB // 2), :] for h in range(H)], axis=1))
            wo = _unpack(jnp.concatenate([woa_v[h] for h in range(H)], axis=1))
            r = jax.lax.dot_general(ctx, wo, NT, preferred_element_type=f32)
            out_v[pl.ds(pl.multiple_of(T + rb * RB, 8), RB), 0:DM] = r.astype(bf16)
            return c
        jax.lax.fori_loop(0, S // RB, oproj, 0)

        xbt_cp.wait()
        transpose_rows(xbt_v, xb_v, DM)
        wob_cp.wait()
        eye = _eye()

        def wob_body(h, c):
            r = jax.lax.dot_general(eye, _unpack(wobt_v[h]), NT, preferred_element_type=f32)
            wob_v[pl.ds(pl.multiple_of(h * (D // 2), D // 2), D // 2), :] = _pack(r.astype(bf16))
            return c
        jax.lax.fori_loop(0, H, wob_body, 0)

        for t, w_hbm in enumerate((wqb_hbm, wkb_hbm, wvb_hbm)):
            def comb(hp, c, t=t, w_hbm=w_hbm):
                ev, od = w_combine(w_hbm, wb_v.at[t], 3 + t, hp)
                wb_v[t, 0, hp] = ev
                wb_v[t, 1, hp] = od
                return c
            jax.lax.fori_loop(0, HP, comb, 0)
        mem_cp.wait()

    pl.run_scoped(
        phase_a,
        pltpu.VMEM((S, DC), bf16),
        pltpu.VMEM((DM, S), bf16),
        pltpu.VMEM((S, DM), bf16),
        pltpu.VMEM((2, HP, DC // 2, D), u32),
        pltpu.VMEM((2, HP, DC // 2, D), u32),
        pltpu.VMEM((2, HP, DM // 2, D), u32),
        pltpu.VMEM((H, DM // 2, D), u32),
        pltpu.VMEM((DM, S), bf16),
        pltpu.VMEM((H, DM // 2, D), u32),
        pltpu.VMEM((H, S // 2, D), u32),
        pltpu.VMEM((H, S // 2, D), u32),
        pltpu.VMEM((H, S // 2, D), u32),
    )

    def out_copy(j, start, size):
        return pltpu.make_async_copy(out_v.at[pl.ds(T + start, size), :],
                                     out_hbm.at[pl.ds(start, size), :], sem.at[SEM_OUT + j])

    def phase_b(qkv_v, o_v, lhs2_v):
        lane = jax.lax.broadcasted_iota(jnp.int32, (1, GW), 1)
        colscale = jnp.where(lane % (3 * D) < D, QSCALE, 1.0).astype(f32)

        def wgroup(g):
            return _unpack(jnp.concatenate(
                [wb_v[t, h % 2, h // 2] for h in range(g * HG, (g + 1) * HG) for t in range(3)], axis=1))

        for g in range(G):
            r = (jnp.dot(xb_v[0:PRE, :], wgroup(g), preferred_element_type=f32) * colscale).astype(bf16)
            for sg in range(PRE // SEG):
                qkv_v[g, sg * L + MEM:(sg + 1) * L, :] = r[sg * SEG:(sg + 1) * SEG, :]

        o_v[0:T, :] = jnp.zeros((T, H * D), bf16)
        row = jax.lax.broadcasted_iota(jnp.int32, (L, L), 0)
        col = jax.lax.broadcasted_iota(jnp.int32, (L, L), 1)
        mask = (row < MEM) | (col <= row)

        def step(s):
            lhs1_v[MEM:MEM + T, :] = xb_v[pl.ds(pl.multiple_of(PRE + T * s, 8), T), :]
            lhs2_v[MEM:MEM + T, :] = o_v[pl.ds(pl.multiple_of(T * s, 8), T), :]
            l1 = lhs1_v[...]
            r0 = pl.multiple_of(L * s, 8)
            rows = []
            for j in range(T // 8):
                cidx = PRE // 8 + (T // 8) * s + j
                rows.append(pl.multiple_of(L * (cidx // 4) + MEM + 8 * (cidx % 4), 8))
            for g in range(G):
                r = (jnp.dot(l1, wgroup(g), preferred_element_type=f32) * colscale).astype(bf16)
                qkv_v[g, pl.ds(r0, MEM), :] = r[0:MEM, :]
                for j in range(T // 8):
                    qkv_v[g, pl.ds(rows[j], 8), :] = r[MEM + 8 * j:MEM + 8 * (j + 1), :]
            scores = []
            for h in range(H):
                g, c0 = h // HG, (h % HG) * 3 * D
                q = qkv_v[g, pl.ds(r0, L), c0:c0 + D]
                k = qkv_v[g, pl.ds(r0, L), c0 + D:c0 + 2 * D]
                scores.append(jax.lax.dot_general(q, k, NT, preferred_element_type=f32))
            for h in range(H):
                g, c0 = h // HG, (h % HG) * 3 * D
                v = qkv_v[g, pl.ds(r0, L), c0 + 2 * D:c0 + 3 * D]
                sc = jnp.where(mask, scores[h], NEG)
                m = jnp.max(sc, axis=1, keepdims=True)
                p = jnp.exp2(sc - m)
                l = jnp.sum(p, axis=1, keepdims=True)
                o = jnp.dot(p.astype(bf16), v, preferred_element_type=f32)
                o = (o * _recip(l)).astype(bf16)
                lhs2_v[0:MEM, h * D:(h + 1) * D] = o[0:MEM, :]
                o_v[pl.ds(pl.multiple_of(T + SEG * s, 8), SEG), h * D:(h + 1) * D] = o[MEM:, :]
            acc = None
            for g in range(G):
                pr = jnp.dot(lhs2_v[:, g * HG * D:(g + 1) * HG * D],
                             _unpack(wob_v[g * HG * D // 2:(g + 1) * HG * D // 2, :]),
                             preferred_element_type=f32)
                acc = pr if acc is None else acc + pr
            accb = acc.astype(bf16)
            lhs1_v[0:MEM, :] = accb[0:MEM, :]
            out_v[pl.ds(pl.multiple_of(T * s, 8), T), DM:2 * DM] = accb[MEM:, :]

        chunk = OUTER * T

        def outer(j, c):
            def inner(i, c2):
                step(j * OUTER + i)
                return c2
            jax.lax.fori_loop(0, OUTER, inner, 0)
            @pl.when(j > 0)
            def _():
                out_copy(j, pl.multiple_of((j - 1) * chunk, 16), chunk).start()
            return c
        nouter = NSEG // OUTER
        jax.lax.fori_loop(0, nouter, outer, 0)

        done = T * (NSEG - 1)
        w0 = (nouter - 1) * chunk
        out_copy(0, w0, done - w0).start()
        r = jnp.dot(o_v[T + done:T + S, :], _unpack(wob_v[...]), preferred_element_type=f32)
        out_v[T + done:T + S, DM:2 * DM] = r.astype(bf16)
        out_copy(nouter, done, S - done).start()
        for j in range(1, nouter):
            out_copy(j, (j - 1) * chunk, chunk).wait()
        out_copy(0, w0, done - w0).wait()
        out_copy(nouter, done, S - done).wait()

    pl.run_scoped(
        phase_b,
        pltpu.VMEM((G, NSEG * L, GW), bf16),
        pltpu.VMEM((T + S, H * D), bf16),
        pltpu.VMEM((MEM + T, H * D), bf16),
    )


@jax.jit
def pallas_concat_heads__compressed_kv_cla__memory_aug_recurrent_mem_tr__prompt_kernel(
    A_x: jax.Array,
    A_c_kv: jax.Array,
    A_w_q: jax.Array,
    A_w_uk: jax.Array,
    A_w_uv: jax.Array,
    A_w_o: jax.Array,
    B_x: jax.Array,
    B_mem0: jax.Array,
    B_Wq: jax.Array,
    B_Wk: jax.Array,
    B_Wv: jax.Array,
    B_Wo: jax.Array,
    B_seg_len=SEG,
):
    def t2(x):
        return jnp.transpose(x, (0, 2, 1)).reshape(DM, S)

    def w3(w):
        return w.reshape(w.shape[0] // 2, 2 * H, D)

    def wo3(w):
        return jnp.transpose(w, (0, 2, 1))

    any_spec = pl.BlockSpec(memory_space=pl.ANY)
    out = pl.pallas_call(
        _kernel,
        out_shape=jax.ShapeDtypeStruct((S, 2 * DM), bf16),
        in_specs=[any_spec] * 12,
        out_specs=any_spec,
        scratch_shapes=[
            pltpu.VMEM((T + S, 2 * DM), bf16),
            pltpu.VMEM((S, DM), bf16),
            pltpu.VMEM((3, 2, HP, DM // 2, D), u32),
            pltpu.VMEM((H * D // 2, DM), u32),
            pltpu.VMEM((MEM + T, DM), bf16),
            pltpu.SemaphoreType.DMA((NSEM,)),
        ],
        compiler_params=pltpu.CompilerParams(vmem_limit_bytes=126 * 1024 * 1024),
    )(t2(A_x), A_c_kv.reshape(S, DC), w3(A_w_q), w3(A_w_uk), w3(A_w_uv), wo3(A_w_o),
      t2(B_x), B_mem0.reshape(MEM, DM), w3(B_Wq), w3(B_Wk), w3(B_Wv), wo3(B_Wo))
    return out.reshape(1, S, 2 * DM)
```

```python
import contextlib

import jax
import jax.numpy as jnp
import jax.experimental.pallas as pl
import jax.experimental.pallas.tpu as pltpu

S = 2048
DM = 576
DC = 512
H = 32
D = 128
MEM = 8
SEG = 32
L = MEM + SEG
NSEG = S // SEG
HP = H // 2

LOG2E = 1.4426950408889634
QSCALE = D ** -0.5 * LOG2E
NEG = -1.0e9 * LOG2E

TQ = 128
RB = 512
HG = 4
G = H // HG
GW = HG * 3 * D
PRE = 8
T = SEG - PRE
OUTER = 8
NOUTER = NSEG // OUTER

bf16 = jnp.bfloat16
f32 = jnp.float32
u32 = jnp.uint32
NT = (((1,), (1,)), ((), ()))

SEM_CKV = 0
SEM_XAT = 4
SEM_XBT = 5
SEM_MEM = 6
SEM_WOA = 7
SEM_WOB = 8
SEM_OUT = 9
SEM_W = SEM_OUT + NOUTER
NSEM = SEM_W + 6 * 32

_PROFILE = False


def _scope(name):
    return jax.named_scope(name) if _PROFILE else contextlib.nullcontext()


def _unpack(w32):
    return pltpu.bitcast(w32, bf16)


def _pack(x):
    return pltpu.bitcast(x, u32)


def _recip(l):
    r = pl.reciprocal(l, approx=True)
    return r * (2.0 - l * r)


def _kernel(xat_hbm, ckv_hbm, wqa_hbm, wuk_hbm, wuv_hbm, woa_hbm,
            xbt_hbm, mem0_hbm, wqb_hbm, wkb_hbm, wvb_hbm, wob_hbm,
            out_hbm,
            out_v, xb_v, xpre_v, wb_v, wob_v, mem_v, sem):

    def w_copy(w_hbm, dst, widx, par, hp):
        return pltpu.make_async_copy(w_hbm.bitcast(u32).at[:, par * HP + hp, :], dst.at[par, hp],
                                     sem.at[SEM_W + widx * 32 + par * HP + hp])

    def w_start(w_hbm, dst, widx, hp):
        for par in range(2):
            w_copy(w_hbm, dst, widx, par, hp).start()

    def w_combine(w_hbm, dst, widx, hp):
        w_copy(w_hbm, dst, widx, 0, hp).wait()
        w_copy(w_hbm, dst, widx, 1, hp).wait()
        a = dst[0, hp]
        b = dst[1, hp]
        ev = (a & u32(0xFFFF)) | (b << 16)
        od = (a >> 16) | (b & u32(0xFFFF0000))
        return ev, od

    wb_hbm = (wqb_hbm, wkb_hbm, wvb_hbm)

    def phase_a(woa_v, xbt_v, wobt_v, q_v, k_v, v_v):
        woa_cp = pltpu.make_async_copy(woa_hbm.bitcast(u32), woa_v, sem.at[SEM_WOA])
        xbt_cp = pltpu.make_async_copy(xbt_hbm, xbt_v, sem.at[SEM_XBT])
        mem_cp = pltpu.make_async_copy(mem0_hbm, mem_v, sem.at[SEM_MEM])
        wob_cp = pltpu.make_async_copy(wob_hbm.bitcast(u32), wobt_v, sem.at[SEM_WOB])

        def store_heads(dst_v, hp, rb, r):
            r = r.astype(bf16)
            rows = slice(rb * RB // 2, (rb + 1) * RB // 2)
            dst_v[2 * hp, rows, :] = _pack(r[:, 0:D])
            dst_v[2 * hp + 1, rows, :] = _pack(r[:, D:2 * D])

        def projections(ckv_v, xat_v, xa_v, wuk_v, wuv_v, wqa_v):
            nck = S // RB
            ahead = 8

            def ckv_cp(j):
                return pltpu.make_async_copy(ckv_hbm.at[j * RB:(j + 1) * RB, :],
                                             ckv_v.at[j * RB:(j + 1) * RB, :], sem.at[SEM_CKV + j])
            xat_cp = pltpu.make_async_copy(xat_hbm, xat_v, sem.at[SEM_XAT])

            with _scope("a_issue0"):
                ckv_cp(0).start()
                w_start(wuk_hbm, wuk_v, 0, 0)
                for j in range(1, nck):
                    ckv_cp(j).start()
                w_start(wuv_hbm, wuv_v, 1, 0)
                for hp in range(1, ahead):
                    w_start(wuk_hbm, wuk_v, 0, hp)
                    w_start(wuv_hbm, wuv_v, 1, hp)
                xat_cp.start()

            def xa_block(t):
                t0 = pl.multiple_of(t * D, D)
                xa_v[pl.ds(t0, D), :] = xat_v[:, pl.ds(t0, D)].T

            def kv_body(hp, c, first=False):
                @pl.when(hp < HP - ahead)
                def _():
                    w_start(wuk_hbm, wuk_v, 0, hp + ahead)
                    w_start(wuv_hbm, wuv_v, 1, hp + ahead)

                @pl.when(hp == ahead)
                def _():
                    xbt_cp.start()
                    mem_cp.start()
                w_start(wqa_hbm, wqa_v, 2, hp)
                for t in range(3):
                    w_start(wb_hbm[t], wb_v.at[t], 3 + t, hp)
                wk = _unpack(jnp.concatenate(w_combine(wuk_hbm, wuk_v, 0, hp), axis=1))
                wv = _unpack(jnp.concatenate(w_combine(wuv_hbm, wuv_v, 1, hp), axis=1))
                if not first:
                    xa_block(hp - 1)
                for rb in range(nck):
                    if first:
                        ckv_cp(rb).wait()
                    lhs = ckv_v[rb * RB:(rb + 1) * RB, :]
                    store_heads(k_v, hp, rb, jnp.dot(lhs, wk, preferred_element_type=f32))
                for rb in range(nck):
                    lhs = ckv_v[rb * RB:(rb + 1) * RB, :]
                    store_heads(v_v, hp, rb, jnp.dot(lhs, wv, preferred_element_type=f32))
                return c

            with _scope("a_kvproj"):
                kv_body(0, 0, first=True)
                xat_cp.wait()
                jax.lax.fori_loop(1, HP, kv_body, 0)
                xa_block(HP - 1)

            woa_cp.start()
            wob_cp.start()
            xbt_cp.wait()

            def q_body(hp, c):
                w = _unpack(jnp.concatenate(w_combine(wqa_hbm, wqa_v, 2, hp), axis=1))
                packed = [w_combine(wb_hbm[t], wb_v.at[t], 3 + t, hp) for t in range(3)]
                for t in range(3):
                    wb_v[t, 0, hp] = packed[t][0]
                    wb_v[t, 1, hp] = packed[t][1]
                t0 = pl.multiple_of(hp * D, D)
                xb = xbt_v[:, pl.ds(t0, D)].T
                xb_v[pl.ds(t0, D), :] = xb
                for sg in range(D // SEG):
                    p0 = pl.multiple_of((hp * (D // SEG) + sg) * PRE, PRE)
                    xpre_v[pl.ds(p0, PRE), :] = xb[sg * SEG:sg * SEG + PRE, :]
                for rb in range(nck):
                    r = jnp.dot(xa_v[rb * RB:(rb + 1) * RB, :], w, preferred_element_type=f32)
                    store_heads(q_v, hp, rb, r * QSCALE)
                return c

            with _scope("a_qproj"):
                jax.lax.fori_loop(0, HP, q_body, 0)

        pl.run_scoped(
            projections,
            pltpu.VMEM((S, DC), bf16),
            pltpu.VMEM((DM, S), bf16),
            pltpu.VMEM((S, DM), bf16),
            pltpu.VMEM((2, HP, DC // 2, D), u32),
            pltpu.VMEM((2, HP, DC // 2, D), u32),
            pltpu.VMEM((2, HP, DM // 2, D), u32),
        )

        def attention(c_v, s_v):
            row = jax.lax.broadcasted_iota(jnp.int32, (TQ, TQ), 0)
            col = jax.lax.broadcasted_iota(jnp.int32, (TQ, TQ), 1)
            tri = col <= row
            nb = S // TQ
            hq = TQ // 2
            npiece = 2
            pw = S // npiece

            def qk_piece(h, j):
                q = _unpack(q_v[h, (nb - 1) * hq:nb * hq, :])
                k = _unpack(k_v[h, j * pw // 2:(j + 1) * pw // 2, :])
                s_v[:, j * pw:(j + 1) * pw] = jax.lax.dot_general(q, k, NT, preferred_element_type=f32)

            def head(h, c):
                def qk(i):
                    q = _unpack(q_v[h, i * hq:(i + 1) * hq, :])
                    k = _unpack(k_v[h, 0:(i + 1) * hq, :])
                    return jax.lax.dot_general(q, k, NT, preferred_element_type=f32)

                hn = jnp.minimum(h + 1, H - 1)
                s_next = s_v[...]
                for i in range(nb - 1, -1, -1):
                    s = s_next
                    if i > 0:
                        s_next = qk(i - 1)
                    if i < npiece:
                        qk_piece(hn, npiece - 1 - i)
                    sd = jnp.where(tri, s[:, i * TQ:], NEG)
                    s = jnp.concatenate([s[:, :i * TQ], sd], axis=1) if i > 0 else sd
                    m = jnp.max(s, axis=1, keepdims=True)
                    p = jnp.exp2(s - m)
                    l = jnp.sum(p, axis=1, keepdims=True)
                    v = _unpack(v_v[h, 0:(i + 1) * hq, :])
                    o = jnp.dot(p.astype(bf16), v, preferred_element_type=f32)
                    c_v[h, i * hq:(i + 1) * hq, :] = _pack((o * _recip(l)).astype(bf16))
                return c
            with _scope("a_attn"):
                for j in range(npiece):
                    qk_piece(0, j)
                jax.lax.fori_loop(0, H, head, 0)

            woa_cp.wait()
            wob_cp.wait()
            nrb = S // RB

            def oproj(rb, c):
                for hh in range(H // nrb):
                    h = rb * (H // nrb) + hh
                    wob_v[pl.ds(pl.multiple_of(h * (D // 2), D // 2), D // 2), :] = _pack(_unpack(wobt_v[h]).T)
                r0 = pl.multiple_of(rb * (RB // 2), RB // 2)
                ctx = _unpack(jnp.concatenate([c_v[h, pl.ds(r0, RB // 2), :] for h in range(H)], axis=1))
                wo = _unpack(jnp.concatenate([woa_v[h] for h in range(H)], axis=1))
                r = jax.lax.dot_general(ctx, wo, NT, preferred_element_type=f32)
                out_v[pl.ds(pl.multiple_of(rb * RB, RB), RB), 0:DM] = r.astype(bf16)
                return c
            with _scope("a_oproj"):
                jax.lax.fori_loop(0, nrb, oproj, 0)

        pl.run_scoped(
            attention,
            pltpu.VMEM((H, S // 2, D), u32),
            pltpu.VMEM((TQ, S), f32),
        )
        mem_cp.wait()

    pl.run_scoped(
        phase_a,
        pltpu.VMEM((H, DM // 2, D), u32),
        pltpu.VMEM((DM, S), bf16),
        pltpu.VMEM((H, DM // 2, D), u32),
        pltpu.VMEM((H, S // 2, D), u32),
        pltpu.VMEM((H, S // 2, D), u32),
        pltpu.VMEM((H, S // 2, D), u32),
    )

    def out_copy(j):
        rows = pl.ds(pl.multiple_of(j * (OUTER * SEG), OUTER * SEG), OUTER * SEG)
        return pltpu.make_async_copy(out_v.at[rows, :], out_hbm.at[rows, :], sem.at[SEM_OUT + j])

    def phase_b(pre_v, post_v):
        lane = jax.lax.broadcasted_iota(jnp.int32, (1, GW), 1)
        colscale = jnp.where(lane % (3 * D) < D, QSCALE, 1.0).astype(f32)

        def wgroup(g):
            return _unpack(jnp.concatenate(
                [wb_v[t, h % 2, h // 2] for h in range(g * HG, (g + 1) * HG) for t in range(3)], axis=1))

        def wogroup(g):
            return _unpack(wob_v[g * HG * D // 2:(g + 1) * HG * D // 2, :])

        with _scope("b_pre"):
            for g in range(G):
                pre_v[g] = (jnp.dot(xpre_v[...], wgroup(g), preferred_element_type=f32) * colscale).astype(bf16)

        ri = jax.lax.broadcasted_iota(jnp.int32, (L, L), 0)
        ci = jax.lax.broadcasted_iota(jnp.int32, (L, L), 1)

        def pos(i):
            return jnp.where(i < T, i + (MEM + PRE), i - T)
        mask = (pos(ri) < MEM) | (pos(ri) >= pos(ci))

        def step(s, mem):
            xt = xb_v[pl.ds(pl.multiple_of(SEG * s + PRE, 8), T), :]
            l1 = jnp.concatenate([xt.astype(f32), mem], axis=0).astype(bf16)
            p0 = pl.multiple_of(PRE * s, 8)
            proj = [(jnp.dot(l1, wgroup(g), preferred_element_type=f32) * colscale).astype(bf16)
                    for g in range(G)]

            def rows(h, t):
                g, c0 = h // HG, (h % HG) * 3 * D + t * D
                return jnp.concatenate([proj[g][:, c0:c0 + D], pre_v[g, pl.ds(p0, PRE), c0:c0 + D]], axis=0)

            scores = [jax.lax.dot_general(rows(h, 0), rows(h, 1), NT, preferred_element_type=f32)
                      for h in range(H)]
            ctx = {}

            def attend(g):
                for h in range(g * HG, (g + 1) * HG):
                    sc = jnp.where(mask, scores[h], NEG)
                    m = jnp.max(sc, axis=1, keepdims=True)
                    p = jnp.exp2(sc - m)
                    l = jnp.sum(p, axis=1, keepdims=True)
                    o = jnp.dot(p.astype(bf16), rows(h, 2), preferred_element_type=f32)
                    o = (o * _recip(l)).astype(bf16)
                    ctx[h] = o[0:T + MEM, :]
                    post_v[pl.ds(pl.multiple_of((PRE * s) % (PRE * OUTER), 8), PRE), h * D:(h + 1) * D] = o[T + MEM:, :]

            parts = []

            def oproj(g):
                lhs = jnp.concatenate([ctx[h] for h in range(g * HG, (g + 1) * HG)], axis=1)
                parts.append(jnp.dot(lhs, wogroup(g), preferred_element_type=f32))

            for t in range(G + 2):
                if t < G:
                    attend(t)
                if t >= 2:
                    oproj(t - 2)
            acc = parts[0]
            for a in parts[1:]:
                acc = acc + a
            accb = acc.astype(bf16)
            out_v[pl.ds(pl.multiple_of(SEG * s + PRE, 8), T), DM:2 * DM] = accb[0:T, :]
            return accb[T:, :].astype(f32)

        def outer(j, mem):
            mem = jax.lax.fori_loop(0, OUTER, lambda i, m: step(j * OUTER + i, m), mem, unroll=2)
            r = jnp.dot(post_v[...], _unpack(wob_v[...]), preferred_element_type=f32).astype(bf16)
            for sg in range(OUTER):
                r0 = pl.multiple_of((j * OUTER + sg) * SEG, SEG)
                out_v[pl.ds(r0, PRE), DM:2 * DM] = r[sg * PRE:(sg + 1) * PRE, :]
            out_copy(j).start()
            return mem
        with _scope("b_loop"):
            jax.lax.fori_loop(0, NOUTER, outer, mem_v[...].astype(f32))
        with _scope("b_outwait"):
            for j in range(NOUTER):
                out_copy(j).wait()

    pl.run_scoped(
        phase_b,
        pltpu.VMEM((G, NSEG * PRE, GW), bf16),
        pltpu.VMEM((OUTER * PRE, H * D), bf16),
    )


@jax.jit
def pallas_concat_heads__compressed_kv_cla__memory_aug_recurrent_mem_tr__prompt_kernel(
    A_x: jax.Array,
    A_c_kv: jax.Array,
    A_w_q: jax.Array,
    A_w_uk: jax.Array,
    A_w_uv: jax.Array,
    A_w_o: jax.Array,
    B_x: jax.Array,
    B_mem0: jax.Array,
    B_Wq: jax.Array,
    B_Wk: jax.Array,
    B_Wv: jax.Array,
    B_Wo: jax.Array,
    B_seg_len=SEG,
):
    def t2(x):
        return jnp.transpose(x, (0, 2, 1)).reshape(DM, S)

    def w3(w):
        return w.reshape(w.shape[0] // 2, 2 * H, D)

    def wo3(w):
        return jnp.transpose(w, (0, 2, 1))

    any_spec = pl.BlockSpec(memory_space=pl.ANY)
    out = pl.pallas_call(
        _kernel,
        out_shape=jax.ShapeDtypeStruct((S, 2 * DM), bf16),
        in_specs=[any_spec] * 12,
        out_specs=any_spec,
        scratch_shapes=[
            pltpu.VMEM((S, 2 * DM), bf16),
            pltpu.VMEM((S, DM), bf16),
            pltpu.VMEM((NSEG * PRE, DM), bf16),
            pltpu.VMEM((3, 2, HP, DM // 2, D), u32),
            pltpu.VMEM((H * D // 2, DM), u32),
            pltpu.VMEM((MEM, DM), bf16),
            pltpu.SemaphoreType.DMA((NSEM,)),
        ],
        compiler_params=pltpu.CompilerParams(vmem_limit_bytes=126 * 1024 * 1024),
    )(t2(A_x), A_c_kv.reshape(S, DC), w3(A_w_q), w3(A_w_uk), w3(A_w_uv), wo3(A_w_o),
      t2(B_x), B_mem0.reshape(MEM, DM), w3(B_Wq), w3(B_Wk), w3(B_Wv), wo3(B_Wo))
    return out.reshape(1, S, 2 * DM)
```

```python
import contextlib

import jax
import jax.numpy as jnp
import jax.experimental.pallas as pl
import jax.experimental.pallas.tpu as pltpu

S = 2048
DM = 576
DC = 512
H = 32
D = 128
MEM = 8
SEG = 32
L = MEM + SEG
NSEG = S // SEG
HP = H // 2

LOG2E = 1.4426950408889634
QSCALE = D ** -0.5 * LOG2E
NEG = -1.0e9 * LOG2E

TQ = 128
RB = 512
HG = 4
G = H // HG
GW = HG * 3 * D
PRE = 8
T = SEG - PRE
OUTER = 8
NOUTER = NSEG // OUTER

bf16 = jnp.bfloat16
f32 = jnp.float32
u32 = jnp.uint32
NT = (((1,), (1,)), ((), ()))

SEM_CKV = 0
SEM_XAT = 4
SEM_XBT = 5
SEM_MEM = 6
SEM_WOA = 7
SEM_WOB = 8
SEM_OUT = 9
SEM_WALL = SEM_OUT + NOUTER
SEM_W = SEM_WALL + 4
NSEM = SEM_W + 2 * 32

_PROFILE = False


def _scope(name):
    return jax.named_scope(name) if _PROFILE else contextlib.nullcontext()


def _unpack(w32):
    return pltpu.bitcast(w32, bf16)


def _pack(x):
    return pltpu.bitcast(x, u32)


def _recip(l):
    r = pl.reciprocal(l, approx=True)
    return r * (2.0 - l * r)


def _kernel(xat_hbm, ckv_hbm, wqa_hbm, wuk_hbm, wuv_hbm, woa_hbm,
            xbt_hbm, mem0_hbm, wqb_hbm, wkb_hbm, wvb_hbm, wob_hbm,
            out_hbm,
            out_v, xb_v, xpre_v, wb_v, wob_v, mem_v, sem):

    def w_copy(w_hbm, dst, slot, par, hp):
        return pltpu.make_async_copy(w_hbm.bitcast(u32).at[:, par * HP + hp, :], dst.at[par, hp], sem.at[slot])

    def w_start(w_hbm, dst, widx, hp):
        for par in range(2):
            w_copy(w_hbm, dst, SEM_W + widx * 32 + par * HP + hp, par, hp).start()

    def w_wait(w_hbm, dst, widx, hp):
        for par in range(2):
            w_copy(w_hbm, dst, SEM_W + widx * 32 + par * HP + hp, par, hp).wait()

    def w_start_shared(w_hbm, dst, widx, hps):
        for hp in hps:
            for par in range(2):
                w_copy(w_hbm, dst, SEM_WALL + widx, par, hp).start()

    def w_wait_shared(dst, widx):
        pltpu.make_async_copy(dst, dst, sem.at[SEM_WALL + widx]).wait()

    def w_combine(dst, hp):
        a = dst[0, hp]
        b = dst[1, hp]
        ev = (a & u32(0xFFFF)) | (b << 16)
        od = (a >> 16) | (b & u32(0xFFFF0000))
        return ev, od

    def w_pair(dst, hp):
        return jnp.concatenate(w_combine(dst, hp), axis=1)

    wb_hbm = (wqb_hbm, wkb_hbm, wvb_hbm)

    def phase_a(woa_v, xbt_v, wobt_v, q_v, k_v, v_v):
        woa_cp = pltpu.make_async_copy(woa_hbm.bitcast(u32), woa_v, sem.at[SEM_WOA])
        xbt_cp = pltpu.make_async_copy(xbt_hbm, xbt_v, sem.at[SEM_XBT])
        mem_cp = pltpu.make_async_copy(mem0_hbm, mem_v.at[0:MEM, :], sem.at[SEM_MEM])
        wob_cp = pltpu.make_async_copy(wob_hbm.bitcast(u32), wobt_v, sem.at[SEM_WOB])

        def store_heads(dst_v, hp, rb, r):
            r = r.astype(bf16)
            rows = slice(rb * RB // 2, (rb + 1) * RB // 2)
            dst_v[2 * hp, rows, :] = _pack(r[:, 0:D])
            dst_v[2 * hp + 1, rows, :] = _pack(r[:, D:2 * D])

        def projections(ckv_v, xat_v, xa_v, wuk_v, wuv_v, wqa_v, wk_v, wq0_v, wq1_v):
            nck = S // RB
            early = 14

            def ckv_cp(j):
                return pltpu.make_async_copy(ckv_hbm.at[j * RB:(j + 1) * RB, :],
                                             ckv_v.at[j * RB:(j + 1) * RB, :], sem.at[SEM_CKV + j])
            xat_cp = pltpu.make_async_copy(xat_hbm, xat_v, sem.at[SEM_XAT])

            with _scope("a_issue0"):
                w_start(wuk_hbm, wuk_v, 0, 0)
                ckv_cp(0).start()
                w_start(wuv_hbm, wuv_v, 1, 0)
                for j in range(1, nck):
                    ckv_cp(j).start()
                for hp in range(1, early):
                    w_start(wuk_hbm, wuk_v, 0, hp)
                    w_start(wuv_hbm, wuv_v, 1, hp)

            def project(dst_v, lhs_v, w, hp, rb, scale=None):
                r = jnp.dot(lhs_v[rb * RB:(rb + 1) * RB, :], _unpack(w), preferred_element_type=f32)
                store_heads(dst_v, hp, rb, r if scale is None else r * scale)

            def kv_first():
                w_wait(wuk_hbm, wuk_v, 0, 0)
                ckv_cp(0).wait()
                wk = w_pair(wuk_v, 0)
                project(k_v, ckv_v, wk, 0, 0)
                w_wait(wuv_hbm, wuv_v, 1, 0)
                wv = w_pair(wuv_v, 0)
                project(v_v, ckv_v, wv, 0, 0)
                for rb in range(1, nck):
                    ckv_cp(rb).wait()
                    project(k_v, ckv_v, wk, 0, rb)
                    project(v_v, ckv_v, wv, 0, rb)
                w_wait(wuk_hbm, wuk_v, 0, 1)
                wk_v[...] = w_pair(wuk_v, 1)

            def kv_body(hp, c, last=False):
                if not last:
                    @pl.when(hp == 4)
                    def _():
                        xat_cp.start()
                        for j in range(early, HP):
                            w_start(wuk_hbm, wuk_v, 0, j)
                            w_start(wuv_hbm, wuv_v, 1, j)
                        w_start_shared(wqa_hbm, wqa_v, 0, range(HP))
                w_wait(wuv_hbm, wuv_v, 1, hp)
                if last:
                    xat_cp.wait()
                    w_wait_shared(wqa_v, 0)
                else:
                    w_wait(wuk_hbm, wuk_v, 0, hp + 1)
                wv = w_pair(wuv_v, hp)
                for rb in range(nck):
                    project(k_v, ckv_v, wk_v[...], hp, rb)
                if last:
                    wq0_v[...] = w_pair(wqa_v, 0)
                    for t in range(S // D):
                        xa_v[t * D:(t + 1) * D, :] = xat_v[:, t * D:(t + 1) * D].T
                else:
                    wk_v[...] = w_pair(wuk_v, hp + 1)
                for rb in range(nck):
                    project(v_v, ckv_v, wv, hp, rb)
                return c

            with _scope("a_kvproj"):
                kv_first()
                jax.lax.fori_loop(1, HP - 1, kv_body, 0)
                kv_body(HP - 1, 0, last=True)

            woa_cp.start()
            wob_cp.start()
            xbt_cp.start()
            mem_cp.start()
            w_start_shared(wqb_hbm, wb_v.at[0], 1, range(HP))
            w_start_shared(wkb_hbm, wb_v.at[1], 2, range(HP // 2))

            def q_body(j, c):
                wq1_v[...] = w_pair(wqa_v, 2 * j + 1)
                for rb in range(nck):
                    project(q_v, xa_v, wq0_v[...], 2 * j, rb, QSCALE)
                wq0_v[...] = w_pair(wqa_v, jnp.minimum(2 * j + 2, HP - 1))
                for rb in range(nck):
                    project(q_v, xa_v, wq1_v[...], 2 * j + 1, rb, QSCALE)
                return c

            with _scope("a_qproj"):
                jax.lax.fori_loop(0, HP // 2, q_body, 0)

            w_start_shared(wkb_hbm, wb_v.at[1], 2, range(HP // 2, HP))
            w_start_shared(wvb_hbm, wb_v.at[2], 3, range(HP))

        pl.run_scoped(
            projections,
            pltpu.VMEM((S, DC), bf16),
            pltpu.VMEM((DM, S), bf16),
            pltpu.VMEM((S, DM), bf16),
            pltpu.VMEM((2, HP, DC // 2, D), u32),
            pltpu.VMEM((2, HP, DC // 2, D), u32),
            pltpu.VMEM((2, HP, DM // 2, D), u32),
            pltpu.VMEM((DC // 2, 2 * D), u32),
            pltpu.VMEM((DM // 2, 2 * D), u32),
            pltpu.VMEM((DM // 2, 2 * D), u32),
        )

        def attention(c_v, s_v):
            row = jax.lax.broadcasted_iota(jnp.int32, (TQ, TQ), 0)
            col = jax.lax.broadcasted_iota(jnp.int32, (TQ, TQ), 1)
            tri = col <= row
            nb = S // TQ
            hq = TQ // 2
            npiece = 2
            pw = S // npiece

            def qk_piece(h, j):
                q = _unpack(q_v[h, (nb - 1) * hq:nb * hq, :])
                k = _unpack(k_v[h, j * pw // 2:(j + 1) * pw // 2, :])
                s_v[:, j * pw:(j + 1) * pw] = jax.lax.dot_general(q, k, NT, preferred_element_type=f32)

            def head(h, c):
                def qk(i):
                    q = _unpack(q_v[h, i * hq:(i + 1) * hq, :])
                    k = _unpack(k_v[h, 0:(i + 1) * hq, :])
                    return jax.lax.dot_general(q, k, NT, preferred_element_type=f32)

                hn = jnp.minimum(h + 1, H - 1)
                s_next = s_v[...]
                for i in range(nb - 1, -1, -1):
                    s = s_next
                    if i > 0:
                        s_next = qk(i - 1)
                    if i < npiece:
                        qk_piece(hn, npiece - 1 - i)
                    sd = jnp.where(tri, s[:, i * TQ:], NEG)
                    s = jnp.concatenate([s[:, :i * TQ], sd], axis=1) if i > 0 else sd
                    m = jnp.max(s, axis=1, keepdims=True)
                    p = jnp.exp2(s - m)
                    l = jnp.sum(p, axis=1, keepdims=True)
                    v = _unpack(v_v[h, 0:(i + 1) * hq, :])
                    o = jnp.dot(p.astype(bf16), v, preferred_element_type=f32)
                    c_v[h, i * hq:(i + 1) * hq, :] = _pack((o * _recip(l)).astype(bf16))
                return c
            with _scope("a_attn"):
                for j in range(npiece):
                    qk_piece(0, j)
                jax.lax.fori_loop(0, H, head, 0)

            woa_cp.wait()
            wob_cp.wait()
            xbt_cp.wait()
            for t in range(3):
                w_wait_shared(wb_v.at[t], 1 + t)
            nrb = S // RB

            def oproj(rb, c):
                for j in range(HP // nrb):
                    hp = rb * (HP // nrb) + j
                    t0 = pl.multiple_of(hp * D, D)
                    xb = xbt_v[:, pl.ds(t0, D)].T
                    xb_v[pl.ds(t0, D), :] = xb
                    for sg in range(D // SEG):
                        p0 = pl.multiple_of((hp * (D // SEG) + sg) * PRE, PRE)
                        xpre_v[pl.ds(p0, PRE), :] = xb[sg * SEG:sg * SEG + PRE, :]
                for hh in range(H // nrb):
                    h = rb * (H // nrb) + hh
                    wob_v[pl.ds(pl.multiple_of(h * (D // 2), D // 2), D // 2), :] = _pack(_unpack(wobt_v[h]).T)
                r0 = pl.multiple_of(rb * (RB // 2), RB // 2)
                ctx = _unpack(jnp.concatenate([c_v[h, pl.ds(r0, RB // 2), :] for h in range(H)], axis=1))
                wo = _unpack(jnp.concatenate([woa_v[h] for h in range(H)], axis=1))
                r = jax.lax.dot_general(ctx, wo, NT, preferred_element_type=f32)
                out_v[pl.ds(pl.multiple_of(rb * RB, RB), RB), 0:DM] = r.astype(bf16)
                return c
            with _scope("a_oproj"):
                jax.lax.fori_loop(0, nrb, oproj, 0)

        pl.run_scoped(
            attention,
            pltpu.VMEM((H, S // 2, D), u32),
            pltpu.VMEM((TQ, S), f32),
        )
        mem_cp.wait()

    pl.run_scoped(
        phase_a,
        pltpu.VMEM((H, DM // 2, D), u32),
        pltpu.VMEM((DM, S), bf16),
        pltpu.VMEM((H, DM // 2, D), u32),
        pltpu.VMEM((H, S // 2, D), u32),
        pltpu.VMEM((H, S // 2, D), u32),
        pltpu.VMEM((H, S // 2, D), u32),
    )

    def out_copy(j):
        rows = pl.ds(pl.multiple_of(j * (OUTER * SEG), OUTER * SEG), OUTER * SEG)
        return pltpu.make_async_copy(out_v.at[rows, :], out_hbm.at[rows, :], sem.at[SEM_OUT + j])

    def phase_b(pre_v, post_v):
        lane = jax.lax.broadcasted_iota(jnp.int32, (1, GW), 1)
        colscale = jnp.where(lane % (3 * D) < D, QSCALE, 1.0).astype(f32)

        def wgroup(g):
            return _unpack(jnp.concatenate(
                [wb_v[t, h % 2, h // 2] for h in range(g * HG, (g + 1) * HG) for t in range(3)], axis=1))

        def wogroup(g):
            return _unpack(wob_v[g * HG * D // 2:(g + 1) * HG * D // 2, :])

        with _scope("b_pre"):
            for g in range(G):
                cols = {}
                for hp in range(g * HG // 2, (g + 1) * HG // 2):
                    for t in range(3):
                        ev, od = w_combine(wb_v.at[t], hp)
                        wb_v[t, 0, hp] = ev
                        wb_v[t, 1, hp] = od
                        cols[2 * hp, t] = ev
                        cols[2 * hp + 1, t] = od
                w = _unpack(jnp.concatenate(
                    [cols[h, t] for h in range(g * HG, (g + 1) * HG) for t in range(3)], axis=1))
                pre_v[g] = (jnp.dot(xpre_v[...], w, preferred_element_type=f32) * colscale).astype(bf16)

        ri = jax.lax.broadcasted_iota(jnp.int32, (L, L), 0)
        ci = jax.lax.broadcasted_iota(jnp.int32, (L, L), 1)

        def pos(i):
            return jnp.where(i < T, i + (MEM + PRE), i - T)
        mask = (pos(ri) < MEM) | (pos(ri) >= pos(ci))

        def step(s, mem):
            xt = xb_v[pl.ds(pl.multiple_of(SEG * s + PRE, 8), T), :]
            l1 = jnp.concatenate([xt.astype(f32), mem], axis=0).astype(bf16)
            p0 = pl.multiple_of(PRE * s, 8)
            proj = [(jnp.dot(l1, wgroup(g), preferred_element_type=f32) * colscale).astype(bf16)
                    for g in range(G)]

            def rows(h, t):
                g, c0 = h // HG, (h % HG) * 3 * D + t * D
                return jnp.concatenate([proj[g][:, c0:c0 + D], pre_v[g, pl.ds(p0, PRE), c0:c0 + D]], axis=0)

            scores = [jax.lax.dot_general(rows(h, 0), rows(h, 1), NT, preferred_element_type=f32)
                      for h in range(H)]
            ctx = {}

            def attend(g):
                for h in range(g * HG, (g + 1) * HG):
                    sc = jnp.where(mask, scores[h], NEG)
                    m = jnp.max(sc, axis=1, keepdims=True)
                    p = jnp.exp2(sc - m)
                    l = jnp.sum(p, axis=1, keepdims=True)
                    o = jnp.dot(p.astype(bf16), rows(h, 2), preferred_element_type=f32)
                    o = (o * _recip(l)).astype(bf16)
                    ctx[h] = o[0:T + MEM, :]
                    post_v[pl.ds(pl.multiple_of((PRE * s) % (PRE * OUTER), 8), PRE), h * D:(h + 1) * D] = o[T + MEM:, :]

            parts = []

            def oproj(g):
                lhs = jnp.concatenate([ctx[h] for h in range(g * HG, (g + 1) * HG)], axis=1)
                parts.append(jnp.dot(lhs, wogroup(g), preferred_element_type=f32))

            for t in range(G + 2):
                if t < G:
                    attend(t)
                if t >= 2:
                    oproj(t - 2)
            acc = parts[0]
            for a in parts[1:]:
                acc = acc + a
            accb = acc.astype(bf16)
            out_v[pl.ds(pl.multiple_of(SEG * s + PRE, 8), T), DM:2 * DM] = accb[0:T, :]
            return accb[T:, :].astype(f32)

        def outer(j, mem):
            mem = jax.lax.fori_loop(0, OUTER, lambda i, m: step(j * OUTER + i, m), mem, unroll=2)
            r = jnp.dot(post_v[...], _unpack(wob_v[...]), preferred_element_type=f32).astype(bf16)
            for sg in range(OUTER):
                r0 = pl.multiple_of((j * OUTER + sg) * SEG, SEG)
                out_v[pl.ds(r0, PRE), DM:2 * DM] = r[sg * PRE:(sg + 1) * PRE, :]
            out_copy(j).start()
            return mem
        with _scope("b_loop"):
            jax.lax.fori_loop(0, NOUTER, outer, mem_v[0:MEM, :].astype(f32))
        with _scope("b_outwait"):
            for j in range(NOUTER):
                out_copy(j).wait()

    pl.run_scoped(
        phase_b,
        pltpu.VMEM((G, NSEG * PRE, GW), bf16),
        pltpu.VMEM((OUTER * PRE, H * D), bf16),
    )


@jax.jit
def pallas_concat_heads__compressed_kv_cla__memory_aug_recurrent_mem_tr__prompt_kernel(
    A_x: jax.Array,
    A_c_kv: jax.Array,
    A_w_q: jax.Array,
    A_w_uk: jax.Array,
    A_w_uv: jax.Array,
    A_w_o: jax.Array,
    B_x: jax.Array,
    B_mem0: jax.Array,
    B_Wq: jax.Array,
    B_Wk: jax.Array,
    B_Wv: jax.Array,
    B_Wo: jax.Array,
    B_seg_len=SEG,
):
    def t2(x):
        return jnp.transpose(x, (0, 2, 1)).reshape(DM, S)

    def w3(w):
        return w.reshape(w.shape[0] // 2, 2 * H, D)

    def wo3(w):
        return jnp.transpose(w, (0, 2, 1))

    any_spec = pl.BlockSpec(memory_space=pl.ANY)
    out = pl.pallas_call(
        _kernel,
        out_shape=jax.ShapeDtypeStruct((S, 2 * DM), bf16),
        in_specs=[any_spec] * 12,
        out_specs=any_spec,
        scratch_shapes=[
            pltpu.VMEM((S, 2 * DM), bf16),
            pltpu.VMEM((S, DM), bf16),
            pltpu.VMEM((NSEG * PRE, DM), bf16),
            pltpu.VMEM((3, 2, HP, DM // 2, D), u32),
            pltpu.VMEM((H * D // 2, DM), u32),
            pltpu.VMEM((8 * MEM, DM), bf16),
            pltpu.SemaphoreType.DMA((NSEM,)),
        ],
        compiler_params=pltpu.CompilerParams(vmem_limit_bytes=126 * 1024 * 1024),
    )(t2(A_x), A_c_kv.reshape(S, DC), w3(A_w_q), w3(A_w_uk), w3(A_w_uv), wo3(A_w_o),
      t2(B_x), B_mem0.reshape(MEM, DM), w3(B_Wq), w3(B_Wk), w3(B_Wv), wo3(B_Wo))
    return out.reshape(1, S, 2 * DM)
```

```python
import contextlib

import jax
import jax.numpy as jnp
import jax.experimental.pallas as pl
import jax.experimental.pallas.tpu as pltpu

S = 2048
DM = 576
DC = 512
H = 32
D = 128
MEM = 8
SEG = 32
L = MEM + SEG
NSEG = S // SEG
HP = H // 2

LOG2E = 1.4426950408889634
QSCALE = D ** -0.5 * LOG2E
NEG = -1.0e9 * LOG2E

TQ = 128
RB = 512
HG = 4
G = H // HG
GW = HG * 3 * D
PRE = 8
T = SEG - PRE
OUTER = 4
NOUTER = NSEG // OUTER

bf16 = jnp.bfloat16
f32 = jnp.float32
u32 = jnp.uint32
NT = (((1,), (1,)), ((), ()))

SEM_CKV = 0
SEM_XAT = 4
SEM_XBT = 5
SEM_MEM = 6
SEM_WOA = 7
SEM_WOB = 8
SEM_OUT = 9
SEM_WALL = SEM_OUT + NOUTER
SEM_W = SEM_WALL + 4
NSEM = SEM_W + 2 * 32

_PROFILE = False


def _scope(name):
    return jax.named_scope(name) if _PROFILE else contextlib.nullcontext()


def _unpack(w32):
    return pltpu.bitcast(w32, bf16)


def _pack(x):
    return pltpu.bitcast(x, u32)


def _recip(l):
    r = pl.reciprocal(l, approx=True)
    return r * (2.0 - l * r)


def _kernel(xat_hbm, ckv_hbm, wqa_hbm, wuk_hbm, wuv_hbm, woa_hbm,
            xbt_hbm, mem0_hbm, wqb_hbm, wkb_hbm, wvb_hbm, wob_hbm,
            out_hbm,
            out_v, xb_v, xpre_v, wb_v, wob_v, mem_v, q_v, k_v, v_v, sem):

    def w_copy(w_hbm, dst, slot, par, hp):
        return pltpu.make_async_copy(w_hbm.bitcast(u32).at[:, par * HP + hp, :], dst.at[par, hp], sem.at[slot])

    def w_start(w_hbm, dst, widx, hp):
        for par in range(2):
            w_copy(w_hbm, dst, SEM_W + widx * 32 + par * HP + hp, par, hp).start()

    def w_wait(w_hbm, dst, widx, hp):
        for par in range(2):
            w_copy(w_hbm, dst, SEM_W + widx * 32 + par * HP + hp, par, hp).wait()

    def w_start_shared(w_hbm, dst, widx, hps):
        for hp in hps:
            for par in range(2):
                w_copy(w_hbm, dst, SEM_WALL + widx, par, hp).start()

    def w_wait_shared(dst, widx):
        pltpu.make_async_copy(dst, dst, sem.at[SEM_WALL + widx]).wait()

    def w_combine(dst, hp):
        a = dst[0, hp]
        b = dst[1, hp]
        ev = (a & u32(0xFFFF)) | (b << 16)
        od = (a >> 16) | (b & u32(0xFFFF0000))
        return ev, od

    def w_pair(dst, hp):
        return jnp.concatenate(w_combine(dst, hp), axis=1)

    wb_hbm = (wqb_hbm, wkb_hbm, wvb_hbm)

    def phase_a(woa_v, xbt_v, wobt_v):
        woa_cp = pltpu.make_async_copy(woa_hbm.bitcast(u32), woa_v, sem.at[SEM_WOA])
        xbt_cp = pltpu.make_async_copy(xbt_hbm, xbt_v, sem.at[SEM_XBT])
        mem_cp = pltpu.make_async_copy(mem0_hbm, mem_v.at[0:MEM, :], sem.at[SEM_MEM])
        wob_cp = pltpu.make_async_copy(wob_hbm.bitcast(u32), wobt_v, sem.at[SEM_WOB])

        def store_heads(dst_v, hp, rb, r):
            r = r.astype(bf16)
            rows = slice(rb * RB // 2, (rb + 1) * RB // 2)
            dst_v[2 * hp, rows, :] = _pack(r[:, 0:D])
            dst_v[2 * hp + 1, rows, :] = _pack(r[:, D:2 * D])

        def projections(ckv_v, xat_v, xa_v, wuk_v, wuv_v, wqa_v, wk_v, wq0_v, wq1_v):
            nck = S // RB
            early = 14

            def ckv_cp(j):
                return pltpu.make_async_copy(ckv_hbm.at[j * RB:(j + 1) * RB, :],
                                             ckv_v.at[j * RB:(j + 1) * RB, :], sem.at[SEM_CKV + j])
            xat_cp = pltpu.make_async_copy(xat_hbm, xat_v, sem.at[SEM_XAT])

            with _scope("a_issue0"):
                w_start(wuk_hbm, wuk_v, 0, 0)
                ckv_cp(0).start()
                w_start(wuv_hbm, wuv_v, 1, 0)
                for j in range(1, nck):
                    ckv_cp(j).start()
                for hp in range(1, early):
                    w_start(wuk_hbm, wuk_v, 0, hp)
                    w_start(wuv_hbm, wuv_v, 1, hp)

            def project(dst_v, lhs_v, w, hp, rb, scale=None):
                r = jnp.dot(lhs_v[rb * RB:(rb + 1) * RB, :], _unpack(w), preferred_element_type=f32)
                store_heads(dst_v, hp, rb, r if scale is None else r * scale)

            def kv_first():
                w_wait(wuk_hbm, wuk_v, 0, 0)
                ckv_cp(0).wait()
                wk = w_pair(wuk_v, 0)
                project(k_v, ckv_v, wk, 0, 0)
                w_wait(wuv_hbm, wuv_v, 1, 0)
                wv = w_pair(wuv_v, 0)
                project(v_v, ckv_v, wv, 0, 0)
                for rb in range(1, nck):
                    ckv_cp(rb).wait()
                    project(k_v, ckv_v, wk, 0, rb)
                    project(v_v, ckv_v, wv, 0, rb)
                w_wait(wuk_hbm, wuk_v, 0, 1)
                wk_v[...] = w_pair(wuk_v, 1)

            def kv_body(hp, c, last=False):
                if not last:
                    @pl.when(hp == 4)
                    def _():
                        xat_cp.start()
                        for j in range(early, HP):
                            w_start(wuk_hbm, wuk_v, 0, j)
                            w_start(wuv_hbm, wuv_v, 1, j)
                        w_start_shared(wqa_hbm, wqa_v, 0, range(HP))
                w_wait(wuv_hbm, wuv_v, 1, hp)
                if last:
                    xat_cp.wait()
                    w_wait_shared(wqa_v, 0)
                else:
                    w_wait(wuk_hbm, wuk_v, 0, hp + 1)
                wv = w_pair(wuv_v, hp)
                for rb in range(nck):
                    project(k_v, ckv_v, wk_v[...], hp, rb)
                if last:
                    wq0_v[...] = w_pair(wqa_v, 0)
                    for t in range(S // D):
                        xa_v[t * D:(t + 1) * D, :] = xat_v[:, t * D:(t + 1) * D].T
                else:
                    wk_v[...] = w_pair(wuk_v, hp + 1)
                for rb in range(nck):
                    project(v_v, ckv_v, wv, hp, rb)
                return c

            with _scope("a_kvproj"):
                kv_first()
                jax.lax.fori_loop(1, HP - 1, kv_body, 0)
                kv_body(HP - 1, 0, last=True)

            woa_cp.start()
            wob_cp.start()
            xbt_cp.start()
            mem_cp.start()
            w_start_shared(wqb_hbm, wb_v.at[0], 1, range(HP))
            w_start_shared(wkb_hbm, wb_v.at[1], 2, range(HP // 2))

            def q_body(j, c):
                wq1_v[...] = w_pair(wqa_v, 2 * j + 1)
                for rb in range(nck):
                    project(q_v, xa_v, wq0_v[...], 2 * j, rb, QSCALE)
                wq0_v[...] = w_pair(wqa_v, jnp.minimum(2 * j + 2, HP - 1))
                for rb in range(nck):
                    project(q_v, xa_v, wq1_v[...], 2 * j + 1, rb, QSCALE)
                return c

            with _scope("a_qproj"):
                jax.lax.fori_loop(0, HP // 2, q_body, 0)

            w_start_shared(wkb_hbm, wb_v.at[1], 2, range(HP // 2, HP))
            w_start_shared(wvb_hbm, wb_v.at[2], 3, range(HP))

        pl.run_scoped(
            projections,
            pltpu.VMEM((S, DC), bf16),
            pltpu.VMEM((DM, S), bf16),
            pltpu.VMEM((S, DM), bf16),
            pltpu.VMEM((2, HP, DC // 2, D), u32),
            pltpu.VMEM((2, HP, DC // 2, D), u32),
            pltpu.VMEM((2, HP, DM // 2, D), u32),
            pltpu.VMEM((DC // 2, 2 * D), u32),
            pltpu.VMEM((DM // 2, 2 * D), u32),
            pltpu.VMEM((DM // 2, 2 * D), u32),
        )

        def attention(c_v, s_v):
            row = jax.lax.broadcasted_iota(jnp.int32, (TQ, TQ), 0)
            col = jax.lax.broadcasted_iota(jnp.int32, (TQ, TQ), 1)
            tri = col <= row
            nb = S // TQ
            hq = TQ // 2
            npiece = 2
            pw = S // npiece

            def qk_piece(h, j):
                q = _unpack(q_v[h, (nb - 1) * hq:nb * hq, :])
                k = _unpack(k_v[h, j * pw // 2:(j + 1) * pw // 2, :])
                s_v[:, j * pw:(j + 1) * pw] = jax.lax.dot_general(q, k, NT, preferred_element_type=f32)

            def head(h, c):
                def qk(i):
                    q = _unpack(q_v[h, i * hq:(i + 1) * hq, :])
                    k = _unpack(k_v[h, 0:(i + 1) * hq, :])
                    return jax.lax.dot_general(q, k, NT, preferred_element_type=f32)

                hn = jnp.minimum(h + 1, H - 1)
                s_next = s_v[...]
                for i in range(nb - 1, -1, -1):
                    s = s_next
                    if i > 0:
                        s_next = qk(i - 1)
                    if i < npiece:
                        qk_piece(hn, npiece - 1 - i)
                    sd = jnp.where(tri, s[:, i * TQ:], NEG)
                    s = jnp.concatenate([s[:, :i * TQ], sd], axis=1) if i > 0 else sd
                    m = jnp.max(s, axis=1, keepdims=True)
                    p = jnp.exp2(s - m)
                    l = jnp.sum(p, axis=1, keepdims=True)
                    v = _unpack(v_v[h, 0:(i + 1) * hq, :])
                    o = jnp.dot(p.astype(bf16), v, preferred_element_type=f32)
                    c_v[h, i * hq:(i + 1) * hq, :] = _pack((o * _recip(l)).astype(bf16))
                return c
            with _scope("a_attn"):
                for j in range(npiece):
                    qk_piece(0, j)
                jax.lax.fori_loop(0, H, head, 0)

            woa_cp.wait()
            wob_cp.wait()
            xbt_cp.wait()
            for t in range(3):
                w_wait_shared(wb_v.at[t], 1 + t)
            nrb = S // RB

            def oproj(rb, c):
                for j in range(HP // nrb):
                    hp = rb * (HP // nrb) + j
                    t0 = pl.multiple_of(hp * D, D)
                    xb = xbt_v[:, pl.ds(t0, D)].T
                    xb_v[pl.ds(t0, D), :] = xb
                    for sg in range(D // SEG):
                        p0 = pl.multiple_of((hp * (D // SEG) + sg) * PRE, PRE)
                        xpre_v[pl.ds(p0, PRE), :] = xb[sg * SEG:sg * SEG + PRE, :]
                for hh in range(H // nrb):
                    h = rb * (H // nrb) + hh
                    wob_v[pl.ds(pl.multiple_of(h * (D // 2), D // 2), D // 2), :] = _pack(_unpack(wobt_v[h]).T)
                r0 = pl.multiple_of(rb * (RB // 2), RB // 2)
                ctx = _unpack(jnp.concatenate([c_v[h, pl.ds(r0, RB // 2), :] for h in range(H)], axis=1))
                wo = _unpack(jnp.concatenate([woa_v[h] for h in range(H)], axis=1))
                r = jax.lax.dot_general(ctx, wo, NT, preferred_element_type=f32)
                out_v[pl.ds(pl.multiple_of(rb * RB, RB), RB), 0:DM] = r.astype(bf16)
                return c
            with _scope("a_oproj"):
                jax.lax.fori_loop(0, nrb, oproj, 0)

        pl.run_scoped(
            attention,
            pltpu.VMEM((H, S // 2, D), u32),
            pltpu.VMEM((TQ, S), f32),
        )
        mem_cp.wait()

    pl.run_scoped(
        phase_a,
        pltpu.VMEM((H, DM // 2, D), u32),
        pltpu.VMEM((DM, S), bf16),
        pltpu.VMEM((H, DM // 2, D), u32),
    )

    def out_copy(j):
        rows = pl.ds(pl.multiple_of(j * (OUTER * SEG), OUTER * SEG), OUTER * SEG)
        return pltpu.make_async_copy(out_v.at[rows, :], out_hbm.at[rows, :], sem.at[SEM_OUT + j])

    def phase_b(pre_v, post_v):
        lane = jax.lax.broadcasted_iota(jnp.int32, (1, GW), 1)
        colscale = jnp.where(lane % (3 * D) < D, QSCALE, 1.0).astype(f32)

        def wgroup(g):
            return _unpack(jnp.concatenate(
                [wb_v[t, h % 2, h // 2] for h in range(g * HG, (g + 1) * HG) for t in range(3)], axis=1))

        def wogroup(g):
            return _unpack(wob_v[g * HG * D // 2:(g + 1) * HG * D // 2, :])

        with _scope("b_pre"):
            for g in range(G):
                cols = {}
                for hp in range(g * HG // 2, (g + 1) * HG // 2):
                    for t in range(3):
                        ev, od = w_combine(wb_v.at[t], hp)
                        wb_v[t, 0, hp] = ev
                        wb_v[t, 1, hp] = od
                        cols[2 * hp, t] = ev
                        cols[2 * hp + 1, t] = od
                w = _unpack(jnp.concatenate(
                    [cols[h, t] for h in range(g * HG, (g + 1) * HG) for t in range(3)], axis=1))
                r = jnp.dot(xpre_v[...], w, preferred_element_type=f32) * colscale
                for hp in range(g * HG // 2, (g + 1) * HG // 2):
                    for t in range(3):
                        c0 = (2 * hp % HG) * 3 * D + t * D
                        two = [r[:, c:c + D].reshape(NSEG, 1, PRE, D) for c in (c0, c0 + 3 * D)]
                        two = jnp.concatenate(two, axis=1).reshape(NSEG * 2 * PRE, D)
                        pre_v[hp * 3 + t] = _pack(two.astype(bf16))

        ri = jax.lax.broadcasted_iota(jnp.int32, (2 * L, 2 * L), 0)
        ci = jax.lax.broadcasted_iota(jnp.int32, (2 * L, 2 * L), 1)

        def second(i):
            return jnp.where(i < 2 * SEG, i // SEG, (i - 2 * SEG) // PRE)

        def pos(i):
            j = i % SEG
            return jnp.where(i < 2 * SEG, jnp.where(j < T, j + (MEM + PRE), j - T), MEM + i % PRE)
        same = second(ri) == second(ci)
        mask = same & ((pos(ri) < MEM) | (pos(ri) >= pos(ci)))
        fill = jnp.where(same, NEG, -jnp.inf).astype(f32)

        def step(s, slot, mem):
            xt = xb_v[pl.ds(pl.multiple_of(SEG * s + PRE, 8), T), :]
            l1 = jnp.concatenate([xt.astype(f32), mem], axis=0).astype(bf16)
            p0 = pl.multiple_of(PRE * s, 8)
            proj = [(jnp.dot(l1, wgroup(g), preferred_element_type=f32) * colscale).astype(bf16)
                    for g in range(G)]

            def rows(hp, t):
                g, c0 = 2 * hp // HG, (2 * hp % HG) * 3 * D + t * D
                return jnp.concatenate([proj[g][:, c0:c0 + D], proj[g][:, c0 + 3 * D:c0 + 4 * D],
                                        _unpack(pre_v[hp * 3 + t, pl.ds(p0, PRE), :])], axis=0)

            scores = [jax.lax.dot_general(rows(hp, 0), rows(hp, 1), NT, preferred_element_type=f32)
                      for hp in range(HP)]
            ctx = {}

            def attend(g):
                for hp in range(g * HG // 2, (g + 1) * HG // 2):
                    sc = jnp.where(mask, scores[hp], fill)
                    m = jnp.max(sc, axis=1, keepdims=True)
                    p = jnp.exp2(sc - m)
                    l = jnp.sum(p, axis=1, keepdims=True)
                    o = jnp.dot(p.astype(bf16), rows(hp, 2), preferred_element_type=f32) * _recip(l)
                    for e in range(2):
                        h = 2 * hp + e
                        ctx[h] = o[e * SEG:(e + 1) * SEG, :].astype(bf16)
                        post_v[slot * PRE:(slot + 1) * PRE, h * D:(h + 1) * D] = o[2 * SEG + e * PRE:2 * SEG + (e + 1) * PRE, :]

            parts = []

            def oproj(g):
                lhs = jnp.concatenate([ctx[h] for h in range(g * HG, (g + 1) * HG)], axis=1)
                parts.append(jnp.dot(lhs, wogroup(g), preferred_element_type=f32))

            for t in range(G + 2):
                if t < G:
                    attend(t)
                if t >= 2:
                    oproj(t - 2)
            acc = parts[0]
            for a in parts[1:]:
                acc = acc + a
            accb = acc.astype(bf16)
            out_v[pl.ds(pl.multiple_of(SEG * s + PRE, 8), T), DM:2 * DM] = accb[0:T, :]
            return accb[T:, :].astype(f32), ctx[H - 1]

        KP = H * D // OUTER

        def partial(rows, i):
            return jnp.dot(rows, _unpack(wob_v[i * KP // 2:(i + 1) * KP // 2, :]), preferred_element_type=f32)

        def finish(j, r):
            r = r.astype(bf16)
            for sg in range(OUTER):
                r0 = pl.multiple_of((j * OUTER + sg) * SEG, SEG)
                out_v[pl.ds(r0, PRE), DM:2 * DM] = r[sg * PRE:(sg + 1) * PRE, :]

        def after(x, late):
            u = _pack(late[0:2 * OUTER * PRE // 2, :])
            zero = (u >> 31) & (~u >> 31)
            return _unpack(_pack(x) | jnp.concatenate([zero] * (x.shape[1] // D), axis=1))

        def outer(j, mem):
            prev = post_v[...].astype(bf16)
            acc = partial(prev[:, 0:KP], 0)
            for i in range(OUTER):
                mem, late = step(j * OUTER + i, i, mem)
                if i + 1 < OUTER:
                    acc = acc + partial(after(prev[:, (i + 1) * KP:(i + 2) * KP], late), i + 1)
            finish(jnp.maximum(j - 1, 0), acc)

            @pl.when(j > 0)
            def _():
                out_copy(j - 1).start()
            return mem
        with _scope("b_loop"):
            post_v[...] = jnp.zeros(post_v.shape, f32)
            jax.lax.fori_loop(0, NOUTER, outer, mem_v[0:MEM, :].astype(f32))
            finish(NOUTER - 1, jnp.dot(post_v[...].astype(bf16), _unpack(wob_v[...]), preferred_element_type=f32))
            out_copy(NOUTER - 1).start()
        with _scope("b_outwait"):
            for j in range(NOUTER):
                out_copy(j).wait()

    pl.run_scoped(
        phase_b,
        pltpu.VMEM((HP * 3, NSEG * PRE, D), u32),
        pltpu.VMEM((OUTER * PRE, H * D), f32),
    )


@jax.jit
def pallas_concat_heads__compressed_kv_cla__memory_aug_recurrent_mem_tr__prompt_kernel(
    A_x: jax.Array,
    A_c_kv: jax.Array,
    A_w_q: jax.Array,
    A_w_uk: jax.Array,
    A_w_uv: jax.Array,
    A_w_o: jax.Array,
    B_x: jax.Array,
    B_mem0: jax.Array,
    B_Wq: jax.Array,
    B_Wk: jax.Array,
    B_Wv: jax.Array,
    B_Wo: jax.Array,
    B_seg_len=SEG,
):
    def t2(x):
        return jnp.transpose(x, (0, 2, 1)).reshape(DM, S)

    def w3(w):
        return w.reshape(w.shape[0] // 2, 2 * H, D)

    def wo3(w):
        return jnp.transpose(w, (0, 2, 1))

    any_spec = pl.BlockSpec(memory_space=pl.ANY)
    out = pl.pallas_call(
        _kernel,
        out_shape=jax.ShapeDtypeStruct((S, 2 * DM), bf16),
        in_specs=[any_spec] * 12,
        out_specs=any_spec,
        scratch_shapes=[
            pltpu.VMEM((S, 2 * DM), bf16),
            pltpu.VMEM((S, DM), bf16),
            pltpu.VMEM((NSEG * PRE, DM), bf16),
            pltpu.VMEM((3, 2, HP, DM // 2, D), u32),
            pltpu.VMEM((H * D // 2, DM), u32),
            pltpu.VMEM((8 * MEM, DM), bf16),
            pltpu.VMEM((H, S // 2, D), u32),
            pltpu.VMEM((H, S // 2, D), u32),
            pltpu.VMEM((H, S // 2, D), u32),
            pltpu.SemaphoreType.DMA((NSEM,)),
        ],
        compiler_params=pltpu.CompilerParams(vmem_limit_bytes=126 * 1024 * 1024),
    )(t2(A_x), A_c_kv.reshape(S, DC), w3(A_w_q), w3(A_w_uk), w3(A_w_uv), wo3(A_w_o),
      t2(B_x), B_mem0.reshape(MEM, DM), w3(B_Wq), w3(B_Wk), w3(B_Wv), wo3(B_Wo))
    return out.reshape(1, S, 2 * DM)
```

```python
import contextlib

import jax
import jax.numpy as jnp
import jax.experimental.pallas as pl
import jax.experimental.pallas.tpu as pltpu

S = 2048
DM = 576
DC = 512
H = 32
D = 128
MEM = 8
SEG = 32
L = MEM + SEG
NSEG = S // SEG
HP = H // 2

LOG2E = 1.4426950408889634
QSCALE = D ** -0.5 * LOG2E
NEG = -1.0e9 * LOG2E

TQ = 128
UH = 2
RB = 512
HG = 4
G = H // HG
GW = HG * 3 * D
PRE = 8
T = SEG - PRE
OUTER = 4
NOUTER = NSEG // OUTER

bf16 = jnp.bfloat16
f32 = jnp.float32
u32 = jnp.uint32
NT = (((1,), (1,)), ((), ()))

SEM_CKV = 0
SEM_XAT = 4
SEM_XBT = 5
SEM_MEM = 6
SEM_WOA = 7
SEM_WOB = 8
SEM_OUT = 9
SEM_WALL = SEM_OUT + NOUTER
SEM_W = SEM_WALL + 4
NSEM = SEM_W + 2 + HP // 2

_PROFILE = False


def _scope(name):
    return jax.named_scope(name) if _PROFILE else contextlib.nullcontext()


def _unpack(w32):
    return pltpu.bitcast(w32, bf16)


def _pack(x):
    return pltpu.bitcast(x, u32)


def _recip(l):
    r = pl.reciprocal(l, approx=True)
    return r * (2.0 - l * r)


def _kernel(xat_hbm, ckv_hbm, wqa_hbm, wuk_hbm, wuv_hbm, woa_hbm,
            xbt_hbm, mem0_hbm, wqb_hbm, wkb_hbm, wvb_hbm, wob_hbm,
            out_hbm,
            out_v, xb_v, xpre_v, wb_v, wob_v, mem_v, q_v, k_v, v_v, sem):

    def w_copy(w_hbm, dst, slot, par, hp):
        return pltpu.make_async_copy(w_hbm.bitcast(u32).at[:, par * HP + hp, :], dst.at[par, hp], sem.at[slot])

    def w_start_shared(w_hbm, dst, widx, hps):
        for hp in hps:
            for par in range(2):
                w_copy(w_hbm, dst, SEM_WALL + widx, par, hp).start()

    def w_wait_shared(dst, widx):
        pltpu.make_async_copy(dst, dst, sem.at[SEM_WALL + widx]).wait()

    def w_combine(dst, hp):
        a = dst[0, hp]
        b = dst[1, hp]
        ev = (a & u32(0xFFFF)) | (b << 16)
        od = (a >> 16) | (b & u32(0xFFFF0000))
        return ev, od

    def w_pair(dst, hp):
        return jnp.concatenate(w_combine(dst, hp), axis=1)

    wb_hbm = (wqb_hbm, wkb_hbm, wvb_hbm)

    def pre_ref(j):
        n = NSEG * PRE
        return q_v.at[j // 2, (j % 2) * n:(j % 2 + 1) * n, :]

    def b_pre():
        lane = jax.lax.broadcasted_iota(jnp.int32, (1, GW), 1)
        colscale = jnp.where(lane % (3 * D) < D, QSCALE, 1.0).astype(f32)

        with _scope("b_pre"):
            for g in range(G):
                cols = {}
                for hp in range(g * HG // 2, (g + 1) * HG // 2):
                    for t in range(3):
                        ev, od = w_combine(wb_v.at[t], hp)
                        wb_v[t, 0, hp] = ev
                        wb_v[t, 1, hp] = od
                        cols[2 * hp, t] = ev
                        cols[2 * hp + 1, t] = od
                w = _unpack(jnp.concatenate(
                    [cols[h, t] for h in range(g * HG, (g + 1) * HG) for t in range(3)], axis=1))
                r = jnp.dot(xpre_v[...], w, preferred_element_type=f32) * colscale
                for hp in range(g * HG // 2, (g + 1) * HG // 2):
                    for t in range(3):
                        c0 = (2 * hp % HG) * 3 * D + t * D
                        two = [r[:, c:c + D].reshape(NSEG, 1, PRE, D) for c in (c0, c0 + 3 * D)]
                        two = jnp.concatenate(two, axis=1).reshape(NSEG * 2 * PRE, D)
                        pre_ref(hp * 3 + t)[...] = _pack(two.astype(bf16))


    def phase_a(woa_v, xbt_v, wobt_v):
        woa_cp = pltpu.make_async_copy(woa_hbm.bitcast(u32), woa_v, sem.at[SEM_WOA])
        xbt_cp = pltpu.make_async_copy(xbt_hbm, xbt_v, sem.at[SEM_XBT])
        mem_cp = pltpu.make_async_copy(mem0_hbm, mem_v.at[0:MEM, :], sem.at[SEM_MEM])
        wob_cp = pltpu.make_async_copy(wob_hbm.bitcast(u32), wobt_v, sem.at[SEM_WOB])

        def store_heads(dst_v, hp, rb, r):
            r = r.astype(bf16)
            rows = slice(rb * RB // 2, (rb + 1) * RB // 2)
            dst_v[2 * hp, rows, :] = _pack(r[:, 0:D])
            dst_v[2 * hp + 1, rows, :] = _pack(r[:, D:2 * D])

        def projections(ckv_v, xat_v, xa_v, wuk_v, wuv_v, wqa_v, wk_v, wq0_v):
            nck = S // RB
            def group(j):
                items = [] if j == 0 else [(wuv_hbm, wuv_v, 2 * j)]
                items += [(wuk_hbm, wuk_v, 2 * j + 1), (wuv_hbm, wuv_v, 2 * j + 1)]
                return items + ([(wuk_hbm, wuk_v, 2 * j + 2)] if 2 * j + 2 < HP else [])

            def group_start(j):
                for w_hbm, dst, hp in group(j):
                    for par in range(2):
                        w_copy(w_hbm, dst, SEM_W + 2 + j, par, hp).start()

            def group_wait(j, n):
                part = wuk_v.at[:, 0:n]
                pltpu.make_async_copy(part, part, sem.at[SEM_W + 2 + j]).wait()

            def first_copies(w_hbm, dst, slot):
                return [w_copy(w_hbm, dst, SEM_W + slot, par, 0) for par in range(2)]

            def first_wait(dst, slot):
                part = dst.at[:, 0:1]
                pltpu.make_async_copy(part, part, sem.at[SEM_W + slot]).wait()

            def ckv_cp(j):
                return pltpu.make_async_copy(ckv_hbm.at[j * RB:(j + 1) * RB, :],
                                             ckv_v.at[j * RB:(j + 1) * RB, :], sem.at[SEM_CKV + j])
            xat_cp = pltpu.make_async_copy(xat_hbm, xat_v, sem.at[SEM_XAT])
            ngrp = HP // 2

            with _scope("a_issue0"):
                for cp in first_copies(wuk_hbm, wuk_v, 0):
                    cp.start()
                ckv_cp(0).start()
                for cp in first_copies(wuv_hbm, wuv_v, 1):
                    cp.start()
                for j in range(1, nck):
                    ckv_cp(j).start()
                for j in range(ngrp - 1):
                    group_start(j)

            def project(dst_v, lhs_v, w, hp, rb, scale=None):
                r = jnp.dot(lhs_v[rb * RB:(rb + 1) * RB, :], _unpack(w), preferred_element_type=f32)
                store_heads(dst_v, hp, rb, r if scale is None else r * scale)

            def project_all(dst_v, w, hp):
                for rb in range(nck):
                    project(dst_v, ckv_v, w, hp, rb)

            def kv_first():
                first_wait(wuk_v, 0)
                ckv_cp(0).wait()
                wk = w_pair(wuk_v, 0)
                project(k_v, ckv_v, wk, 0, 0)
                first_wait(wuv_v, 1)
                wv = w_pair(wuv_v, 0)
                project(v_v, ckv_v, wv, 0, 0)
                ckv_cp(1).wait()
                project(k_v, ckv_v, wk, 0, 1)
                project(v_v, ckv_v, wv, 0, 1)
                for rb in range(2, nck):
                    ckv_cp(rb).wait()
                for rb in range(2, nck):
                    project(k_v, ckv_v, wk, 0, rb)
                    project(v_v, ckv_v, wv, 0, rb)
                group_wait(0, len(group(0)))
                project_all(k_v, w_pair(wuk_v, 1), 1)
                wk_v[...] = w_pair(wuk_v, 2)
                project_all(v_v, w_pair(wuv_v, 1), 1)

            def kv_body(j, c, last=False):
                if not last:
                    @pl.when(j == 2)
                    def _():
                        xat_cp.start()
                        group_start(ngrp - 1)
                        w_start_shared(wqa_hbm, wqa_v, 0, range(HP))
                group_wait(j, len(group(ngrp - 1 if last else 1)))
                if last:
                    xat_cp.wait()
                    w_wait_shared(wqa_v, 0)
                project_all(k_v, wk_v[...], 2 * j)
                project_all(v_v, w_pair(wuv_v, 2 * j), 2 * j)
                project_all(k_v, w_pair(wuk_v, 2 * j + 1), 2 * j + 1)
                if last:
                    wq0_v[...] = w_pair(wqa_v, 0)
                    for t in range(S // D):
                        xa_v[t * D:(t + 1) * D, :] = xat_v[:, t * D:(t + 1) * D].T
                else:
                    wk_v[...] = w_pair(wuk_v, 2 * j + 2)
                project_all(v_v, w_pair(wuv_v, 2 * j + 1), 2 * j + 1)
                return c

            with _scope("a_kvproj"):
                kv_first()
                jax.lax.fori_loop(1, ngrp - 1, kv_body, 0)
                kv_body(ngrp - 1, 0, last=True)

            woa_cp.start()
            wob_cp.start()
            xbt_cp.start()
            mem_cp.start()
            w_start_shared(wqb_hbm, wb_v.at[0], 1, range(HP))
            w_start_shared(wkb_hbm, wb_v.at[1], 2, range(HP // 2))

            with _scope("a_qproj"):
                for hp in range(HP):
                    wq = wq0_v[...] if hp == 0 else w_pair(wqa_v, hp)
                    for rb in range(nck):
                        project(q_v, xa_v, wq, hp, rb, QSCALE)

        pl.run_scoped(
            projections,
            pltpu.VMEM((S, DC), bf16),
            pltpu.VMEM((DM, S), bf16),
            pltpu.VMEM((S, DM), bf16),
            pltpu.VMEM((2, HP, DC // 2, D), u32),
            pltpu.VMEM((2, HP, DC // 2, D), u32),
            pltpu.VMEM((2, HP, DM // 2, D), u32),
            pltpu.VMEM((DC // 2, 2 * D), u32),
            pltpu.VMEM((DM // 2, 2 * D), u32),
        )

        def attention(c_v, s_v):
            row = jax.lax.broadcasted_iota(jnp.int32, (TQ, TQ), 0)
            col = jax.lax.broadcasted_iota(jnp.int32, (TQ, TQ), 1)
            tri = col <= row
            nb = S // TQ
            hq = TQ // 2
            npiece = 2
            pw = S // npiece

            def qk_piece(h, j):
                q = _unpack(q_v[h, (nb - 1) * hq:nb * hq, :])
                k = _unpack(k_v[h, j * pw // 2:(j + 1) * pw // 2, :])
                s_v[:, j * pw:(j + 1) * pw] = jax.lax.dot_general(q, k, NT, preferred_element_type=f32)

            def qk(h, i, j0=0, j1=None):
                j1 = i + 1 if j1 is None else j1
                q = _unpack(q_v[h, i * hq:(i + 1) * hq, :])
                k = _unpack(k_v[h, j0 * hq:j1 * hq, :])
                return jax.lax.dot_general(q, k, NT, preferred_element_type=f32)

            def heads(j, c):
                @pl.when(j == 0)
                def _():
                    w_start_shared(wkb_hbm, wb_v.at[1], 2, range(HP // 2, HP))
                    w_start_shared(wvb_hbm, wb_v.at[2], 3, range(HP))

                s_next = s_v[...]
                for e in range(UH):
                    h = j * UH + e
                    hn = jnp.minimum(h + 1, H - 1) if e == UH - 1 else h + 1
                    pieces = []
                    for i in range(nb - 1, -1, -1):
                        s = s_next
                        if i > 0:
                            s_next = qk(h, i - 1)
                        if i < npiece:
                            if e == UH - 1:
                                qk_piece(hn, npiece - 1 - i)
                            else:
                                jj = npiece - 1 - i
                                pieces.append(qk(hn, nb - 1, jj * nb // npiece, (jj + 1) * nb // npiece))
                        sd = jnp.where(tri, s[:, i * TQ:], NEG)
                        s = jnp.concatenate([s[:, :i * TQ], sd], axis=1) if i > 0 else sd
                        m = jnp.max(s, axis=1, keepdims=True)
                        p = jnp.exp2(s - m)
                        l = jnp.sum(p, axis=1, keepdims=True)
                        v = _unpack(v_v[h, 0:(i + 1) * hq, :])
                        o = jnp.dot(p.astype(bf16), v, preferred_element_type=f32)
                        c_v[h, i * hq:(i + 1) * hq, :] = _pack((o * _recip(l)).astype(bf16))
                    if e < UH - 1:
                        s_next = jnp.concatenate(pieces, axis=1)
                return c
            with _scope("a_attn"):
                for j in range(npiece):
                    qk_piece(0, j)
                jax.lax.fori_loop(0, H // UH, heads, 0)

            woa_cp.wait()
            wob_cp.wait()
            xbt_cp.wait()
            mem_cp.wait()
            for t in range(3):
                w_wait_shared(wb_v.at[t], 1 + t)
            nrb = S // RB

            def oproj(rb, c):
                for j in range(HP // nrb):
                    hp = rb * (HP // nrb) + j
                    t0 = hp * D
                    xb = xbt_v[:, t0:t0 + D].T
                    xb_v[t0:t0 + D, :] = xb
                    for sg in range(D // SEG):
                        p0 = (hp * (D // SEG) + sg) * PRE
                        xpre_v[p0:p0 + PRE, :] = xb[sg * SEG:sg * SEG + PRE, :]
                for hh in range(H // nrb):
                    h = rb * (H // nrb) + hh
                    wob_v[h * (D // 2):(h + 1) * (D // 2), :] = _pack(_unpack(wobt_v[h]).T)
                r0 = rb * (RB // 2)
                ctx = _unpack(jnp.concatenate([c_v[h, r0:r0 + RB // 2, :] for h in range(H)], axis=1))
                wo = _unpack(jnp.concatenate([woa_v[h] for h in range(H)], axis=1))
                for t in range(RB // D):
                    r = jax.lax.dot_general(wo, ctx[t * D:(t + 1) * D, :], NT, preferred_element_type=f32)
                    out_v[rb * RB + t * D:rb * RB + (t + 1) * D, 0:DM] = r.T.astype(bf16)
                return c
            with _scope("a_oproj"):
                for rb in range(nrb):
                    oproj(rb, 0)
            b_pre()

        pl.run_scoped(
            attention,
            pltpu.VMEM((H, S // 2, D), u32),
            pltpu.VMEM((TQ, S), f32),
        )

    pl.run_scoped(
        phase_a,
        pltpu.VMEM((H, DM // 2, D), u32),
        pltpu.VMEM((DM, S), bf16),
        pltpu.VMEM((H, DM // 2, D), u32),
    )

    def out_copy(j):
        rows = pl.ds(pl.multiple_of(j * (OUTER * SEG), OUTER * SEG), OUTER * SEG)
        return pltpu.make_async_copy(out_v.at[rows, :], out_hbm.at[rows, :], sem.at[SEM_OUT + j])

    def phase_b(post_v):
        lane = jax.lax.broadcasted_iota(jnp.int32, (1, GW), 1)
        colscale = jnp.where(lane % (3 * D) < D, QSCALE, 1.0).astype(f32)

        def wgroup(g):
            return _unpack(jnp.concatenate(
                [wb_v[t, h % 2, h // 2] for h in range(g * HG, (g + 1) * HG) for t in range(3)], axis=1))

        def wogroup(g):
            return _unpack(wob_v[g * HG * D // 2:(g + 1) * HG * D // 2, :])

        ri = jax.lax.broadcasted_iota(jnp.int32, (2 * L, 2 * L), 0)
        ci = jax.lax.broadcasted_iota(jnp.int32, (2 * L, 2 * L), 1)

        def second(i):
            return jnp.where(i < 2 * SEG, i // SEG, (i - 2 * SEG) // PRE)

        def pos(i):
            j = i % SEG
            return jnp.where(i < 2 * SEG, jnp.where(j < T, j + (MEM + PRE), j - T), MEM + i % PRE)
        same = second(ri) == second(ci)
        mask = same & ((pos(ri) < MEM) | (pos(ri) >= pos(ci)))
        fill = jnp.where(same, NEG, -jnp.inf).astype(f32)

        def step(s, slot, mem):
            xt = xb_v[pl.ds(pl.multiple_of(SEG * s + PRE, 8), T), :]
            l1 = jnp.concatenate([xt.astype(f32), mem], axis=0).astype(bf16)
            p0 = pl.multiple_of(PRE * s, 8)
            proj = [(jnp.dot(l1, wgroup(g), preferred_element_type=f32) * colscale).astype(bf16)
                    for g in range(G)]

            def rows(hp, t):
                g, c0 = 2 * hp // HG, (2 * hp % HG) * 3 * D + t * D
                return jnp.concatenate([proj[g][:, c0:c0 + D], proj[g][:, c0 + 3 * D:c0 + 4 * D],
                                        _unpack(pre_ref(hp * 3 + t)[pl.ds(p0, PRE), :])], axis=0)

            scores = [jax.lax.dot_general(rows(hp, 0), rows(hp, 1), NT, preferred_element_type=f32)
                      for hp in range(HP)]
            ctx = {}

            def attend(g):
                for hp in range(g * HG // 2, (g + 1) * HG // 2):
                    sc = jnp.where(mask, scores[hp], fill)
                    m = jnp.max(sc, axis=1, keepdims=True)
                    p = jnp.exp2(sc - m)
                    l = jnp.sum(p, axis=1, keepdims=True)
                    o = jnp.dot(p.astype(bf16), rows(hp, 2), preferred_element_type=f32) * _recip(l)
                    for e in range(2):
                        h = 2 * hp + e
                        ctx[h] = o[e * SEG:(e + 1) * SEG, :].astype(bf16)
                        post_v[slot * PRE:(slot + 1) * PRE, h * D:(h + 1) * D] = o[2 * SEG + e * PRE:2 * SEG + (e + 1) * PRE, :]

            parts = []

            def oproj(g):
                lhs = jnp.concatenate([ctx[h] for h in range(g * HG, (g + 1) * HG)], axis=1)
                parts.append(jnp.dot(lhs, wogroup(g), preferred_element_type=f32))

            for t in range(G + 2):
                if t < G:
                    attend(t)
                if t >= 2:
                    oproj(t - 2)
            acc = parts[0]
            for a in parts[1:]:
                acc = acc + a
            accb = acc.astype(bf16)
            out_v[pl.ds(pl.multiple_of(SEG * s + PRE, 8), T), DM:2 * DM] = accb[0:T, :]
            return accb[T:, :].astype(f32), ctx[H - 1]

        KP = H * D // OUTER

        def partial(rows, i):
            return jnp.dot(rows, _unpack(wob_v[i * KP // 2:(i + 1) * KP // 2, :]), preferred_element_type=f32)

        def finish(j, r):
            r = r.astype(bf16)
            for sg in range(OUTER):
                r0 = pl.multiple_of((j * OUTER + sg) * SEG, SEG)
                out_v[pl.ds(r0, PRE), DM:2 * DM] = r[sg * PRE:(sg + 1) * PRE, :]

        def after(x, late):
            u = _pack(late[0:2 * OUTER * PRE // 2, :])
            zero = (u >> 31) & (~u >> 31)
            return _unpack(_pack(x) | jnp.concatenate([zero] * (x.shape[1] // D), axis=1))

        def outer(j, mem):
            prev = post_v[...].astype(bf16)
            acc = partial(prev[:, 0:KP], 0)
            for i in range(OUTER):
                mem, late = step(j * OUTER + i, i, mem)
                if i + 1 < OUTER:
                    acc = acc + partial(after(prev[:, (i + 1) * KP:(i + 2) * KP], late), i + 1)
            finish(jnp.maximum(j - 1, 0), acc)

            @pl.when(j > 0)
            def _():
                out_copy(j - 1).start()
            return mem
        with _scope("b_loop"):
            post_v[...] = jnp.zeros(post_v.shape, f32)
            jax.lax.fori_loop(0, NOUTER, outer, mem_v[0:MEM, :].astype(f32))
            finish(NOUTER - 1, jnp.dot(post_v[...].astype(bf16), _unpack(wob_v[...]), preferred_element_type=f32))
            out_copy(NOUTER - 1).start()
        with _scope("b_outwait"):
            for j in range(NOUTER):
                out_copy(j).wait()

    pl.run_scoped(
        phase_b,
        pltpu.VMEM((OUTER * PRE, H * D), f32),
    )


@jax.jit
def pallas_concat_heads__compressed_kv_cla__memory_aug_recurrent_mem_tr__prompt_kernel(
    A_x: jax.Array,
    A_c_kv: jax.Array,
    A_w_q: jax.Array,
    A_w_uk: jax.Array,
    A_w_uv: jax.Array,
    A_w_o: jax.Array,
    B_x: jax.Array,
    B_mem0: jax.Array,
    B_Wq: jax.Array,
    B_Wk: jax.Array,
    B_Wv: jax.Array,
    B_Wo: jax.Array,
    B_seg_len=SEG,
):
    def t2(x):
        return jnp.transpose(x, (0, 2, 1)).reshape(DM, S)

    def w3(w):
        return w.reshape(w.shape[0] // 2, 2 * H, D)

    def wo3(w):
        return jnp.transpose(w, (0, 2, 1))

    any_spec = pl.BlockSpec(memory_space=pl.ANY)
    out = pl.pallas_call(
        _kernel,
        out_shape=jax.ShapeDtypeStruct((S, 2 * DM), bf16),
        in_specs=[any_spec] * 12,
        out_specs=any_spec,
        scratch_shapes=[
            pltpu.VMEM((S, 2 * DM), bf16),
            pltpu.VMEM((S, DM), bf16),
            pltpu.VMEM((NSEG * PRE, DM), bf16),
            pltpu.VMEM((3, 2, HP, DM // 2, D), u32),
            pltpu.VMEM((H * D // 2, DM), u32),
            pltpu.VMEM((8 * MEM, DM), bf16),
            pltpu.VMEM((H, S // 2, D), u32),
            pltpu.VMEM((H, S // 2, D), u32),
            pltpu.VMEM((H, S // 2, D), u32),
            pltpu.SemaphoreType.DMA((NSEM,)),
        ],
        compiler_params=pltpu.CompilerParams(vmem_limit_bytes=126 * 1024 * 1024),
    )(t2(A_x), A_c_kv.reshape(S, DC), w3(A_w_q), w3(A_w_uk), w3(A_w_uv), wo3(A_w_o),
      t2(B_x), B_mem0.reshape(MEM, DM), w3(B_Wq), w3(B_Wk), w3(B_Wv), wo3(B_Wo))
    return out.reshape(1, S, 2 * DM)
```

```python
import contextlib

import jax
import jax.numpy as jnp
import jax.experimental.pallas as pl
import jax.experimental.pallas.tpu as pltpu

S = 2048
DM = 576
DC = 512
H = 32
D = 128
MEM = 8
SEG = 32
L = MEM + SEG
NSEG = S // SEG
HP = H // 2

LOG2E = 1.4426950408889634
QSCALE = D ** -0.5 * LOG2E
NEG = -1.0e9 * LOG2E

TQ = 128
UH = 4
ANCHOR_LAG = 2000
ANCHOR_MIN = 6
RB = 512
HG = 4
G = H // HG
GW = HG * 3 * D
PRE = 8
T = SEG - PRE
OUTER = 4
NOUTER = NSEG // OUTER

bf16 = jnp.bfloat16
f32 = jnp.float32
u32 = jnp.uint32
NT = (((1,), (1,)), ((), ()))

SEM_CKV = 0
SEM_XAT = 4
SEM_XBT = 5
SEM_MEM = 6
SEM_WOA = 7
SEM_WOB = 8
SEM_OUT = 9
SEM_WALL = SEM_OUT + NOUTER
SEM_W = SEM_WALL + 4
NSEM = SEM_W + 2 + HP // 2

_PROFILE = False


def _scope(name):
    return jax.named_scope(name) if _PROFILE else contextlib.nullcontext()


def _unpack(w32):
    return pltpu.bitcast(w32, bf16)


def _pack(x):
    return pltpu.bitcast(x, u32)


def _recip(l):
    r = pl.reciprocal(l, approx=True)
    return r * (2.0 - l * r)


def _kernel(xat_hbm, ckv_hbm, wqa_hbm, wuk_hbm, wuv_hbm, woa_hbm,
            xbt_hbm, mem0_hbm, wqb_hbm, wkb_hbm, wvb_hbm, wob_hbm,
            out_hbm,
            out_v, xb_v, xpre_v, wb_v, wob_v, mem_v, q_v, k_v, v_v, sem):

    def w_copy(w_hbm, dst, slot, par, hp):
        return pltpu.make_async_copy(w_hbm.bitcast(u32).at[:, par * HP + hp, :], dst.at[par, hp], sem.at[slot])

    def w_start_shared(w_hbm, dst, widx, hps):
        for hp in hps:
            for par in range(2):
                w_copy(w_hbm, dst, SEM_WALL + widx, par, hp).start()

    def w_wait_shared(dst, widx):
        pltpu.make_async_copy(dst, dst, sem.at[SEM_WALL + widx]).wait()

    def w_combine(dst, hp):
        a = dst[0, hp]
        b = dst[1, hp]
        ev = (a & u32(0xFFFF)) | (b << 16)
        od = (a >> 16) | (b & u32(0xFFFF0000))
        return ev, od

    def w_pair(dst, hp):
        return jnp.concatenate(w_combine(dst, hp), axis=1)

    wb_hbm = (wqb_hbm, wkb_hbm, wvb_hbm)

    def pre_ref(j):
        n = NSEG * PRE
        return q_v.at[j // 2, (j % 2) * n:(j % 2 + 1) * n, :]

    def b_pre():
        lane = jax.lax.broadcasted_iota(jnp.int32, (1, GW), 1)
        colscale = jnp.where(lane % (3 * D) < D, QSCALE, 1.0).astype(f32)

        with _scope("b_pre"):
            for g in range(G):
                cols = {}
                for hp in range(g * HG // 2, (g + 1) * HG // 2):
                    for t in range(3):
                        ev, od = w_combine(wb_v.at[t], hp)
                        wb_v[t, 0, hp] = ev
                        wb_v[t, 1, hp] = od
                        cols[2 * hp, t] = ev
                        cols[2 * hp + 1, t] = od
                w = _unpack(jnp.concatenate(
                    [cols[h, t] for h in range(g * HG, (g + 1) * HG) for t in range(3)], axis=1))
                r = jnp.dot(xpre_v[...], w, preferred_element_type=f32) * colscale
                for hp in range(g * HG // 2, (g + 1) * HG // 2):
                    for t in range(3):
                        c0 = (2 * hp % HG) * 3 * D + t * D
                        two = [r[:, c:c + D].reshape(NSEG, 1, PRE, D) for c in (c0, c0 + 3 * D)]
                        two = jnp.concatenate(two, axis=1).reshape(NSEG * 2 * PRE, D)
                        pre_ref(hp * 3 + t)[...] = _pack(two.astype(bf16))


    def phase_a(woa_v, xbt_v, wobt_v):
        woa_cp = pltpu.make_async_copy(woa_hbm.bitcast(u32), woa_v, sem.at[SEM_WOA])
        xbt_cp = pltpu.make_async_copy(xbt_hbm, xbt_v, sem.at[SEM_XBT])
        mem_cp = pltpu.make_async_copy(mem0_hbm, mem_v.at[0:MEM, :], sem.at[SEM_MEM])
        wob_cp = pltpu.make_async_copy(wob_hbm.bitcast(u32), wobt_v, sem.at[SEM_WOB])

        def store_heads(dst_v, hp, rb, r):
            r = r.astype(bf16)
            rows = slice(rb * RB // 2, (rb + 1) * RB // 2)
            dst_v[2 * hp, rows, :] = _pack(r[:, 0:D])
            dst_v[2 * hp + 1, rows, :] = _pack(r[:, D:2 * D])

        def projections(ckv_v, xat_v, xa_v, wuk_v, wuv_v, wqa_v, wk_v, wq0_v):
            nck = S // RB
            def group(j):
                items = [] if j == 0 else [(wuv_hbm, wuv_v, 2 * j)]
                items += [(wuk_hbm, wuk_v, 2 * j + 1), (wuv_hbm, wuv_v, 2 * j + 1)]
                return items + ([(wuk_hbm, wuk_v, 2 * j + 2)] if 2 * j + 2 < HP else [])

            def group_start(j):
                for w_hbm, dst, hp in group(j):
                    for par in range(2):
                        w_copy(w_hbm, dst, SEM_W + 2 + j, par, hp).start()

            def group_wait(j, n):
                part = wuk_v.at[:, 0:n]
                pltpu.make_async_copy(part, part, sem.at[SEM_W + 2 + j]).wait()

            def first_copies(w_hbm, dst, slot):
                return [w_copy(w_hbm, dst, SEM_W + slot, par, 0) for par in range(2)]

            def first_wait(dst, slot):
                part = dst.at[:, 0:1]
                pltpu.make_async_copy(part, part, sem.at[SEM_W + slot]).wait()

            def ckv_cp(j):
                return pltpu.make_async_copy(ckv_hbm.at[j * RB:(j + 1) * RB, :],
                                             ckv_v.at[j * RB:(j + 1) * RB, :], sem.at[SEM_CKV + j])
            xat_cp = pltpu.make_async_copy(xat_hbm, xat_v, sem.at[SEM_XAT])
            ngrp = HP // 2

            with _scope("a_issue0"):
                for cp in first_copies(wuk_hbm, wuk_v, 0):
                    cp.start()
                ckv_cp(0).start()
                for cp in first_copies(wuv_hbm, wuv_v, 1):
                    cp.start()
                for j in range(1, nck):
                    ckv_cp(j).start()
                for j in range(ngrp - 1):
                    group_start(j)

            def project(dst_v, lhs_v, w, hp, rb, scale=None):
                r = jnp.dot(lhs_v[rb * RB:(rb + 1) * RB, :], _unpack(w), preferred_element_type=f32)
                store_heads(dst_v, hp, rb, r if scale is None else r * scale)

            def project_all(dst_v, w, hp):
                for rb in range(nck):
                    project(dst_v, ckv_v, w, hp, rb)

            def kv_first():
                first_wait(wuk_v, 0)
                ckv_cp(0).wait()
                wk = w_pair(wuk_v, 0)
                project(k_v, ckv_v, wk, 0, 0)
                first_wait(wuv_v, 1)
                wv = w_pair(wuv_v, 0)
                project(v_v, ckv_v, wv, 0, 0)
                ckv_cp(1).wait()
                project(k_v, ckv_v, wk, 0, 1)
                project(v_v, ckv_v, wv, 0, 1)
                for rb in range(2, nck):
                    ckv_cp(rb).wait()
                for rb in range(2, nck):
                    project(k_v, ckv_v, wk, 0, rb)
                    project(v_v, ckv_v, wv, 0, rb)
                group_wait(0, len(group(0)))
                project_all(k_v, w_pair(wuk_v, 1), 1)
                wk_v[...] = w_pair(wuk_v, 2)
                project_all(v_v, w_pair(wuv_v, 1), 1)

            def kv_body(j, c, last=False):
                if not last:
                    @pl.when(j == 2)
                    def _():
                        xat_cp.start()
                        group_start(ngrp - 1)
                        w_start_shared(wqa_hbm, wqa_v, 0, range(HP))
                group_wait(j, len(group(ngrp - 1 if last else 1)))
                if last:
                    xat_cp.wait()
                    w_wait_shared(wqa_v, 0)
                project_all(k_v, wk_v[...], 2 * j)
                project_all(v_v, w_pair(wuv_v, 2 * j), 2 * j)
                project_all(k_v, w_pair(wuk_v, 2 * j + 1), 2 * j + 1)
                if last:
                    wq0_v[...] = w_pair(wqa_v, 0)
                    for t in range(S // D):
                        xa_v[t * D:(t + 1) * D, :] = xat_v[:, t * D:(t + 1) * D].T
                else:
                    wk_v[...] = w_pair(wuk_v, 2 * j + 2)
                project_all(v_v, w_pair(wuv_v, 2 * j + 1), 2 * j + 1)
                return c

            with _scope("a_kvproj"):
                kv_first()
                jax.lax.fori_loop(1, ngrp - 1, kv_body, 0)
                kv_body(ngrp - 1, 0, last=True)

            woa_cp.start()
            wob_cp.start()
            xbt_cp.start()
            mem_cp.start()
            w_start_shared(wqb_hbm, wb_v.at[0], 1, range(HP))
            w_start_shared(wkb_hbm, wb_v.at[1], 2, range(HP // 2))

            with _scope("a_qproj"):
                for hp in range(HP):
                    wq = wq0_v[...] if hp == 0 else w_pair(wqa_v, hp)
                    for rb in range(nck):
                        project(q_v, xa_v, wq, hp, rb, QSCALE)

        pl.run_scoped(
            projections,
            pltpu.VMEM((S, DC), bf16),
            pltpu.VMEM((DM, S), bf16),
            pltpu.VMEM((S, DM), bf16),
            pltpu.VMEM((2, HP, DC // 2, D), u32),
            pltpu.VMEM((2, HP, DC // 2, D), u32),
            pltpu.VMEM((2, HP, DM // 2, D), u32),
            pltpu.VMEM((DC // 2, 2 * D), u32),
            pltpu.VMEM((DM // 2, 2 * D), u32),
        )

        def attention(c_v, s_v):
            row = jax.lax.broadcasted_iota(jnp.int32, (TQ, TQ), 0)
            col = jax.lax.broadcasted_iota(jnp.int32, (TQ, TQ), 1)
            tri = col <= row
            nb = S // TQ
            hq = TQ // 2
            npiece = 2
            pw = S // npiece

            def qk_piece(h, j):
                q = _unpack(q_v[h, (nb - 1) * hq:nb * hq, :])
                k = _unpack(k_v[h, j * pw // 2:(j + 1) * pw // 2, :])
                s_v[:, j * pw:(j + 1) * pw] = jax.lax.dot_general(q, k, NT, preferred_element_type=f32)

            def qk(h, i, j0=0, j1=None):
                j1 = i + 1 if j1 is None else j1
                q = _unpack(q_v[h, i * hq:(i + 1) * hq, :])
                k = _unpack(k_v[h, j0 * hq:j1 * hq, :])
                return jax.lax.dot_general(q, k, NT, preferred_element_type=f32)

            def anchor_plan():
                ops = []
                for e in range(UH):
                    for i in range(nb - 1, -1, -1):
                        if i > 0:
                            ops.append(("qk", e, i - 1, 32 * i))
                        if i < npiece:
                            ops.append(("piece", e, i, 32 * nb // npiece))
                        ops.append(("pv", e, i, 32 * (i + 1)))
                t, start, end = 0, [], []
                for op in ops:
                    start.append(t)
                    t += op[3]
                    end.append(t)
                plan = {}
                for a, op in enumerate(ops):
                    if op[0] != "pv" or op[2] < ANCHOR_MIN:
                        continue
                    for b in range(a + 1, len(ops)):
                        if ops[b][0] == "qk" and start[b] >= end[a] + ANCHOR_LAG:
                            plan.setdefault((ops[b][1], ops[b][2]), []).append((op[1], op[2]))
                            break
                return plan

            def heads(j, c):
                @pl.when(j == 0)
                def _():
                    w_start_shared(wkb_hbm, wb_v.at[1], 2, range(HP // 2, HP))
                    w_start_shared(wvb_hbm, wb_v.at[2], 3, range(HP))

                plan = anchor_plan()

                def gated_qk(e, i):
                    h = j * UH + e
                    if (e, i) not in plan:
                        return qk(h, i)
                    w = None
                    for ea, ia in plan[e, i]:
                        u = c_v[j * UH + ea, ia * hq:(ia + 1) * hq, :]
                        for r in range(0, hq, 8):
                            w = u[r:r + 8] if w is None else w | u[r:r + 8]
                    zero = (w >> 31) >> 1
                    q = q_v[h, i * hq:(i + 1) * hq, :]
                    q = _unpack(jnp.concatenate([q[0:8] | zero, q[8:]], axis=0))
                    k = _unpack(k_v[h, 0:(i + 1) * hq, :])
                    return jax.lax.dot_general(q, k, NT, preferred_element_type=f32)

                s_next = s_v[...]
                for e in range(UH):
                    h = j * UH + e
                    hn = jnp.minimum(h + 1, H - 1) if e == UH - 1 else h + 1
                    pieces = []
                    for i in range(nb - 1, -1, -1):
                        s = s_next
                        if i > 0:
                            s_next = gated_qk(e, i - 1)
                        if i < npiece:
                            if e == UH - 1:
                                qk_piece(hn, npiece - 1 - i)
                            else:
                                jj = npiece - 1 - i
                                pieces.append(qk(hn, nb - 1, jj * nb // npiece, (jj + 1) * nb // npiece))
                        sd = jnp.where(tri, s[:, i * TQ:], NEG)
                        s = jnp.concatenate([s[:, :i * TQ], sd], axis=1) if i > 0 else sd
                        m = jnp.max(s, axis=1, keepdims=True)
                        p = jnp.exp2(s - m)
                        l = jnp.sum(p, axis=1, keepdims=True)
                        v = _unpack(v_v[h, 0:(i + 1) * hq, :])
                        o = jnp.dot(p.astype(bf16), v, preferred_element_type=f32)
                        c_v[h, i * hq:(i + 1) * hq, :] = _pack((o * _recip(l)).astype(bf16))
                    if e < UH - 1:
                        s_next = jnp.concatenate(pieces, axis=1)
                return c
            with _scope("a_attn"):
                for j in range(npiece):
                    qk_piece(0, j)
                jax.lax.fori_loop(0, H // UH, heads, 0)

            woa_cp.wait()
            wob_cp.wait()
            xbt_cp.wait()
            mem_cp.wait()
            for t in range(3):
                w_wait_shared(wb_v.at[t], 1 + t)
            nrb = S // RB

            def oproj(rb, c):
                for j in range(HP // nrb):
                    hp = rb * (HP // nrb) + j
                    t0 = hp * D
                    xb = xbt_v[:, t0:t0 + D].T
                    xb_v[t0:t0 + D, :] = xb
                    for sg in range(D // SEG):
                        p0 = (hp * (D // SEG) + sg) * PRE
                        xpre_v[p0:p0 + PRE, :] = xb[sg * SEG:sg * SEG + PRE, :]
                for hh in range(H // nrb):
                    h = rb * (H // nrb) + hh
                    wob_v[h * (D // 2):(h + 1) * (D // 2), :] = _pack(_unpack(wobt_v[h]).T)
                r0 = rb * (RB // 2)
                ctx = _unpack(jnp.concatenate([c_v[h, r0:r0 + RB // 2, :] for h in range(H)], axis=1))
                wo = _unpack(jnp.concatenate([woa_v[h] for h in range(H)], axis=1))
                for t in range(RB // D):
                    r = jax.lax.dot_general(wo, ctx[t * D:(t + 1) * D, :], NT, preferred_element_type=f32)
                    out_v[rb * RB + t * D:rb * RB + (t + 1) * D, 0:DM] = r.T.astype(bf16)
                return c
            with _scope("a_oproj"):
                for rb in range(nrb):
                    oproj(rb, 0)
            b_pre()

        pl.run_scoped(
            attention,
            pltpu.VMEM((H, S // 2, D), u32),
            pltpu.VMEM((TQ, S), f32),
        )

    pl.run_scoped(
        phase_a,
        pltpu.VMEM((H, DM // 2, D), u32),
        pltpu.VMEM((DM, S), bf16),
        pltpu.VMEM((H, DM // 2, D), u32),
    )

    def out_copy(j):
        rows = pl.ds(pl.multiple_of(j * (OUTER * SEG), OUTER * SEG), OUTER * SEG)
        return pltpu.make_async_copy(out_v.at[rows, :], out_hbm.at[rows, :], sem.at[SEM_OUT + j])

    def phase_b(post_v):
        lane = jax.lax.broadcasted_iota(jnp.int32, (1, GW), 1)
        colscale = jnp.where(lane % (3 * D) < D, QSCALE, 1.0).astype(f32)

        def wgroup(g):
            return _unpack(jnp.concatenate(
                [wb_v[t, h % 2, h // 2] for h in range(g * HG, (g + 1) * HG) for t in range(3)], axis=1))

        def wogroup(g):
            return _unpack(wob_v[g * HG * D // 2:(g + 1) * HG * D // 2, :])

        ri = jax.lax.broadcasted_iota(jnp.int32, (2 * L, 2 * L), 0)
        ci = jax.lax.broadcasted_iota(jnp.int32, (2 * L, 2 * L), 1)

        def second(i):
            return jnp.where(i < 2 * SEG, i // SEG, (i - 2 * SEG) // PRE)

        def pos(i):
            j = i % SEG
            return jnp.where(i < 2 * SEG, jnp.where(j < T, j + (MEM + PRE), j - T), MEM + i % PRE)
        same = second(ri) == second(ci)
        mask = same & ((pos(ri) < MEM) | (pos(ri) >= pos(ci)))
        fill = jnp.where(same, NEG, -jnp.inf).astype(f32)

        def step(s, slot, mem):
            xt = xb_v[pl.ds(pl.multiple_of(SEG * s + PRE, 8), T), :]
            l1 = jnp.concatenate([xt.astype(f32), mem], axis=0).astype(bf16)
            p0 = pl.multiple_of(PRE * s, 8)
            proj = [(jnp.dot(l1, wgroup(g), preferred_element_type=f32) * colscale).astype(bf16)
                    for g in range(G)]

            def rows(hp, t):
                g, c0 = 2 * hp // HG, (2 * hp % HG) * 3 * D + t * D
                return jnp.concatenate([proj[g][:, c0:c0 + D], proj[g][:, c0 + 3 * D:c0 + 4 * D],
                                        _unpack(pre_ref(hp * 3 + t)[pl.ds(p0, PRE), :])], axis=0)

            scores = [jax.lax.dot_general(rows(hp, 0), rows(hp, 1), NT, preferred_element_type=f32)
                      for hp in range(HP)]
            ctx = {}

            def attend(g):
                for hp in range(g * HG // 2, (g + 1) * HG // 2):
                    sc = jnp.where(mask, scores[hp], fill)
                    m = jnp.max(sc, axis=1, keepdims=True)
                    p = jnp.exp2(sc - m)
                    l = jnp.sum(p, axis=1, keepdims=True)
                    o = jnp.dot(p.astype(bf16), rows(hp, 2), preferred_element_type=f32) * _recip(l)
                    for e in range(2):
                        h = 2 * hp + e
                        ctx[h] = o[e * SEG:(e + 1) * SEG, :].astype(bf16)
                        post_v[slot * PRE:(slot + 1) * PRE, h * D:(h + 1) * D] = o[2 * SEG + e * PRE:2 * SEG + (e + 1) * PRE, :]

            parts = []

            def oproj(g):
                lhs = jnp.concatenate([ctx[h] for h in range(g * HG, (g + 1) * HG)], axis=1)
                parts.append(jnp.dot(lhs, wogroup(g), preferred_element_type=f32))

            for t in range(G + 2):
                if t < G:
                    attend(t)
                if t >= 2:
                    oproj(t - 2)
            acc = parts[0]
            for a in parts[1:]:
                acc = acc + a
            accb = acc.astype(bf16)
            out_v[pl.ds(pl.multiple_of(SEG * s + PRE, 8), T), DM:2 * DM] = accb[0:T, :]
            return accb[T:, :].astype(f32), ctx[H - 1]

        KP = H * D // OUTER

        def partial(rows, i):
            return jnp.dot(rows, _unpack(wob_v[i * KP // 2:(i + 1) * KP // 2, :]), preferred_element_type=f32)

        def finish(j, r):
            r = r.astype(bf16)
            for sg in range(OUTER):
                r0 = pl.multiple_of((j * OUTER + sg) * SEG, SEG)
                out_v[pl.ds(r0, PRE), DM:2 * DM] = r[sg * PRE:(sg + 1) * PRE, :]

        def after(x, late):
            u = _pack(late[0:2 * OUTER * PRE // 2, :])
            zero = (u >> 31) & (~u >> 31)
            return _unpack(_pack(x) | jnp.concatenate([zero] * (x.shape[1] // D), axis=1))

        def outer(j, mem):
            prev = post_v[...].astype(bf16)
            acc = partial(prev[:, 0:KP], 0)
            for i in range(OUTER):
                mem, late = step(j * OUTER + i, i, mem)
                if i + 1 < OUTER:
                    acc = acc + partial(after(prev[:, (i + 1) * KP:(i + 2) * KP], late), i + 1)
            finish(jnp.maximum(j - 1, 0), acc)

            @pl.when(j > 0)
            def _():
                out_copy(j - 1).start()
            return mem
        with _scope("b_loop"):
            post_v[...] = jnp.zeros(post_v.shape, f32)
            jax.lax.fori_loop(0, NOUTER, outer, mem_v[0:MEM, :].astype(f32))
            finish(NOUTER - 1, jnp.dot(post_v[...].astype(bf16), _unpack(wob_v[...]), preferred_element_type=f32))
            out_copy(NOUTER - 1).start()
        with _scope("b_outwait"):
            for j in range(NOUTER):
                out_copy(j).wait()

    pl.run_scoped(
        phase_b,
        pltpu.VMEM((OUTER * PRE, H * D), f32),
    )


@jax.jit
def pallas_concat_heads__compressed_kv_cla__memory_aug_recurrent_mem_tr__prompt_kernel(
    A_x: jax.Array,
    A_c_kv: jax.Array,
    A_w_q: jax.Array,
    A_w_uk: jax.Array,
    A_w_uv: jax.Array,
    A_w_o: jax.Array,
    B_x: jax.Array,
    B_mem0: jax.Array,
    B_Wq: jax.Array,
    B_Wk: jax.Array,
    B_Wv: jax.Array,
    B_Wo: jax.Array,
    B_seg_len=SEG,
):
    def t2(x):
        return jnp.transpose(x, (0, 2, 1)).reshape(DM, S)

    def w3(w):
        return w.reshape(w.shape[0] // 2, 2 * H, D)

    def wo3(w):
        return jnp.transpose(w, (0, 2, 1))

    any_spec = pl.BlockSpec(memory_space=pl.ANY)
    out = pl.pallas_call(
        _kernel,
        out_shape=jax.ShapeDtypeStruct((S, 2 * DM), bf16),
        in_specs=[any_spec] * 12,
        out_specs=any_spec,
        scratch_shapes=[
            pltpu.VMEM((S, 2 * DM), bf16),
            pltpu.VMEM((S, DM), bf16),
            pltpu.VMEM((NSEG * PRE, DM), bf16),
            pltpu.VMEM((3, 2, HP, DM // 2, D), u32),
            pltpu.VMEM((H * D // 2, DM), u32),
            pltpu.VMEM((8 * MEM, DM), bf16),
            pltpu.VMEM((H, S // 2, D), u32),
            pltpu.VMEM((H, S // 2, D), u32),
            pltpu.VMEM((H, S // 2, D), u32),
            pltpu.SemaphoreType.DMA((NSEM,)),
        ],
        compiler_params=pltpu.CompilerParams(vmem_limit_bytes=126 * 1024 * 1024),
    )(t2(A_x), A_c_kv.reshape(S, DC), w3(A_w_q), w3(A_w_uk), w3(A_w_uv), wo3(A_w_o),
      t2(B_x), B_mem0.reshape(MEM, DM), w3(B_Wq), w3(B_Wk), w3(B_Wv), wo3(B_Wo))
    return out.reshape(1, S, 2 * DM)
```

```python
import contextlib

import jax
import jax.numpy as jnp
import jax.experimental.pallas as pl
import jax.experimental.pallas.tpu as pltpu

S = 2048
DM = 576
DC = 512
H = 32
D = 128
MEM = 8
SEG = 32
L = MEM + SEG
NSEG = S // SEG
HP = H // 2

LOG2E = 1.4426950408889634
QSCALE = D ** -0.5 * LOG2E
NEG = -1.0e9 * LOG2E

TQ = 128
UH = 4
ANCHOR_LAG = 2000
ANCHOR_MIN = 6
RB = 512
HG = 4
G = H // HG
GW = HG * 3 * D
PRE = 8
T = SEG - PRE
OUTER = 4
NOUTER = NSEG // OUTER

bf16 = jnp.bfloat16
f32 = jnp.float32
u32 = jnp.uint32
NT = (((1,), (1,)), ((), ()))

SEM_CKV = 0
SEM_XAT = 5
SEM_XBT = 6
SEM_MEM = 7
SEM_WOA = 8
SEM_WOB = 9
SEM_OUT = 10
SEM_WALL = SEM_OUT + NOUTER
SEM_W = SEM_WALL + 4
NSEM = SEM_W + 3 + HP // 2

_PROFILE = False


def _scope(name):
    return jax.named_scope(name) if _PROFILE else contextlib.nullcontext()


def _unpack(w32):
    return pltpu.bitcast(w32, bf16)


def _pack(x):
    return pltpu.bitcast(x, u32)


def _lo(w):
    return pltpu.bitcast(w << 16, f32)


def _hi(w):
    return pltpu.bitcast(w & u32(0xFFFF0000), f32)


def _strassen_lhs(a11, a12, a21, a22):
    return [a11 + a22, a21 + a22, a11, a22, a11 + a12, a21 - a11, a12 - a22]


def _strassen_rhs(b11, b12, b21, b22):
    return [b11 + b22, b11, b12 - b22, b21 - b11, b22, b11 + b12, b21 + b22]


def _sum_words(combine, x11, x12, x21, x22, raw_idx, raw):
    lo = combine(_lo(x11), _lo(x12), _lo(x21), _lo(x22))
    hi = combine(_hi(x11), _hi(x12), _hi(x21), _hi(x22))
    words = [pltpu.bitcast(pltpu.pack_elementwise([a, b], packed_dtype=bf16), u32) for a, b in zip(lo, hi)]
    for i, r in zip(raw_idx, raw):
        words[i] = r
    return words


def _strassen(lhs, rhs, dims=(((1,), (0,)), ((), ())), order=0):
    def m(i):
        return jax.lax.dot_general(lhs(i - 1), rhs(i - 1), dims, preferred_element_type=f32)
    if order == 0:
        m1 = m(1)
        m2 = m(2)
        c22 = m1 - m2
        m4 = m(4)
        c11 = m1 + m4
        c21 = m2 + m4
        c22 = c22 + m(6)
        m3 = m(3)
        c22 = c22 + m3
        m5 = m(5)
        c11 = c11 - m5
        c12 = m3 + m5
        c11 = c11 + m(7)
        return c11, c12, c21, c22
    m3 = m(3)
    m4 = m(4)
    m5 = m(5)
    c12 = m3 + m5
    c11 = m4 - m5
    m2 = m(2)
    c21 = m4 + m2
    c22 = m3 - m2
    m1 = m(1)
    c11 = c11 + m1
    c22 = c22 + m1
    c22 = c22 + m(6)
    c11 = c11 + m(7)
    return c11, c12, c21, c22


def _rhs_words(s0, s1, z0, z1):
    per = [_strassen_rhs(_lo(s), _hi(s), _lo(z), _hi(z)) for s, z in ((s0, z0), (s1, z1))]
    words = [pltpu.bitcast(pltpu.pack_elementwise([per[0][i], per[1][i]], packed_dtype=bf16), u32)
             for i in range(7)]
    words[1] = (s0 & u32(0xFFFF)) | (s1 << 16)
    words[4] = (z0 >> 16) | (z1 & u32(0xFFFF0000))
    return words


def _recip(l):
    r = pl.reciprocal(l, approx=True)
    return r * (2.0 - l * r)


def _kernel(xat_hbm, ckv_hbm, wqa_hbm, wuk_hbm, wuv_hbm, woa_hbm,
            xbt_hbm, mem0_hbm, wqb_hbm, wkb_hbm, wvb_hbm, wob_hbm,
            out_hbm,
            out_v, xb_v, xpre_v, wb_v, wob_v, mem_v, q_v, k_v, v_v, sem):

    def w_copy(w_hbm, dst, slot, par, hp):
        return pltpu.make_async_copy(w_hbm.bitcast(u32).at[:, par * HP + hp, :], dst.at[par, hp], sem.at[slot])

    def w_start_shared(w_hbm, dst, widx, hps):
        for hp in hps:
            for par in range(2):
                w_copy(w_hbm, dst, SEM_WALL + widx, par, hp).start()

    def w_wait_shared(dst, widx):
        pltpu.make_async_copy(dst, dst, sem.at[SEM_WALL + widx]).wait()

    def w_combine(dst, hp):
        a = dst[0, hp]
        b = dst[1, hp]
        ev = (a & u32(0xFFFF)) | (b << 16)
        od = (a >> 16) | (b & u32(0xFFFF0000))
        return ev, od

    def w_pair(dst, hp):
        return jnp.concatenate(w_combine(dst, hp), axis=1)

    wb_hbm = (wqb_hbm, wkb_hbm, wvb_hbm)

    def pre_ref(j):
        n = NSEG * PRE
        return q_v.at[j // 2, (j % 2) * n:(j % 2 + 1) * n, :]

    def lp_prep(lp_v):
        nr = NSEG * PRE // 2
        kh = DC // 2
        x = xpre_v[:, 0:DC].astype(f32)
        for i, o in enumerate(_strassen_lhs(x[:nr, :kh], x[:nr, kh:], x[nr:, :kh], x[nr:, kh:])):
            lp_v[i] = _pack(o.astype(bf16))

    def b_pre(lp_v):
        nr = NSEG * PRE // 2
        kh = DC // 2
        n = kh // 2
        PG = 1
        SP = nr
        with _scope("b_pre"):
            for g in range(HP // PG):
                ts, rem = [], [[], []]
                combos = [(hp, t) for hp in range(g * PG, (g + 1) * PG) for t in range(3)]
                for hp, t in combos:
                    s0, s1 = wb_v[t, 0, hp], wb_v[t, 1, hp]
                    ev = (s0 & u32(0xFFFF)) | (s1 << 16)
                    od = (s0 >> 16) | (s1 & u32(0xFFFF0000))
                    wb_v[t, 0, hp] = ev
                    wb_v[t, 1, hp] = od
                    ts.append(_rhs_words(s0[:n], s1[:n], s0[n:2 * n], s1[n:2 * n]))
                    rem[0].append(ev[2 * n:])
                    rem[1].append(od[2 * n:])
                tw = [jnp.concatenate([x_[i] for x_ in ts], axis=1) for i in range(7)]
                remw = _unpack(jnp.concatenate(rem[0] + rem[1], axis=1))
                nc = len(combos)
                for sub in range(nr // SP):
                    r0 = sub * SP
                    c = _strassen(lambda i: _unpack(lp_v[i, r0 // 2:(r0 + SP) // 2, :]), lambda i: _unpack(tw[i]))
                    for half in range(2):
                        x0 = half * nr + r0
                        r = jnp.dot(xpre_v[x0:x0 + SP, DC:DM], remw, preferred_element_type=f32)
                        r = jnp.concatenate([c[2 * half], c[2 * half + 1]], axis=1) + r
                        for ci_, (hp, t) in enumerate(combos):
                            two = [r[:, cc * D:(cc + 1) * D] for cc in (ci_, nc + ci_)]
                            if t == 0:
                                two = [y * QSCALE for y in two]
                            two = [y.reshape(SP // PRE, 1, PRE, D) for y in two]
                            two = jnp.concatenate(two, axis=1).reshape(2 * SP, D)
                            pre_ref(hp * 3 + t)[x0:x0 + SP, :] = _pack(two.astype(bf16))


    def phase_a(woa_v, xbt_v, wobt_v, lp_v):
        woa_cp = pltpu.make_async_copy(woa_hbm.bitcast(u32), woa_v, sem.at[SEM_WOA])
        xbt_cp = pltpu.make_async_copy(xbt_hbm, xbt_v, sem.at[SEM_XBT])
        mem_cp = pltpu.make_async_copy(mem0_hbm, mem_v.at[0:MEM, :], sem.at[SEM_MEM])
        wob_cp = pltpu.make_async_copy(wob_hbm.bitcast(u32), wobt_v, sem.at[SEM_WOB])

        def projections(ckv_v, xat_v, xa_v, wuk_v, wuv_v, wqa_v, tkv_v, lq_v, la_v):
            UR = 2 * D
            NU = S // UR
            kh = DC // 2
            ngrp = HP // 2

            def batch_start(pairs, slot):
                for hp in pairs:
                    for w_hbm, dst in ((wuk_hbm, wuk_v), (wuv_hbm, wuv_v)):
                        for par in range(2):
                            w_copy(w_hbm, dst, SEM_W + slot, par, hp).start()

            def batch_wait(npairs, slot):
                part = wuk_v.at[:, 0:2 * npairs]
                pltpu.make_async_copy(part, part, sem.at[SEM_W + slot]).wait()

            def group(j):
                return [hp for hp in (2 * j + 1, 2 * j + 2) if hp < HP]

            def first_copies(w_hbm, dst, slot):
                return [w_copy(w_hbm, dst, SEM_W + slot, par, 0) for par in range(2)]

            def first_wait(dst, slot):
                part = dst.at[:, 0:1]
                pltpu.make_async_copy(part, part, sem.at[SEM_W + slot]).wait()

            pieces = [(0, 1), (1, 2), (2, 4), (4, 6), (6, 8)]

            def ckv_cp(j):
                rows = slice(pieces[j][0] * UR, pieces[j][1] * UR)
                return pltpu.make_async_copy(ckv_hbm.at[rows, :], ckv_v.at[rows, :], sem.at[SEM_CKV + j])
            xat_cp = pltpu.make_async_copy(xat_hbm, xat_v, sem.at[SEM_XAT])

            with _scope("a_issue0"):
                for cp in first_copies(wuk_hbm, wuk_v, 0) + first_copies(wuv_hbm, wuv_v, 1):
                    cp.start()
                for j in range(4):
                    ckv_cp(j).start()
                batch_start([1], 2)
                ckv_cp(4).start()
                batch_start([2], 3)
                for j in range(1, ngrp - 1):
                    batch_start(group(j), 3 + j)

            def lhs_prep(src_v, dst_v, u):
                c = src_v[u * UR:(u + 1) * UR, 0:DC].astype(f32)
                ops = _strassen_lhs(c[:D, :kh], c[:D, kh:], c[D:, :kh], c[D:, kh:])
                for i, o in enumerate(ops):
                    dst_v[i, u * D // 2:(u + 1) * D // 2, :] = _pack(o.astype(bf16))

            def rhs_words(w_v, hp):
                n = kh // 2
                s0, s1 = w_v[0, hp, 0:n, :], w_v[1, hp, 0:n, :]
                z0, z1 = w_v[0, hp, n:2 * n, :], w_v[1, hp, n:2 * n, :]
                return _rhs_words(s0, s1, z0, z1)

            def rhs_kv(hp):
                return [jnp.concatenate([a, b], axis=1) for a, b in zip(rhs_words(wuk_v, hp), rhs_words(wuv_v, hp))]

            def items(lst):
                return lambda i: lst[i]

            def project_kv(t, hp, u0, u1):
                c = _strassen(lambda i: _unpack(la_v[i, u0 * D // 2:u1 * D // 2, :]), lambda i: _unpack(t(i)), order=1)
                for u in range(u0, u1):
                    rows = slice((u - u0) * D, (u - u0 + 1) * D)
                    top = u * D
                    for blk, h, p0 in ((c[0], 2 * hp, top), (c[1], 2 * hp + 1, top),
                                       (c[2], 2 * hp, top + D // 2), (c[3], 2 * hp + 1, top + D // 2)):
                        blk = blk[rows, :].astype(bf16)
                        k_v[h, p0:p0 + D // 2, :] = _pack(blk[:, 0:D])
                        v_v[h, p0:p0 + D // 2, :] = _pack(blk[:, D:2 * D])

            KU = 2

            def project_pair(t, hp):
                for u in range(0, NU, KU):
                    project_kv(t, hp, u, u + KU)

            def kv_first():
                first_wait(wuk_v, 0)
                first_wait(wuv_v, 1)
                t = items(rhs_kv(0))
                for j in range(4):
                    ckv_cp(j).wait()
                    for u in range(*pieces[j]):
                        lhs_prep(ckv_v, la_v, u)
                    project_kv(t, 0, *pieces[j])
                ckv_cp(4).wait()
                batch_wait(1, 2)
                for u in range(*pieces[4]):
                    lhs_prep(ckv_v, la_v, u)
                project_kv(t, 0, *pieces[4])
                t1 = items(rhs_kv(1))
                project_kv(t1, 1, 0, 2)
                batch_wait(1, 3)
                for i, w in enumerate(rhs_kv(2)):
                    tkv_v[i] = w
                for u in range(2, NU, 2):
                    project_kv(t1, 1, u, u + 2)

            def kv_body(j, c):
                @pl.when(j == 2)
                def _():
                    xat_cp.start()
                    batch_start(group(ngrp - 1), 3 + ngrp - 1)
                    w_start_shared(wqa_hbm, wqa_v, 0, range(HP))
                    xbt_cp.start()
                batch_wait(2, 3 + j)
                project_pair(lambda i: tkv_v[i], 2 * j)
                t1 = items(rhs_kv(2 * j + 1))
                for i, w in enumerate(rhs_kv(2 * j + 2)):
                    tkv_v[i] = w
                project_pair(t1, 2 * j + 1)
                return c

            with _scope("a_kvproj"):
                kv_first()
                jax.lax.fori_loop(1, ngrp - 1, kv_body, 0)

            woa_cp.start()
            wob_cp.start()
            mem_cp.start()
            w_start_shared(wqb_hbm, wb_v.at[0], 1, range(HP))
            w_start_shared(wkb_hbm, wb_v.at[1], 2, range(HP // 2))

            def q_rhs(hp):
                t = [jnp.concatenate([a, b], axis=1) for a, b in zip(rhs_words(wqa_v, hp), rhs_words(wqa_v, hp + 1))]
                rem = []
                for e in range(2):
                    for p in (hp, hp + 1):
                        a, b = wqa_v[0, p, kh:, :], wqa_v[1, p, kh:, :]
                        rem.append((a & u32(0xFFFF)) | (b << 16) if e == 0 else (a >> 16) | (b & u32(0xFFFF0000)))
                return t, jnp.concatenate(rem, axis=1)

            def project_q(t, rem, hp, u):
                c = _strassen(lambda i: _unpack(lq_v[i, u * D // 2:(u + 1) * D // 2, :]), lambda i: _unpack(t[i]))
                for half in range(2):
                    x0 = u * UR + half * D
                    r = jnp.dot(xa_v[x0:x0 + D, DC:DM], _unpack(rem), preferred_element_type=f32)
                    r = (jnp.concatenate([c[2 * half], c[2 * half + 1]], axis=1) + r) * QSCALE
                    r = r.astype(bf16)
                    for n, h in enumerate((2 * hp, 2 * hp + 2, 2 * hp + 1, 2 * hp + 3)):
                        q_v[h, x0 // 2:(x0 + D) // 2, :] = _pack(r[:, n * D:(n + 1) * D])

            def xa_prep(u):
                for t in range(u * UR // D, (u + 1) * UR // D):
                    xa_v[t * D:(t + 1) * D, :] = xat_v[:, t * D:(t + 1) * D].T
                lhs_prep(xa_v, lq_v, u)

            def xb_prep(t):
                t0 = t * D
                xb = xbt_v[:, t0:t0 + D].T
                xb_v[t0:t0 + D, :] = xb
                for sg in range(D // SEG):
                    p0 = (t * (D // SEG) + sg) * PRE
                    xpre_v[p0:p0 + PRE, :] = xb[sg * SEG:sg * SEG + PRE, :]

            with _scope("a_qproj"):
                j = ngrp - 1
                batch_wait(1, 3 + j)
                xat_cp.wait()
                xbt_cp.wait()
                w_wait_shared(wqa_v, 0)
                t14 = lambda i: tkv_v[i]
                t15 = items(rhs_kv(2 * j + 1))
                kv = [(t14, 2 * j, u) for u in range(0, NU, 2)] + [(t15, 2 * j + 1, u) for u in range(0, NU, 2)]
                t, rem = q_rhs(0)
                for u in range(NU):
                    project_kv(kv[u][0], kv[u][1], kv[u][2], kv[u][2] + 2)
                    xa_prep(u)
                    project_q(t, rem, 0, u)
                XG = 4
                nx = 0
                for hp in range(2, HP, 2):
                    t, rem = q_rhs(hp)
                    for u in range(NU):
                        project_q(t, rem, hp, u)
                        if u == 0:
                            for _ in range(XG):
                                if nx < S // D:
                                    xb_prep(nx)
                                    nx += 1
                                    if nx == S // D:
                                        lp_prep(lp_v)

        pl.run_scoped(
            projections,
            pltpu.VMEM((S, DC), bf16),
            pltpu.VMEM((DM, S), bf16),
            pltpu.VMEM((S, DM), bf16),
            pltpu.VMEM((2, HP, DC // 2, D), u32),
            pltpu.VMEM((2, HP, DC // 2, D), u32),
            pltpu.VMEM((2, HP, DM // 2, D), u32),
            pltpu.VMEM((7, DC // 4, 2 * D), u32),
            pltpu.VMEM((7, S // 4, DC // 2), u32),
            pltpu.VMEM((7, S // 4, DC // 2), u32),
        )

        def attention(c_v, s_v):
            row = jax.lax.broadcasted_iota(jnp.int32, (TQ, TQ), 0)
            col = jax.lax.broadcasted_iota(jnp.int32, (TQ, TQ), 1)
            tri = col <= row
            nb = S // TQ
            hq = TQ // 2
            npiece = 2
            pw = S // npiece

            def qk_piece(h, j):
                q = _unpack(q_v[h, (nb - 1) * hq:nb * hq, :])
                k = _unpack(k_v[h, j * pw // 2:(j + 1) * pw // 2, :])
                s_v[:, j * pw:(j + 1) * pw] = jax.lax.dot_general(q, k, NT, preferred_element_type=f32)

            def qk(h, i, j0=0, j1=None):
                j1 = i + 1 if j1 is None else j1
                q = _unpack(q_v[h, i * hq:(i + 1) * hq, :])
                k = _unpack(k_v[h, j0 * hq:j1 * hq, :])
                return jax.lax.dot_general(q, k, NT, preferred_element_type=f32)

            def anchor_plan():
                ops = []
                for e in range(UH):
                    for i in range(nb - 1, -1, -1):
                        if i > 0:
                            ops.append(("qk", e, i - 1, 32 * i))
                        if i < npiece:
                            ops.append(("piece", e, i, 32 * nb // npiece))
                        ops.append(("pv", e, i, 32 * (i + 1)))
                t, start, end = 0, [], []
                for op in ops:
                    start.append(t)
                    t += op[3]
                    end.append(t)
                plan = {}
                for a, op in enumerate(ops):
                    if op[0] != "pv" or op[2] < ANCHOR_MIN:
                        continue
                    for b in range(a + 1, len(ops)):
                        if ops[b][0] == "qk" and start[b] >= end[a] + ANCHOR_LAG:
                            plan.setdefault((ops[b][1], ops[b][2]), []).append((op[1], op[2]))
                            break
                return plan

            def heads(j, c):
                @pl.when(j == 0)
                def _():
                    w_start_shared(wkb_hbm, wb_v.at[1], 2, range(HP // 2, HP))
                    w_start_shared(wvb_hbm, wb_v.at[2], 3, range(HP))

                plan = anchor_plan()

                def gated_qk(e, i):
                    h = j * UH + e
                    if (e, i) not in plan:
                        return qk(h, i)
                    w = None
                    for ea, ia in plan[e, i]:
                        u = c_v[j * UH + ea, ia * hq:(ia + 1) * hq, :]
                        for r in range(0, hq, 8):
                            w = u[r:r + 8] if w is None else w | u[r:r + 8]
                    zero = (w >> 31) >> 1
                    q = q_v[h, i * hq:(i + 1) * hq, :]
                    q = _unpack(jnp.concatenate([q[0:8] | zero, q[8:]], axis=0))
                    k = _unpack(k_v[h, 0:(i + 1) * hq, :])
                    return jax.lax.dot_general(q, k, NT, preferred_element_type=f32)

                s_next = s_v[...]
                for e in range(UH):
                    h = j * UH + e
                    hn = jnp.minimum(h + 1, H - 1) if e == UH - 1 else h + 1
                    pieces = []
                    for i in range(nb - 1, -1, -1):
                        s = s_next
                        if i > 0:
                            s_next = gated_qk(e, i - 1)
                        if i < npiece:
                            if e == UH - 1:
                                qk_piece(hn, npiece - 1 - i)
                            else:
                                jj = npiece - 1 - i
                                pieces.append(qk(hn, nb - 1, jj * nb // npiece, (jj + 1) * nb // npiece))
                        sd = jnp.where(tri, s[:, i * TQ:], NEG)
                        s = jnp.concatenate([s[:, :i * TQ], sd], axis=1) if i > 0 else sd
                        m = jnp.max(s, axis=1, keepdims=True)
                        p = jnp.exp2(s - m)
                        l = jnp.sum(p, axis=1, keepdims=True)
                        v = _unpack(v_v[h, 0:(i + 1) * hq, :])
                        o = jnp.dot(p.astype(bf16), v, preferred_element_type=f32)
                        c_v[h, i * hq:(i + 1) * hq, :] = _pack((o * _recip(l)).astype(bf16))
                    if e < UH - 1:
                        s_next = jnp.concatenate(pieces, axis=1)
                return c
            with _scope("a_attn"):
                for j in range(npiece):
                    qk_piece(0, j)
                jax.lax.fori_loop(0, H // UH, heads, 0)

            woa_cp.wait()
            wob_cp.wait()
            mem_cp.wait()
            for t in range(3):
                w_wait_shared(wb_v.at[t], 1 + t)
            mh = DM // 4

            def wo_prep(hh):
                a11, a21 = woa_v[hh, 0:mh, :], woa_v[hh, mh:2 * mh, :]
                a12, a22 = woa_v[hh + HP, 0:mh, :], woa_v[hh + HP, mh:2 * mh, :]
                for i, w in enumerate(_sum_words(_strassen_lhs, a11, a12, a21, a22, (2, 3), (a11, a22))):
                    if i not in (2, 3):
                        k_v[hh, i * mh:(i + 1) * mh, :] = w

            def wob_prep(h):
                wob_v[h * (D // 2):(h + 1) * (D // 2), :] = _pack(_unpack(wobt_v[h]).T)

            def oproj(tp):
                w0 = tp * D
                per = []
                for hh in range(HP):
                    b11, b21 = c_v[hh, w0:w0 + D // 2, :], c_v[hh + HP, w0:w0 + D // 2, :]
                    b12, b22 = c_v[hh, w0 + D // 2:w0 + D, :], c_v[hh + HP, w0 + D // 2:w0 + D, :]
                    per.append(_sum_words(_strassen_rhs, b11, b12, b21, b22, (1, 4), (b11, b22)))

                def lhs(i):
                    if i == 2:
                        return _unpack(jnp.concatenate([woa_v[hh, 0:mh, :] for hh in range(HP)], axis=1))
                    if i == 3:
                        return _unpack(jnp.concatenate([woa_v[hh + HP, mh:2 * mh, :] for hh in range(HP)], axis=1))
                    return _unpack(jnp.concatenate([k_v[hh, i * mh:(i + 1) * mh, :] for hh in range(HP)], axis=1))

                def rhs(i):
                    return _unpack(jnp.concatenate([per[hh][i] for hh in range(HP)], axis=1))
                c11, c12, c21, c22 = _strassen(lhs, rhs, NT)
                t0 = 2 * tp * D
                out_v[t0:t0 + D, 0:DM] = jnp.concatenate([c11, c21], axis=0).T.astype(bf16)
                out_v[t0 + D:t0 + 2 * D, 0:DM] = jnp.concatenate([c12, c22], axis=0).T.astype(bf16)

            b_pre(lp_v)
            with _scope("a_oproj"):
                for hh in range(HP):
                    wo_prep(hh)
                for tp in range(S // D // 2):
                    oproj(tp)
                    for h in range(4 * tp, 4 * tp + 4):
                        wob_prep(h)

        pl.run_scoped(
            attention,
            pltpu.VMEM((H, S // 2, D), u32),
            pltpu.VMEM((TQ, S), f32),
        )

    pl.run_scoped(
        phase_a,
        pltpu.VMEM((H, DM // 2, D), u32),
        pltpu.VMEM((DM, S), bf16),
        pltpu.VMEM((H, DM // 2, D), u32),
        pltpu.VMEM((7, NSEG * PRE // 4, DC // 2), u32),
    )

    def out_copy(j):
        rows = pl.ds(pl.multiple_of(j * (OUTER * SEG), OUTER * SEG), OUTER * SEG)
        return pltpu.make_async_copy(out_v.at[rows, :], out_hbm.at[rows, :], sem.at[SEM_OUT + j])

    def phase_b(post_v):
        lane = jax.lax.broadcasted_iota(jnp.int32, (1, GW), 1)
        colscale = jnp.where(lane % (3 * D) < D, QSCALE, 1.0).astype(f32)

        def wgroup(g):
            return _unpack(jnp.concatenate(
                [wb_v[t, h % 2, h // 2] for h in range(g * HG, (g + 1) * HG) for t in range(3)], axis=1))

        def wogroup(g):
            return _unpack(wob_v[g * HG * D // 2:(g + 1) * HG * D // 2, :])

        ri = jax.lax.broadcasted_iota(jnp.int32, (2 * L, 2 * L), 0)
        ci = jax.lax.broadcasted_iota(jnp.int32, (2 * L, 2 * L), 1)

        def second(i):
            return jnp.where(i < 2 * SEG, i // SEG, (i - 2 * SEG) // PRE)

        def pos(i):
            j = i % SEG
            return jnp.where(i < 2 * SEG, jnp.where(j < T, j + (MEM + PRE), j - T), MEM + i % PRE)
        same = second(ri) == second(ci)
        mask = same & ((pos(ri) < MEM) | (pos(ri) >= pos(ci)))
        fill = jnp.where(same, NEG, -jnp.inf).astype(f32)

        def step(s, slot, mem):
            xt = xb_v[pl.ds(pl.multiple_of(SEG * s + PRE, 8), T), :]
            l1 = jnp.concatenate([xt.astype(f32), mem], axis=0).astype(bf16)
            p0 = pl.multiple_of(PRE * s, 8)
            proj = [(jnp.dot(l1, wgroup(g), preferred_element_type=f32) * colscale).astype(bf16)
                    for g in range(G)]

            def rows(hp, t):
                g, c0 = 2 * hp // HG, (2 * hp % HG) * 3 * D + t * D
                return jnp.concatenate([proj[g][:, c0:c0 + D], proj[g][:, c0 + 3 * D:c0 + 4 * D],
                                        _unpack(pre_ref(hp * 3 + t)[pl.ds(p0, PRE), :])], axis=0)

            scores = [jax.lax.dot_general(rows(hp, 0), rows(hp, 1), NT, preferred_element_type=f32)
                      for hp in range(HP)]
            ctx = {}

            def attend(g):
                for hp in range(g * HG // 2, (g + 1) * HG // 2):
                    sc = jnp.where(mask, scores[hp], fill)
                    m = jnp.max(sc, axis=1, keepdims=True)
                    p = jnp.exp2(sc - m)
                    l = jnp.sum(p, axis=1, keepdims=True)
                    o = jnp.dot(p.astype(bf16), rows(hp, 2), preferred_element_type=f32) * _recip(l)
                    for e in range(2):
                        h = 2 * hp + e
                        ctx[h] = o[e * SEG:(e + 1) * SEG, :].astype(bf16)
                        post_v[slot * PRE:(slot + 1) * PRE, h * D:(h + 1) * D] = o[2 * SEG + e * PRE:2 * SEG + (e + 1) * PRE, :]

            parts = []

            def oproj(g):
                lhs = jnp.concatenate([ctx[h] for h in range(g * HG, (g + 1) * HG)], axis=1)
                parts.append(jnp.dot(lhs, wogroup(g), preferred_element_type=f32))

            for t in range(G + 2):
                if t < G:
                    attend(t)
                if t >= 2:
                    oproj(t - 2)
            acc = parts[0]
            for a in parts[1:]:
                acc = acc + a
            accb = acc.astype(bf16)
            out_v[pl.ds(pl.multiple_of(SEG * s + PRE, 8), T), DM:2 * DM] = accb[0:T, :]
            return accb[T:, :].astype(f32), ctx[H - 1]

        KP = H * D // OUTER

        def partial(rows, i):
            return jnp.dot(rows, _unpack(wob_v[i * KP // 2:(i + 1) * KP // 2, :]), preferred_element_type=f32)

        def finish(j, r):
            r = r.astype(bf16)
            for sg in range(OUTER):
                r0 = pl.multiple_of((j * OUTER + sg) * SEG, SEG)
                out_v[pl.ds(r0, PRE), DM:2 * DM] = r[sg * PRE:(sg + 1) * PRE, :]

        def after(x, late):
            u = _pack(late[0:2 * OUTER * PRE // 2, :])
            zero = (u >> 31) & (~u >> 31)
            return _unpack(_pack(x) | jnp.concatenate([zero] * (x.shape[1] // D), axis=1))

        def outer(j, mem):
            prev = post_v[...].astype(bf16)
            acc = partial(prev[:, 0:KP], 0)
            for i in range(OUTER):
                mem, late = step(j * OUTER + i, i, mem)
                if i + 1 < OUTER:
                    acc = acc + partial(after(prev[:, (i + 1) * KP:(i + 2) * KP], late), i + 1)
            finish(jnp.maximum(j - 1, 0), acc)

            @pl.when(j > 0)
            def _():
                out_copy(j - 1).start()
            return mem
        with _scope("b_loop"):
            post_v[...] = jnp.zeros(post_v.shape, f32)
            jax.lax.fori_loop(0, NOUTER, outer, mem_v[0:MEM, :].astype(f32))
            finish(NOUTER - 1, jnp.dot(post_v[...].astype(bf16), _unpack(wob_v[...]), preferred_element_type=f32))
            out_copy(NOUTER - 1).start()
        with _scope("b_outwait"):
            for j in range(NOUTER):
                out_copy(j).wait()

    pl.run_scoped(
        phase_b,
        pltpu.VMEM((OUTER * PRE, H * D), f32),
    )


@jax.jit
def pallas_concat_heads__compressed_kv_cla__memory_aug_recurrent_mem_tr__prompt_kernel(
    A_x: jax.Array,
    A_c_kv: jax.Array,
    A_w_q: jax.Array,
    A_w_uk: jax.Array,
    A_w_uv: jax.Array,
    A_w_o: jax.Array,
    B_x: jax.Array,
    B_mem0: jax.Array,
    B_Wq: jax.Array,
    B_Wk: jax.Array,
    B_Wv: jax.Array,
    B_Wo: jax.Array,
    B_seg_len=SEG,
):
    def t2(x):
        return jnp.transpose(x, (0, 2, 1)).reshape(DM, S)

    def w3(w):
        return w.reshape(w.shape[0] // 2, 2 * H, D)

    def wo3(w):
        return jnp.transpose(w, (0, 2, 1))

    any_spec = pl.BlockSpec(memory_space=pl.ANY)
    out = pl.pallas_call(
        _kernel,
        out_shape=jax.ShapeDtypeStruct((S, 2 * DM), bf16),
        in_specs=[any_spec] * 12,
        out_specs=any_spec,
        scratch_shapes=[
            pltpu.VMEM((S, 2 * DM), bf16),
            pltpu.VMEM((S, DM), bf16),
            pltpu.VMEM((NSEG * PRE, DM), bf16),
            pltpu.VMEM((3, 2, HP, DM // 2, D), u32),
            pltpu.VMEM((H * D // 2, DM), u32),
            pltpu.VMEM((8 * MEM, DM), bf16),
            pltpu.VMEM((H, S // 2, D), u32),
            pltpu.VMEM((H, S // 2, D), u32),
            pltpu.VMEM((H, S // 2, D), u32),
            pltpu.SemaphoreType.DMA((NSEM,)),
        ],
        compiler_params=pltpu.CompilerParams(vmem_limit_bytes=126 * 1024 * 1024),
    )(t2(A_x), A_c_kv.reshape(S, DC), w3(A_w_q), w3(A_w_uk), w3(A_w_uv), wo3(A_w_o),
      t2(B_x), B_mem0.reshape(MEM, DM), w3(B_Wq), w3(B_Wk), w3(B_Wv), wo3(B_Wo))
    return out.reshape(1, S, 2 * DM)
```

```python
import contextlib

import jax
import jax.numpy as jnp
import jax.experimental.pallas as pl
import jax.experimental.pallas.tpu as pltpu

S = 2048
DM = 576
DC = 512
H = 32
D = 128
MEM = 8
SEG = 32
L = MEM + SEG
NSEG = S // SEG
HP = H // 2
HD = D // 2
KM = DM - 3 * HD
DMP = DM + HD

LOG2E = 1.4426950408889634
QSCALE = D ** -0.5 * LOG2E
NEG = -1.0e9 * LOG2E

TQ = 128
UH = 4
ANCHOR_LAG = 2000
ANCHOR_MIN = 6
RB = 512
HG = 4
G = H // HG
PRE = 8
T = SEG - PRE
OUTER = 4
NOUTER = NSEG // OUTER

bf16 = jnp.bfloat16
f32 = jnp.float32
u32 = jnp.uint32
NT = (((1,), (1,)), ((), ()))

SEM_CKV = 0
SEM_XAT = 5
SEM_XBT = 6
SEM_MEM = 7
SEM_WOA = 8
SEM_WOB = 9
SEM_OUT = 10
SEM_WALL = SEM_OUT + NOUTER
SEM_W = SEM_WALL + 4
NSEM = SEM_W + 3 + HP // 2

_PROFILE = False


def _scope(name):
    return jax.named_scope(name) if _PROFILE else contextlib.nullcontext()


def _unpack(w32):
    return pltpu.bitcast(w32, bf16)


def _pack(x):
    return pltpu.bitcast(x, u32)


def _lo(w):
    return pltpu.bitcast(w << 16, f32)


def _hi(w):
    return pltpu.bitcast(w & u32(0xFFFF0000), f32)


def _words(even, odd):
    return pltpu.bitcast(pltpu.pack_elementwise([even, odd], packed_dtype=bf16), u32)


def _strassen_lhs(a11, a12, a21, a22):
    return [a11 + a22, a21 + a22, a11, a22, a11 + a12, a21 - a11, a12 - a22]


def _strassen_rhs(b11, b12, b21, b22):
    return [b11 + b22, b11, b12 - b22, b21 - b11, b22, b11 + b12, b21 + b22]


def _sum_words(combine, x11, x12, x21, x22, raw_idx, raw):
    lo = combine(_lo(x11), _lo(x12), _lo(x21), _lo(x22))
    hi = combine(_hi(x11), _hi(x12), _hi(x21), _hi(x22))
    words = [pltpu.bitcast(pltpu.pack_elementwise([a, b], packed_dtype=bf16), u32) for a, b in zip(lo, hi)]
    for i, r in zip(raw_idx, raw):
        words[i] = r
    return words


def _strassen(lhs, rhs, dims=(((1,), (0,)), ((), ())), order=0):
    def m(i):
        return jax.lax.dot_general(lhs(i - 1), rhs(i - 1), dims, preferred_element_type=f32)
    if order == 0:
        m1 = m(1)
        m2 = m(2)
        c22 = m1 - m2
        m4 = m(4)
        c11 = m1 + m4
        c21 = m2 + m4
        c22 = c22 + m(6)
        m3 = m(3)
        c22 = c22 + m3
        m5 = m(5)
        c11 = c11 - m5
        c12 = m3 + m5
        c11 = c11 + m(7)
        return c11, c12, c21, c22
    m3 = m(3)
    m4 = m(4)
    m5 = m(5)
    c12 = m3 + m5
    c11 = m4 - m5
    m2 = m(2)
    c21 = m4 + m2
    c22 = m3 - m2
    m1 = m(1)
    c11 = c11 + m1
    c22 = c22 + m1
    c22 = c22 + m(6)
    c11 = c11 + m(7)
    return c11, c12, c21, c22


def _rhs_words(s0, s1, z0, z1):
    per = [_strassen_rhs(_lo(s), _hi(s), _lo(z), _hi(z)) for s, z in ((s0, z0), (s1, z1))]
    words = [pltpu.bitcast(pltpu.pack_elementwise([per[0][i], per[1][i]], packed_dtype=bf16), u32)
             for i in range(7)]
    words[1] = (s0 & u32(0xFFFF)) | (s1 << 16)
    words[4] = (z0 >> 16) | (z1 & u32(0xFFFF0000))
    return words


def _recip(l):
    r = pl.reciprocal(l, approx=True)
    return r * (2.0 - l * r)


def _kernel(xat_hbm, ckv_hbm, wqa_hbm, wuk_hbm, wuv_hbm, woa_hbm,
            xbt_hbm, mem0_hbm, wqb_hbm, wkb_hbm, wvb_hbm, wob_hbm,
            out_hbm,
            out_v, xb_v, xpre_v, wb_v, wob_v, wos_v, mem_v, q_v, k_v, v_v, sem):

    def w_copy(w_hbm, dst, slot, par, hp):
        return pltpu.make_async_copy(w_hbm.bitcast(u32).at[:, par * HP + hp, :], dst.at[par, hp], sem.at[slot])

    def w_start_shared(w_hbm, dst, widx, hps):
        for hp in hps:
            for par in range(2):
                w_copy(w_hbm, dst, SEM_WALL + widx, par, hp).start()

    def w_wait_shared(dst, widx):
        pltpu.make_async_copy(dst, dst, sem.at[SEM_WALL + widx]).wait()

    def w_combine(dst, hp):
        a = dst[0, hp]
        b = dst[1, hp]
        ev = (a & u32(0xFFFF)) | (b << 16)
        od = (a >> 16) | (b & u32(0xFFFF0000))
        return ev, od

    def w_pair(dst, hp):
        return jnp.concatenate(w_combine(dst, hp), axis=1)

    wb_hbm = (wqb_hbm, wkb_hbm, wvb_hbm)

    def pre_ref(j):
        n = NSEG * PRE
        return q_v.at[j // 2, (j % 2) * n:(j % 2 + 1) * n, :]

    def lp_prep(lp_v):
        nr = NSEG * PRE // 2
        kh = DC // 2
        x = xpre_v[:, 0:DC].astype(f32)
        for i, o in enumerate(_strassen_lhs(x[:nr, :kh], x[:nr, kh:], x[nr:, :kh], x[nr:, kh:])):
            lp_v[i] = _pack(o.astype(bf16))

    def b_pre(lp_v):
        nr = NSEG * PRE // 2
        kh = DC // 2
        n = kh // 2
        PG = 1
        SP = nr
        with _scope("b_pre"):
            for g in range(HP // PG):
                ts, rem = [], [[], []]
                combos = [(hp, t) for hp in range(g * PG, (g + 1) * PG) for t in range(3)]
                for hp, t in combos:
                    s0, s1 = wb_v[t, 0, hp], wb_v[t, 1, hp]
                    ev = (s0 & u32(0xFFFF)) | (s1 << 16)
                    od = (s0 >> 16) | (s1 & u32(0xFFFF0000))
                    a, b = (KM + HD) // 2, (KM + 2 * HD) // 2
                    c = DM // 2
                    d12 = _words(_lo(s0[a:b]) - _hi(s0[a:b]), _lo(s1[a:b]) - _hi(s1[a:b]))
                    d21 = _words(_hi(s0[b:c]) - _lo(s0[b:c]), _hi(s1[b:c]) - _lo(s1[b:c]))
                    wb_v[t, 0, hp] = jnp.concatenate([ev[:a], d12, ev[b:]], axis=0)
                    wb_v[t, 1, hp] = jnp.concatenate([od[:a], d21, od[a:b]], axis=0)
                    ts.append(_rhs_words(s0[:n], s1[:n], s0[n:2 * n], s1[n:2 * n]))
                    rem[0].append(ev[2 * n:])
                    rem[1].append(od[2 * n:])
                tw = [jnp.concatenate([x_[i] for x_ in ts], axis=1) for i in range(7)]
                remw = _unpack(jnp.concatenate(rem[0] + rem[1], axis=1))
                nc = len(combos)
                for sub in range(nr // SP):
                    r0 = sub * SP
                    c = _strassen(lambda i: _unpack(lp_v[i, r0 // 2:(r0 + SP) // 2, :]), lambda i: _unpack(tw[i]))
                    for half in range(2):
                        x0 = half * nr + r0
                        r = jnp.dot(xpre_v[x0:x0 + SP, DC:DM], remw, preferred_element_type=f32)
                        r = jnp.concatenate([c[2 * half], c[2 * half + 1]], axis=1) + r
                        for ci_, (hp, t) in enumerate(combos):
                            two = [r[:, cc * D:(cc + 1) * D] for cc in (ci_, nc + ci_)]
                            if t == 0:
                                two = [y * QSCALE for y in two]
                            two = [y.reshape(SP // PRE, 1, PRE, D) for y in two]
                            two = jnp.concatenate(two, axis=1).reshape(2 * SP, D)
                            pre_ref(hp * 3 + t)[x0:x0 + SP, :] = _pack(two.astype(bf16))


    def phase_a(woa_v, xbt_v, wobt_v, lp_v):
        woa_cp = pltpu.make_async_copy(woa_hbm.bitcast(u32), woa_v, sem.at[SEM_WOA])
        xbt_cp = pltpu.make_async_copy(xbt_hbm, xbt_v, sem.at[SEM_XBT])
        mem_cp = pltpu.make_async_copy(mem0_hbm, mem_v.at[0:MEM, :], sem.at[SEM_MEM])
        wob_cp = pltpu.make_async_copy(wob_hbm.bitcast(u32), wobt_v, sem.at[SEM_WOB])

        def projections(ckv_v, xat_v, xa_v, wuk_v, wuv_v, wqa_v, tkv_v, lq_v, la_v):
            UR = 2 * D
            NU = S // UR
            kh = DC // 2
            ngrp = HP // 2

            def batch_start(pairs, slot):
                for hp in pairs:
                    for w_hbm, dst in ((wuk_hbm, wuk_v), (wuv_hbm, wuv_v)):
                        for par in range(2):
                            w_copy(w_hbm, dst, SEM_W + slot, par, hp).start()

            def batch_wait(npairs, slot):
                part = wuk_v.at[:, 0:2 * npairs]
                pltpu.make_async_copy(part, part, sem.at[SEM_W + slot]).wait()

            def group(j):
                return [hp for hp in (2 * j + 1, 2 * j + 2) if hp < HP]

            def first_copies(w_hbm, dst, slot):
                return [w_copy(w_hbm, dst, SEM_W + slot, par, 0) for par in range(2)]

            def first_wait(dst, slot):
                part = dst.at[:, 0:1]
                pltpu.make_async_copy(part, part, sem.at[SEM_W + slot]).wait()

            pieces = [(0, 1), (1, 2), (2, 4), (4, 6), (6, 8)]

            def ckv_cp(j):
                rows = slice(pieces[j][0] * UR, pieces[j][1] * UR)
                return pltpu.make_async_copy(ckv_hbm.at[rows, :], ckv_v.at[rows, :], sem.at[SEM_CKV + j])
            xat_cp = pltpu.make_async_copy(xat_hbm, xat_v, sem.at[SEM_XAT])

            with _scope("a_issue0"):
                for cp in first_copies(wuk_hbm, wuk_v, 0) + first_copies(wuv_hbm, wuv_v, 1):
                    cp.start()
                for j in range(4):
                    ckv_cp(j).start()
                batch_start([1], 2)
                ckv_cp(4).start()
                batch_start([2], 3)
                for j in range(1, ngrp - 1):
                    batch_start(group(j), 3 + j)

            def lhs_prep(src_v, dst_v, u):
                c = src_v[u * UR:(u + 1) * UR, 0:DC].astype(f32)
                ops = _strassen_lhs(c[:D, :kh], c[:D, kh:], c[D:, :kh], c[D:, kh:])
                for i, o in enumerate(ops):
                    dst_v[i, u * D // 2:(u + 1) * D // 2, :] = _pack(o.astype(bf16))

            def rhs_words(w_v, hp):
                n = kh // 2
                s0, s1 = w_v[0, hp, 0:n, :], w_v[1, hp, 0:n, :]
                z0, z1 = w_v[0, hp, n:2 * n, :], w_v[1, hp, n:2 * n, :]
                return _rhs_words(s0, s1, z0, z1)

            def rhs_kv(hp):
                return [jnp.concatenate([a, b], axis=1) for a, b in zip(rhs_words(wuk_v, hp), rhs_words(wuv_v, hp))]

            def items(lst):
                return lambda i: lst[i]

            def project_kv(t, hp, u0, u1):
                c = _strassen(lambda i: _unpack(la_v[i, u0 * D // 2:u1 * D // 2, :]), lambda i: _unpack(t(i)), order=1)
                for u in range(u0, u1):
                    rows = slice((u - u0) * D, (u - u0 + 1) * D)
                    top = u * D
                    for blk, h, p0 in ((c[0], 2 * hp, top), (c[1], 2 * hp + 1, top),
                                       (c[2], 2 * hp, top + D // 2), (c[3], 2 * hp + 1, top + D // 2)):
                        blk = blk[rows, :].astype(bf16)
                        k_v[h, p0:p0 + D // 2, :] = _pack(blk[:, 0:D])
                        v_v[h, p0:p0 + D // 2, :] = _pack(blk[:, D:2 * D])

            KU = 2

            def project_pair(t, hp):
                for u in range(0, NU, KU):
                    project_kv(t, hp, u, u + KU)

            def kv_first():
                first_wait(wuk_v, 0)
                first_wait(wuv_v, 1)
                t = items(rhs_kv(0))
                for j in range(4):
                    ckv_cp(j).wait()
                    for u in range(*pieces[j]):
                        lhs_prep(ckv_v, la_v, u)
                    project_kv(t, 0, *pieces[j])
                ckv_cp(4).wait()
                batch_wait(1, 2)
                for u in range(*pieces[4]):
                    lhs_prep(ckv_v, la_v, u)
                project_kv(t, 0, *pieces[4])
                t1 = items(rhs_kv(1))
                project_kv(t1, 1, 0, 2)
                batch_wait(1, 3)
                for i, w in enumerate(rhs_kv(2)):
                    tkv_v[i] = w
                for u in range(2, NU, 2):
                    project_kv(t1, 1, u, u + 2)

            def kv_body(j, c):
                @pl.when(j == 2)
                def _():
                    xat_cp.start()
                    batch_start(group(ngrp - 1), 3 + ngrp - 1)
                    w_start_shared(wqa_hbm, wqa_v, 0, range(HP))
                    xbt_cp.start()
                batch_wait(2, 3 + j)
                project_pair(lambda i: tkv_v[i], 2 * j)
                t1 = items(rhs_kv(2 * j + 1))
                for i, w in enumerate(rhs_kv(2 * j + 2)):
                    tkv_v[i] = w
                project_pair(t1, 2 * j + 1)
                return c

            with _scope("a_kvproj"):
                kv_first()
                jax.lax.fori_loop(1, ngrp - 1, kv_body, 0)

            woa_cp.start()
            wob_cp.start()
            mem_cp.start()
            w_start_shared(wqb_hbm, wb_v.at[0], 1, range(HP))
            w_start_shared(wkb_hbm, wb_v.at[1], 2, range(HP // 2))

            def q_rhs(hp):
                t = [jnp.concatenate([a, b], axis=1) for a, b in zip(rhs_words(wqa_v, hp), rhs_words(wqa_v, hp + 1))]
                rem = []
                for e in range(2):
                    for p in (hp, hp + 1):
                        a, b = wqa_v[0, p, kh:, :], wqa_v[1, p, kh:, :]
                        rem.append((a & u32(0xFFFF)) | (b << 16) if e == 0 else (a >> 16) | (b & u32(0xFFFF0000)))
                return t, jnp.concatenate(rem, axis=1)

            def project_q(t, rem, hp, u):
                c = _strassen(lambda i: _unpack(lq_v[i, u * D // 2:(u + 1) * D // 2, :]), lambda i: _unpack(t[i]))
                for half in range(2):
                    x0 = u * UR + half * D
                    r = jnp.dot(xa_v[x0:x0 + D, DC:DM], _unpack(rem), preferred_element_type=f32)
                    r = (jnp.concatenate([c[2 * half], c[2 * half + 1]], axis=1) + r) * QSCALE
                    r = r.astype(bf16)
                    for n, h in enumerate((2 * hp, 2 * hp + 2, 2 * hp + 1, 2 * hp + 3)):
                        q_v[h, x0 // 2:(x0 + D) // 2, :] = _pack(r[:, n * D:(n + 1) * D])

            def xa_prep(u):
                for t in range(u * UR // D, (u + 1) * UR // D):
                    xa_v[t * D:(t + 1) * D, :] = xat_v[:, t * D:(t + 1) * D].T
                lhs_prep(xa_v, lq_v, u)

            def xb_prep(t):
                t0 = t * D
                xt = xbt_v[:, t0:t0 + D]
                xb = jnp.concatenate([xt, xt[DM - HD:]], axis=0).T
                xb_v[t0:t0 + D, :] = xb
                for sg in range(D // SEG):
                    p0 = (t * (D // SEG) + sg) * PRE
                    xpre_v[p0:p0 + PRE, :] = xb[sg * SEG:sg * SEG + PRE, 0:DM]

            with _scope("a_qproj"):
                j = ngrp - 1
                batch_wait(1, 3 + j)
                xat_cp.wait()
                xbt_cp.wait()
                w_wait_shared(wqa_v, 0)
                t14 = lambda i: tkv_v[i]
                t15 = items(rhs_kv(2 * j + 1))
                kv = [(t14, 2 * j, u) for u in range(0, NU, 2)] + [(t15, 2 * j + 1, u) for u in range(0, NU, 2)]
                t, rem = q_rhs(0)
                for u in range(NU):
                    project_kv(kv[u][0], kv[u][1], kv[u][2], kv[u][2] + 2)
                    xa_prep(u)
                    project_q(t, rem, 0, u)
                XG = 4
                nx = 0
                for hp in range(2, HP, 2):
                    t, rem = q_rhs(hp)
                    for u in range(NU):
                        project_q(t, rem, hp, u)
                        if u == 0:
                            for _ in range(XG):
                                if nx < S // D:
                                    xb_prep(nx)
                                    nx += 1
                                    if nx == S // D:
                                        lp_prep(lp_v)

        pl.run_scoped(
            projections,
            pltpu.VMEM((S, DC), bf16),
            pltpu.VMEM((DM, S), bf16),
            pltpu.VMEM((S, DM), bf16),
            pltpu.VMEM((2, HP, DC // 2, D), u32),
            pltpu.VMEM((2, HP, DC // 2, D), u32),
            pltpu.VMEM((2, HP, DM // 2, D), u32),
            pltpu.VMEM((7, DC // 4, 2 * D), u32),
            pltpu.VMEM((7, S // 4, DC // 2), u32),
            pltpu.VMEM((7, S // 4, DC // 2), u32),
        )

        def attention(c_v, s_v):
            row = jax.lax.broadcasted_iota(jnp.int32, (TQ, TQ), 0)
            col = jax.lax.broadcasted_iota(jnp.int32, (TQ, TQ), 1)
            tri = col <= row
            nb = S // TQ
            hq = TQ // 2
            npiece = 2
            pw = S // npiece

            def qk_piece(h, j):
                q = _unpack(q_v[h, (nb - 1) * hq:nb * hq, :])
                k = _unpack(k_v[h, j * pw // 2:(j + 1) * pw // 2, :])
                s_v[:, j * pw:(j + 1) * pw] = jax.lax.dot_general(q, k, NT, preferred_element_type=f32)

            def qk(h, i, j0=0, j1=None):
                j1 = i + 1 if j1 is None else j1
                q = _unpack(q_v[h, i * hq:(i + 1) * hq, :])
                k = _unpack(k_v[h, j0 * hq:j1 * hq, :])
                return jax.lax.dot_general(q, k, NT, preferred_element_type=f32)

            def anchor_plan():
                ops = []
                for e in range(UH):
                    for i in range(nb - 1, -1, -1):
                        if i > 0:
                            ops.append(("qk", e, i - 1, 32 * i))
                        if i < npiece:
                            ops.append(("piece", e, i, 32 * nb // npiece))
                        ops.append(("pv", e, i, 32 * (i + 1)))
                t, start, end = 0, [], []
                for op in ops:
                    start.append(t)
                    t += op[3]
                    end.append(t)
                plan = {}
                for a, op in enumerate(ops):
                    if op[0] != "pv" or op[2] < ANCHOR_MIN:
                        continue
                    for b in range(a + 1, len(ops)):
                        if ops[b][0] == "qk" and start[b] >= end[a] + ANCHOR_LAG:
                            plan.setdefault((ops[b][1], ops[b][2]), []).append((op[1], op[2]))
                            break
                return plan

            def heads(j, c):
                @pl.when(j == 0)
                def _():
                    w_start_shared(wkb_hbm, wb_v.at[1], 2, range(HP // 2, HP))
                    w_start_shared(wvb_hbm, wb_v.at[2], 3, range(HP))

                plan = anchor_plan()

                def gated_qk(e, i):
                    h = j * UH + e
                    if (e, i) not in plan:
                        return qk(h, i)
                    w = None
                    for ea, ia in plan[e, i]:
                        u = c_v[j * UH + ea, ia * hq:(ia + 1) * hq, :]
                        for r in range(0, hq, 8):
                            w = u[r:r + 8] if w is None else w | u[r:r + 8]
                    zero = (w >> 31) >> 1
                    q = q_v[h, i * hq:(i + 1) * hq, :]
                    q = _unpack(jnp.concatenate([q[0:8] | zero, q[8:]], axis=0))
                    k = _unpack(k_v[h, 0:(i + 1) * hq, :])
                    return jax.lax.dot_general(q, k, NT, preferred_element_type=f32)

                s_next = s_v[...]
                for e in range(UH):
                    h = j * UH + e
                    hn = jnp.minimum(h + 1, H - 1) if e == UH - 1 else h + 1
                    pieces = []
                    for i in range(nb - 1, -1, -1):
                        s = s_next
                        if i > 0:
                            s_next = gated_qk(e, i - 1)
                        if i < npiece:
                            if e == UH - 1:
                                qk_piece(hn, npiece - 1 - i)
                            else:
                                jj = npiece - 1 - i
                                pieces.append(qk(hn, nb - 1, jj * nb // npiece, (jj + 1) * nb // npiece))
                        sd = jnp.where(tri, s[:, i * TQ:], NEG)
                        s = jnp.concatenate([s[:, :i * TQ], sd], axis=1) if i > 0 else sd
                        m = jnp.max(s, axis=1, keepdims=True)
                        p = jnp.exp2(s - m)
                        l = jnp.sum(p, axis=1, keepdims=True)
                        v = _unpack(v_v[h, 0:(i + 1) * hq, :])
                        o = jnp.dot(p.astype(bf16), v, preferred_element_type=f32)
                        c_v[h, i * hq:(i + 1) * hq, :] = _pack((o * _recip(l)).astype(bf16))
                    if e < UH - 1:
                        s_next = jnp.concatenate(pieces, axis=1)
                return c
            with _scope("a_attn"):
                for j in range(npiece):
                    qk_piece(0, j)
                jax.lax.fori_loop(0, H // UH, heads, 0)

            woa_cp.wait()
            wob_cp.wait()
            mem_cp.wait()
            for t in range(3):
                w_wait_shared(wb_v.at[t], 1 + t)
            mh = DM // 4

            def wo_prep(hh):
                a11, a21 = woa_v[hh, 0:mh, :], woa_v[hh, mh:2 * mh, :]
                a12, a22 = woa_v[hh + HP, 0:mh, :], woa_v[hh + HP, mh:2 * mh, :]
                for i, w in enumerate(_sum_words(_strassen_lhs, a11, a12, a21, a22, (2, 3), (a11, a22))):
                    if i not in (2, 3):
                        k_v[hh, i * mh:(i + 1) * mh, :] = w

            def wob_prep(hp):
                w1, w2 = _unpack(wobt_v[2 * hp]), _unpack(wobt_v[2 * hp + 1])
                a, b = KM + HD, KM + 2 * HD
                d12 = (w1[a:b].astype(f32) - w2[a:b].astype(f32)).astype(bf16)
                d21 = (w2[b:].astype(f32) - w1[b:].astype(f32)).astype(bf16)
                rows = slice(hp * HD, (hp + 1) * HD)
                wob_v[0, rows, :] = _pack(jnp.concatenate([w1[:a], d12], axis=0).T)
                wob_v[1, rows, :] = _pack(jnp.concatenate([w2[:a], d21], axis=0).T)
                wos_v[rows, :] = _pack(jnp.concatenate([w1[b:], w2[a:b]], axis=0).T)

            def oproj(tp):
                w0 = tp * D
                per = []
                for hh in range(HP):
                    b11, b21 = c_v[hh, w0:w0 + D // 2, :], c_v[hh + HP, w0:w0 + D // 2, :]
                    b12, b22 = c_v[hh, w0 + D // 2:w0 + D, :], c_v[hh + HP, w0 + D // 2:w0 + D, :]
                    per.append(_sum_words(_strassen_rhs, b11, b12, b21, b22, (1, 4), (b11, b22)))

                def lhs(i):
                    if i == 2:
                        return _unpack(jnp.concatenate([woa_v[hh, 0:mh, :] for hh in range(HP)], axis=1))
                    if i == 3:
                        return _unpack(jnp.concatenate([woa_v[hh + HP, mh:2 * mh, :] for hh in range(HP)], axis=1))
                    return _unpack(jnp.concatenate([k_v[hh, i * mh:(i + 1) * mh, :] for hh in range(HP)], axis=1))

                def rhs(i):
                    return _unpack(jnp.concatenate([per[hh][i] for hh in range(HP)], axis=1))
                c11, c12, c21, c22 = _strassen(lhs, rhs, NT)
                t0 = 2 * tp * D
                out_v[t0:t0 + D, 0:DM] = jnp.concatenate([c11, c21], axis=0).T.astype(bf16)
                out_v[t0 + D:t0 + 2 * D, 0:DM] = jnp.concatenate([c12, c22], axis=0).T.astype(bf16)

            b_pre(lp_v)
            with _scope("a_oproj"):
                for hh in range(HP):
                    wo_prep(hh)
                for tp in range(S // D // 2):
                    oproj(tp)
                    for hp in range(2 * tp, 2 * tp + 2):
                        wob_prep(hp)

        pl.run_scoped(
            attention,
            pltpu.VMEM((H, S // 2, D), u32),
            pltpu.VMEM((TQ, S), f32),
        )

    pl.run_scoped(
        phase_a,
        pltpu.VMEM((H, DM // 2, D), u32),
        pltpu.VMEM((DM, S), bf16),
        pltpu.VMEM((H, DM // 2, D), u32),
        pltpu.VMEM((7, NSEG * PRE // 4, DC // 2), u32),
    )

    def out_copy(j):
        rows = pl.ds(pl.multiple_of(j * (OUTER * SEG), OUTER * SEG), OUTER * SEG)
        return pltpu.make_async_copy(out_v.at[rows, :], out_hbm.at[rows, :], sem.at[SEM_OUT + j])

    def phase_b(post_v):
        GP = HG // 2
        GC = GP * 3 * D
        KA = KM + 2 * HD
        lane = jax.lax.broadcasted_iota(jnp.int32, (1, GC), 1)
        colscale = jnp.where(lane % (3 * D) < D, QSCALE, 1.0).astype(f32)
        low = jax.lax.broadcasted_iota(jnp.int32, (1, D), 1) < HD

        def swap(x):
            return pltpu.roll(x, HD, 1)

        def wgroup(g):
            cols = [(hp, t) for hp in range(g * GP, (g + 1) * GP) for t in range(3)]
            own = [_unpack(jnp.concatenate([wb_v[t, e, hp, 0:KA // 2, :] for hp, t in cols], axis=1)) for e in range(2)]
            both = jnp.concatenate([jnp.concatenate([wb_v[t, e, hp, KA // 2:, :] for hp, t in cols], axis=1)
                                    for e in range(2)], axis=0)
            return own[0], own[1], _unpack(both)

        def out_project(even, odd, both, p0, p1):
            rows = slice(p0 * HD, p1 * HD)
            return [jnp.dot(even, _unpack(wob_v[0, rows, :]), preferred_element_type=f32),
                    jnp.dot(odd, _unpack(wob_v[1, rows, :]), preferred_element_type=f32),
                    jnp.dot(both, _unpack(wos_v[rows, :]), preferred_element_type=f32)]

        def out_add(acc, part):
            e, o, b = part
            new = [e[:, :KM] + o[:, :KM], e[:, KM:], o[:, KM:], b]
            return new if acc is None else [x + y for x, y in zip(acc, new)]

        def out_finish(acc):
            main, e, o, b = acc
            mid = e + jnp.where(low, o, b)
            last = jnp.where(low, swap(o) + b, o + swap(b))
            return jnp.concatenate([main, mid, last], axis=1)

        ri = jax.lax.broadcasted_iota(jnp.int32, (2 * L, 2 * L), 0)
        ci = jax.lax.broadcasted_iota(jnp.int32, (2 * L, 2 * L), 1)

        def second(i):
            return jnp.where(i < 2 * SEG, i // SEG, (i - 2 * SEG) // PRE)

        def pos(i):
            j = i % SEG
            return jnp.where(i < 2 * SEG, jnp.where(j < T, j + (MEM + PRE), j - T), MEM + i % PRE)
        same = second(ri) == second(ci)
        mask = same & ((pos(ri) < MEM) | (pos(ri) >= pos(ci)))
        fill = jnp.where(same, NEG, -jnp.inf).astype(f32)

        def step(s, slot, mem):
            xt = xb_v[pl.ds(pl.multiple_of(SEG * s + PRE, 8), T), :]
            l1 = jnp.concatenate([xt.astype(f32), mem], axis=0)
            mid, last = l1[:, KM:KA], l1[:, KA:]
            l_even = l1[:, :KA].astype(bf16)
            l_odd = jnp.concatenate([l1[:, :KM], jnp.where(low, mid, last)], axis=1).astype(bf16)
            l_both = jnp.where(low, last, mid).astype(bf16)
            p0 = pl.multiple_of(PRE * s, 8)
            proj = []
            for g in range(G):
                w_even, w_odd, w_both = wgroup(g)
                both = jnp.dot(l_both, w_both, preferred_element_type=f32)
                even = jnp.dot(l_even, w_even, preferred_element_type=f32)
                odd = jnp.dot(l_odd, w_odd, preferred_element_type=f32)
                proj.append([((x + both) * colscale).astype(bf16) for x in (even, odd)])

            def rows(hp, t):
                g, c0 = hp // GP, (hp % GP) * 3 * D + t * D
                return jnp.concatenate([proj[g][0][:, c0:c0 + D], proj[g][1][:, c0:c0 + D],
                                        _unpack(pre_ref(hp * 3 + t)[pl.ds(p0, PRE), :])], axis=0)

            scores = [jax.lax.dot_general(rows(hp, 0), rows(hp, 1), NT, preferred_element_type=f32)
                      for hp in range(HP)]
            ctx = {}

            def attend(g):
                for hp in range(g * HG // 2, (g + 1) * HG // 2):
                    sc = jnp.where(mask, scores[hp], fill)
                    m = jnp.max(sc, axis=1, keepdims=True)
                    p = jnp.exp2(sc - m)
                    l = jnp.sum(p, axis=1, keepdims=True)
                    o = jnp.dot(p.astype(bf16), rows(hp, 2), preferred_element_type=f32) * _recip(l)
                    ctx[hp] = [o[0:SEG, :].astype(bf16), o[SEG:2 * SEG, :].astype(bf16),
                               (o[0:SEG, :] + o[SEG:2 * SEG, :]).astype(bf16)]
                    for e in range(2):
                        post_v[e, slot * PRE:(slot + 1) * PRE, hp * D:(hp + 1) * D] = o[2 * SEG + e * PRE:2 * SEG + (e + 1) * PRE, :]

            parts = []

            def oproj(g):
                lhs = [jnp.concatenate([ctx[hp][e] for hp in range(g * GP, (g + 1) * GP)], axis=1) for e in range(3)]
                parts.append(out_project(*lhs, g * GP, (g + 1) * GP))

            for t in range(G + 2):
                if t < G:
                    attend(t)
                if t >= 2:
                    oproj(t - 2)
            acc = None
            for a in parts:
                acc = out_add(acc, a)
            accb = out_finish(acc).astype(bf16)
            out_v[pl.ds(pl.multiple_of(SEG * s + PRE, 8), T), DM:2 * DM] = accb[0:T, 0:DM]
            return accb[T:, :].astype(f32), ctx[HP - 1][1]

        PP = HP // OUTER

        def deferred_rows():
            even, odd = post_v[0], post_v[1]
            return even.astype(bf16), odd.astype(bf16), (even + odd).astype(bf16)

        def finish(j, acc):
            r = out_finish(acc).astype(bf16)
            for sg in range(OUTER):
                r0 = pl.multiple_of((j * OUTER + sg) * SEG, SEG)
                out_v[pl.ds(r0, PRE), DM:2 * DM] = r[sg * PRE:(sg + 1) * PRE, 0:DM]

        def after(x, late):
            u = _pack(late[0:2 * OUTER * PRE // 2, :])
            zero = (u >> 31) & (~u >> 31)
            return _unpack(_pack(x) | jnp.concatenate([zero] * (x.shape[1] // D), axis=1))

        def outer(j, mem):
            prev = deferred_rows()

            def partial(i, late):
                x = [p[:, i * PP * D:(i + 1) * PP * D] for p in prev]
                if late is not None:
                    x = [after(p, late) for p in x]
                return out_project(*x, i * PP, (i + 1) * PP)
            acc = out_add(None, partial(0, None))
            for i in range(OUTER):
                mem, late = step(j * OUTER + i, i, mem)
                if i + 1 < OUTER:
                    acc = out_add(acc, partial(i + 1, late))
            finish(jnp.maximum(j - 1, 0), acc)

            @pl.when(j > 0)
            def _():
                out_copy(j - 1).start()
            return mem
        with _scope("b_loop"):
            post_v[...] = jnp.zeros(post_v.shape, f32)
            mem0 = mem_v[0:MEM, :].astype(f32)
            jax.lax.fori_loop(0, NOUTER, outer, jnp.concatenate([mem0, mem0[:, DM - HD:]], axis=1))
            finish(NOUTER - 1, out_add(None, out_project(*deferred_rows(), 0, HP)))
            out_copy(NOUTER - 1).start()
        with _scope("b_outwait"):
            for j in range(NOUTER):
                out_copy(j).wait()

    pl.run_scoped(
        phase_b,
        pltpu.VMEM((2, OUTER * PRE, HP * D), f32),
    )


@jax.jit
def pallas_concat_heads__compressed_kv_cla__memory_aug_recurrent_mem_tr__prompt_kernel(
    A_x: jax.Array,
    A_c_kv: jax.Array,
    A_w_q: jax.Array,
    A_w_uk: jax.Array,
    A_w_uv: jax.Array,
    A_w_o: jax.Array,
    B_x: jax.Array,
    B_mem0: jax.Array,
    B_Wq: jax.Array,
    B_Wk: jax.Array,
    B_Wv: jax.Array,
    B_Wo: jax.Array,
    B_seg_len=SEG,
):
    def t2(x):
        return jnp.transpose(x, (0, 2, 1)).reshape(DM, S)

    def w3(w):
        return w.reshape(w.shape[0] // 2, 2 * H, D)

    def wo3(w):
        return jnp.transpose(w, (0, 2, 1))

    any_spec = pl.BlockSpec(memory_space=pl.ANY)
    out = pl.pallas_call(
        _kernel,
        out_shape=jax.ShapeDtypeStruct((S, 2 * DM), bf16),
        in_specs=[any_spec] * 12,
        out_specs=any_spec,
        scratch_shapes=[
            pltpu.VMEM((S, 2 * DM), bf16),
            pltpu.VMEM((S, DMP), bf16),
            pltpu.VMEM((NSEG * PRE, DM), bf16),
            pltpu.VMEM((3, 2, HP, DM // 2, D), u32),
            pltpu.VMEM((2, HP * D // 2, KM + 2 * HD), u32),
            pltpu.VMEM((HP * D // 2, D), u32),
            pltpu.VMEM((8 * MEM, DM), bf16),
            pltpu.VMEM((H, S // 2, D), u32),
            pltpu.VMEM((H, S // 2, D), u32),
            pltpu.VMEM((H, S // 2, D), u32),
            pltpu.SemaphoreType.DMA((NSEM,)),
        ],
        compiler_params=pltpu.CompilerParams(vmem_limit_bytes=126 * 1024 * 1024),
    )(t2(A_x), A_c_kv.reshape(S, DC), w3(A_w_q), w3(A_w_uk), w3(A_w_uv), wo3(A_w_o),
      t2(B_x), B_mem0.reshape(MEM, DM), w3(B_Wq), w3(B_Wk), w3(B_Wv), wo3(B_Wo))
    return out.reshape(1, S, 2 * DM)
```

```python
import contextlib

import jax
import jax.numpy as jnp
import jax.experimental.pallas as pl
import jax.experimental.pallas.tpu as pltpu

S = 2048
DM = 576
DC = 512
H = 32
D = 128
MEM = 8
SEG = 32
L = MEM + SEG
NSEG = S // SEG
HP = H // 2
HD = D // 2
KM = DM - 3 * HD
DMP = DM + HD

LOG2E = 1.4426950408889634
QSCALE = D ** -0.5 * LOG2E
NEG = -1.0e9 * LOG2E

TQ = 128
UH = 4
ANCHOR_LAG = 2000
ANCHOR_MIN = 6
RB = 512
HG = 4
G = H // HG
PRE = 8
T = SEG - PRE
OUTER = 4
NOUTER = NSEG // OUTER

bf16 = jnp.bfloat16
f32 = jnp.float32
u32 = jnp.uint32
NT = (((1,), (1,)), ((), ()))

SEM_CKV = 0
SEM_XAT = 5
SEM_XBT = 6
SEM_MEM = 7
SEM_WOA = 8
SEM_WOB = 9
SEM_OUT = 10
SEM_WALL = SEM_OUT + NOUTER
SEM_W = SEM_WALL + 4
NSEM = SEM_W + 3 + HP // 2

_PROFILE = False
PG = 1

def _scope(name):
    return jax.named_scope(name) if _PROFILE else contextlib.nullcontext()


def _unpack(w32):
    return pltpu.bitcast(w32, bf16)


def _pack(x):
    return pltpu.bitcast(x, u32)


def _lo(w):
    return pltpu.bitcast(w << 16, f32)


def _hi(w):
    return pltpu.bitcast(w & u32(0xFFFF0000), f32)


def _words(even, odd):
    return pltpu.bitcast(pltpu.pack_elementwise([even, odd], packed_dtype=bf16), u32)


def _strassen_lhs(a11, a12, a21, a22):
    return [a11 + a22, a21 + a22, a11, a22, a11 + a12, a21 - a11, a12 - a22]


def _strassen_rhs(b11, b12, b21, b22):
    return [b11 + b22, b11, b12 - b22, b21 - b11, b22, b11 + b12, b21 + b22]


def _sum_words(combine, x11, x12, x21, x22, raw_idx, raw):
    lo = combine(_lo(x11), _lo(x12), _lo(x21), _lo(x22))
    hi = combine(_hi(x11), _hi(x12), _hi(x21), _hi(x22))
    words = [pltpu.bitcast(pltpu.pack_elementwise([a, b], packed_dtype=bf16), u32) for a, b in zip(lo, hi)]
    for i, r in zip(raw_idx, raw):
        words[i] = r
    return words


def _strassen(lhs, rhs, dims=(((1,), (0,)), ((), ())), order=0):
    def m(i):
        return jax.lax.dot_general(lhs(i - 1), rhs(i - 1), dims, preferred_element_type=f32)
    if order == 0:
        m1 = m(1)
        m2 = m(2)
        c22 = m1 - m2
        m4 = m(4)
        c11 = m1 + m4
        c21 = m2 + m4
        c22 = c22 + m(6)
        m3 = m(3)
        c22 = c22 + m3
        m5 = m(5)
        c11 = c11 - m5
        c12 = m3 + m5
        c11 = c11 + m(7)
        return c11, c12, c21, c22
    m3 = m(3)
    m4 = m(4)
    m5 = m(5)
    c12 = m3 + m5
    c11 = m4 - m5
    m2 = m(2)
    c21 = m4 + m2
    c22 = m3 - m2
    m1 = m(1)
    c11 = c11 + m1
    c22 = c22 + m1
    c22 = c22 + m(6)
    c11 = c11 + m(7)
    return c11, c12, c21, c22


def _rhs_words(s0, s1, z0, z1):
    per = [_strassen_rhs(_lo(s), _hi(s), _lo(z), _hi(z)) for s, z in ((s0, z0), (s1, z1))]
    words = [pltpu.bitcast(pltpu.pack_elementwise([per[0][i], per[1][i]], packed_dtype=bf16), u32)
             for i in range(7)]
    words[1] = (s0 & u32(0xFFFF)) | (s1 << 16)
    words[4] = (z0 >> 16) | (z1 & u32(0xFFFF0000))
    return words


_L233 = (((0, 1, 1), (1, 0, 1)), ((0, 1, 1),), ((0, 0, 1), (1, 0, -1)), ((0, 1, 1), (1, 1, -1)), ((1, 0, 1),),
         ((0, 0, -1), (0, 1, -1)), ((1, 0, 1), (1, 1, 1)), ((0, 0, 1), (0, 2, 1), (1, 0, -1)), ((1, 2, 1),),
         ((0, 2, 1),), ((1, 0, 1), (1, 2, 1), (0, 0, -1), (0, 2, -1)), ((0, 0, -1), (0, 2, -1)),
         ((1, 1, 1), (1, 2, 1), (0, 1, -1)), ((1, 1, -1), (1, 2, -1)),
         ((0, 1, 1), (0, 2, 1), (1, 1, -1), (1, 2, -1)))
_R233 = (((0, 1, 1), (1, 0, 1)), ((1, 1, 1), (1, 2, 1), (0, 1, -1)), ((0, 0, 1), (0, 1, 1), (2, 0, -1)),
         ((2, 1, 1), (1, 0, -1), (1, 1, -1)), ((0, 0, 1), (0, 2, 1), (1, 0, -1)), ((0, 1, 1),), ((1, 0, 1),),
         ((0, 2, 1), (2, 0, 1)), ((2, 0, 1), (2, 2, 1), (1, 2, -1)), ((2, 1, 1), (2, 2, 1), (0, 2, -1)),
         ((2, 0, 1),), ((0, 2, 1),), ((1, 2, 1), (2, 1, 1)), ((1, 2, 1),), ((2, 1, 1),))
_PIECES = ((0, 32, 64), (128, 160, 96), (192, 224, 256))


def _signed_sum(terms, get):
    acc = None
    for a, b, c in terms:
        x = get(a, b)
        if acc is None:
            acc = x if c > 0 else -x
        else:
            acc = acc + x if c > 0 else acc - x
    return acc


def _lhs233(y1, y2, store):
    low = jax.lax.broadcasted_iota(jnp.int32, (1, D), 1) < HD
    base = {}
    for i in range(2):
        t1 = [y1[i][:, c * D:(c + 1) * D] for c in range(5)]
        t2 = [y2[i][:, c * D:(c + 1) * D] for c in range(5)]
        r1, r2 = pltpu.roll(t1[1], HD, 1), pltpu.roll(t2[1], HD, 1)
        for k in range(3):
            a1, a2 = t1[(0, 2, 3)[k]], t2[(0, 2, 3)[k]]
            lo1 = (t1[1], r1, t1[4])[k]
            hi1, hi2 = (r1, t1[1], t1[4])[k], (r2, t2[1], t2[4])[k]
            base[i, k] = (jnp.where(low, a1, a1 - a2), jnp.where(low, a2, hi2 - hi1), jnp.where(low, lo1, a2))
    for r, terms in enumerate(_L233):
        for p in range(3):
            store(r, p, _pack(_signed_sum(terms, lambda i, k: base[i, k][p]).astype(bf16)))


def _rhs233(slabs):
    def chunk(j, par, k):
        s = slabs[j][par]
        a, b, c = _PIECES[k]
        return s[a:a + 96] if k != 1 else jnp.concatenate([s[a:a + 64], s[c:c + 32]], axis=0)

    def words(r):
        terms = _R233[r]
        if len(terms) == 1:
            k, j, _ = terms[0]
            s0, s1 = chunk(j, 0, k), chunk(j, 1, k)
            return (s0 & u32(0xFFFF)) | (s1 << 16), (s0 >> 16) | (s1 & u32(0xFFFF0000))
        half = [[_signed_sum(terms, lambda k, j: f(chunk(j, par, k))) for par in range(2)] for f in (_lo, _hi)]
        return _words(*half[0]), _words(*half[1])
    return words


def _passes(w):
    return (w[0:64], jnp.concatenate([w[0:32], w[64:96]], axis=0), jnp.concatenate([w[64:96], w[32:64]], axis=0))


def _mm233(product):
    def add(a, b):
        return [x + y for x, y in zip(a, b)]

    def sub(a, b):
        return [x - y for x, y in zip(a, b)]
    p13 = product(13)
    s1 = add(product(12), p13)
    s2 = add(s1, product(14))
    p11 = product(11)
    z = add(s2, p11)
    yield (0, 2), sub(product(9), z)
    s3 = add(product(7), p11)
    s4 = add(s3, product(10))
    y = add(s4, p13)
    yield (1, 2), sub(product(8), y)
    p4 = product(4)
    c10 = add(s4, p4)
    c00 = add(s3, p4)
    p6 = product(6)
    yield (1, 0), add(c10, p6)
    c11 = sub(s1, p6)
    p5 = product(5)
    c01 = sub(s2, p5)
    c00 = add(c00, p5)
    p1 = product(1)
    yield (0, 1), add(c01, p1)
    c11 = add(c11, p1)
    p0 = product(0)
    c00 = add(c00, p0)
    c11 = add(c11, p0)
    yield (1, 1), add(c11, product(3))
    yield (0, 0), add(c00, product(2))


def _recip(l):
    r = pl.reciprocal(l, approx=True)
    return r * (2.0 - l * r)


def _kernel(xat_hbm, ckv_hbm, wqa_hbm, wuk_hbm, wuv_hbm, woa_hbm,
            xbt_hbm, mem0_hbm, wqb_hbm, wkb_hbm, wvb_hbm, wob_hbm,
            out_hbm,
            out_v, xb_v, xpre_v, wb_v, wob_v, wos_v, mem_v, q_v, k_v, v_v, sem):

    def w_copy(w_hbm, dst, slot, par, hp):
        return pltpu.make_async_copy(w_hbm.bitcast(u32).at[:, par * HP + hp, :], dst.at[par, hp], sem.at[slot])

    def w_start_shared(w_hbm, dst, widx, hps):
        for hp in hps:
            for par in range(2):
                w_copy(w_hbm, dst, SEM_WALL + widx, par, hp).start()

    def w_wait_shared(dst, widx):
        pltpu.make_async_copy(dst, dst, sem.at[SEM_WALL + widx]).wait()

    def w_combine(dst, hp):
        a = dst[0, hp]
        b = dst[1, hp]
        ev = (a & u32(0xFFFF)) | (b << 16)
        od = (a >> 16) | (b & u32(0xFFFF0000))
        return ev, od

    def w_pair(dst, hp):
        return jnp.concatenate(w_combine(dst, hp), axis=1)

    wb_hbm = (wqb_hbm, wkb_hbm, wvb_hbm)

    def pre_ref(j):
        n = NSEG * PRE
        return q_v.at[j // 2, (j % 2) * n:(j % 2 + 1) * n, :]

    def lp_prep(lp_v):
        nr = NSEG * PRE // 4
        x = xpre_v[...].astype(f32)

        def store(r, p, w):
            lp_v[r, p] = w
        _lhs233([x[0:nr], x[2 * nr:3 * nr]], [x[nr:2 * nr], x[3 * nr:]], store)

    def b_pre(lp_v):
        nr = NSEG * PRE // 4
        with _scope("b_pre"):
            for g in range(HP // PG):
                hps = range(g * PG, (g + 1) * PG)
                slabs = {}
                for hp in hps:
                    for t in range(3):
                        s0, s1 = wb_v[t, 0, hp], wb_v[t, 1, hp]
                        slabs[hp, t] = (s0, s1)
                        ev = (s0 & u32(0xFFFF)) | (s1 << 16)
                        od = (s0 >> 16) | (s1 & u32(0xFFFF0000))
                        a, b = (KM + HD) // 2, (KM + 2 * HD) // 2
                        d12 = _words(_lo(s0[a:b]) - _hi(s0[a:b]), _lo(s1[a:b]) - _hi(s1[a:b]))
                        d21 = _words(_hi(s0[b:]) - _lo(s0[b:]), _hi(s1[b:]) - _lo(s1[b:]))
                        wb_v[t, 0, hp] = jnp.concatenate([ev[:a], d12, ev[b:]], axis=0)
                        wb_v[t, 1, hp] = jnp.concatenate([od[:a], d21, od[a:b]], axis=0)
                rhs = [_rhs233([slabs[hp, t] for t in range(3)]) for hp in hps]

                def product(r):
                    w = jnp.concatenate([x for f in rhs for x in f(r)], axis=1)
                    wa, wb, wc = _passes(w)
                    c = jnp.dot(_unpack(lp_v[r, 2]), _unpack(wc), preferred_element_type=f32)
                    a = jnp.dot(_unpack(lp_v[r, 0]), _unpack(wa), preferred_element_type=f32)
                    b = jnp.dot(_unpack(lp_v[r, 1]), _unpack(wb), preferred_element_type=f32)
                    return [a + c, b + c]
                for (i, t), blk in _mm233(product):
                    for y in range(2):
                        x0 = (2 * i + y) * nr
                        for n, hp in enumerate(hps):
                            two = [blk[y][:, (2 * n + e) * D:(2 * n + e + 1) * D] for e in range(2)]
                            if t == 0:
                                two = [z * QSCALE for z in two]
                            two = [z.reshape(nr // PRE, 1, PRE, D) for z in two]
                            two = jnp.concatenate(two, axis=1).reshape(2 * nr, D)
                            pre_ref(hp * 3 + t)[x0:x0 + nr, :] = _pack(two.astype(bf16))


    def phase_a(woa_v, xbt_v, wobt_v, lp_v):
        woa_cp = pltpu.make_async_copy(woa_hbm.bitcast(u32), woa_v, sem.at[SEM_WOA])
        xbt_cp = pltpu.make_async_copy(xbt_hbm, xbt_v, sem.at[SEM_XBT])
        mem_cp = pltpu.make_async_copy(mem0_hbm, mem_v.at[0:MEM, :], sem.at[SEM_MEM])
        wob_cp = pltpu.make_async_copy(wob_hbm.bitcast(u32), wobt_v, sem.at[SEM_WOB])

        def projections(ckv_v, xat_v, xa_v, wuk_v, wuv_v, wqa_v, tkv_v, lq_v, la_v):
            UR = 2 * D
            NU = S // UR
            kh = DC // 2
            ngrp = HP // 2

            def batch_start(pairs, slot):
                for hp in pairs:
                    for w_hbm, dst in ((wuk_hbm, wuk_v), (wuv_hbm, wuv_v)):
                        for par in range(2):
                            w_copy(w_hbm, dst, SEM_W + slot, par, hp).start()

            def batch_wait(npairs, slot):
                part = wuk_v.at[:, 0:2 * npairs]
                pltpu.make_async_copy(part, part, sem.at[SEM_W + slot]).wait()

            def group(j):
                return [hp for hp in (2 * j + 1, 2 * j + 2) if hp < HP]

            def first_copies(w_hbm, dst, slot):
                return [w_copy(w_hbm, dst, SEM_W + slot, par, 0) for par in range(2)]

            def first_wait(dst, slot):
                part = dst.at[:, 0:1]
                pltpu.make_async_copy(part, part, sem.at[SEM_W + slot]).wait()

            pieces = [(0, 1), (1, 2), (2, 4), (4, 6), (6, 8)]

            def ckv_cp(j):
                rows = slice(pieces[j][0] * UR, pieces[j][1] * UR)
                return pltpu.make_async_copy(ckv_hbm.at[rows, :], ckv_v.at[rows, :], sem.at[SEM_CKV + j])
            xat_cp = pltpu.make_async_copy(xat_hbm, xat_v, sem.at[SEM_XAT])

            with _scope("a_issue0"):
                for cp in first_copies(wuk_hbm, wuk_v, 0) + first_copies(wuv_hbm, wuv_v, 1):
                    cp.start()
                for j in range(4):
                    ckv_cp(j).start()
                batch_start([1], 2)
                ckv_cp(4).start()
                batch_start([2], 3)
                for j in range(1, ngrp - 1):
                    batch_start(group(j), 3 + j)

            def lhs_prep(src_v, dst_v, u):
                c = src_v[u * UR:(u + 1) * UR, 0:DC].astype(f32)
                ops = _strassen_lhs(c[:D, :kh], c[:D, kh:], c[D:, :kh], c[D:, kh:])
                for i, o in enumerate(ops):
                    dst_v[i, u * D // 2:(u + 1) * D // 2, :] = _pack(o.astype(bf16))

            def rhs_words(w_v, hp):
                n = kh // 2
                s0, s1 = w_v[0, hp, 0:n, :], w_v[1, hp, 0:n, :]
                z0, z1 = w_v[0, hp, n:2 * n, :], w_v[1, hp, n:2 * n, :]
                return _rhs_words(s0, s1, z0, z1)

            def rhs_kv(hp):
                return [jnp.concatenate([a, b], axis=1) for a, b in zip(rhs_words(wuk_v, hp), rhs_words(wuv_v, hp))]

            def items(lst):
                return lambda i: lst[i]

            def project_kv(t, hp, u0, u1):
                c = _strassen(lambda i: _unpack(la_v[i, u0 * D // 2:u1 * D // 2, :]), lambda i: _unpack(t(i)), order=1)
                for u in range(u0, u1):
                    rows = slice((u - u0) * D, (u - u0 + 1) * D)
                    top = u * D
                    for blk, h, p0 in ((c[0], 2 * hp, top), (c[1], 2 * hp + 1, top),
                                       (c[2], 2 * hp, top + D // 2), (c[3], 2 * hp + 1, top + D // 2)):
                        blk = blk[rows, :].astype(bf16)
                        k_v[h, p0:p0 + D // 2, :] = _pack(blk[:, 0:D])
                        v_v[h, p0:p0 + D // 2, :] = _pack(blk[:, D:2 * D])

            KU = 2

            def project_pair(t, hp):
                for u in range(0, NU, KU):
                    project_kv(t, hp, u, u + KU)

            def kv_first():
                first_wait(wuk_v, 0)
                first_wait(wuv_v, 1)
                t = items(rhs_kv(0))
                for j in range(4):
                    ckv_cp(j).wait()
                    for u in range(*pieces[j]):
                        lhs_prep(ckv_v, la_v, u)
                    project_kv(t, 0, *pieces[j])
                ckv_cp(4).wait()
                batch_wait(1, 2)
                for u in range(*pieces[4]):
                    lhs_prep(ckv_v, la_v, u)
                project_kv(t, 0, *pieces[4])
                t1 = items(rhs_kv(1))
                project_kv(t1, 1, 0, 2)
                batch_wait(1, 3)
                for i, w in enumerate(rhs_kv(2)):
                    tkv_v[i] = w
                for u in range(2, NU, 2):
                    project_kv(t1, 1, u, u + 2)

            def kv_body(j, c):
                @pl.when(j == 2)
                def _():
                    xat_cp.start()
                    batch_start(group(ngrp - 1), 3 + ngrp - 1)
                    w_start_shared(wqa_hbm, wqa_v, 0, range(HP))
                    xbt_cp.start()
                batch_wait(2, 3 + j)
                project_pair(lambda i: tkv_v[i], 2 * j)
                t1 = items(rhs_kv(2 * j + 1))
                for i, w in enumerate(rhs_kv(2 * j + 2)):
                    tkv_v[i] = w
                project_pair(t1, 2 * j + 1)
                return c

            with _scope("a_kvproj"):
                kv_first()
                jax.lax.fori_loop(1, ngrp - 1, kv_body, 0)

            woa_cp.start()
            wob_cp.start()
            mem_cp.start()
            w_start_shared(wqb_hbm, wb_v.at[0], 1, range(HP))
            w_start_shared(wkb_hbm, wb_v.at[1], 2, range(HP // 2))

            def q_rhs(hp):
                t = [jnp.concatenate([a, b], axis=1) for a, b in zip(rhs_words(wqa_v, hp), rhs_words(wqa_v, hp + 1))]
                rem = []
                for e in range(2):
                    for p in (hp, hp + 1):
                        a, b = wqa_v[0, p, kh:, :], wqa_v[1, p, kh:, :]
                        rem.append((a & u32(0xFFFF)) | (b << 16) if e == 0 else (a >> 16) | (b & u32(0xFFFF0000)))
                return t, jnp.concatenate(rem, axis=1)

            def project_q(t, rem, hp, u):
                c = _strassen(lambda i: _unpack(lq_v[i, u * D // 2:(u + 1) * D // 2, :]), lambda i: _unpack(t[i]))
                for half in range(2):
                    x0 = u * UR + half * D
                    r = jnp.dot(xa_v[x0:x0 + D, DC:DM], _unpack(rem), preferred_element_type=f32)
                    r = (jnp.concatenate([c[2 * half], c[2 * half + 1]], axis=1) + r) * QSCALE
                    r = r.astype(bf16)
                    for n, h in enumerate((2 * hp, 2 * hp + 2, 2 * hp + 1, 2 * hp + 3)):
                        q_v[h, x0 // 2:(x0 + D) // 2, :] = _pack(r[:, n * D:(n + 1) * D])

            def xa_prep(u):
                for t in range(u * UR // D, (u + 1) * UR // D):
                    xa_v[t * D:(t + 1) * D, :] = xat_v[:, t * D:(t + 1) * D].T
                lhs_prep(xa_v, lq_v, u)

            def xb_prep(t):
                t0 = t * D
                xt = xbt_v[:, t0:t0 + D]
                xb = jnp.concatenate([xt, xt[DM - HD:]], axis=0).T
                xb_v[t0:t0 + D, :] = xb
                for sg in range(D // SEG):
                    p0 = (t * (D // SEG) + sg) * PRE
                    xpre_v[p0:p0 + PRE, :] = xb[sg * SEG:sg * SEG + PRE, :]

            with _scope("a_qproj"):
                j = ngrp - 1
                batch_wait(1, 3 + j)
                xat_cp.wait()
                xbt_cp.wait()
                w_wait_shared(wqa_v, 0)
                t14 = lambda i: tkv_v[i]
                t15 = items(rhs_kv(2 * j + 1))
                kv = [(t14, 2 * j, u) for u in range(0, NU, 2)] + [(t15, 2 * j + 1, u) for u in range(0, NU, 2)]
                t, rem = q_rhs(0)
                for u in range(NU):
                    project_kv(kv[u][0], kv[u][1], kv[u][2], kv[u][2] + 2)
                    xa_prep(u)
                    project_q(t, rem, 0, u)
                XG = 4
                nx = 0
                for hp in range(2, HP, 2):
                    t, rem = q_rhs(hp)
                    for u in range(NU):
                        project_q(t, rem, hp, u)
                        if u == 0:
                            for _ in range(XG):
                                if nx < S // D:
                                    xb_prep(nx)
                                    nx += 1
                                    if nx == S // D:
                                        lp_prep(lp_v)

        pl.run_scoped(
            projections,
            pltpu.VMEM((S, DC), bf16),
            pltpu.VMEM((DM, S), bf16),
            pltpu.VMEM((S, DM), bf16),
            pltpu.VMEM((2, HP, DC // 2, D), u32),
            pltpu.VMEM((2, HP, DC // 2, D), u32),
            pltpu.VMEM((2, HP, DM // 2, D), u32),
            pltpu.VMEM((7, DC // 4, 2 * D), u32),
            pltpu.VMEM((7, S // 4, DC // 2), u32),
            pltpu.VMEM((7, S // 4, DC // 2), u32),
        )

        def attention(c_v, s_v):
            row = jax.lax.broadcasted_iota(jnp.int32, (TQ, TQ), 0)
            col = jax.lax.broadcasted_iota(jnp.int32, (TQ, TQ), 1)
            tri = col <= row
            nb = S // TQ
            hq = TQ // 2
            npiece = 2
            pw = S // npiece

            def qk_piece(h, j):
                q = _unpack(q_v[h, (nb - 1) * hq:nb * hq, :])
                k = _unpack(k_v[h, j * pw // 2:(j + 1) * pw // 2, :])
                s_v[:, j * pw:(j + 1) * pw] = jax.lax.dot_general(q, k, NT, preferred_element_type=f32)

            def qk(h, i, j0=0, j1=None):
                j1 = i + 1 if j1 is None else j1
                q = _unpack(q_v[h, i * hq:(i + 1) * hq, :])
                k = _unpack(k_v[h, j0 * hq:j1 * hq, :])
                return jax.lax.dot_general(q, k, NT, preferred_element_type=f32)

            def anchor_plan():
                ops = []
                for e in range(UH):
                    for i in range(nb - 1, -1, -1):
                        if i > 0:
                            ops.append(("qk", e, i - 1, 32 * i))
                        if i < npiece:
                            ops.append(("piece", e, i, 32 * nb // npiece))
                        ops.append(("pv", e, i, 32 * (i + 1)))
                t, start, end = 0, [], []
                for op in ops:
                    start.append(t)
                    t += op[3]
                    end.append(t)
                plan = {}
                for a, op in enumerate(ops):
                    if op[0] != "pv" or op[2] < ANCHOR_MIN:
                        continue
                    for b in range(a + 1, len(ops)):
                        if ops[b][0] == "qk" and start[b] >= end[a] + ANCHOR_LAG:
                            plan.setdefault((ops[b][1], ops[b][2]), []).append((op[1], op[2]))
                            break
                return plan

            def heads(j, c):
                @pl.when(j == 0)
                def _():
                    w_start_shared(wkb_hbm, wb_v.at[1], 2, range(HP // 2, HP))
                    w_start_shared(wvb_hbm, wb_v.at[2], 3, range(HP))

                plan = anchor_plan()

                def gated_qk(e, i):
                    h = j * UH + e
                    if (e, i) not in plan:
                        return qk(h, i)
                    w = None
                    for ea, ia in plan[e, i]:
                        u = c_v[j * UH + ea, ia * hq:(ia + 1) * hq, :]
                        for r in range(0, hq, 8):
                            w = u[r:r + 8] if w is None else w | u[r:r + 8]
                    zero = (w >> 31) >> 1
                    q = q_v[h, i * hq:(i + 1) * hq, :]
                    q = _unpack(jnp.concatenate([q[0:8] | zero, q[8:]], axis=0))
                    k = _unpack(k_v[h, 0:(i + 1) * hq, :])
                    return jax.lax.dot_general(q, k, NT, preferred_element_type=f32)

                s_next = s_v[...]
                for e in range(UH):
                    h = j * UH + e
                    hn = jnp.minimum(h + 1, H - 1) if e == UH - 1 else h + 1
                    pieces = []
                    for i in range(nb - 1, -1, -1):
                        s = s_next
                        if i > 0:
                            s_next = gated_qk(e, i - 1)
                        if i < npiece:
                            if e == UH - 1:
                                qk_piece(hn, npiece - 1 - i)
                            else:
                                jj = npiece - 1 - i
                                pieces.append(qk(hn, nb - 1, jj * nb // npiece, (jj + 1) * nb // npiece))
                        sd = jnp.where(tri, s[:, i * TQ:], NEG)
                        s = jnp.concatenate([s[:, :i * TQ], sd], axis=1) if i > 0 else sd
                        m = jnp.max(s, axis=1, keepdims=True)
                        p = jnp.exp2(s - m)
                        l = jnp.sum(p, axis=1, keepdims=True)
                        v = _unpack(v_v[h, 0:(i + 1) * hq, :])
                        o = jnp.dot(p.astype(bf16), v, preferred_element_type=f32)
                        c_v[h, i * hq:(i + 1) * hq, :] = _pack((o * _recip(l)).astype(bf16))
                    if e < UH - 1:
                        s_next = jnp.concatenate(pieces, axis=1)
                return c
            with _scope("a_attn"):
                for j in range(npiece):
                    qk_piece(0, j)
                jax.lax.fori_loop(0, H // UH, heads, 0)

            woa_cp.wait()
            wob_cp.wait()
            mem_cp.wait()
            for t in range(3):
                w_wait_shared(wb_v.at[t], 1 + t)
            mh = DM // 4

            def wo_prep(hh):
                a11, a21 = woa_v[hh, 0:mh, :], woa_v[hh, mh:2 * mh, :]
                a12, a22 = woa_v[hh + HP, 0:mh, :], woa_v[hh + HP, mh:2 * mh, :]
                for i, w in enumerate(_sum_words(_strassen_lhs, a11, a12, a21, a22, (2, 3), (a11, a22))):
                    if i not in (2, 3):
                        k_v[hh, i * mh:(i + 1) * mh, :] = w

            def wob_prep(hp):
                w1, w2 = _unpack(wobt_v[2 * hp]), _unpack(wobt_v[2 * hp + 1])
                a, b = KM + HD, KM + 2 * HD
                d12 = (w1[a:b].astype(f32) - w2[a:b].astype(f32)).astype(bf16)
                d21 = (w2[b:].astype(f32) - w1[b:].astype(f32)).astype(bf16)
                rows = slice(hp * HD, (hp + 1) * HD)
                wob_v[0, rows, :] = _pack(jnp.concatenate([w1[:a], d12], axis=0).T)
                wob_v[1, rows, :] = _pack(jnp.concatenate([w2[:a], d21], axis=0).T)
                wos_v[rows, :] = _pack(jnp.concatenate([w1[b:], w2[a:b]], axis=0).T)

            def oproj(tp):
                w0 = tp * D
                per = []
                for hh in range(HP):
                    b11, b21 = c_v[hh, w0:w0 + D // 2, :], c_v[hh + HP, w0:w0 + D // 2, :]
                    b12, b22 = c_v[hh, w0 + D // 2:w0 + D, :], c_v[hh + HP, w0 + D // 2:w0 + D, :]
                    per.append(_sum_words(_strassen_rhs, b11, b12, b21, b22, (1, 4), (b11, b22)))

                def lhs(i):
                    if i == 2:
                        return _unpack(jnp.concatenate([woa_v[hh, 0:mh, :] for hh in range(HP)], axis=1))
                    if i == 3:
                        return _unpack(jnp.concatenate([woa_v[hh + HP, mh:2 * mh, :] for hh in range(HP)], axis=1))
                    return _unpack(jnp.concatenate([k_v[hh, i * mh:(i + 1) * mh, :] for hh in range(HP)], axis=1))

                def rhs(i):
                    return _unpack(jnp.concatenate([per[hh][i] for hh in range(HP)], axis=1))
                c11, c12, c21, c22 = _strassen(lhs, rhs, NT)
                t0 = 2 * tp * D
                out_v[t0:t0 + D, 0:DM] = jnp.concatenate([c11, c21], axis=0).T.astype(bf16)
                out_v[t0 + D:t0 + 2 * D, 0:DM] = jnp.concatenate([c12, c22], axis=0).T.astype(bf16)

            b_pre(lp_v)
            with _scope("a_oproj"):
                for hh in range(HP):
                    wo_prep(hh)
                for tp in range(S // D // 2):
                    oproj(tp)
                    for hp in range(2 * tp, 2 * tp + 2):
                        wob_prep(hp)

        pl.run_scoped(
            attention,
            pltpu.VMEM((H, S // 2, D), u32),
            pltpu.VMEM((TQ, S), f32),
        )

    pl.run_scoped(
        phase_a,
        pltpu.VMEM((H, DM // 2, D), u32),
        pltpu.VMEM((DM, S), bf16),
        pltpu.VMEM((H, DM // 2, D), u32),
        pltpu.VMEM((15, 3, NSEG * PRE // 8, D), u32),
    )

    def out_copy(j):
        rows = pl.ds(pl.multiple_of(j * (OUTER * SEG), OUTER * SEG), OUTER * SEG)
        return pltpu.make_async_copy(out_v.at[rows, :], out_hbm.at[rows, :], sem.at[SEM_OUT + j])

    def phase_b(post_v):
        GP = HG // 2
        GC = GP * 3 * D
        KA = KM + 2 * HD
        lane = jax.lax.broadcasted_iota(jnp.int32, (1, GC), 1)
        colscale = jnp.where(lane % (3 * D) < D, QSCALE, 1.0).astype(f32)
        low = jax.lax.broadcasted_iota(jnp.int32, (1, D), 1) < HD

        def swap(x):
            return pltpu.roll(x, HD, 1)

        def wgroup(g):
            cols = [(hp, t) for hp in range(g * GP, (g + 1) * GP) for t in range(3)]
            own = [_unpack(jnp.concatenate([wb_v[t, e, hp, 0:KA // 2, :] for hp, t in cols], axis=1)) for e in range(2)]
            both = jnp.concatenate([jnp.concatenate([wb_v[t, e, hp, KA // 2:, :] for hp, t in cols], axis=1)
                                    for e in range(2)], axis=0)
            return own[0], own[1], _unpack(both)

        def out_project(even, odd, both, p0, p1):
            rows = slice(p0 * HD, p1 * HD)
            return [jnp.dot(even, _unpack(wob_v[0, rows, :]), preferred_element_type=f32),
                    jnp.dot(odd, _unpack(wob_v[1, rows, :]), preferred_element_type=f32),
                    jnp.dot(both, _unpack(wos_v[rows, :]), preferred_element_type=f32)]

        def out_add(acc, part):
            e, o, b = part
            new = [e[:, :KM] + o[:, :KM], e[:, KM:], o[:, KM:], b]
            return new if acc is None else [x + y for x, y in zip(acc, new)]

        def out_finish(acc):
            main, e, o, b = acc
            mid = e + jnp.where(low, o, b)
            last = jnp.where(low, swap(o) + b, o + swap(b))
            return jnp.concatenate([main, mid, last], axis=1)

        ri = jax.lax.broadcasted_iota(jnp.int32, (2 * L, 2 * L), 0)
        ci = jax.lax.broadcasted_iota(jnp.int32, (2 * L, 2 * L), 1)

        def second(i):
            return jnp.where(i < 2 * SEG, i // SEG, (i - 2 * SEG) // PRE)

        def pos(i):
            j = i % SEG
            return jnp.where(i < 2 * SEG, jnp.where(j < T, j + (MEM + PRE), j - T), MEM + i % PRE)
        same = second(ri) == second(ci)
        mask = same & ((pos(ri) < MEM) | (pos(ri) >= pos(ci)))
        fill = jnp.where(same, NEG, -jnp.inf).astype(f32)

        def step(s, slot, mem):
            xt = xb_v[pl.ds(pl.multiple_of(SEG * s + PRE, 8), T), :]
            l1 = jnp.concatenate([xt.astype(f32), mem], axis=0)
            mid, last = l1[:, KM:KA], l1[:, KA:]
            l_even = l1[:, :KA].astype(bf16)
            l_odd = jnp.concatenate([l1[:, :KM], jnp.where(low, mid, last)], axis=1).astype(bf16)
            l_both = jnp.where(low, last, mid).astype(bf16)
            p0 = pl.multiple_of(PRE * s, 8)
            proj = []
            for g in range(G):
                w_even, w_odd, w_both = wgroup(g)
                both = jnp.dot(l_both, w_both, preferred_element_type=f32)
                even = jnp.dot(l_even, w_even, preferred_element_type=f32)
                odd = jnp.dot(l_odd, w_odd, preferred_element_type=f32)
                proj.append([((x + both) * colscale).astype(bf16) for x in (even, odd)])

            def rows(hp, t):
                g, c0 = hp // GP, (hp % GP) * 3 * D + t * D
                return jnp.concatenate([proj[g][0][:, c0:c0 + D], proj[g][1][:, c0:c0 + D],
                                        _unpack(pre_ref(hp * 3 + t)[pl.ds(p0, PRE), :])], axis=0)

            scores = [jax.lax.dot_general(rows(hp, 0), rows(hp, 1), NT, preferred_element_type=f32)
                      for hp in range(HP)]
            ctx = {}

            def attend(g):
                for hp in range(g * HG // 2, (g + 1) * HG // 2):
                    sc = jnp.where(mask, scores[hp], fill)
                    m = jnp.max(sc, axis=1, keepdims=True)
                    p = jnp.exp2(sc - m)
                    l = jnp.sum(p, axis=1, keepdims=True)
                    o = jnp.dot(p.astype(bf16), rows(hp, 2), preferred_element_type=f32) * _recip(l)
                    ctx[hp] = [o[0:SEG, :].astype(bf16), o[SEG:2 * SEG, :].astype(bf16),
                               (o[0:SEG, :] + o[SEG:2 * SEG, :]).astype(bf16)]
                    for e in range(2):
                        post_v[e, slot * PRE:(slot + 1) * PRE, hp * D:(hp + 1) * D] = o[2 * SEG + e * PRE:2 * SEG + (e + 1) * PRE, :]

            parts = []

            def oproj(g):
                lhs = [jnp.concatenate([ctx[hp][e] for hp in range(g * GP, (g + 1) * GP)], axis=1) for e in range(3)]
                parts.append(out_project(*lhs, g * GP, (g + 1) * GP))

            for t in range(G + 2):
                if t < G:
                    attend(t)
                if t >= 2:
                    oproj(t - 2)
            acc = None
            for a in parts:
                acc = out_add(acc, a)
            accb = out_finish(acc).astype(bf16)
            out_v[pl.ds(pl.multiple_of(SEG * s + PRE, 8), T), DM:2 * DM] = accb[0:T, 0:DM]
            return accb[T:, :].astype(f32), ctx[HP - 1][1]

        PP = HP // OUTER

        def deferred_rows():
            even, odd = post_v[0], post_v[1]
            return even.astype(bf16), odd.astype(bf16), (even + odd).astype(bf16)

        def finish(j, acc):
            r = out_finish(acc).astype(bf16)
            for sg in range(OUTER):
                r0 = pl.multiple_of((j * OUTER + sg) * SEG, SEG)
                out_v[pl.ds(r0, PRE), DM:2 * DM] = r[sg * PRE:(sg + 1) * PRE, 0:DM]

        def after(x, late):
            u = _pack(late[0:2 * OUTER * PRE // 2, :])
            zero = (u >> 31) & (~u >> 31)
            return _unpack(_pack(x) | jnp.concatenate([zero] * (x.shape[1] // D), axis=1))

        def outer(j, mem):
            prev = deferred_rows()

            def partial(i, late):
                x = [after(p[:, i * PP * D:(i + 1) * PP * D], late) for p in prev]
                return out_project(*x, i * PP, (i + 1) * PP)
            acc = None
            for i in range(OUTER):
                mem, late = step(j * OUTER + i, i, mem)
                acc = out_add(acc, partial(i, late))
            finish(jnp.maximum(j - 1, 0), acc)

            @pl.when(j > 0)
            def _():
                out_copy(j - 1).start()
            return mem
        with _scope("b_loop"):
            post_v[...] = jnp.zeros(post_v.shape, f32)
            mem0 = mem_v[0:MEM, :].astype(f32)
            jax.lax.fori_loop(0, NOUTER, outer, jnp.concatenate([mem0, mem0[:, DM - HD:]], axis=1))
            finish(NOUTER - 1, out_add(None, out_project(*deferred_rows(), 0, HP)))
            out_copy(NOUTER - 1).start()
        with _scope("b_outwait"):
            for j in range(NOUTER):
                out_copy(j).wait()

    pl.run_scoped(
        phase_b,
        pltpu.VMEM((2, OUTER * PRE, HP * D), f32),
    )


@jax.jit
def pallas_concat_heads__compressed_kv_cla__memory_aug_recurrent_mem_tr__prompt_kernel(
    A_x: jax.Array,
    A_c_kv: jax.Array,
    A_w_q: jax.Array,
    A_w_uk: jax.Array,
    A_w_uv: jax.Array,
    A_w_o: jax.Array,
    B_x: jax.Array,
    B_mem0: jax.Array,
    B_Wq: jax.Array,
    B_Wk: jax.Array,
    B_Wv: jax.Array,
    B_Wo: jax.Array,
    B_seg_len=SEG,
):
    def t2(x):
        return jnp.transpose(x, (0, 2, 1)).reshape(DM, S)

    def w3(w):
        return w.reshape(w.shape[0] // 2, 2 * H, D)

    def wo3(w):
        return jnp.transpose(w, (0, 2, 1))

    any_spec = pl.BlockSpec(memory_space=pl.ANY)
    out = pl.pallas_call(
        _kernel,
        out_shape=jax.ShapeDtypeStruct((S, 2 * DM), bf16),
        in_specs=[any_spec] * 12,
        out_specs=any_spec,
        scratch_shapes=[
            pltpu.VMEM((S, 2 * DM), bf16),
            pltpu.VMEM((S, DMP), bf16),
            pltpu.VMEM((NSEG * PRE, DMP), bf16),
            pltpu.VMEM((3, 2, HP, DM // 2, D), u32),
            pltpu.VMEM((2, HP * D // 2, KM + 2 * HD), u32),
            pltpu.VMEM((HP * D // 2, D), u32),
            pltpu.VMEM((8 * MEM, DM), bf16),
            pltpu.VMEM((H, S // 2, D), u32),
            pltpu.VMEM((H, S // 2, D), u32),
            pltpu.VMEM((H, S // 2, D), u32),
            pltpu.SemaphoreType.DMA((NSEM,)),
        ],
        compiler_params=pltpu.CompilerParams(vmem_limit_bytes=126 * 1024 * 1024),
    )(t2(A_x), A_c_kv.reshape(S, DC), w3(A_w_q), w3(A_w_uk), w3(A_w_uv), wo3(A_w_o),
      t2(B_x), B_mem0.reshape(MEM, DM), w3(B_Wq), w3(B_Wk), w3(B_Wv), wo3(B_Wo))
    return out.reshape(1, S, 2 * DM)
```

```python
import contextlib

import jax
import jax.numpy as jnp
import jax.experimental.pallas as pl
import jax.experimental.pallas.tpu as pltpu

S = 2048
DM = 576
DC = 512
H = 32
D = 128
MEM = 8
SEG = 32
L = MEM + SEG
NSEG = S // SEG
HP = H // 2
HD = D // 2
KM = DM - 3 * HD
DMP = DM + HD

LOG2E = 1.4426950408889634
QSCALE = D ** -0.5 * LOG2E
NEG = -1.0e9 * LOG2E

TQ = 128
UH = 4
ANCHOR_LAG = 2000
ANCHOR_MIN = 6
RB = 512
HG = 4
G = H // HG
PRE = 8
T = SEG - PRE
OUTER = 4
NOUTER = NSEG // OUTER

bf16 = jnp.bfloat16
f32 = jnp.float32
u32 = jnp.uint32
NT = (((1,), (1,)), ((), ()))

SEM_CKV = 0
SEM_XAT = 5
SEM_XBT = 6
SEM_MEM = 7
SEM_WOA = 8
SEM_WOB = 9
SEM_OUT = 10
SEM_WALL = SEM_OUT + NOUTER
SEM_W = SEM_WALL + 4
NSEM = SEM_W + 3 + HP // 2

_PROFILE = False
PG = 1
QS = 2

def _scope(name):
    return jax.named_scope(name) if _PROFILE else contextlib.nullcontext()


def _unpack(w32):
    return pltpu.bitcast(w32, bf16)


def _pack(x):
    return pltpu.bitcast(x, u32)


def _lo(w):
    return pltpu.bitcast(w << 16, f32)


def _hi(w):
    return pltpu.bitcast(w & u32(0xFFFF0000), f32)


def _words(even, odd):
    return pltpu.bitcast(pltpu.pack_elementwise([even, odd], packed_dtype=bf16), u32)


def _strassen_lhs(a11, a12, a21, a22):
    return [a11 + a22, a21 + a22, a11, a22, a11 + a12, a21 - a11, a12 - a22]


def _strassen_rhs(b11, b12, b21, b22):
    return [b11 + b22, b11, b12 - b22, b21 - b11, b22, b11 + b12, b21 + b22]


def _sum_words(combine, x11, x12, x21, x22, raw_idx, raw):
    lo = combine(_lo(x11), _lo(x12), _lo(x21), _lo(x22))
    hi = combine(_hi(x11), _hi(x12), _hi(x21), _hi(x22))
    words = [pltpu.bitcast(pltpu.pack_elementwise([a, b], packed_dtype=bf16), u32) for a, b in zip(lo, hi)]
    for i, r in zip(raw_idx, raw):
        words[i] = r
    return words


def _strassen(lhs, rhs, dims=(((1,), (0,)), ((), ())), order=0):
    def m(i):
        return jax.lax.dot_general(lhs(i - 1), rhs(i - 1), dims, preferred_element_type=f32)
    if order == 0:
        m1 = m(1)
        m2 = m(2)
        c22 = m1 - m2
        m4 = m(4)
        c11 = m1 + m4
        c21 = m2 + m4
        c22 = c22 + m(6)
        m3 = m(3)
        c22 = c22 + m3
        m5 = m(5)
        c11 = c11 - m5
        c12 = m3 + m5
        c11 = c11 + m(7)
        return c11, c12, c21, c22
    m3 = m(3)
    m4 = m(4)
    m5 = m(5)
    c12 = m3 + m5
    c11 = m4 - m5
    m2 = m(2)
    c21 = m4 + m2
    c22 = m3 - m2
    m1 = m(1)
    c11 = c11 + m1
    c22 = c22 + m1
    c22 = c22 + m(6)
    c11 = c11 + m(7)
    return c11, c12, c21, c22


def _rhs_words(s0, s1, z0, z1):
    per = [_strassen_rhs(_lo(s), _hi(s), _lo(z), _hi(z)) for s, z in ((s0, z0), (s1, z1))]
    words = [pltpu.bitcast(pltpu.pack_elementwise([per[0][i], per[1][i]], packed_dtype=bf16), u32)
             for i in range(7)]
    words[1] = (s0 & u32(0xFFFF)) | (s1 << 16)
    words[4] = (z0 >> 16) | (z1 & u32(0xFFFF0000))
    return words


_L233 = (((0, 1, 1), (1, 0, 1)), ((0, 1, 1),), ((0, 0, 1), (1, 0, -1)), ((0, 1, 1), (1, 1, -1)), ((1, 0, 1),),
         ((0, 0, -1), (0, 1, -1)), ((1, 0, 1), (1, 1, 1)), ((0, 0, 1), (0, 2, 1), (1, 0, -1)), ((1, 2, 1),),
         ((0, 2, 1),), ((1, 0, 1), (1, 2, 1), (0, 0, -1), (0, 2, -1)), ((0, 0, -1), (0, 2, -1)),
         ((1, 1, 1), (1, 2, 1), (0, 1, -1)), ((1, 1, -1), (1, 2, -1)),
         ((0, 1, 1), (0, 2, 1), (1, 1, -1), (1, 2, -1)))
_R233 = (((0, 1, 1), (1, 0, 1)), ((1, 1, 1), (1, 2, 1), (0, 1, -1)), ((0, 0, 1), (0, 1, 1), (2, 0, -1)),
         ((2, 1, 1), (1, 0, -1), (1, 1, -1)), ((0, 0, 1), (0, 2, 1), (1, 0, -1)), ((0, 1, 1),), ((1, 0, 1),),
         ((0, 2, 1), (2, 0, 1)), ((2, 0, 1), (2, 2, 1), (1, 2, -1)), ((2, 1, 1), (2, 2, 1), (0, 2, -1)),
         ((2, 0, 1),), ((0, 2, 1),), ((1, 2, 1), (2, 1, 1)), ((1, 2, 1),), ((2, 1, 1),))
_PIECES = ((0, 32, 64), (128, 160, 96), (192, 224, 256))


def _signed_sum(terms, get):
    acc = None
    for a, b, c in terms:
        x = get(a, b)
        if acc is None:
            acc = x if c > 0 else -x
        else:
            acc = acc + x if c > 0 else acc - x
    return acc


def _lhs233(y1, y2, store, extra=()):
    low = jax.lax.broadcasted_iota(jnp.int32, (1, D), 1) < HD
    base = {}
    for i in range(2):
        t1 = [y1[i][:, c * D:(c + 1) * D] for c in range(5)]
        t2 = [y2[i][:, c * D:(c + 1) * D] for c in range(5)]
        r1, r2 = pltpu.roll(t1[1], HD, 1), pltpu.roll(t2[1], HD, 1)
        for k in range(3):
            a1, a2 = t1[(0, 2, 3)[k]], t2[(0, 2, 3)[k]]
            lo1 = (t1[1], r1, t1[4])[k]
            hi1, hi2 = (r1, t1[1], t1[4])[k], (r2, t2[1], t2[4])[k]
            base[i, k] = (jnp.where(low, a1, a1 - a2), jnp.where(low, a2, hi2 - hi1), jnp.where(low, lo1, a2))
    for r, terms in enumerate(_L233 + extra):
        for p in range(3):
            store(r, p, _pack(_signed_sum(terms, lambda i, k: base[i, k][p]).astype(bf16)))


def _rhs233(slabs):
    def chunk(j, par, k):
        s = slabs[j][par]
        a, b, c = _PIECES[k]
        return s[a:a + 96] if k != 1 else jnp.concatenate([s[a:a + 64], s[c:c + 32]], axis=0)

    def words(r):
        terms = _R233[r]
        if len(terms) == 1:
            k, j, _ = terms[0]
            s0, s1 = chunk(j, 0, k), chunk(j, 1, k)
            return (s0 & u32(0xFFFF)) | (s1 << 16), (s0 >> 16) | (s1 & u32(0xFFFF0000))
        half = [[_signed_sum(terms, lambda k, j: f(chunk(j, par, k))) for par in range(2)] for f in (_lo, _hi)]
        return _words(*half[0]), _words(*half[1])
    return words


def _passes(w):
    return (w[0:64], jnp.concatenate([w[0:32], w[64:96]], axis=0), jnp.concatenate([w[64:96], w[32:64]], axis=0))


def _mm233(product):
    def add(a, b):
        return [x + y for x, y in zip(a, b)]

    def sub(a, b):
        return [x - y for x, y in zip(a, b)]
    p13 = product(13)
    s1 = add(product(12), p13)
    s2 = add(s1, product(14))
    p11 = product(11)
    z = add(s2, p11)
    yield (0, 2), sub(product(9), z)
    s3 = add(product(7), p11)
    s4 = add(s3, product(10))
    y = add(s4, p13)
    yield (1, 2), sub(product(8), y)
    p4 = product(4)
    c10 = add(s4, p4)
    c00 = add(s3, p4)
    p6 = product(6)
    yield (1, 0), add(c10, p6)
    c11 = sub(s1, p6)
    p5 = product(5)
    c01 = sub(s2, p5)
    c00 = add(c00, p5)
    p1 = product(1)
    yield (0, 1), add(c01, p1)
    c11 = add(c11, p1)
    p0 = product(0)
    c00 = add(c00, p0)
    c11 = add(c11, p0)
    yield (1, 1), add(c11, product(3))
    yield (0, 0), add(c00, product(2))


def _recip(l):
    r = pl.reciprocal(l, approx=True)
    return r * (2.0 - l * r)


def _kernel(xat_hbm, ckv_hbm, wqa_hbm, wuk_hbm, wuv_hbm, woa_hbm,
            xbt_hbm, mem0_hbm, wqb_hbm, wkb_hbm, wvb_hbm, wob_hbm,
            out_hbm,
            out_v, xb_v, xpre_v, wb_v, wob_v, wos_v, mem_v, q_v, kv_v, sem):

    def w_copy(w_hbm, dst, slot, par, hp):
        return pltpu.make_async_copy(w_hbm.bitcast(u32).at[:, par * HP + hp, :], dst.at[par, hp], sem.at[slot])

    def w_start_shared(w_hbm, dst, widx, hps):
        for hp in hps:
            for par in range(2):
                w_copy(w_hbm, dst, SEM_WALL + widx, par, hp).start()

    def w_wait_shared(dst, widx):
        pltpu.make_async_copy(dst, dst, sem.at[SEM_WALL + widx]).wait()

    def w_combine(dst, hp):
        a = dst[0, hp]
        b = dst[1, hp]
        ev = (a & u32(0xFFFF)) | (b << 16)
        od = (a >> 16) | (b & u32(0xFFFF0000))
        return ev, od

    def w_pair(dst, hp):
        return jnp.concatenate(w_combine(dst, hp), axis=1)

    wb_hbm = (wqb_hbm, wkb_hbm, wvb_hbm)

    def pre_ref(j):
        n = NSEG * PRE
        return q_v.at[j // 4], (j % 4 // 2) * n, (j % 2) * D

    def lp_prep(lp_v):
        nr = NSEG * PRE // 4
        x = xpre_v[...].astype(f32)

        def store(r, p, w):
            lp_v.at[r][:, p * D:(p + 1) * D] = w
        _lhs233([x[0:nr], x[2 * nr:3 * nr]], [x[nr:2 * nr], x[3 * nr:]], store)

    def b_pre(lp_v):
        nr = NSEG * PRE // 4
        with _scope("b_pre"):
            for g in range(HP // PG):
                hps = range(g * PG, (g + 1) * PG)
                slabs = {}
                for hp in hps:
                    for t in range(3):
                        s0, s1 = wb_v[t, 0, hp], wb_v[t, 1, hp]
                        slabs[hp, t] = (s0, s1)
                        ev = (s0 & u32(0xFFFF)) | (s1 << 16)
                        od = (s0 >> 16) | (s1 & u32(0xFFFF0000))
                        a, b = (KM + HD) // 2, (KM + 2 * HD) // 2
                        d12 = _words(_lo(s0[a:b]) - _hi(s0[a:b]), _lo(s1[a:b]) - _hi(s1[a:b]))
                        d21 = _words(_hi(s0[b:]) - _lo(s0[b:]), _hi(s1[b:]) - _lo(s1[b:]))
                        wb_v[t, 0, hp] = jnp.concatenate([ev[:a], d12, ev[b:]], axis=0)
                        wb_v[t, 1, hp] = jnp.concatenate([od[:a], d21, od[a:b]], axis=0)
                rhs = [_rhs233([slabs[hp, t] for t in range(3)]) for hp in hps]

                def product(r):
                    wa, wb, wc = _passes(jnp.concatenate([x for f in rhs for x in f(r)], axis=1))
                    c = jnp.dot(_unpack(lp_v[r, :, 2 * D:3 * D]), _unpack(wc), preferred_element_type=f32)
                    a = jnp.dot(_unpack(lp_v[r, :, 0:D]), _unpack(wa), preferred_element_type=f32)
                    b = jnp.dot(_unpack(lp_v[r, :, D:2 * D]), _unpack(wb), preferred_element_type=f32)
                    return [a + c, b + c]
                for (i, t), blk in _mm233(product):
                    for y in range(2):
                        x0 = (2 * i + y) * nr
                        for n, hp in enumerate(hps):
                            two = [blk[y][:, (2 * n + e) * D:(2 * n + e + 1) * D] for e in range(2)]
                            if t == 0:
                                two = [z * QSCALE for z in two]
                            two = [z.reshape(nr // PRE, 1, PRE, D) for z in two]
                            two = jnp.concatenate(two, axis=1).reshape(2 * nr, D)
                            ref, r0, l0 = pre_ref(hp * 3 + t)
                            ref[r0 + x0:r0 + x0 + nr, l0:l0 + D] = _pack(two.astype(bf16))

    def phase_a(woa_v, xbt_v, wobt_v, lp_v):
        woa_cp = pltpu.make_async_copy(woa_hbm.bitcast(u32), woa_v, sem.at[SEM_WOA])
        xbt_cp = pltpu.make_async_copy(xbt_hbm, xbt_v, sem.at[SEM_XBT])
        mem_cp = pltpu.make_async_copy(mem0_hbm, mem_v.at[0:MEM, :], sem.at[SEM_MEM])
        wob_cp = pltpu.make_async_copy(wob_hbm.bitcast(u32), wobt_v, sem.at[SEM_WOB])

        def projections(ckv_v, xat_v, wuk_v, wuv_v, wqa_v, tkv_v, lq_v, la_v):
            UR = 2 * D
            NU = S // UR
            kh = DC // 2
            ngrp = HP // 2

            def batch_start(pairs, slot):
                for hp in pairs:
                    for w_hbm, dst in ((wuk_hbm, wuk_v), (wuv_hbm, wuv_v)):
                        for par in range(2):
                            w_copy(w_hbm, dst, SEM_W + slot, par, hp).start()

            def batch_wait(npairs, slot):
                part = wuk_v.at[:, 0:2 * npairs]
                pltpu.make_async_copy(part, part, sem.at[SEM_W + slot]).wait()

            def group(j):
                return [hp for hp in (2 * j + 1, 2 * j + 2) if hp < HP]

            def first_copies(w_hbm, dst, slot):
                return [w_copy(w_hbm, dst, SEM_W + slot, par, 0) for par in range(2)]

            def first_wait(dst, slot):
                part = dst.at[:, 0:1]
                pltpu.make_async_copy(part, part, sem.at[SEM_W + slot]).wait()

            pieces = [(0, 1), (1, 2), (2, 4), (4, 6), (6, 8)]

            def ckv_cp(j):
                rows = slice(pieces[j][0] * UR, pieces[j][1] * UR)
                return pltpu.make_async_copy(ckv_hbm.at[rows, :], ckv_v.at[rows, :], sem.at[SEM_CKV + j])
            xat_cp = pltpu.make_async_copy(xat_hbm, xat_v, sem.at[SEM_XAT])

            with _scope("a_issue0"):
                for cp in first_copies(wuk_hbm, wuk_v, 0) + first_copies(wuv_hbm, wuv_v, 1):
                    cp.start()
                for j in range(4):
                    ckv_cp(j).start()
                batch_start([1], 2)
                ckv_cp(4).start()
                batch_start([2], 3)
                for j in range(1, ngrp - 1):
                    batch_start(group(j), 3 + j)

            def lhs_prep(src_v, dst_v, u):
                c = src_v[u * UR:(u + 1) * UR, 0:DC].astype(f32)
                ops = _strassen_lhs(c[:D, :kh], c[:D, kh:], c[D:, :kh], c[D:, kh:])
                for i, o in enumerate(ops):
                    dst_v.at[i][u * D // 2:(u + 1) * D // 2, :] = _pack(o.astype(bf16))

            def rhs_words(w_v, hp):
                n = kh // 2
                s0, s1 = w_v[0, hp, 0:n, :], w_v[1, hp, 0:n, :]
                z0, z1 = w_v[0, hp, n:2 * n, :], w_v[1, hp, n:2 * n, :]
                return _rhs_words(s0, s1, z0, z1)

            def rhs_kv(hp):
                return [jnp.concatenate([a, b], axis=1) for a, b in zip(rhs_words(wuk_v, hp), rhs_words(wuv_v, hp))]

            def items(lst):
                return lambda i: lst[i]

            def project_kv(t, hp, u0, u1):
                c = _strassen(lambda i: _unpack(la_v[i, u0 * D // 2:u1 * D // 2, :]), lambda i: _unpack(t(i)), order=1)
                for u in range(u0, u1):
                    rows = slice((u - u0) * D, (u - u0 + 1) * D)
                    top = u * D
                    for blk, h, p0 in ((c[0], 2 * hp, top), (c[1], 2 * hp + 1, top),
                                       (c[2], 2 * hp, top + D // 2), (c[3], 2 * hp + 1, top + D // 2)):
                        kv_v.at[h][p0:p0 + D // 2, :] = _pack(blk[rows, :].astype(bf16))

            KU = 2

            def project_pair(t, hp):
                for u in range(0, NU, KU):
                    project_kv(t, hp, u, u + KU)

            def kv_first():
                first_wait(wuk_v, 0)
                first_wait(wuv_v, 1)
                t = items(rhs_kv(0))
                for j in range(4):
                    ckv_cp(j).wait()
                    for u in range(*pieces[j]):
                        lhs_prep(ckv_v, la_v, u)
                    project_kv(t, 0, *pieces[j])
                ckv_cp(4).wait()
                batch_wait(1, 2)
                for u in range(*pieces[4]):
                    lhs_prep(ckv_v, la_v, u)
                project_kv(t, 0, *pieces[4])
                t1 = items(rhs_kv(1))
                project_kv(t1, 1, 0, 2)
                batch_wait(1, 3)
                for i, w in enumerate(rhs_kv(2)):
                    tkv_v[i] = w
                for u in range(2, NU, 2):
                    project_kv(t1, 1, u, u + 2)

            def kv_body(j, c):
                @pl.when(j == 2)
                def _():
                    xat_cp.start()
                    batch_start(group(ngrp - 1), 3 + ngrp - 1)
                    w_start_shared(wqa_hbm, wqa_v, 0, range(HP))
                    xbt_cp.start()
                batch_wait(2, 3 + j)
                project_pair(lambda i: tkv_v[i], 2 * j)
                t1 = items(rhs_kv(2 * j + 1))
                for i, w in enumerate(rhs_kv(2 * j + 2)):
                    tkv_v[i] = w
                project_pair(t1, 2 * j + 1)
                return c

            with _scope("a_kvproj"):
                kv_first()
                jax.lax.fori_loop(1, ngrp - 1, kv_body, 0)

            woa_cp.start()
            wob_cp.start()
            mem_cp.start()
            w_start_shared(wqb_hbm, wb_v.at[0], 1, range(HP))
            w_start_shared(wkb_hbm, wb_v.at[1], 2, range(HP // 2))

            QB = 4 * D
            plain = {(0, 0): 15, (0, 1): 1, (0, 2): 9, (1, 0): 4, (1, 1): 16, (1, 2): 8}

            def xa_prep(b):
                x = []
                for t in range(4 * b, 4 * b + 4):
                    xt = xat_v[:, t * D:(t + 1) * D]
                    x.append(jnp.concatenate([xt, xt[DM - HD:]], axis=0).astype(f32).T)

                def store(r, p, w):
                    lq_v.at[r][b * HD:(b + 1) * HD, p * D:(p + 1) * D] = w
                _lhs233([x[0], x[2]], [x[1], x[3]], store, extra=(((0, 0, 1),), ((1, 1, 1),)))

            def q_store(blk, hp, x0):
                q_v.at[hp][x0 // 2:(x0 + blk.shape[0]) // 2, :] = _pack((blk * QSCALE).astype(bf16))

            def q_rhs(hp):
                f = _rhs233([(wqa_v[0, hp + n], wqa_v[1, hp + n]) for n in range(3)])
                return [_passes(jnp.concatenate(f(r), axis=1)) for r in range(15)]

            def project_q(t, hp, b):
                nr = D // QS
                for s in range(QS):
                    rows = slice(b * HD + s * nr // 2, b * HD + (s + 1) * nr // 2)

                    def product(r):
                        wa, wb, wc = t[r]
                        c = jnp.dot(_unpack(lq_v[r, rows, 2 * D:3 * D]), _unpack(wc), preferred_element_type=f32)
                        a = jnp.dot(_unpack(lq_v[r, rows, 0 * D:1 * D]), _unpack(wa), preferred_element_type=f32)
                        b = jnp.dot(_unpack(lq_v[r, rows, 1 * D:2 * D]), _unpack(wb), preferred_element_type=f32)
                        return [a + c, b + c]
                    for (i, j), blk in _mm233(product):
                        for y in range(2):
                            q_store(blk[y], hp + j, b * QB + (2 * i + y) * D + s * nr)

            def project_q_last(hp):
                s0, s1 = wqa_v[0, hp], wqa_v[1, hp]
                w = jnp.concatenate([(s0 & u32(0xFFFF)) | (s1 << 16), (s0 >> 16) | (s1 & u32(0xFFFF0000))], axis=1)
                per = [_passes(jnp.concatenate([w[a:a + 64], w[c:c + 32]] if k == 1 else [w[a:a + 96]], axis=0))
                       for k, (a, _, c) in enumerate(_PIECES)]
                wp = [_unpack(jnp.concatenate([per[k][p] for k in range(3)], axis=0)) for p in range(3)]
                for b in range(S // QB):
                    rows = slice(b * HD, (b + 1) * HD)
                    for i in range(2):
                        a, bb, c = [jnp.dot(_unpack(jnp.concatenate([lq_v[plain[i, k], rows, p * D:(p + 1) * D] for k in range(3)], axis=1)),
                                            wp[p], preferred_element_type=f32) for p in range(3)]
                        q_store(a + c, hp, b * QB + 2 * i * D)
                        q_store(bb + c, hp, b * QB + (2 * i + 1) * D)

            def xb_prep(t):
                t0 = pl.multiple_of(t * D, D)
                xt = xbt_v[:, pl.ds(t0, D)]
                xb = jnp.concatenate([xt, xt[DM - HD:]], axis=0).T
                xb_v[pl.ds(t0, D), :] = xb
                for sg in range(D // SEG):
                    p0 = pl.multiple_of((t * (D // SEG) + sg) * PRE, PRE)
                    xpre_v[pl.ds(p0, PRE), :] = xb[sg * SEG:sg * SEG + PRE, :]

            with _scope("a_qproj"):
                j = ngrp - 1
                batch_wait(1, 3 + j)
                xat_cp.wait()
                xbt_cp.wait()
                w_wait_shared(wqa_v, 0)
                t14 = lambda i: tkv_v[i]
                t15 = items(rhs_kv(2 * j + 1))
                kv = [(t14, 2 * j, u) for u in range(0, NU, 2)] + [(t15, 2 * j + 1, u) for u in range(0, NU, 2)]
                t = q_rhs(0)
                for b in range(S // QB):
                    xa_prep(b)
                    for u in (2 * b, 2 * b + 1):
                        project_kv(kv[u][0], kv[u][1], kv[u][2], kv[u][2] + 2)
                    project_q(t, 0, b)
                XG = 4

                def q_body(j, c):
                    hp = 3 * j
                    for n in range(XG):
                        xb_prep((j - 1) * XG + n)
                    t = q_rhs(hp)
                    for b in range(S // QB):
                        project_q(t, hp, b)
                    return c
                jax.lax.fori_loop(1, 5, q_body, 0)
                lp_prep(lp_v)
                project_q_last(HP - 1)

        pl.run_scoped(
            projections,
            pltpu.VMEM((S, DC), bf16),
            pltpu.VMEM((DM, S), bf16),
            pltpu.VMEM((2, HP, DC // 2, D), u32),
            pltpu.VMEM((2, HP, DC // 2, D), u32),
            pltpu.VMEM((2, HP, DM // 2, D), u32),
            pltpu.VMEM((7, DC // 4, 2 * D), u32),
            pltpu.VMEM((17, S // 8, 3 * D), u32),
            pltpu.VMEM((7, S // 4, DC // 2), u32),
        )

        def attention(c_v, s_v):
            row = jax.lax.broadcasted_iota(jnp.int32, (TQ, TQ), 0)
            col = jax.lax.broadcasted_iota(jnp.int32, (TQ, TQ), 1)
            tri = col <= row
            nb = S // TQ
            hq = TQ // 2
            npiece = 2
            pw = S // npiece

            def q_rows(h, r0, r1):
                return q_v[h[0], r0:r1, h[1] * D:(h[1] + 1) * D]

            def head(h):
                return 2 * h[0] + h[1]

            def qk_piece(h, j):
                q = _unpack(q_rows(h, (nb - 1) * hq, nb * hq))
                k = _unpack(kv_v[head(h), j * pw // 2:(j + 1) * pw // 2, 0:D])
                s_v[:, j * pw:(j + 1) * pw] = jax.lax.dot_general(q, k, NT, preferred_element_type=f32)

            def qk(h, i, j0=0, j1=None):
                j1 = i + 1 if j1 is None else j1
                q = _unpack(q_rows(h, i * hq, (i + 1) * hq))
                k = _unpack(kv_v[head(h), j0 * hq:j1 * hq, 0:D])
                return jax.lax.dot_general(q, k, NT, preferred_element_type=f32)

            def anchor_plan():
                ops = []
                for e in range(UH):
                    for i in range(nb - 1, -1, -1):
                        if i > 0:
                            ops.append(("qk", e, i - 1, 32 * i))
                        if i < npiece:
                            ops.append(("piece", e, i, 32 * nb // npiece))
                        ops.append(("pv", e, i, 32 * (i + 1)))
                t, start, end = 0, [], []
                for op in ops:
                    start.append(t)
                    t += op[3]
                    end.append(t)
                plan = {}
                for a, op in enumerate(ops):
                    if op[0] != "pv" or op[2] < ANCHOR_MIN:
                        continue
                    for b in range(a + 1, len(ops)):
                        if ops[b][0] == "qk" and start[b] >= end[a] + ANCHOR_LAG:
                            plan.setdefault((ops[b][1], ops[b][2]), []).append((op[1], op[2]))
                            break
                return plan

            def heads(j, c):
                @pl.when(j == 0)
                def _():
                    w_start_shared(wkb_hbm, wb_v.at[1], 2, range(HP // 2, HP))
                    w_start_shared(wvb_hbm, wb_v.at[2], 3, range(HP))

                plan = anchor_plan()

                def gated_qk(e, i):
                    h = (j * (UH // 2) + e // 2, e % 2)
                    if (e, i) not in plan:
                        return qk(h, i)
                    w = None
                    for ea, ia in plan[e, i]:
                        u = c_v[j * (UH // 2) + ea // 2, ia * hq:(ia + 1) * hq, (ea % 2) * D:(ea % 2 + 1) * D]
                        for r in range(0, hq, 8):
                            w = u[r:r + 8] if w is None else w | u[r:r + 8]
                    zero = (w >> 31) >> 1
                    q = q_rows(h, i * hq, (i + 1) * hq)
                    q = _unpack(jnp.concatenate([q[0:8] | zero, q[8:]], axis=0))
                    k = _unpack(kv_v[head(h), 0:(i + 1) * hq, 0:D])
                    return jax.lax.dot_general(q, k, NT, preferred_element_type=f32)

                s_next = s_v[...]
                for e in range(UH):
                    h = (j * (UH // 2) + e // 2, e % 2)
                    if e == UH - 1:
                        hn = (jnp.minimum(h[0] + 1, HP - 1), 0)
                    else:
                        hn = (j * (UH // 2) + (e + 1) // 2, (e + 1) % 2)
                    pieces = []
                    for i in range(nb - 1, -1, -1):
                        s = s_next
                        if i > 0:
                            s_next = gated_qk(e, i - 1)
                        if i < npiece:
                            if e == UH - 1:
                                qk_piece(hn, npiece - 1 - i)
                            else:
                                jj = npiece - 1 - i
                                pieces.append(qk(hn, nb - 1, jj * nb // npiece, (jj + 1) * nb // npiece))
                        sd = jnp.where(tri, s[:, i * TQ:], NEG)
                        s = jnp.concatenate([s[:, :i * TQ], sd], axis=1) if i > 0 else sd
                        m = jnp.max(s, axis=1, keepdims=True)
                        p = jnp.exp2(s - m)
                        l = jnp.sum(p, axis=1, keepdims=True)
                        v = _unpack(kv_v[head(h), 0:(i + 1) * hq, D:2 * D])
                        o = jnp.dot(p.astype(bf16), v, preferred_element_type=f32)
                        c_v.at[h[0]][i * hq:(i + 1) * hq, h[1] * D:(h[1] + 1) * D] = _pack((o * _recip(l)).astype(bf16))
                    if e < UH - 1:
                        s_next = jnp.concatenate(pieces, axis=1)
                return c
            with _scope("a_attn"):
                for j in range(npiece):
                    qk_piece((0, 0), j)
                jax.lax.fori_loop(0, H // UH, heads, 0)

            woa_cp.wait()
            wob_cp.wait()
            mem_cp.wait()
            for t in range(3):
                w_wait_shared(wb_v.at[t], 1 + t)
            mh = DM // 4

            def wo_prep(hh):
                a11, a21 = woa_v[hh, 0:mh, :], woa_v[hh, mh:2 * mh, :]
                a12, a22 = woa_v[hh + HP, 0:mh, :], woa_v[hh + HP, mh:2 * mh, :]
                for i, w in enumerate(_sum_words(_strassen_lhs, a11, a12, a21, a22, (2, 3), (a11, a22))):
                    if i not in (2, 3):
                        kv_v[hh, i * mh:(i + 1) * mh, 0:D] = w

            def wob_prep(hp):
                w1, w2 = _unpack(wobt_v[2 * hp]), _unpack(wobt_v[2 * hp + 1])
                a, b = KM + HD, KM + 2 * HD
                d12 = (w1[a:b].astype(f32) - w2[a:b].astype(f32)).astype(bf16)
                d21 = (w2[b:].astype(f32) - w1[b:].astype(f32)).astype(bf16)
                rows = slice(hp * HD, (hp + 1) * HD)
                wob_v[0, rows, :] = _pack(jnp.concatenate([w1[:a], d12], axis=0).T)
                wob_v[1, rows, :] = _pack(jnp.concatenate([w2[:a], d21], axis=0).T)
                wos_v[rows, :] = _pack(jnp.concatenate([w1[b:], w2[a:b]], axis=0).T)

            def oproj(tp):
                w0 = tp * D
                per = []
                for hh in range(HP):
                    def ctx(h, r0):
                        return c_v[h // 2, r0:r0 + D // 2, (h % 2) * D:(h % 2 + 1) * D]
                    b11, b21 = ctx(hh, w0), ctx(hh + HP, w0)
                    b12, b22 = ctx(hh, w0 + D // 2), ctx(hh + HP, w0 + D // 2)
                    per.append(_sum_words(_strassen_rhs, b11, b12, b21, b22, (1, 4), (b11, b22)))

                def lhs(i):
                    if i == 2:
                        return _unpack(jnp.concatenate([woa_v[hh, 0:mh, :] for hh in range(HP)], axis=1))
                    if i == 3:
                        return _unpack(jnp.concatenate([woa_v[hh + HP, mh:2 * mh, :] for hh in range(HP)], axis=1))
                    return _unpack(jnp.concatenate([kv_v[hh, i * mh:(i + 1) * mh, 0:D] for hh in range(HP)], axis=1))

                def rhs(i):
                    return _unpack(jnp.concatenate([per[hh][i] for hh in range(HP)], axis=1))
                c11, c12, c21, c22 = _strassen(lhs, rhs, NT)
                t0 = 2 * tp * D
                out_v[t0:t0 + D, 0:DM] = jnp.concatenate([c11, c21], axis=0).T.astype(bf16)
                out_v[t0 + D:t0 + 2 * D, 0:DM] = jnp.concatenate([c12, c22], axis=0).T.astype(bf16)

            b_pre(lp_v)
            with _scope("a_oproj"):
                for hh in range(HP):
                    wo_prep(hh)
                for tp in range(S // D // 2):
                    oproj(tp)
                    for hp in range(2 * tp, 2 * tp + 2):
                        wob_prep(hp)

        pl.run_scoped(
            attention,
            pltpu.VMEM((HP, S // 2, 2 * D), u32),
            pltpu.VMEM((TQ, S), f32),
        )

    pl.run_scoped(
        phase_a,
        pltpu.VMEM((H, DM // 2, D), u32),
        pltpu.VMEM((DM, S), bf16),
        pltpu.VMEM((H, DM // 2, D), u32),
        pltpu.VMEM((15, NSEG * PRE // 8, 3 * D), u32),
    )

    def out_copy(j):
        rows = pl.ds(pl.multiple_of(j * (OUTER * SEG), OUTER * SEG), OUTER * SEG)
        return pltpu.make_async_copy(out_v.at[rows, :], out_hbm.at[rows, :], sem.at[SEM_OUT + j])

    def phase_b(post_v):
        GP = HG // 2
        GC = GP * 3 * D
        KA = KM + 2 * HD
        lane = jax.lax.broadcasted_iota(jnp.int32, (1, GC), 1)
        colscale = jnp.where(lane % (3 * D) < D, QSCALE, 1.0).astype(f32)
        low = jax.lax.broadcasted_iota(jnp.int32, (1, D), 1) < HD

        def swap(x):
            return pltpu.roll(x, HD, 1)

        def wgroup(g):
            cols = [(hp, t) for hp in range(g * GP, (g + 1) * GP) for t in range(3)]
            own = [_unpack(jnp.concatenate([wb_v[t, e, hp, 0:KA // 2, :] for hp, t in cols], axis=1)) for e in range(2)]
            both = jnp.concatenate([jnp.concatenate([wb_v[t, e, hp, KA // 2:, :] for hp, t in cols], axis=1)
                                    for e in range(2)], axis=0)
            return own[0], own[1], _unpack(both)

        def out_project(even, odd, both, p0, p1):
            rows = slice(p0 * HD, p1 * HD)
            return [jnp.dot(even, _unpack(wob_v[0, rows, :]), preferred_element_type=f32),
                    jnp.dot(odd, _unpack(wob_v[1, rows, :]), preferred_element_type=f32),
                    jnp.dot(both, _unpack(wos_v[rows, :]), preferred_element_type=f32)]

        def out_add(acc, part):
            e, o, b = part
            new = [e[:, :KM] + o[:, :KM], e[:, KM:], o[:, KM:], b]
            return new if acc is None else [x + y for x, y in zip(acc, new)]

        def out_finish(acc):
            main, e, o, b = acc
            mid = e + jnp.where(low, o, b)
            last = jnp.where(low, swap(o) + b, o + swap(b))
            return jnp.concatenate([main, mid, last], axis=1)

        ri = jax.lax.broadcasted_iota(jnp.int32, (2 * L, 2 * L), 0)
        ci = jax.lax.broadcasted_iota(jnp.int32, (2 * L, 2 * L), 1)

        def second(i):
            return jnp.where(i < 2 * SEG, i // SEG, (i - 2 * SEG) // PRE)

        def pos(i):
            j = i % SEG
            return jnp.where(i < 2 * SEG, jnp.where(j < T, j + (MEM + PRE), j - T), MEM + i % PRE)
        same = second(ri) == second(ci)
        mask = same & ((pos(ri) < MEM) | (pos(ri) >= pos(ci)))
        fill = jnp.where(same, NEG, -jnp.inf).astype(f32)

        def step(s, slot, mem):
            xt = xb_v[pl.ds(pl.multiple_of(SEG * s + PRE, 8), T), :]
            l1 = jnp.concatenate([xt.astype(f32), mem], axis=0)
            mid, last = l1[:, KM:KA], l1[:, KA:]
            l_even = l1[:, :KA].astype(bf16)
            l_odd = jnp.concatenate([l1[:, :KM], jnp.where(low, mid, last)], axis=1).astype(bf16)
            l_both = jnp.where(low, last, mid).astype(bf16)
            p0 = pl.multiple_of(PRE * s, 8)
            proj = []
            for g in range(G):
                w_even, w_odd, w_both = wgroup(g)
                both = jnp.dot(l_both, w_both, preferred_element_type=f32)
                even = jnp.dot(l_even, w_even, preferred_element_type=f32)
                odd = jnp.dot(l_odd, w_odd, preferred_element_type=f32)
                proj.append([(x + both) * colscale for x in (even, odd)])

            def rows(hp, t):
                g, c0 = hp // GP, (hp % GP) * 3 * D + t * D
                ref, r0, l0 = pre_ref(hp * 3 + t)
                return jnp.concatenate([proj[g][0][:, c0:c0 + D], proj[g][1][:, c0:c0 + D],
                                        _unpack(ref[pl.ds(r0 + p0, PRE), l0:l0 + D]).astype(f32)], axis=0).astype(bf16)

            scores = [jax.lax.dot_general(rows(hp, 0), rows(hp, 1), NT, preferred_element_type=f32)
                      for hp in range(HP)]
            ctx = {}

            def attend(g):
                for hp in range(g * HG // 2, (g + 1) * HG // 2):
                    sc = jnp.where(mask, scores[hp], fill)
                    m = jnp.max(sc, axis=1, keepdims=True)
                    p = jnp.exp2(sc - m)
                    l = jnp.sum(p, axis=1, keepdims=True)
                    o = jnp.dot(p.astype(bf16), rows(hp, 2), preferred_element_type=f32) * _recip(l)
                    ctx[hp] = [o[0:SEG, :], o[SEG:2 * SEG, :], o[0:SEG, :] + o[SEG:2 * SEG, :]]
                    for e in range(2):
                        post_v[e, slot * PRE:(slot + 1) * PRE, hp * D:(hp + 1) * D] = o[2 * SEG + e * PRE:2 * SEG + (e + 1) * PRE, :]

            parts = []

            def oproj(g):
                lhs = [jnp.concatenate([ctx[hp][e] for hp in range(g * GP, (g + 1) * GP)], axis=1).astype(bf16)
                       for e in range(3)]
                parts.append(out_project(*lhs, g * GP, (g + 1) * GP))

            for t in range(G + 2):
                if t < G:
                    attend(t)
                if t >= 2:
                    oproj(t - 2)
            acc = None
            for a in parts:
                acc = out_add(acc, a)
            accb = out_finish(acc).astype(bf16)
            out_v[pl.ds(pl.multiple_of(SEG * s + PRE, 8), T), DM:2 * DM] = accb[0:T, 0:DM]
            return accb[T:, :].astype(f32), ctx[HP - 1][1]

        PP = HP // OUTER

        def deferred_rows():
            even, odd = post_v[0], post_v[1]
            return even, odd, even + odd

        def finish(j, acc):
            r = out_finish(acc).astype(bf16)
            for sg in range(OUTER):
                r0 = pl.multiple_of((j * OUTER + sg) * SEG, SEG)
                out_v[pl.ds(r0, PRE), DM:2 * DM] = r[sg * PRE:(sg + 1) * PRE, 0:DM]

        def after(x, late):
            u = pltpu.bitcast(late[0:8, :], u32)
            zero = (u >> 31) & (~u >> 31)
            top = pltpu.bitcast(x[0:8], u32) | jnp.concatenate([zero] * (x.shape[1] // D), axis=1)
            return jnp.concatenate([pltpu.bitcast(top, f32), x[8:]], axis=0).astype(bf16)

        def outer(j, mem):
            prev = deferred_rows()

            def partial(i, late):
                x = [after(p[:, i * PP * D:(i + 1) * PP * D], late) for p in prev]
                return out_project(*x, i * PP, (i + 1) * PP)
            acc = None
            for i in range(OUTER):
                mem, late = step(j * OUTER + i, i, mem)
                acc = out_add(acc, partial(i, late))
            finish(jnp.maximum(j - 1, 0), acc)

            @pl.when(j > 0)
            def _():
                out_copy(j - 1).start()
            return mem
        with _scope("b_loop"):
            post_v[...] = jnp.zeros(post_v.shape, f32)
            mem0 = mem_v[0:MEM, :].astype(f32)
            jax.lax.fori_loop(0, NOUTER, outer, jnp.concatenate([mem0, mem0[:, DM - HD:]], axis=1))
            finish(NOUTER - 1, out_add(None, out_project(*[x.astype(bf16) for x in deferred_rows()], 0, HP)))
            out_copy(NOUTER - 1).start()
        with _scope("b_outwait"):
            for j in range(NOUTER):
                out_copy(j).wait()

    pl.run_scoped(
        phase_b,
        pltpu.VMEM((2, OUTER * PRE, HP * D), f32),
    )


@jax.jit
def pallas_concat_heads__compressed_kv_cla__memory_aug_recurrent_mem_tr__prompt_kernel(
    A_x: jax.Array,
    A_c_kv: jax.Array,
    A_w_q: jax.Array,
    A_w_uk: jax.Array,
    A_w_uv: jax.Array,
    A_w_o: jax.Array,
    B_x: jax.Array,
    B_mem0: jax.Array,
    B_Wq: jax.Array,
    B_Wk: jax.Array,
    B_Wv: jax.Array,
    B_Wo: jax.Array,
    B_seg_len=SEG,
):
    def t2(x):
        return jnp.transpose(x, (0, 2, 1)).reshape(DM, S)

    def w3(w):
        return w.reshape(w.shape[0] // 2, 2 * H, D)

    def wo3(w):
        return jnp.transpose(w, (0, 2, 1))

    any_spec = pl.BlockSpec(memory_space=pl.ANY)
    out = pl.pallas_call(
        _kernel,
        out_shape=jax.ShapeDtypeStruct((S, 2 * DM), bf16),
        in_specs=[any_spec] * 12,
        out_specs=any_spec,
        scratch_shapes=[
            pltpu.VMEM((S, 2 * DM), bf16),
            pltpu.VMEM((S, DMP), bf16),
            pltpu.VMEM((NSEG * PRE, DMP), bf16),
            pltpu.VMEM((3, 2, HP, DM // 2, D), u32),
            pltpu.VMEM((2, HP * D // 2, KM + 2 * HD), u32),
            pltpu.VMEM((HP * D // 2, D), u32),
            pltpu.VMEM((8 * MEM, DM), bf16),
            pltpu.VMEM((HP, S // 2, 2 * D), u32),
            pltpu.VMEM((H, S // 2, 2 * D), u32),
            pltpu.SemaphoreType.DMA((NSEM,)),
        ],
        compiler_params=pltpu.CompilerParams(vmem_limit_bytes=126 * 1024 * 1024),
    )(t2(A_x), A_c_kv.reshape(S, DC), w3(A_w_q), w3(A_w_uk), w3(A_w_uv), wo3(A_w_o),
      t2(B_x), B_mem0.reshape(MEM, DM), w3(B_Wq), w3(B_Wk), w3(B_Wv), wo3(B_Wo))
    return out.reshape(1, S, 2 * DM)
```

```python
import contextlib

import jax
import jax.numpy as jnp
import jax.experimental.pallas as pl
import jax.experimental.pallas.tpu as pltpu

S = 2048
DM = 576
DC = 512
H = 32
D = 128
MEM = 8
SEG = 32
L = MEM + SEG
NSEG = S // SEG
HP = H // 2
HD = D // 2
KM = DM - 3 * HD
DMP = DM + HD

LOG2E = 1.4426950408889634
QSCALE = D ** -0.5 * LOG2E
NEG = -1.0e9 * LOG2E

TQ = 128
UH = 4
ANCHOR_LAG = 2000
ANCHOR_MIN = 6
RB = 512
HG = 4
G = H // HG
PRE = 8
T = SEG - PRE
OUTER = 4
NOUTER = NSEG // OUTER

bf16 = jnp.bfloat16
f32 = jnp.float32
u32 = jnp.uint32
NT = (((1,), (1,)), ((), ()))

SEM_CKV = 0
SEM_XAT = 5
SEM_XBT = 6
SEM_MEM = 7
SEM_WOA = 8
SEM_WOB = 9
SEM_OUT = 10
SEM_WALL = SEM_OUT + NOUTER
SEM_W = SEM_WALL + 4
NSEM = SEM_W + 6

_PROFILE = False
KU = 2
CL = 16
CR = 8
PG = 1
QS = 2

def _scope(name):
    return jax.named_scope(name) if _PROFILE else contextlib.nullcontext()


def _unpack(w32):
    return pltpu.bitcast(w32, bf16)


def _pack(x):
    return pltpu.bitcast(x, u32)


def _lo(w):
    return pltpu.bitcast(w << 16, f32)


def _hi(w):
    return pltpu.bitcast(w & u32(0xFFFF0000), f32)


def _words(even, odd):
    return pltpu.bitcast(pltpu.pack_elementwise([even, odd], packed_dtype=bf16), u32)


def _strassen_lhs(a11, a12, a21, a22):
    return [a11 + a22, a21 + a22, a11, a22, a11 + a12, a21 - a11, a12 - a22]


def _strassen_rhs(b11, b12, b21, b22):
    return [b11 + b22, b11, b12 - b22, b21 - b11, b22, b11 + b12, b21 + b22]


def _sum_words(combine, x11, x12, x21, x22, raw_idx, raw):
    lo = combine(_lo(x11), _lo(x12), _lo(x21), _lo(x22))
    hi = combine(_hi(x11), _hi(x12), _hi(x21), _hi(x22))
    words = [pltpu.bitcast(pltpu.pack_elementwise([a, b], packed_dtype=bf16), u32) for a, b in zip(lo, hi)]
    for i, r in zip(raw_idx, raw):
        words[i] = r
    return words


def _strassen(lhs, rhs, dims=(((1,), (0,)), ((), ())), order=0):
    def m(i):
        return jax.lax.dot_general(lhs(i - 1), rhs(i - 1), dims, preferred_element_type=f32)
    if order == 0:
        m1 = m(1)
        m2 = m(2)
        c22 = m1 - m2
        m4 = m(4)
        c11 = m1 + m4
        c21 = m2 + m4
        c22 = c22 + m(6)
        m3 = m(3)
        c22 = c22 + m3
        m5 = m(5)
        c11 = c11 - m5
        c12 = m3 + m5
        c11 = c11 + m(7)
        return c11, c12, c21, c22
    m3 = m(3)
    m4 = m(4)
    m5 = m(5)
    c12 = m3 + m5
    c11 = m4 - m5
    m2 = m(2)
    c21 = m4 + m2
    c22 = m3 - m2
    m1 = m(1)
    c11 = c11 + m1
    c22 = c22 + m1
    c22 = c22 + m(6)
    c11 = c11 + m(7)
    return c11, c12, c21, c22


def _rhs_words(s0, s1, z0, z1):
    per = [_strassen_rhs(_lo(s), _hi(s), _lo(z), _hi(z)) for s, z in ((s0, z0), (s1, z1))]
    words = [pltpu.bitcast(pltpu.pack_elementwise([per[0][i], per[1][i]], packed_dtype=bf16), u32)
             for i in range(7)]
    words[1] = (s0 & u32(0xFFFF)) | (s1 << 16)
    words[4] = (z0 >> 16) | (z1 & u32(0xFFFF0000))
    return words


_L233 = (((0, 1, 1), (1, 0, 1)), ((0, 1, 1),), ((0, 0, 1), (1, 0, -1)), ((0, 1, 1), (1, 1, -1)), ((1, 0, 1),),
         ((0, 0, -1), (0, 1, -1)), ((1, 0, 1), (1, 1, 1)), ((0, 0, 1), (0, 2, 1), (1, 0, -1)), ((1, 2, 1),),
         ((0, 2, 1),), ((1, 0, 1), (1, 2, 1), (0, 0, -1), (0, 2, -1)), ((0, 0, -1), (0, 2, -1)),
         ((1, 1, 1), (1, 2, 1), (0, 1, -1)), ((1, 1, -1), (1, 2, -1)),
         ((0, 1, 1), (0, 2, 1), (1, 1, -1), (1, 2, -1)))
_R233 = (((0, 1, 1), (1, 0, 1)), ((1, 1, 1), (1, 2, 1), (0, 1, -1)), ((0, 0, 1), (0, 1, 1), (2, 0, -1)),
         ((2, 1, 1), (1, 0, -1), (1, 1, -1)), ((0, 0, 1), (0, 2, 1), (1, 0, -1)), ((0, 1, 1),), ((1, 0, 1),),
         ((0, 2, 1), (2, 0, 1)), ((2, 0, 1), (2, 2, 1), (1, 2, -1)), ((2, 1, 1), (2, 2, 1), (0, 2, -1)),
         ((2, 0, 1),), ((0, 2, 1),), ((1, 2, 1), (2, 1, 1)), ((1, 2, 1),), ((2, 1, 1),))
_PIECES = ((0, 32, 64), (128, 160, 96), (192, 224, 256))


def _signed_sum(terms, get):
    acc = None
    for a, b, c in terms:
        x = get(a, b)
        if acc is None:
            acc = x if c > 0 else -x
        else:
            acc = acc + x if c > 0 else acc - x
    return acc


def _lhs233(y1, y2, store, extra=()):
    low = jax.lax.broadcasted_iota(jnp.int32, (1, D), 1) < HD
    base = {}
    for i in range(2):
        t1 = [y1[i][:, c * D:(c + 1) * D] for c in range(5)]
        t2 = [y2[i][:, c * D:(c + 1) * D] for c in range(5)]
        r1, r2 = pltpu.roll(t1[1], HD, 1), pltpu.roll(t2[1], HD, 1)
        for k in range(3):
            a1, a2 = t1[(0, 2, 3)[k]], t2[(0, 2, 3)[k]]
            lo1 = (t1[1], r1, t1[4])[k]
            hi1, hi2 = (r1, t1[1], t1[4])[k], (r2, t2[1], t2[4])[k]
            base[i, k] = (jnp.where(low, a1, a1 - a2), jnp.where(low, a2, hi2 - hi1), jnp.where(low, lo1, a2))
    for r, terms in enumerate(_L233 + extra):
        for p in range(3):
            store(r, p, _pack(_signed_sum(terms, lambda i, k: base[i, k][p]).astype(bf16)))


def _rhs233(slabs):
    def chunk(j, par, k):
        s = slabs[j][par]
        a, b, c = _PIECES[k]
        return s[a:a + 96] if k != 1 else jnp.concatenate([s[a:a + 64], s[c:c + 32]], axis=0)

    def words(r):
        terms = _R233[r]
        if len(terms) == 1:
            k, j, _ = terms[0]
            s0, s1 = chunk(j, 0, k), chunk(j, 1, k)
            return (s0 & u32(0xFFFF)) | (s1 << 16), (s0 >> 16) | (s1 & u32(0xFFFF0000))
        half = [[_signed_sum(terms, lambda k, j: f(chunk(j, par, k))) for par in range(2)] for f in (_lo, _hi)]
        return _words(*half[0]), _words(*half[1])
    return words


def _passes(w):
    return (w[0:64], jnp.concatenate([w[0:32], w[64:96]], axis=0), jnp.concatenate([w[64:96], w[32:64]], axis=0))


def _mm233(product):
    def add(a, b):
        return [x + y for x, y in zip(a, b)]

    def sub(a, b):
        return [x - y for x, y in zip(a, b)]
    p13 = product(13)
    s1 = add(product(12), p13)
    s2 = add(s1, product(14))
    p11 = product(11)
    z = add(s2, p11)
    yield (0, 2), sub(product(9), z)
    s3 = add(product(7), p11)
    s4 = add(s3, product(10))
    y = add(s4, p13)
    yield (1, 2), sub(product(8), y)
    p4 = product(4)
    c10 = add(s4, p4)
    c00 = add(s3, p4)
    p6 = product(6)
    yield (1, 0), add(c10, p6)
    c11 = sub(s1, p6)
    p5 = product(5)
    c01 = sub(s2, p5)
    c00 = add(c00, p5)
    p1 = product(1)
    yield (0, 1), add(c01, p1)
    c11 = add(c11, p1)
    p0 = product(0)
    c00 = add(c00, p0)
    c11 = add(c11, p0)
    yield (1, 1), add(c11, product(3))
    yield (0, 0), add(c00, product(2))


_A424_TEMPS = ((3, 7, -1), (5, 7, -1), (0, 6, -1), (2, 6, -1), (4, 9, -1))
_A424_ROWS = (((4, 1), (0, -1)), ((1, 1), (5, -1)), ((4, 1), (1, -1)), ((0, 1), (1, -1)), ((4, 1),), ((5, 1), (4, -1)), ((1, 1),), ((12, 1),), ((3, 1), (1, -1)), ((2, 1), (1, -1)), ((1, 1), (10, -1)), ((2, 1), (0, -1)), ((10, 1),), ((2, 1),), ((6, 1),), ((2, 1), (3, -1)), ((6, 1), (12, -1)), ((8, 1), (2, -1)), ((8, 1), (11, -1)), ((8, 1),), ((7, 1),), ((8, 1), (10, -1)), ((9, 1),), ((4, 1), (11, 1)), ((2, 1), (9, 1)), ((5, 1), (8, 1)))
_B424_TEMPS = ((0, 2, 1), (2, 3, -1), (5, 6, -1), (7, 9, -1), (4, 8, 1), (1, 10, 1))
_B424_ROWS = (((0, 1), (1, 1)), ((4, 1), (5, 1)), ((1, 1), (4, -1)), ((1, 1),), ((0, 1), (4, 1)), ((4, 1),), ((1, 1), (5, 1)), ((12, 1),), ((5, 1), (7, -1)), ((1, 1), (7, 1)), ((13, 1),), ((1, 1), (3, -1)), ((2, 1), (13, -1)), ((3, 1), (7, 1)), ((2, 1),), ((7, 1),), ((8, 1),), ((11, 1),), ((9, 1),), ((6, 1), (11, -1)), ((6, 1),), ((9, 1), (10, -1)), ((6, 1), (12, 1)), ((3, 1), (8, 1)), ((7, 1), (8, -1)), ((4, 1), (6, 1), (7, 1)))
_POST424 = ((0,), (0,), (0,), (-1, 2, 0), (-1, 2, 1), (0,), (-1, 3, 5), (0,), (1, 6, 7), (2, 0, 8), (0,), (1, 7, 9), (-1, 4, 9), (2, 8, 10), (0,), (1, 5, 12), (1, 11, 12), (2, 1, 13), (2, 9, 14), (0,), (-1, 15, 7), (1, 9, 15), (0,), (0,), (1, 18, 19), (-1, 5, 19), (1, 12, 20), (0,), (-1, 12, 23), (0,), (1, 21, 25), (-1, 22, 25), (0,), (1, 24, 28), (1, 27, 28), (0,), (1, 26, 31), (2, 3, 32), (0,), (1, 29, 33), (-1, 17, 33), (2, 2, 34), (0,), (-1, 22, 36), (-1, 31, 36), (2, 5, 37), (2, 7, 38), (0,), (1, 35, 39), (2, 12, 40), (0,), (1, 31, 41), (-1, 39, 42), (0,), (1, 36, 44), (-1, 33, 45), (1, 43, 46), (1, 30, 46), (-1, 46, 41), (2, 15, 49), (0,), (1, 42, 50), (-1, 48, 51), (0,), (1, 51, 53), (1, 16, 53), (1, 33, 53), (-1, 36, 54), (2, 6, 54), (2, 14, 56), (0,), (1, 52, 58), (2, 13, 59), (0,), (-1, 57, 60), (1, 55, 60), (2, 10, 62), (0,), (1, 47, 63), (0,), (-1, 61, 65), (1, 64, 65), (2, 11, 67), (0,), (1, 66, 68), (2, 4, 69))


def _plain(rows, r):
    return rows[r][0][0] if len(rows[r]) == 1 and rows[r][0][0] < 8 else None


def _operands(block, temps, rows, which):
    x = {}

    def get(v):
        if v not in x:
            if v < 8:
                x[v] = block(v)
            else:
                a, b, c = temps[v - 8]
                x[v] = get(a) + get(b) if c > 0 else get(a) - get(b)
        return x[v]
    out = {}
    for r in which:
        acc = get(rows[r][0][0])
        for v, c in rows[r][1:]:
            acc = acc + get(v) if c > 0 else acc - get(v)
        out[r] = acc
    return out


def _mm424(product, store):
    val, r = [], 0
    for ins in _POST424:
        if ins[0] == 0:
            val.append(product(r))
            r += 1
        elif ins[0] == 2:
            store(ins[1] // 4, ins[1] % 4, val[ins[2]])
        else:
            val.append(val[ins[1]] + val[ins[2]] if ins[0] > 0 else val[ins[1]] - val[ins[2]])


def _recip(l):
    r = pl.reciprocal(l, approx=True)
    return r * (2.0 - l * r)


def _kernel(xat_hbm, ckv_hbm, wqa_hbm, wuk_hbm, wuv_hbm, woa_hbm,
            xbt_hbm, mem0_hbm, wqb_hbm, wkb_hbm, wvb_hbm, wob_hbm,
            out_hbm,
            out_v, xb_v, xpre_v, wb_v, wob_v, wos_v, mem_v, q_v, kv_v, sem):

    def w_copy(w_hbm, dst, slot, par, hp):
        return pltpu.make_async_copy(w_hbm.bitcast(u32).at[:, par * HP + hp, :], dst.at[par, hp], sem.at[slot])

    def w_start_shared(w_hbm, dst, widx, hps):
        for hp in hps:
            for par in range(2):
                w_copy(w_hbm, dst, SEM_WALL + widx, par, hp).start()

    def w_wait_shared(dst, widx):
        pltpu.make_async_copy(dst, dst, sem.at[SEM_WALL + widx]).wait()

    def w_combine(dst, hp):
        a = dst[0, hp]
        b = dst[1, hp]
        ev = (a & u32(0xFFFF)) | (b << 16)
        od = (a >> 16) | (b & u32(0xFFFF0000))
        return ev, od

    def w_pair(dst, hp):
        return jnp.concatenate(w_combine(dst, hp), axis=1)

    wb_hbm = (wqb_hbm, wkb_hbm, wvb_hbm)

    def pre_ref(j):
        n = NSEG * PRE
        return q_v.at[j // 4], (j % 4 // 2) * n, (j % 2) * D

    def lp_prep(lp_v):
        nr = NSEG * PRE // 4
        x = xpre_v[...].astype(f32)

        def store(r, p, w):
            lp_v.at[r][:, p * D:(p + 1) * D] = w
        _lhs233([x[0:nr], x[2 * nr:3 * nr]], [x[nr:2 * nr], x[3 * nr:]], store)

    def b_pre(lp_v):
        nr = NSEG * PRE // 4
        with _scope("b_pre"):
            for g in range(HP // PG):
                hps = range(g * PG, (g + 1) * PG)
                slabs = {}
                for hp in hps:
                    for t in range(3):
                        s0, s1 = wb_v[t, 0, hp], wb_v[t, 1, hp]
                        slabs[hp, t] = (s0, s1)
                        ev = (s0 & u32(0xFFFF)) | (s1 << 16)
                        od = (s0 >> 16) | (s1 & u32(0xFFFF0000))
                        a, b = (KM + HD) // 2, (KM + 2 * HD) // 2
                        d12 = _words(_lo(s0[a:b]) - _hi(s0[a:b]), _lo(s1[a:b]) - _hi(s1[a:b]))
                        d21 = _words(_hi(s0[b:]) - _lo(s0[b:]), _hi(s1[b:]) - _lo(s1[b:]))
                        wb_v[t, 0, hp] = jnp.concatenate([ev[:a], d12, ev[b:]], axis=0)
                        wb_v[t, 1, hp] = jnp.concatenate([od[:a], d21, od[a:b]], axis=0)
                rhs = [_rhs233([slabs[hp, t] for t in range(3)]) for hp in hps]

                def product(r):
                    wa, wb, wc = _passes(jnp.concatenate([x for f in rhs for x in f(r)], axis=1))
                    c = jnp.dot(_unpack(lp_v[r, :, 2 * D:3 * D]), _unpack(wc), preferred_element_type=f32)
                    a = jnp.dot(_unpack(lp_v[r, :, 0:D]), _unpack(wa), preferred_element_type=f32)
                    b = jnp.dot(_unpack(lp_v[r, :, D:2 * D]), _unpack(wb), preferred_element_type=f32)
                    return [a + c, b + c]
                for (i, t), blk in _mm233(product):
                    for y in range(2):
                        x0 = (2 * i + y) * nr
                        for n, hp in enumerate(hps):
                            two = [blk[y][:, (2 * n + e) * D:(2 * n + e + 1) * D] for e in range(2)]
                            if t == 0:
                                two = [z * QSCALE for z in two]
                            two = [z.reshape(nr // PRE, 1, PRE, D) for z in two]
                            two = jnp.concatenate(two, axis=1).reshape(2 * nr, D)
                            ref, r0, l0 = pre_ref(hp * 3 + t)
                            ref[r0 + x0:r0 + x0 + nr, l0:l0 + D] = _pack(two.astype(bf16))

    def phase_a(woa_v, xbt_v, wobt_v, lp_v):
        woa_cp = pltpu.make_async_copy(woa_hbm.bitcast(u32), woa_v, sem.at[SEM_WOA])
        xbt_cp = pltpu.make_async_copy(xbt_hbm, xbt_v, sem.at[SEM_XBT])
        mem_cp = pltpu.make_async_copy(mem0_hbm, mem_v.at[0:MEM, :], sem.at[SEM_MEM])
        wob_cp = pltpu.make_async_copy(wob_hbm.bitcast(u32), wobt_v, sem.at[SEM_WOB])

        def projections(ckv_v, xat_v, wuk_v, wuv_v, wqa_v, lq_v):
            UR = 2 * D
            NU = S // UR
            QR = UR // 4
            kh = DC // 2
            NG = H // 4

            batches = [(0, 1), (2, 4), (4, 8), (8, 12), (12, 16), (1, 2)]

            def batch_start(n):
                for hp in range(*batches[n]):
                    for w_hbm, dst in ((wuk_hbm, wuk_v), (wuv_hbm, wuv_v)):
                        for par in range(2):
                            w_copy(w_hbm, dst, SEM_W + n, par, hp).start()

            def batch_wait(npairs, slot):
                part = wuk_v.at[:, 0:2 * npairs]
                pltpu.make_async_copy(part, part, sem.at[SEM_W + slot]).wait()

            pieces = [(0, 1), (1, 2), (2, 4), (4, 6), (6, 8)]

            def ckv_cp(j):
                rows = slice(pieces[j][0] * UR, pieces[j][1] * UR)
                return pltpu.make_async_copy(ckv_hbm.at[rows, :], ckv_v.at[rows, :], sem.at[SEM_CKV + j])
            xat_cp = pltpu.make_async_copy(xat_hbm, xat_v, sem.at[SEM_XAT])

            with _scope("a_issue0"):
                ckv_cp(0).start()
                batch_start(0)
                ckv_cp(1).start()
                batch_start(5)
                for j in range(2, 5):
                    ckv_cp(j).start()
                for n in range(1, 5):
                    batch_start(n)

            slot_of = {}
            for r in range(26):
                if _plain(_A424_ROWS, r) is None:
                    slot_of[r] = len(slot_of)

            def la_ref(n):
                return q_v.at[3 + n // 4], (n % 4) * (S // 8)

            def t_ref(n):
                return q_v.at[9 + n // 8], (n % 8) * (kh // 2)

            def t_get(n):
                ref, r0 = t_ref(n)
                return ref[r0:r0 + kh // 2, :]

            def lhs_prep(u):
                for c0 in range(0, QR, CL):
                    def block(v):
                        r0 = u * UR + v // 2 * QR + c0
                        return ckv_v[r0:r0 + CL, v % 2 * kh:(v % 2 + 1) * kh].astype(f32)
                    for r, o in _operands(block, _A424_TEMPS, _A424_ROWS, slot_of).items():
                        ref, r0 = la_ref(slot_of[r])
                        p0 = r0 + (u * QR + c0) // 2
                        ref[p0:p0 + CL // 2, :] = _pack(o.astype(bf16))

            def lhs(r, u0, u1):
                v = _plain(_A424_ROWS, r)
                if v is None:
                    ref, r0 = la_ref(slot_of[r])
                    return _unpack(ref[r0 + u0 * QR // 2:r0 + u1 * QR // 2, :])
                i, k = v // 2, v % 2
                return jnp.concatenate([ckv_v[u * UR + i * QR:u * UR + (i + 1) * QR, k * kh:(k + 1) * kh]
                                        for u in range(u0, u1)], axis=0)

            def put_chunk(g, par, c, m, sub=range(26)):
                zero = None if m is None else (pltpu.bitcast(m[0:8, 0:D], u32) >> 31) >> 1
                n = kh // 2
                for e, w_v in enumerate((wuk_v, wuv_v)):
                    raw = {}

                    def words(p, v):
                        if (p, v // 2) not in raw:
                            w = w_v[p, 2 * g + v // 2 % 2, v // 4 * n + c * CR:v // 4 * n + (c + 1) * CR, :]
                            raw[p, v // 2] = w if zero is None else w | zero
                        return raw[p, v // 2]
                    sums = [r for r in sub if _plain(_B424_ROWS, r) is None]
                    ops = [_operands(lambda v: (_hi if v % 2 else _lo)(words(p, v)), _B424_TEMPS, _B424_ROWS, sums)
                           for p in range(2)]
                    for r in sub:
                        v = _plain(_B424_ROWS, r)
                        if v is None:
                            w = _words(ops[0][r], ops[1][r])
                        elif v % 2 == 0:
                            w = (words(0, v) & u32(0xFFFF)) | (words(1, v) << 16)
                        else:
                            w = (words(0, v) >> 16) | (words(1, v) & u32(0xFFFF0000))
                        ref, r0 = t_ref(26 * par + r)
                        ref[r0 + c * CR:r0 + (c + 1) * CR, e * D:(e + 1) * D] = w

            def project_kv(par, g, u0, u1, hooks=None, pre=None):
                def product(r):
                    if pre and r in pre:
                        pre[r]()
                    m = jnp.dot(lhs(r, u0, u1), _unpack(t_get(26 * par + r)), preferred_element_type=f32)
                    if hooks:
                        for c in hooks[1].get(r, ()):
                            put_chunk(hooks[0], 1 - par, c, m)
                    return m

                def store(i, j, blk):
                    for u in range(u0, u1):
                        p0 = (u * UR + i * QR) // 2
                        kv_v.at[4 * g + j][p0:p0 + QR // 2, :] = _pack(blk[(u - u0) * QR:(u - u0 + 1) * QR, :].astype(bf16))
                _mm424(product, store)

            def put_rhs(g, par, which):
                for c in range(kh // 2 // CR):
                    put_chunk(g, par, c, None, which)

            def hook_plan(npiece):
                nch = kh // 2 // CR
                plan = [{} for _ in range(npiece)]
                for c in range(nch):
                    sl = c * (npiece * 26 - 8) // nch
                    plan[sl // 26].setdefault(sl % 26, []).append(c)
                return plan

            def project_group(par, g, nxt):
                plan = hook_plan(NU // KU)
                for u in range(0, NU, KU):
                    project_kv(par, g, u, u + KU, (nxt, plan[u // KU]))

            def kv_first():
                ckv_cp(0).wait()
                lhs_prep(0)
                batch_wait(1, 0)
                put_rhs(0, 0, range(0, 7))
                ckv_cp(1).wait()
                lhs_prep(1)

                def rest():
                    batch_wait(1, 5)
                    for r in (7, 14, 20):
                        put_rhs(0, 0, range(r, {7: 14, 14: 20, 20: 26}[r]))
                project_kv(0, 0, 0, 2, pre={7: rest})
                ckv_cp(2).wait()
                lhs_prep(2)
                lhs_prep(3)
                ckv_cp(3).wait()
                lhs_prep(4)
                lhs_prep(5)
                project_kv(0, 0, 2, 4)
                ckv_cp(4).wait()
                batch_wait(2, 1)
                lhs_prep(6)
                lhs_prep(7)
                plan = hook_plan(2)
                for u in range(4, 8, 2):
                    project_kv(0, 0, u, u + 2, (1, plan[(u - 4) // 2]))

            def kv_body(j, c):
                @pl.when(j == 0)
                def _():
                    xat_cp.start()
                    w_start_shared(wqa_hbm, wqa_v, 0, range(HP))
                    xbt_cp.start()
                batch_wait(4, 2 + j)
                project_group(1, 2 * j + 1, 2 * j + 2)
                project_group(0, 2 * j + 2, 2 * j + 3)
                return c

            with _scope("a_kvproj"):
                kv_first()
                jax.lax.fori_loop(0, NG // 2 - 1, kv_body, 0)

            woa_cp.start()
            wob_cp.start()
            mem_cp.start()
            w_start_shared(wqb_hbm, wb_v.at[0], 1, range(HP))
            w_start_shared(wkb_hbm, wb_v.at[1], 2, range(HP // 2))

            QB = 4 * D
            plain = {(0, 0): 15, (0, 1): 1, (0, 2): 9, (1, 0): 4, (1, 1): 16, (1, 2): 8}

            def xa_prep(b):
                x = []
                for t in range(4 * b, 4 * b + 4):
                    xt = xat_v[:, t * D:(t + 1) * D]
                    x.append(jnp.concatenate([xt, xt[DM - HD:]], axis=0).astype(f32).T)

                def store(r, p, w):
                    lq_v.at[r][b * HD:(b + 1) * HD, p * D:(p + 1) * D] = w
                _lhs233([x[0], x[2]], [x[1], x[3]], store, extra=(((0, 0, 1),), ((1, 1, 1),)))

            def q_store(blk, hp, x0):
                q_v.at[hp][x0 // 2:(x0 + blk.shape[0]) // 2, :] = _pack((blk * QSCALE).astype(bf16))

            def q_rhs(hp):
                f = _rhs233([(wqa_v[0, hp + n], wqa_v[1, hp + n]) for n in range(3)])
                return [_passes(jnp.concatenate(f(r), axis=1)) for r in range(15)]

            def project_q(t, hp, b):
                nr = D // QS
                for s in range(QS):
                    rows = slice(b * HD + s * nr // 2, b * HD + (s + 1) * nr // 2)

                    def product(r):
                        wa, wb, wc = t[r]
                        c = jnp.dot(_unpack(lq_v[r, rows, 2 * D:3 * D]), _unpack(wc), preferred_element_type=f32)
                        a = jnp.dot(_unpack(lq_v[r, rows, 0 * D:1 * D]), _unpack(wa), preferred_element_type=f32)
                        b = jnp.dot(_unpack(lq_v[r, rows, 1 * D:2 * D]), _unpack(wb), preferred_element_type=f32)
                        return [a + c, b + c]
                    for (i, j), blk in _mm233(product):
                        for y in range(2):
                            q_store(blk[y], hp + j, b * QB + (2 * i + y) * D + s * nr)

            def project_q_last(hp):
                s0, s1 = wqa_v[0, hp], wqa_v[1, hp]
                w = jnp.concatenate([(s0 & u32(0xFFFF)) | (s1 << 16), (s0 >> 16) | (s1 & u32(0xFFFF0000))], axis=1)
                per = [_passes(jnp.concatenate([w[a:a + 64], w[c:c + 32]] if k == 1 else [w[a:a + 96]], axis=0))
                       for k, (a, _, c) in enumerate(_PIECES)]
                wp = [_unpack(jnp.concatenate([per[k][p] for k in range(3)], axis=0)) for p in range(3)]
                for b in range(S // QB):
                    rows = slice(b * HD, (b + 1) * HD)
                    for i in range(2):
                        a, bb, c = [jnp.dot(_unpack(jnp.concatenate([lq_v[plain[i, k], rows, p * D:(p + 1) * D] for k in range(3)], axis=1)),
                                            wp[p], preferred_element_type=f32) for p in range(3)]
                        q_store(a + c, hp, b * QB + 2 * i * D)
                        q_store(bb + c, hp, b * QB + (2 * i + 1) * D)

            def xb_prep(t):
                t0 = pl.multiple_of(t * D, D)
                xt = xbt_v[:, pl.ds(t0, D)]
                xb = jnp.concatenate([xt, xt[DM - HD:]], axis=0).T
                xb_v[pl.ds(t0, D), :] = xb
                for sg in range(D // SEG):
                    p0 = pl.multiple_of((t * (D // SEG) + sg) * PRE, PRE)
                    xpre_v[pl.ds(p0, PRE), :] = xb[sg * SEG:sg * SEG + PRE, :]

            with _scope("a_qproj"):
                xat_cp.wait()
                xbt_cp.wait()
                w_wait_shared(wqa_v, 0)
                t = q_rhs(0)
                for b in range(S // QB):
                    xa_prep(b)
                    for u in range(0, NU, KU):
                        if u // 2 == b:
                            project_kv(1, NG - 1, u, u + KU)
                    project_q(t, 0, b)
                XG = 4

                def q_body(j, c):
                    hp = 3 * j
                    for n in range(XG):
                        xb_prep((j - 1) * XG + n)
                    t = q_rhs(hp)
                    for b in range(S // QB):
                        project_q(t, hp, b)
                    return c
                jax.lax.fori_loop(1, 5, q_body, 0)
                lp_prep(lp_v)
                project_q_last(HP - 1)

        pl.run_scoped(
            projections,
            pltpu.VMEM((S, DC), bf16),
            pltpu.VMEM((DM, S), bf16),
            pltpu.VMEM((2, HP, DC // 2, D), u32),
            pltpu.VMEM((2, HP, DC // 2, D), u32),
            pltpu.VMEM((2, HP, DM // 2, D), u32),
            pltpu.VMEM((17, S // 8, 3 * D), u32),
        )

        def attention(c_v, s_v):
            row = jax.lax.broadcasted_iota(jnp.int32, (TQ, TQ), 0)
            col = jax.lax.broadcasted_iota(jnp.int32, (TQ, TQ), 1)
            tri = col <= row
            nb = S // TQ
            hq = TQ // 2
            npiece = 2
            pw = S // npiece

            def q_rows(h, r0, r1):
                return q_v[h[0], r0:r1, h[1] * D:(h[1] + 1) * D]

            def head(h):
                return 2 * h[0] + h[1]

            def qk_piece(h, j):
                q = _unpack(q_rows(h, (nb - 1) * hq, nb * hq))
                k = _unpack(kv_v[head(h), j * pw // 2:(j + 1) * pw // 2, 0:D])
                s_v[:, j * pw:(j + 1) * pw] = jax.lax.dot_general(q, k, NT, preferred_element_type=f32)

            def qk(h, i, j0=0, j1=None):
                j1 = i + 1 if j1 is None else j1
                q = _unpack(q_rows(h, i * hq, (i + 1) * hq))
                k = _unpack(kv_v[head(h), j0 * hq:j1 * hq, 0:D])
                return jax.lax.dot_general(q, k, NT, preferred_element_type=f32)

            def anchor_plan():
                ops = []
                for e in range(UH):
                    for i in range(nb - 1, -1, -1):
                        if i > 0:
                            ops.append(("qk", e, i - 1, 32 * i))
                        if i < npiece:
                            ops.append(("piece", e, i, 32 * nb // npiece))
                        ops.append(("pv", e, i, 32 * (i + 1)))
                t, start, end = 0, [], []
                for op in ops:
                    start.append(t)
                    t += op[3]
                    end.append(t)
                plan = {}
                for a, op in enumerate(ops):
                    if op[0] != "pv" or op[2] < ANCHOR_MIN:
                        continue
                    for b in range(a + 1, len(ops)):
                        if ops[b][0] == "qk" and start[b] >= end[a] + ANCHOR_LAG:
                            plan.setdefault((ops[b][1], ops[b][2]), []).append((op[1], op[2]))
                            break
                return plan

            def heads(j, c):
                @pl.when(j == 0)
                def _():
                    w_start_shared(wkb_hbm, wb_v.at[1], 2, range(HP // 2, HP))
                    w_start_shared(wvb_hbm, wb_v.at[2], 3, range(HP))

                plan = anchor_plan()

                def gated_qk(e, i):
                    h = (j * (UH // 2) + e // 2, e % 2)
                    if (e, i) not in plan:
                        return qk(h, i)
                    w = None
                    for ea, ia in plan[e, i]:
                        u = c_v[j * (UH // 2) + ea // 2, ia * hq:(ia + 1) * hq, (ea % 2) * D:(ea % 2 + 1) * D]
                        for r in range(0, hq, 8):
                            w = u[r:r + 8] if w is None else w | u[r:r + 8]
                    zero = (w >> 31) >> 1
                    q = q_rows(h, i * hq, (i + 1) * hq)
                    q = _unpack(jnp.concatenate([q[0:8] | zero, q[8:]], axis=0))
                    k = _unpack(kv_v[head(h), 0:(i + 1) * hq, 0:D])
                    return jax.lax.dot_general(q, k, NT, preferred_element_type=f32)

                s_next = s_v[...]
                for e in range(UH):
                    h = (j * (UH // 2) + e // 2, e % 2)
                    if e == UH - 1:
                        hn = (jnp.minimum(h[0] + 1, HP - 1), 0)
                    else:
                        hn = (j * (UH // 2) + (e + 1) // 2, (e + 1) % 2)
                    pieces = []
                    for i in range(nb - 1, -1, -1):
                        s = s_next
                        if i > 0:
                            s_next = gated_qk(e, i - 1)
                        if i < npiece:
                            if e == UH - 1:
                                qk_piece(hn, npiece - 1 - i)
                            else:
                                jj = npiece - 1 - i
                                pieces.append(qk(hn, nb - 1, jj * nb // npiece, (jj + 1) * nb // npiece))
                        sd = jnp.where(tri, s[:, i * TQ:], NEG)
                        s = jnp.concatenate([s[:, :i * TQ], sd], axis=1) if i > 0 else sd
                        m = jnp.max(s, axis=1, keepdims=True)
                        p = jnp.exp2(s - m)
                        l = jnp.sum(p, axis=1, keepdims=True)
                        v = _unpack(kv_v[head(h), 0:(i + 1) * hq, D:2 * D])
                        o = jnp.dot(p.astype(bf16), v, preferred_element_type=f32)
                        c_v.at[h[0]][i * hq:(i + 1) * hq, h[1] * D:(h[1] + 1) * D] = _pack((o * _recip(l)).astype(bf16))
                    if e < UH - 1:
                        s_next = jnp.concatenate(pieces, axis=1)
                return c
            with _scope("a_attn"):
                for j in range(npiece):
                    qk_piece((0, 0), j)
                jax.lax.fori_loop(0, H // UH, heads, 0)

            woa_cp.wait()
            wob_cp.wait()
            mem_cp.wait()
            for t in range(3):
                w_wait_shared(wb_v.at[t], 1 + t)
            mh = DM // 4

            def wo_prep(hh):
                a11, a21 = woa_v[hh, 0:mh, :], woa_v[hh, mh:2 * mh, :]
                a12, a22 = woa_v[hh + HP, 0:mh, :], woa_v[hh + HP, mh:2 * mh, :]
                for i, w in enumerate(_sum_words(_strassen_lhs, a11, a12, a21, a22, (2, 3), (a11, a22))):
                    if i not in (2, 3):
                        kv_v[hh, i * mh:(i + 1) * mh, 0:D] = w

            def wob_prep(hp):
                w1, w2 = _unpack(wobt_v[2 * hp]), _unpack(wobt_v[2 * hp + 1])
                a, b = KM + HD, KM + 2 * HD
                d12 = (w1[a:b].astype(f32) - w2[a:b].astype(f32)).astype(bf16)
                d21 = (w2[b:].astype(f32) - w1[b:].astype(f32)).astype(bf16)
                rows = slice(hp * HD, (hp + 1) * HD)
                wob_v[0, rows, :] = _pack(jnp.concatenate([w1[:a], d12], axis=0).T)
                wob_v[1, rows, :] = _pack(jnp.concatenate([w2[:a], d21], axis=0).T)
                wos_v[rows, :] = _pack(jnp.concatenate([w1[b:], w2[a:b]], axis=0).T)

            def oproj(tp):
                w0 = tp * D
                per = []
                for hh in range(HP):
                    def ctx(h, r0):
                        return c_v[h // 2, r0:r0 + D // 2, (h % 2) * D:(h % 2 + 1) * D]
                    b11, b21 = ctx(hh, w0), ctx(hh + HP, w0)
                    b12, b22 = ctx(hh, w0 + D // 2), ctx(hh + HP, w0 + D // 2)
                    per.append(_sum_words(_strassen_rhs, b11, b12, b21, b22, (1, 4), (b11, b22)))

                def lhs(i):
                    if i == 2:
                        return _unpack(jnp.concatenate([woa_v[hh, 0:mh, :] for hh in range(HP)], axis=1))
                    if i == 3:
                        return _unpack(jnp.concatenate([woa_v[hh + HP, mh:2 * mh, :] for hh in range(HP)], axis=1))
                    return _unpack(jnp.concatenate([kv_v[hh, i * mh:(i + 1) * mh, 0:D] for hh in range(HP)], axis=1))

                def rhs(i):
                    return _unpack(jnp.concatenate([per[hh][i] for hh in range(HP)], axis=1))
                c11, c12, c21, c22 = _strassen(lhs, rhs, NT)
                t0 = 2 * tp * D
                out_v[t0:t0 + D, 0:DM] = jnp.concatenate([c11, c21], axis=0).T.astype(bf16)
                out_v[t0 + D:t0 + 2 * D, 0:DM] = jnp.concatenate([c12, c22], axis=0).T.astype(bf16)

            b_pre(lp_v)
            with _scope("a_oproj"):
                for hh in range(HP):
                    wo_prep(hh)
                for tp in range(S // D // 2):
                    oproj(tp)
                    for hp in range(2 * tp, 2 * tp + 2):
                        wob_prep(hp)

        pl.run_scoped(
            attention,
            pltpu.VMEM((HP, S // 2, 2 * D), u32),
            pltpu.VMEM((TQ, S), f32),
        )

    pl.run_scoped(
        phase_a,
        pltpu.VMEM((H, DM // 2, D), u32),
        pltpu.VMEM((DM, S), bf16),
        pltpu.VMEM((H, DM // 2, D), u32),
        pltpu.VMEM((15, NSEG * PRE // 8, 3 * D), u32),
    )

    def out_copy(j):
        rows = pl.ds(pl.multiple_of(j * (OUTER * SEG), OUTER * SEG), OUTER * SEG)
        return pltpu.make_async_copy(out_v.at[rows, :], out_hbm.at[rows, :], sem.at[SEM_OUT + j])

    def phase_b(post_v):
        GP = HG // 2
        GC = GP * 3 * D
        KA = KM + 2 * HD
        lane = jax.lax.broadcasted_iota(jnp.int32, (1, GC), 1)
        colscale = jnp.where(lane % (3 * D) < D, QSCALE, 1.0).astype(f32)
        low = jax.lax.broadcasted_iota(jnp.int32, (1, D), 1) < HD

        def swap(x):
            return pltpu.roll(x, HD, 1)

        def wgroup(g):
            cols = [(hp, t) for hp in range(g * GP, (g + 1) * GP) for t in range(3)]
            own = [_unpack(jnp.concatenate([wb_v[t, e, hp, 0:KA // 2, :] for hp, t in cols], axis=1)) for e in range(2)]
            both = jnp.concatenate([jnp.concatenate([wb_v[t, e, hp, KA // 2:, :] for hp, t in cols], axis=1)
                                    for e in range(2)], axis=0)
            return own[0], own[1], _unpack(both)

        def out_project(even, odd, both, p0, p1):
            rows = slice(p0 * HD, p1 * HD)
            return [jnp.dot(even, _unpack(wob_v[0, rows, :]), preferred_element_type=f32),
                    jnp.dot(odd, _unpack(wob_v[1, rows, :]), preferred_element_type=f32),
                    jnp.dot(both, _unpack(wos_v[rows, :]), preferred_element_type=f32)]

        def out_add(acc, part):
            e, o, b = part
            new = [e[:, :KM] + o[:, :KM], e[:, KM:], o[:, KM:], b]
            return new if acc is None else [x + y for x, y in zip(acc, new)]

        def out_finish(acc):
            main, e, o, b = acc
            mid = e + jnp.where(low, o, b)
            last = jnp.where(low, swap(o) + b, o + swap(b))
            return jnp.concatenate([main, mid, last], axis=1)

        ri = jax.lax.broadcasted_iota(jnp.int32, (2 * L, 2 * L), 0)
        ci = jax.lax.broadcasted_iota(jnp.int32, (2 * L, 2 * L), 1)

        def second(i):
            return jnp.where(i < 2 * SEG, i // SEG, (i - 2 * SEG) // PRE)

        def pos(i):
            j = i % SEG
            return jnp.where(i < 2 * SEG, jnp.where(j < T, j + (MEM + PRE), j - T), MEM + i % PRE)
        same = second(ri) == second(ci)
        mask = same & ((pos(ri) < MEM) | (pos(ri) >= pos(ci)))
        fill = jnp.where(same, NEG, -jnp.inf).astype(f32)

        def step(s, slot, mem):
            xt = xb_v[pl.ds(pl.multiple_of(SEG * s + PRE, 8), T), :]
            l1 = jnp.concatenate([xt.astype(f32), mem], axis=0)
            mid, last = l1[:, KM:KA], l1[:, KA:]
            l_even = l1[:, :KA].astype(bf16)
            l_odd = jnp.concatenate([l1[:, :KM], jnp.where(low, mid, last)], axis=1).astype(bf16)
            l_both = jnp.where(low, last, mid).astype(bf16)
            p0 = pl.multiple_of(PRE * s, 8)
            proj = []
            for g in range(G):
                w_even, w_odd, w_both = wgroup(g)
                both = jnp.dot(l_both, w_both, preferred_element_type=f32)
                even = jnp.dot(l_even, w_even, preferred_element_type=f32)
                odd = jnp.dot(l_odd, w_odd, preferred_element_type=f32)
                proj.append([(x + both) * colscale for x in (even, odd)])

            def rows(hp, t):
                g, c0 = hp // GP, (hp % GP) * 3 * D + t * D
                ref, r0, l0 = pre_ref(hp * 3 + t)
                return jnp.concatenate([proj[g][0][:, c0:c0 + D], proj[g][1][:, c0:c0 + D],
                                        _unpack(ref[pl.ds(r0 + p0, PRE), l0:l0 + D]).astype(f32)], axis=0).astype(bf16)

            scores = [jax.lax.dot_general(rows(hp, 0), rows(hp, 1), NT, preferred_element_type=f32)
                      for hp in range(HP)]
            ctx = {}

            def attend(g):
                for hp in range(g * HG // 2, (g + 1) * HG // 2):
                    sc = jnp.where(mask, scores[hp], fill)
                    m = jnp.max(sc, axis=1, keepdims=True)
                    p = jnp.exp2(sc - m)
                    l = jnp.sum(p, axis=1, keepdims=True)
                    o = jnp.dot(p.astype(bf16), rows(hp, 2), preferred_element_type=f32) * _recip(l)
                    ctx[hp] = [o[0:SEG, :], o[SEG:2 * SEG, :], o[0:SEG, :] + o[SEG:2 * SEG, :]]
                    for e in range(2):
                        post_v[e, slot * PRE:(slot + 1) * PRE, hp * D:(hp + 1) * D] = o[2 * SEG + e * PRE:2 * SEG + (e + 1) * PRE, :]

            parts = []

            def oproj(g):
                lhs = [jnp.concatenate([ctx[hp][e] for hp in range(g * GP, (g + 1) * GP)], axis=1).astype(bf16)
                       for e in range(3)]
                parts.append(out_project(*lhs, g * GP, (g + 1) * GP))

            for t in range(G + 2):
                if t < G:
                    attend(t)
                if t >= 2:
                    oproj(t - 2)
            acc = None
            for a in parts:
                acc = out_add(acc, a)
            accb = out_finish(acc).astype(bf16)
            out_v[pl.ds(pl.multiple_of(SEG * s + PRE, 8), T), DM:2 * DM] = accb[0:T, 0:DM]
            return accb[T:, :].astype(f32), ctx[HP - 1][1]

        PP = HP // OUTER

        def deferred_rows():
            even, odd = post_v[0], post_v[1]
            return even, odd, even + odd

        def finish(j, acc):
            r = out_finish(acc).astype(bf16)
            for sg in range(OUTER):
                r0 = pl.multiple_of((j * OUTER + sg) * SEG, SEG)
                out_v[pl.ds(r0, PRE), DM:2 * DM] = r[sg * PRE:(sg + 1) * PRE, 0:DM]

        def after(x, late):
            u = pltpu.bitcast(late[0:8, :], u32)
            zero = (u >> 31) & (~u >> 31)
            top = pltpu.bitcast(x[0:8], u32) | jnp.concatenate([zero] * (x.shape[1] // D), axis=1)
            return jnp.concatenate([pltpu.bitcast(top, f32), x[8:]], axis=0).astype(bf16)

        def outer(j, mem):
            prev = deferred_rows()

            def partial(i, late):
                x = [after(p[:, i * PP * D:(i + 1) * PP * D], late) for p in prev]
                return out_project(*x, i * PP, (i + 1) * PP)
            acc = None
            for i in range(OUTER):
                mem, late = step(j * OUTER + i, i, mem)
                acc = out_add(acc, partial(i, late))
            finish(jnp.maximum(j - 1, 0), acc)

            @pl.when(j > 0)
            def _():
                out_copy(j - 1).start()
            return mem
        with _scope("b_loop"):
            post_v[...] = jnp.zeros(post_v.shape, f32)
            mem0 = mem_v[0:MEM, :].astype(f32)
            jax.lax.fori_loop(0, NOUTER, outer, jnp.concatenate([mem0, mem0[:, DM - HD:]], axis=1))
            finish(NOUTER - 1, out_add(None, out_project(*[x.astype(bf16) for x in deferred_rows()], 0, HP)))
            out_copy(NOUTER - 1).start()
        with _scope("b_outwait"):
            for j in range(NOUTER):
                out_copy(j).wait()

    pl.run_scoped(
        phase_b,
        pltpu.VMEM((2, OUTER * PRE, HP * D), f32),
    )


@jax.jit
def pallas_concat_heads__compressed_kv_cla__memory_aug_recurrent_mem_tr__prompt_kernel(
    A_x: jax.Array,
    A_c_kv: jax.Array,
    A_w_q: jax.Array,
    A_w_uk: jax.Array,
    A_w_uv: jax.Array,
    A_w_o: jax.Array,
    B_x: jax.Array,
    B_mem0: jax.Array,
    B_Wq: jax.Array,
    B_Wk: jax.Array,
    B_Wv: jax.Array,
    B_Wo: jax.Array,
    B_seg_len=SEG,
):
    def t2(x):
        return jnp.transpose(x, (0, 2, 1)).reshape(DM, S)

    def w3(w):
        return w.reshape(w.shape[0] // 2, 2 * H, D)

    def wo3(w):
        return jnp.transpose(w, (0, 2, 1))

    any_spec = pl.BlockSpec(memory_space=pl.ANY)
    out = pl.pallas_call(
        _kernel,
        out_shape=jax.ShapeDtypeStruct((S, 2 * DM), bf16),
        in_specs=[any_spec] * 12,
        out_specs=any_spec,
        scratch_shapes=[
            pltpu.VMEM((S, 2 * DM), bf16),
            pltpu.VMEM((S, DMP), bf16),
            pltpu.VMEM((NSEG * PRE, DMP), bf16),
            pltpu.VMEM((3, 2, HP, DM // 2, D), u32),
            pltpu.VMEM((2, HP * D // 2, KM + 2 * HD), u32),
            pltpu.VMEM((HP * D // 2, D), u32),
            pltpu.VMEM((8 * MEM, DM), bf16),
            pltpu.VMEM((HP, S // 2, 2 * D), u32),
            pltpu.VMEM((H, S // 2, 2 * D), u32),
            pltpu.SemaphoreType.DMA((NSEM,)),
        ],
        compiler_params=pltpu.CompilerParams(vmem_limit_bytes=126 * 1024 * 1024),
    )(t2(A_x), A_c_kv.reshape(S, DC), w3(A_w_q), w3(A_w_uk), w3(A_w_uv), wo3(A_w_o),
      t2(B_x), B_mem0.reshape(MEM, DM), w3(B_Wq), w3(B_Wk), w3(B_Wv), wo3(B_Wo))
    return out.reshape(1, S, 2 * DM)
```

```python
import contextlib

import jax
import jax.numpy as jnp
import jax.experimental.pallas as pl
import jax.experimental.pallas.tpu as pltpu

S = 2048
DM = 576
DC = 512
H = 32
D = 128
MEM = 8
SEG = 32
L = MEM + SEG
NSEG = S // SEG
HP = H // 2
HD = D // 2
KM = DM - 3 * HD
DMP = DM + HD

LOG2E = 1.4426950408889634
QSCALE = D ** -0.5 * LOG2E
NEG = -1.0e9 * LOG2E

TQ = 128
UH = 4
ANCHOR_LAG = 2000
ANCHOR_MIN = 6
RB = 512
HG = 4
G = H // HG
PRE = 8
T = SEG - PRE
OUTER = 4
NOUTER = NSEG // OUTER

bf16 = jnp.bfloat16
f32 = jnp.float32
u32 = jnp.uint32
NT = (((1,), (1,)), ((), ()))

SEM_CKV = 0
SEM_XAT = 5
SEM_XBT = 6
SEM_MEM = 7
SEM_WOA = 8
SEM_WOB = 9
SEM_OUT = 10
SEM_WALL = SEM_OUT + NOUTER
SEM_W = SEM_WALL + 4
NSEM = SEM_W + 6

_PROFILE = False
KU = 2
CL = 16
CR = 8
PVT = 5
PG = 1
QS = 2

def _scope(name):
    return jax.named_scope(name) if _PROFILE else contextlib.nullcontext()


def _unpack(w32):
    return pltpu.bitcast(w32, bf16)


def _pack(x):
    return pltpu.bitcast(x, u32)


def _lo(w):
    return pltpu.bitcast(w << 16, f32)


def _hi(w):
    return pltpu.bitcast(w & u32(0xFFFF0000), f32)


def _words(even, odd):
    return pltpu.bitcast(pltpu.pack_elementwise([even, odd], packed_dtype=bf16), u32)


def _strassen_lhs(a11, a12, a21, a22):
    return [a11 + a22, a21 + a22, a11, a22, a11 + a12, a21 - a11, a12 - a22]


def _strassen_rhs(b11, b12, b21, b22):
    return [b11 + b22, b11, b12 - b22, b21 - b11, b22, b11 + b12, b21 + b22]


def _sum_words(combine, x11, x12, x21, x22, raw_idx, raw):
    lo = combine(_lo(x11), _lo(x12), _lo(x21), _lo(x22))
    hi = combine(_hi(x11), _hi(x12), _hi(x21), _hi(x22))
    words = [pltpu.bitcast(pltpu.pack_elementwise([a, b], packed_dtype=bf16), u32) for a, b in zip(lo, hi)]
    for i, r in zip(raw_idx, raw):
        words[i] = r
    return words


def _strassen(lhs, rhs, dims=(((1,), (0,)), ((), ())), order=0):
    def m(i):
        return jax.lax.dot_general(lhs(i - 1), rhs(i - 1), dims, preferred_element_type=f32)
    if order == 0:
        m1 = m(1)
        m2 = m(2)
        c22 = m1 - m2
        m4 = m(4)
        c11 = m1 + m4
        c21 = m2 + m4
        c22 = c22 + m(6)
        m3 = m(3)
        c22 = c22 + m3
        m5 = m(5)
        c11 = c11 - m5
        c12 = m3 + m5
        c11 = c11 + m(7)
        return c11, c12, c21, c22
    m3 = m(3)
    m4 = m(4)
    m5 = m(5)
    c12 = m3 + m5
    c11 = m4 - m5
    m2 = m(2)
    c21 = m4 + m2
    c22 = m3 - m2
    m1 = m(1)
    c11 = c11 + m1
    c22 = c22 + m1
    c22 = c22 + m(6)
    c11 = c11 + m(7)
    return c11, c12, c21, c22


def _rhs_words(s0, s1, z0, z1):
    per = [_strassen_rhs(_lo(s), _hi(s), _lo(z), _hi(z)) for s, z in ((s0, z0), (s1, z1))]
    words = [pltpu.bitcast(pltpu.pack_elementwise([per[0][i], per[1][i]], packed_dtype=bf16), u32)
             for i in range(7)]
    words[1] = (s0 & u32(0xFFFF)) | (s1 << 16)
    words[4] = (z0 >> 16) | (z1 & u32(0xFFFF0000))
    return words


_L233 = (((0, 1, 1), (1, 0, 1)), ((0, 1, 1),), ((0, 0, 1), (1, 0, -1)), ((0, 1, 1), (1, 1, -1)), ((1, 0, 1),),
         ((0, 0, -1), (0, 1, -1)), ((1, 0, 1), (1, 1, 1)), ((0, 0, 1), (0, 2, 1), (1, 0, -1)), ((1, 2, 1),),
         ((0, 2, 1),), ((1, 0, 1), (1, 2, 1), (0, 0, -1), (0, 2, -1)), ((0, 0, -1), (0, 2, -1)),
         ((1, 1, 1), (1, 2, 1), (0, 1, -1)), ((1, 1, -1), (1, 2, -1)),
         ((0, 1, 1), (0, 2, 1), (1, 1, -1), (1, 2, -1)))
_R233 = (((0, 1, 1), (1, 0, 1)), ((1, 1, 1), (1, 2, 1), (0, 1, -1)), ((0, 0, 1), (0, 1, 1), (2, 0, -1)),
         ((2, 1, 1), (1, 0, -1), (1, 1, -1)), ((0, 0, 1), (0, 2, 1), (1, 0, -1)), ((0, 1, 1),), ((1, 0, 1),),
         ((0, 2, 1), (2, 0, 1)), ((2, 0, 1), (2, 2, 1), (1, 2, -1)), ((2, 1, 1), (2, 2, 1), (0, 2, -1)),
         ((2, 0, 1),), ((0, 2, 1),), ((1, 2, 1), (2, 1, 1)), ((1, 2, 1),), ((2, 1, 1),))
_PIECES = ((0, 32, 64), (128, 160, 96), (192, 224, 256))


def _signed_sum(terms, get):
    acc = None
    for a, b, c in terms:
        x = get(a, b)
        if acc is None:
            acc = x if c > 0 else -x
        else:
            acc = acc + x if c > 0 else acc - x
    return acc


def _lhs233(y1, y2, store, extra=()):
    low = jax.lax.broadcasted_iota(jnp.int32, (1, D), 1) < HD
    base = {}
    for i in range(2):
        t1 = [y1[i][:, c * D:(c + 1) * D] for c in range(5)]
        t2 = [y2[i][:, c * D:(c + 1) * D] for c in range(5)]
        r1, r2 = pltpu.roll(t1[1], HD, 1), pltpu.roll(t2[1], HD, 1)
        for k in range(3):
            a1, a2 = t1[(0, 2, 3)[k]], t2[(0, 2, 3)[k]]
            lo1 = (t1[1], r1, t1[4])[k]
            hi1, hi2 = (r1, t1[1], t1[4])[k], (r2, t2[1], t2[4])[k]
            base[i, k] = (jnp.where(low, a1, a1 - a2), jnp.where(low, a2, hi2 - hi1), jnp.where(low, lo1, a2))
    for r, terms in enumerate(_L233 + extra):
        for p in range(3):
            store(r, p, _pack(_signed_sum(terms, lambda i, k: base[i, k][p]).astype(bf16)))


def _rhs233(slabs):
    def chunk(j, par, k):
        s = slabs[j][par]
        a, b, c = _PIECES[k]
        return s[a:a + 96] if k != 1 else jnp.concatenate([s[a:a + 64], s[c:c + 32]], axis=0)

    def words(r):
        terms = _R233[r]
        if len(terms) == 1:
            k, j, _ = terms[0]
            s0, s1 = chunk(j, 0, k), chunk(j, 1, k)
            return (s0 & u32(0xFFFF)) | (s1 << 16), (s0 >> 16) | (s1 & u32(0xFFFF0000))
        half = [[_signed_sum(terms, lambda k, j: f(chunk(j, par, k))) for par in range(2)] for f in (_lo, _hi)]
        return _words(*half[0]), _words(*half[1])
    return words


def _passes(w):
    return (w[0:64], jnp.concatenate([w[0:32], w[64:96]], axis=0), jnp.concatenate([w[64:96], w[32:64]], axis=0))


def _mm233(product):
    def add(a, b):
        return [x + y for x, y in zip(a, b)]

    def sub(a, b):
        return [x - y for x, y in zip(a, b)]
    p13 = product(13)
    s1 = add(product(12), p13)
    s2 = add(s1, product(14))
    p11 = product(11)
    yield (0, 2), sub(sub(product(9), s2), p11)
    s3 = add(product(7), p11)
    s4 = add(s3, product(10))
    yield (1, 2), sub(sub(product(8), s4), p13)
    p4 = product(4)
    p6 = product(6)
    yield (1, 0), add(add(p6, s4), p4)
    c11 = sub(s1, p6)
    p5 = product(5)
    p1 = product(1)
    yield (0, 1), sub(add(p1, s2), p5)
    c11 = add(c11, p1)
    p0 = product(0)
    yield (1, 1), add(add(product(3), c11), p0)
    yield (0, 0), add(add(add(add(product(2), s3), p4), p5), p0)


_A424_TEMPS = ((3, 7, -1), (5, 7, -1), (0, 6, -1), (2, 6, -1), (4, 9, -1))
_A424_ROWS = (((4, 1), (0, -1)), ((1, 1), (5, -1)), ((4, 1), (1, -1)), ((0, 1), (1, -1)), ((4, 1),), ((5, 1), (4, -1)), ((1, 1),), ((12, 1),), ((3, 1), (1, -1)), ((2, 1), (1, -1)), ((1, 1), (10, -1)), ((2, 1), (0, -1)), ((10, 1),), ((2, 1),), ((6, 1),), ((2, 1), (3, -1)), ((6, 1), (12, -1)), ((8, 1), (2, -1)), ((8, 1), (11, -1)), ((8, 1),), ((7, 1),), ((8, 1), (10, -1)), ((9, 1),), ((4, 1), (11, 1)), ((2, 1), (9, 1)), ((5, 1), (8, 1)))
_B424_TEMPS = ((0, 2, 1), (2, 3, -1), (5, 6, -1), (7, 9, -1), (4, 8, 1), (1, 10, 1))
_B424_ROWS = (((0, 1), (1, 1)), ((4, 1), (5, 1)), ((1, 1), (4, -1)), ((1, 1),), ((0, 1), (4, 1)), ((4, 1),), ((1, 1), (5, 1)), ((12, 1),), ((5, 1), (7, -1)), ((1, 1), (7, 1)), ((13, 1),), ((1, 1), (3, -1)), ((2, 1), (13, -1)), ((3, 1), (7, 1)), ((2, 1),), ((7, 1),), ((8, 1),), ((11, 1),), ((9, 1),), ((6, 1), (11, -1)), ((6, 1),), ((9, 1), (10, -1)), ((6, 1), (12, 1)), ((3, 1), (8, 1)), ((7, 1), (8, -1)), ((4, 1), (6, 1), (7, 1)))
_POST424 = ((0,), (0,), (0,), (-1, 2, 0), (-1, 2, 1), (0,), (-1, 3, 5), (0,), (1, 6, 7), (2, 0, 8), (0,), (1, 7, 9), (-1, 4, 9), (2, 8, 10), (0,), (1, 5, 12), (1, 11, 12), (2, 1, 13), (2, 9, 14), (0,), (-1, 15, 7), (1, 9, 15), (0,), (0,), (1, 18, 19), (-1, 5, 19), (1, 12, 20), (0,), (-1, 12, 23), (0,), (1, 21, 25), (-1, 22, 25), (0,), (1, 24, 28), (1, 27, 28), (0,), (1, 26, 31), (2, 3, 32), (0,), (1, 29, 33), (-1, 17, 33), (2, 2, 34), (0,), (-1, 22, 36), (-1, 31, 36), (2, 5, 37), (2, 7, 38), (0,), (1, 35, 39), (2, 12, 40), (0,), (1, 31, 41), (-1, 39, 42), (0,), (1, 36, 44), (-1, 33, 45), (1, 43, 46), (1, 30, 46), (-1, 46, 41), (2, 15, 49), (0,), (1, 42, 50), (-1, 48, 51), (0,), (1, 51, 53), (1, 16, 53), (1, 33, 53), (-1, 36, 54), (2, 6, 54), (2, 14, 56), (0,), (1, 52, 58), (2, 13, 59), (0,), (-1, 57, 60), (1, 55, 60), (2, 10, 62), (0,), (1, 47, 63), (0,), (-1, 61, 65), (1, 64, 65), (2, 11, 67), (0,), (1, 66, 68), (2, 4, 69))


def _plain(rows, r):
    return rows[r][0][0] if len(rows[r]) == 1 and rows[r][0][0] < 8 else None


def _operands(block, temps, rows, which):
    x = {}

    def get(v):
        if v not in x:
            if v < 8:
                x[v] = block(v)
            else:
                a, b, c = temps[v - 8]
                x[v] = get(a) + get(b) if c > 0 else get(a) - get(b)
        return x[v]
    out = {}
    for r in which:
        acc = get(rows[r][0][0])
        for v, c in rows[r][1:]:
            acc = acc + get(v) if c > 0 else acc - get(v)
        out[r] = acc
    return out


def _mm424(product, store):
    val, r = [], 0
    for ins in _POST424:
        if ins[0] == 0:
            val.append(product(r))
            r += 1
        elif ins[0] == 2:
            store(ins[1] // 4, ins[1] % 4, val[ins[2]])
        else:
            val.append(val[ins[1]] + val[ins[2]] if ins[0] > 0 else val[ins[1]] - val[ins[2]])


def _recip(l):
    r = pl.reciprocal(l, approx=True)
    return r * (2.0 - l * r)


def _kernel(xat_hbm, ckv_hbm, wqa_hbm, wuk_hbm, wuv_hbm, woa_hbm,
            xbt_hbm, mem0_hbm, wqb_hbm, wkb_hbm, wvb_hbm, wob_hbm,
            out_hbm,
            out_v, xb_v, xpre_v, wb_v, wob_v, wos_v, mem_v, q_v, kv_v, sem):

    def w_copy(w_hbm, dst, slot, par, hp):
        return pltpu.make_async_copy(w_hbm.bitcast(u32).at[:, par * HP + hp, :], dst.at[par, hp], sem.at[slot])

    def w_start_shared(w_hbm, dst, widx, hps):
        for hp in hps:
            for par in range(2):
                w_copy(w_hbm, dst, SEM_WALL + widx, par, hp).start()

    def w_wait_shared(dst, widx):
        pltpu.make_async_copy(dst, dst, sem.at[SEM_WALL + widx]).wait()

    def w_combine(dst, hp):
        a = dst[0, hp]
        b = dst[1, hp]
        ev = (a & u32(0xFFFF)) | (b << 16)
        od = (a >> 16) | (b & u32(0xFFFF0000))
        return ev, od

    def w_pair(dst, hp):
        return jnp.concatenate(w_combine(dst, hp), axis=1)

    wb_hbm = (wqb_hbm, wkb_hbm, wvb_hbm)

    def pre_ref(j):
        n = NSEG * PRE
        return q_v.at[j // 4], (j % 4 // 2) * n, (j % 2) * D

    def lp_prep(lp_v):
        nr = NSEG * PRE // 4
        x = xpre_v[...].astype(f32)

        def store(r, p, w):
            lp_v.at[r][:, p * D:(p + 1) * D] = w
        _lhs233([x[0:nr], x[2 * nr:3 * nr]], [x[nr:2 * nr], x[3 * nr:]], store)

    def b_pre(lp_v):
        nr = NSEG * PRE // 4
        with _scope("b_pre"):
            for g in range(HP // PG):
                hps = range(g * PG, (g + 1) * PG)
                slabs = {}
                for hp in hps:
                    for t in range(3):
                        s0, s1 = wb_v[t, 0, hp], wb_v[t, 1, hp]
                        slabs[hp, t] = (s0, s1)
                        ev = (s0 & u32(0xFFFF)) | (s1 << 16)
                        od = (s0 >> 16) | (s1 & u32(0xFFFF0000))
                        a, b = (KM + HD) // 2, (KM + 2 * HD) // 2
                        d12 = _words(_lo(s0[a:b]) - _hi(s0[a:b]), _lo(s1[a:b]) - _hi(s1[a:b]))
                        d21 = _words(_hi(s0[b:]) - _lo(s0[b:]), _hi(s1[b:]) - _lo(s1[b:]))
                        wb_v[t, 0, hp] = jnp.concatenate([ev[:a], d12, ev[b:]], axis=0)
                        wb_v[t, 1, hp] = jnp.concatenate([od[:a], d21, od[a:b]], axis=0)
                rhs = [_rhs233([slabs[hp, t] for t in range(3)]) for hp in hps]

                def product(r):
                    ws = [x for f in rhs for x in f(r)]
                    res = []
                    for w in ws:
                        wa, wb, wc = _passes(w)
                        c = jnp.dot(_unpack(lp_v[r, :, 2 * D:3 * D]), _unpack(wc), preferred_element_type=f32)
                        a = jnp.dot(_unpack(lp_v[r, :, 0:D]), _unpack(wa), preferred_element_type=f32)
                        b = jnp.dot(_unpack(lp_v[r, :, D:2 * D]), _unpack(wb), preferred_element_type=f32)
                        res.append((a + c, b + c))
                    return [jnp.concatenate([x[y] for x in res], axis=1) for y in range(2)]
                for (i, t), blk in _mm233(product):
                    for y in range(2):
                        x0 = (2 * i + y) * nr
                        for n, hp in enumerate(hps):
                            two = [blk[y][:, (2 * n + e) * D:(2 * n + e + 1) * D] for e in range(2)]
                            if t == 0:
                                two = [z * QSCALE for z in two]
                            two = [z.reshape(nr // PRE, 1, PRE, D) for z in two]
                            two = jnp.concatenate(two, axis=1).reshape(2 * nr, D)
                            ref, r0, l0 = pre_ref(hp * 3 + t)
                            ref[r0 + x0:r0 + x0 + nr, l0:l0 + D] = _pack(two.astype(bf16))

    def phase_a(woa_v, xbt_v, wobt_v, lp_v):
        woa_cp = pltpu.make_async_copy(woa_hbm.bitcast(u32), woa_v, sem.at[SEM_WOA])
        xbt_cp = pltpu.make_async_copy(xbt_hbm, xbt_v, sem.at[SEM_XBT])
        mem_cp = pltpu.make_async_copy(mem0_hbm, mem_v.at[0:MEM, :], sem.at[SEM_MEM])
        wob_cp = pltpu.make_async_copy(wob_hbm.bitcast(u32), wobt_v, sem.at[SEM_WOB])

        def projections(ckv_v, xat_v, wuk_v, wuv_v, wqa_v, lq_v):
            UR = 2 * D
            NU = S // UR
            QR = UR // 4
            kh = DC // 2
            NG = H // 4

            batches = [(0, 1), (2, 4), (4, 8), (8, 12), (12, 16), (1, 2)]

            def batch_start(n):
                for hp in range(*batches[n]):
                    for w_hbm, dst in ((wuk_hbm, wuk_v), (wuv_hbm, wuv_v)):
                        for par in range(2):
                            w_copy(w_hbm, dst, SEM_W + n, par, hp).start()

            def batch_wait(npairs, slot):
                part = wuk_v.at[:, 0:2 * npairs]
                pltpu.make_async_copy(part, part, sem.at[SEM_W + slot]).wait()

            pieces = [(0, 1), (1, 2), (2, 4), (4, 6), (6, 8)]

            def ckv_cp(j):
                rows = slice(pieces[j][0] * UR, pieces[j][1] * UR)
                return pltpu.make_async_copy(ckv_hbm.at[rows, :], ckv_v.at[rows, :], sem.at[SEM_CKV + j])
            xat_cp = pltpu.make_async_copy(xat_hbm, xat_v, sem.at[SEM_XAT])

            with _scope("a_issue0"):
                ckv_cp(0).start()
                batch_start(0)
                ckv_cp(1).start()
                batch_start(5)
                for j in range(2, 5):
                    ckv_cp(j).start()
                for n in range(1, 5):
                    batch_start(n)

            slot_of = {}
            for r in range(26):
                if _plain(_A424_ROWS, r) is None:
                    slot_of[r] = len(slot_of)

            def la_ref(n):
                return q_v.at[3 + n // 4], (n % 4) * (S // 8)

            def t_ref(n):
                return q_v.at[9 + n // 8], (n % 8) * (kh // 2)

            def t_get(n):
                ref, r0 = t_ref(n)
                return ref[r0:r0 + kh // 2, :]

            def lhs_prep(u):
                for c0 in range(0, QR, CL):
                    def block(v):
                        r0 = u * UR + v // 2 * QR + c0
                        return ckv_v[r0:r0 + CL, v % 2 * kh:(v % 2 + 1) * kh].astype(f32)
                    for r, o in _operands(block, _A424_TEMPS, _A424_ROWS, slot_of).items():
                        ref, r0 = la_ref(slot_of[r])
                        p0 = r0 + (u * QR + c0) // 2
                        ref[p0:p0 + CL // 2, :] = _pack(o.astype(bf16))

            def lhs(r, u0, u1):
                v = _plain(_A424_ROWS, r)
                if v is None:
                    ref, r0 = la_ref(slot_of[r])
                    return _unpack(ref[r0 + u0 * QR // 2:r0 + u1 * QR // 2, :])
                i, k = v // 2, v % 2
                return jnp.concatenate([ckv_v[u * UR + i * QR:u * UR + (i + 1) * QR, k * kh:(k + 1) * kh]
                                        for u in range(u0, u1)], axis=0)

            def put_chunk(g, par, c, m, sub=range(26)):
                zero = None if m is None else (pltpu.bitcast(m[0:8, 0:D], u32) >> 31) >> 1
                n = kh // 2
                for e, w_v in enumerate((wuk_v, wuv_v)):
                    raw = {}

                    def words(p, v):
                        if (p, v // 2) not in raw:
                            w = w_v[p, 2 * g + v // 2 % 2, v // 4 * n + c * CR:v // 4 * n + (c + 1) * CR, :]
                            raw[p, v // 2] = w if zero is None else w | zero
                        return raw[p, v // 2]
                    sums = [r for r in sub if _plain(_B424_ROWS, r) is None]
                    ops = [_operands(lambda v: (_hi if v % 2 else _lo)(words(p, v)), _B424_TEMPS, _B424_ROWS, sums)
                           for p in range(2)]
                    for r in sub:
                        v = _plain(_B424_ROWS, r)
                        if v is None:
                            w = _words(ops[0][r], ops[1][r])
                        elif v % 2 == 0:
                            w = (words(0, v) & u32(0xFFFF)) | (words(1, v) << 16)
                        else:
                            w = (words(0, v) >> 16) | (words(1, v) & u32(0xFFFF0000))
                        ref, r0 = t_ref(26 * par + r)
                        ref[r0 + c * CR:r0 + (c + 1) * CR, e * D:(e + 1) * D] = w

            def project_kv(par, g, u0, u1, hooks=None, pre=None):
                def product(r):
                    if pre and r in pre:
                        pre[r]()
                    m = jnp.dot(lhs(r, u0, u1), _unpack(t_get(26 * par + r)), preferred_element_type=f32)
                    if hooks:
                        for c in hooks[1].get(r, ()):
                            put_chunk(hooks[0], 1 - par, c, m)
                    return m

                def store(i, j, blk):
                    for u in range(u0, u1):
                        p0 = (u * UR + i * QR) // 2
                        kv_v.at[4 * g + j][p0:p0 + QR // 2, :] = _pack(blk[(u - u0) * QR:(u - u0 + 1) * QR, :].astype(bf16))
                _mm424(product, store)

            def put_rhs(g, par, which):
                for c in range(kh // 2 // CR):
                    put_chunk(g, par, c, None, which)

            def hook_plan(npiece):
                nch = kh // 2 // CR
                plan = [{} for _ in range(npiece)]
                for c in range(nch):
                    sl = c * (npiece * 26 - 8) // nch
                    plan[sl // 26].setdefault(sl % 26, []).append(c)
                return plan

            def project_group(par, g, nxt):
                plan = hook_plan(NU // KU)
                for u in range(0, NU, KU):
                    project_kv(par, g, u, u + KU, (nxt, plan[u // KU]))

            def kv_first():
                ckv_cp(0).wait()
                lhs_prep(0)
                batch_wait(1, 0)
                put_rhs(0, 0, range(0, 7))
                ckv_cp(1).wait()
                lhs_prep(1)

                def rest():
                    batch_wait(1, 5)
                    for r in (7, 14, 20):
                        put_rhs(0, 0, range(r, {7: 14, 14: 20, 20: 26}[r]))
                project_kv(0, 0, 0, 2, pre={7: rest})
                ckv_cp(2).wait()
                lhs_prep(2)
                lhs_prep(3)
                ckv_cp(3).wait()
                lhs_prep(4)
                lhs_prep(5)
                project_kv(0, 0, 2, 4)
                ckv_cp(4).wait()
                batch_wait(2, 1)
                lhs_prep(6)
                lhs_prep(7)
                plan = hook_plan(2)
                for u in range(4, 8, 2):
                    project_kv(0, 0, u, u + 2, (1, plan[(u - 4) // 2]))

            def kv_body(j, c):
                @pl.when(j == 0)
                def _():
                    xat_cp.start()
                    w_start_shared(wqa_hbm, wqa_v, 0, range(HP))
                    xbt_cp.start()
                batch_wait(4, 2 + j)
                project_group(1, 2 * j + 1, 2 * j + 2)
                project_group(0, 2 * j + 2, 2 * j + 3)
                return c

            with _scope("a_kvproj"):
                kv_first()
                jax.lax.fori_loop(0, NG // 2 - 1, kv_body, 0)

            woa_cp.start()
            wob_cp.start()
            mem_cp.start()
            w_start_shared(wqb_hbm, wb_v.at[0], 1, range(HP))
            w_start_shared(wkb_hbm, wb_v.at[1], 2, range(HP // 2))

            QB = 4 * D
            plain = {(0, 0): 15, (0, 1): 1, (0, 2): 9, (1, 0): 4, (1, 1): 16, (1, 2): 8}

            def xa_prep(b):
                x = []
                for t in range(4 * b, 4 * b + 4):
                    xt = xat_v[:, t * D:(t + 1) * D]
                    x.append(jnp.concatenate([xt, xt[DM - HD:]], axis=0).astype(f32).T)

                def store(r, p, w):
                    lq_v.at[r][b * HD:(b + 1) * HD, p * D:(p + 1) * D] = w
                _lhs233([x[0], x[2]], [x[1], x[3]], store, extra=(((0, 0, 1),), ((1, 1, 1),)))

            def q_store(blk, hp, x0):
                q_v.at[hp][x0 // 2:(x0 + blk.shape[0]) // 2, :] = _pack((blk * QSCALE).astype(bf16))

            def q_rhs(hp):
                f = _rhs233([(wqa_v[0, hp + n], wqa_v[1, hp + n]) for n in range(3)])
                return [_passes(jnp.concatenate(f(r), axis=1)) for r in range(15)]

            def project_q(t, hp, b):
                nr = D // QS
                for s in range(QS):
                    rows = slice(b * HD + s * nr // 2, b * HD + (s + 1) * nr // 2)

                    def product(r):
                        wa, wb, wc = t[r]
                        c = jnp.dot(_unpack(lq_v[r, rows, 2 * D:3 * D]), _unpack(wc), preferred_element_type=f32)
                        a = jnp.dot(_unpack(lq_v[r, rows, 0 * D:1 * D]), _unpack(wa), preferred_element_type=f32)
                        b = jnp.dot(_unpack(lq_v[r, rows, 1 * D:2 * D]), _unpack(wb), preferred_element_type=f32)
                        return [a + c, b + c]
                    for (i, j), blk in _mm233(product):
                        for y in range(2):
                            q_store(blk[y], hp + j, b * QB + (2 * i + y) * D + s * nr)

            def project_q_last(hp):
                s0, s1 = wqa_v[0, hp], wqa_v[1, hp]
                w = jnp.concatenate([(s0 & u32(0xFFFF)) | (s1 << 16), (s0 >> 16) | (s1 & u32(0xFFFF0000))], axis=1)
                per = [_passes(jnp.concatenate([w[a:a + 64], w[c:c + 32]] if k == 1 else [w[a:a + 96]], axis=0))
                       for k, (a, _, c) in enumerate(_PIECES)]
                wp = [_unpack(jnp.concatenate([per[k][p] for k in range(3)], axis=0)) for p in range(3)]
                for b in range(S // QB):
                    rows = slice(b * HD, (b + 1) * HD)
                    for i in range(2):
                        a, bb, c = [jnp.dot(_unpack(jnp.concatenate([lq_v[plain[i, k], rows, p * D:(p + 1) * D] for k in range(3)], axis=1)),
                                            wp[p], preferred_element_type=f32) for p in range(3)]
                        q_store(a + c, hp, b * QB + 2 * i * D)
                        q_store(bb + c, hp, b * QB + (2 * i + 1) * D)

            def xb_prep(t):
                t0 = pl.multiple_of(t * D, D)
                xt = xbt_v[:, pl.ds(t0, D)]
                xb = jnp.concatenate([xt, xt[DM - HD:]], axis=0).T
                xb_v[pl.ds(t0, D), :] = xb
                for sg in range(D // SEG):
                    p0 = pl.multiple_of((t * (D // SEG) + sg) * PRE, PRE)
                    xpre_v[pl.ds(p0, PRE), :] = xb[sg * SEG:sg * SEG + PRE, :]

            with _scope("a_qproj"):
                xat_cp.wait()
                xbt_cp.wait()
                w_wait_shared(wqa_v, 0)
                t = q_rhs(0)
                for b in range(S // QB):
                    xa_prep(b)
                    for u in range(0, NU, KU):
                        if u // 2 == b:
                            project_kv(1, NG - 1, u, u + KU)
                    project_q(t, 0, b)
                XG = 4

                def q_body(j, c):
                    hp = 3 * j
                    for n in range(XG):
                        xb_prep((j - 1) * XG + n)
                    t = q_rhs(hp)
                    for b in range(S // QB):
                        project_q(t, hp, b)
                    return c
                jax.lax.fori_loop(1, 5, q_body, 0)
                lp_prep(lp_v)
                project_q_last(HP - 1)

        pl.run_scoped(
            projections,
            pltpu.VMEM((S, DC), bf16),
            pltpu.VMEM((DM, S), bf16),
            pltpu.VMEM((2, HP, DC // 2, D), u32),
            pltpu.VMEM((2, HP, DC // 2, D), u32),
            pltpu.VMEM((2, HP, DM // 2, D), u32),
            pltpu.VMEM((17, S // 8, 3 * D), u32),
        )

        def attention(c_v, s_v):
            row = jax.lax.broadcasted_iota(jnp.int32, (TQ, TQ), 0)
            col = jax.lax.broadcasted_iota(jnp.int32, (TQ, TQ), 1)
            tri = col <= row
            nb = S // TQ
            hq = TQ // 2
            npiece = 2
            pw = S // npiece

            def q_rows(h, r0, r1):
                return q_v[h[0], r0:r1, h[1] * D:(h[1] + 1) * D]

            def head(h):
                return 2 * h[0] + h[1]

            def qk_piece(h, j):
                q = _unpack(q_rows(h, (nb - 1) * hq, nb * hq))
                k = _unpack(kv_v[head(h), j * pw // 2:(j + 1) * pw // 2, 0:D])
                s_v[:, j * pw:(j + 1) * pw] = jax.lax.dot_general(q, k, NT, preferred_element_type=f32)

            def qk(h, i, j0=0, j1=None):
                j1 = i + 1 if j1 is None else j1
                q = _unpack(q_rows(h, i * hq, (i + 1) * hq))
                k = _unpack(kv_v[head(h), j0 * hq:j1 * hq, 0:D])
                return jax.lax.dot_general(q, k, NT, preferred_element_type=f32)

            def pv_shared(p, hd, i):
                low = jax.lax.broadcasted_iota(jnp.int32, (1, TQ), 1) < HD
                qr = TQ // 4

                def mm(x, w):
                    return jnp.dot(x.astype(bf16), _unpack(w), preferred_element_type=f32)
                pa, pd = p[:, (i - 1) * TQ:i * TQ], p[:, i * TQ:]
                y1a, y2a, y1d, y2d = pa[0:qr], pa[qr:2 * qr], pd[0:qr], pd[qr:2 * qr]
                va = kv_v[hd, (i - 1) * hq:i * hq, D:2 * D]
                vd = kv_v[hd, i * hq:(i + 1) * hq, D:2 * D]
                la = jnp.where(low, y1a, y1a - y2a)
                lb = jnp.where(low, y2a, pltpu.roll(y2d - y1d, HD, 1))
                lc = jnp.where(low, y1d, y2a)
                o = None
                if i > 1:
                    o = mm(p[:, :(i - 1) * TQ], kv_v[hd, 0:(i - 1) * hq, D:2 * D])
                o2 = mm(jnp.concatenate([la, pa[2 * qr:]], axis=0), va)
                o3 = mm(pd[2 * qr:], vd)
                ob = mm(lb, jnp.concatenate([va[0:qr], vd[0:qr]], axis=0))
                oc = mm(lc, jnp.concatenate([vd[0:qr], va[qr:]], axis=0))
                r = jnp.concatenate([o2[0:qr] + oc, ob + oc, o2[qr:] + o3], axis=0)
                return r if o is None else o + r

            def anchor_plan():
                ops = []
                for e in range(UH):
                    for i in range(nb - 1, -1, -1):
                        if i > 0:
                            ops.append(("qk", e, i - 1, 32 * i))
                        if i < npiece:
                            ops.append(("piece", e, i, 32 * nb // npiece))
                        ops.append(("pv", e, i, 32 * (i + 1)))
                t, start, end = 0, [], []
                for op in ops:
                    start.append(t)
                    t += op[3]
                    end.append(t)
                plan = {}
                for a, op in enumerate(ops):
                    if op[0] != "pv" or op[2] < ANCHOR_MIN:
                        continue
                    for b in range(a + 1, len(ops)):
                        if ops[b][0] == "qk" and start[b] >= end[a] + ANCHOR_LAG:
                            plan.setdefault((ops[b][1], ops[b][2]), []).append((op[1], op[2]))
                            break
                return plan

            def heads(j, c):
                @pl.when(j == 0)
                def _():
                    w_start_shared(wkb_hbm, wb_v.at[1], 2, range(HP // 2, HP))
                    w_start_shared(wvb_hbm, wb_v.at[2], 3, range(HP))

                plan = anchor_plan()

                def gated_qk(e, i):
                    h = (j * (UH // 2) + e // 2, e % 2)
                    if (e, i) not in plan:
                        return qk(h, i)
                    w = None
                    for ea, ia in plan[e, i]:
                        u = c_v[j * (UH // 2) + ea // 2, ia * hq:(ia + 1) * hq, (ea % 2) * D:(ea % 2 + 1) * D]
                        for r in range(0, hq, 8):
                            w = u[r:r + 8] if w is None else w | u[r:r + 8]
                    zero = (w >> 31) >> 1
                    q = q_rows(h, i * hq, (i + 1) * hq)
                    q = _unpack(jnp.concatenate([q[0:8] | zero, q[8:]], axis=0))
                    k = _unpack(kv_v[head(h), 0:(i + 1) * hq, 0:D])
                    return jax.lax.dot_general(q, k, NT, preferred_element_type=f32)

                s_next = s_v[...]
                for e in range(UH):
                    h = (j * (UH // 2) + e // 2, e % 2)
                    if e == UH - 1:
                        hn = (jnp.minimum(h[0] + 1, HP - 1), 0)
                    else:
                        hn = (j * (UH // 2) + (e + 1) // 2, (e + 1) % 2)
                    pieces = []
                    for i in range(nb - 1, -1, -1):
                        s = s_next
                        if i > 0:
                            s_next = gated_qk(e, i - 1)
                        if i < npiece:
                            if e == UH - 1:
                                qk_piece(hn, npiece - 1 - i)
                            else:
                                jj = npiece - 1 - i
                                pieces.append(qk(hn, nb - 1, jj * nb // npiece, (jj + 1) * nb // npiece))
                        sd = jnp.where(tri, s[:, i * TQ:], NEG)
                        s = jnp.concatenate([s[:, :i * TQ], sd], axis=1) if i > 0 else sd
                        m = jnp.max(s, axis=1, keepdims=True)
                        p = jnp.exp2(s - m)
                        l = jnp.sum(p, axis=1, keepdims=True)
                        if i < PVT:
                            v = _unpack(kv_v[head(h), 0:(i + 1) * hq, D:2 * D])
                            o = jnp.dot(p.astype(bf16), v, preferred_element_type=f32)
                        else:
                            o = pv_shared(p, head(h), i)
                        c_v.at[h[0]][i * hq:(i + 1) * hq, h[1] * D:(h[1] + 1) * D] = _pack((o * _recip(l)).astype(bf16))
                    if e < UH - 1:
                        s_next = jnp.concatenate(pieces, axis=1)
                return c
            with _scope("a_attn"):
                for j in range(npiece):
                    qk_piece((0, 0), j)
                jax.lax.fori_loop(0, H // UH, heads, 0)

            woa_cp.wait()
            wob_cp.wait()
            mem_cp.wait()
            for t in range(3):
                w_wait_shared(wb_v.at[t], 1 + t)
            mh = DM // 4

            def wo_prep(hh):
                a11, a21 = woa_v[hh, 0:mh, :], woa_v[hh, mh:2 * mh, :]
                a12, a22 = woa_v[hh + HP, 0:mh, :], woa_v[hh + HP, mh:2 * mh, :]
                for i, w in enumerate(_sum_words(_strassen_lhs, a11, a12, a21, a22, (2, 3), (a11, a22))):
                    if i not in (2, 3):
                        kv_v[hh, i * mh:(i + 1) * mh, 0:D] = w

            def wob_prep(hp):
                w1, w2 = _unpack(wobt_v[2 * hp]), _unpack(wobt_v[2 * hp + 1])
                a, b = KM + HD, KM + 2 * HD
                d12 = (w1[a:b].astype(f32) - w2[a:b].astype(f32)).astype(bf16)
                d21 = (w2[b:].astype(f32) - w1[b:].astype(f32)).astype(bf16)
                rows = slice(hp * HD, (hp + 1) * HD)
                wob_v[0, rows, :] = _pack(jnp.concatenate([w1[:a], d12], axis=0).T)
                wob_v[1, rows, :] = _pack(jnp.concatenate([w2[:a], d21], axis=0).T)
                wos_v[rows, :] = _pack(jnp.concatenate([w1[b:], w2[a:b]], axis=0).T)

            def oproj(tp):
                w0 = tp * D
                per = []
                for hh in range(HP):
                    def ctx(h, r0):
                        return c_v[h // 2, r0:r0 + D // 2, (h % 2) * D:(h % 2 + 1) * D]
                    b11, b21 = ctx(hh, w0), ctx(hh + HP, w0)
                    b12, b22 = ctx(hh, w0 + D // 2), ctx(hh + HP, w0 + D // 2)
                    per.append(_sum_words(_strassen_rhs, b11, b12, b21, b22, (1, 4), (b11, b22)))

                def lhs(i):
                    if i == 2:
                        return _unpack(jnp.concatenate([woa_v[hh, 0:mh, :] for hh in range(HP)], axis=1))
                    if i == 3:
                        return _unpack(jnp.concatenate([woa_v[hh + HP, mh:2 * mh, :] for hh in range(HP)], axis=1))
                    return _unpack(jnp.concatenate([kv_v[hh, i * mh:(i + 1) * mh, 0:D] for hh in range(HP)], axis=1))

                def rhs(i):
                    return _unpack(jnp.concatenate([per[hh][i] for hh in range(HP)], axis=1))
                c11, c12, c21, c22 = _strassen(lhs, rhs, NT)
                t0 = 2 * tp * D
                out_v[t0:t0 + D, 0:DM] = jnp.concatenate([c11, c21], axis=0).T.astype(bf16)
                out_v[t0 + D:t0 + 2 * D, 0:DM] = jnp.concatenate([c12, c22], axis=0).T.astype(bf16)

            b_pre(lp_v)
            with _scope("a_oproj"):
                for hh in range(HP):
                    wo_prep(hh)
                for tp in range(S // D // 2):
                    oproj(tp)
                    for hp in range(2 * tp, 2 * tp + 2):
                        wob_prep(hp)

        pl.run_scoped(
            attention,
            pltpu.VMEM((HP, S // 2, 2 * D), u32),
            pltpu.VMEM((TQ, S), f32),
        )

    pl.run_scoped(
        phase_a,
        pltpu.VMEM((H, DM // 2, D), u32),
        pltpu.VMEM((DM, S), bf16),
        pltpu.VMEM((H, DM // 2, D), u32),
        pltpu.VMEM((15, NSEG * PRE // 8, 3 * D), u32),
    )

    def out_copy(j):
        rows = pl.ds(pl.multiple_of(j * (OUTER * SEG), OUTER * SEG), OUTER * SEG)
        return pltpu.make_async_copy(out_v.at[rows, :], out_hbm.at[rows, :], sem.at[SEM_OUT + j])

    def phase_b(post_v):
        GP = HG // 2
        GC = GP * 3 * D
        KA = KM + 2 * HD
        lane = jax.lax.broadcasted_iota(jnp.int32, (1, GC), 1)
        colscale = jnp.where(lane % (3 * D) < D, QSCALE, 1.0).astype(f32)
        low = jax.lax.broadcasted_iota(jnp.int32, (1, D), 1) < HD

        def swap(x):
            return pltpu.roll(x, HD, 1)

        def wgroup(g):
            cols = [(hp, t) for hp in range(g * GP, (g + 1) * GP) for t in range(3)]
            own = [_unpack(jnp.concatenate([wb_v[t, e, hp, 0:KA // 2, :] for hp, t in cols], axis=1)) for e in range(2)]
            both = jnp.concatenate([jnp.concatenate([wb_v[t, e, hp, KA // 2:, :] for hp, t in cols], axis=1)
                                    for e in range(2)], axis=0)
            return own[0], own[1], _unpack(both)

        def out_project(even, odd, both, p0, p1):
            rows = slice(p0 * HD, p1 * HD)
            return [jnp.dot(even, _unpack(wob_v[0, rows, :]), preferred_element_type=f32),
                    jnp.dot(odd, _unpack(wob_v[1, rows, :]), preferred_element_type=f32),
                    jnp.dot(both, _unpack(wos_v[rows, :]), preferred_element_type=f32)]

        def out_add(acc, part):
            e, o, b = part
            new = [e[:, :KM] + o[:, :KM], e[:, KM:], o[:, KM:], b]
            return new if acc is None else [x + y for x, y in zip(acc, new)]

        def out_finish(acc):
            main, e, o, b = acc
            mid = e + jnp.where(low, o, b)
            last = jnp.where(low, swap(o) + b, o + swap(b))
            return jnp.concatenate([main, mid, last], axis=1)

        ri = jax.lax.broadcasted_iota(jnp.int32, (2 * L, 2 * L), 0)
        ci = jax.lax.broadcasted_iota(jnp.int32, (2 * L, 2 * L), 1)

        def second(i):
            return jnp.where(i < 2 * SEG, i // SEG, (i - 2 * SEG) // PRE)

        def pos(i):
            j = i % SEG
            return jnp.where(i < 2 * SEG, jnp.where(j < T, j + (MEM + PRE), j - T), MEM + i % PRE)
        same = second(ri) == second(ci)
        mask = same & ((pos(ri) < MEM) | (pos(ri) >= pos(ci)))
        fill = jnp.where(same, NEG, -jnp.inf).astype(f32)

        def step(s, slot, mem):
            xt = xb_v[pl.ds(pl.multiple_of(SEG * s + PRE, 8), T), :]
            l1 = jnp.concatenate([xt.astype(f32), mem], axis=0)
            mid, last = l1[:, KM:KA], l1[:, KA:]
            l_even = l1[:, :KA].astype(bf16)
            l_odd = jnp.concatenate([l1[:, :KM], jnp.where(low, mid, last)], axis=1).astype(bf16)
            l_both = jnp.where(low, last, mid).astype(bf16)
            p0 = pl.multiple_of(PRE * s, 8)
            proj = []
            for g in range(G):
                w_even, w_odd, w_both = wgroup(g)
                both = jnp.dot(l_both, w_both, preferred_element_type=f32)
                even = jnp.dot(l_even, w_even, preferred_element_type=f32)
                odd = jnp.dot(l_odd, w_odd, preferred_element_type=f32)
                proj.append([(x + both) * colscale for x in (even, odd)])

            def rows(hp, t):
                g, c0 = hp // GP, (hp % GP) * 3 * D + t * D
                ref, r0, l0 = pre_ref(hp * 3 + t)
                return jnp.concatenate([proj[g][0][:, c0:c0 + D], proj[g][1][:, c0:c0 + D],
                                        _unpack(ref[pl.ds(r0 + p0, PRE), l0:l0 + D]).astype(f32)], axis=0).astype(bf16)

            scores = [jax.lax.dot_general(rows(hp, 0), rows(hp, 1), NT, preferred_element_type=f32)
                      for hp in range(HP)]
            ctx = {}

            def attend(g):
                for hp in range(g * HG // 2, (g + 1) * HG // 2):
                    sc = jnp.where(mask, scores[hp], fill)
                    m = jnp.max(sc, axis=1, keepdims=True)
                    p = jnp.exp2(sc - m)
                    l = jnp.sum(p, axis=1, keepdims=True)
                    o = jnp.dot(p.astype(bf16), rows(hp, 2), preferred_element_type=f32) * _recip(l)
                    ctx[hp] = [o[0:SEG, :], o[SEG:2 * SEG, :], o[0:SEG, :] + o[SEG:2 * SEG, :]]
                    for e in range(2):
                        post_v[e, slot * PRE:(slot + 1) * PRE, hp * D:(hp + 1) * D] = o[2 * SEG + e * PRE:2 * SEG + (e + 1) * PRE, :]

            parts = []

            def oproj(g):
                lhs = [jnp.concatenate([ctx[hp][e] for hp in range(g * GP, (g + 1) * GP)], axis=1).astype(bf16)
                       for e in range(3)]
                parts.append(out_project(*lhs, g * GP, (g + 1) * GP))

            for t in range(G + 2):
                if t < G:
                    attend(t)
                if t >= 2:
                    oproj(t - 2)
            acc = None
            for a in parts:
                acc = out_add(acc, a)
            accb = out_finish(acc).astype(bf16)
            out_v[pl.ds(pl.multiple_of(SEG * s + PRE, 8), T), DM:2 * DM] = accb[0:T, 0:DM]
            return accb[T:, :].astype(f32), ctx[HP - 1][1]

        PP = HP // OUTER

        def deferred_rows():
            even, odd = post_v[0], post_v[1]
            return even, odd, even + odd

        def finish(j, acc):
            r = out_finish(acc).astype(bf16)
            for sg in range(OUTER):
                r0 = pl.multiple_of((j * OUTER + sg) * SEG, SEG)
                out_v[pl.ds(r0, PRE), DM:2 * DM] = r[sg * PRE:(sg + 1) * PRE, 0:DM]

        def after(x, late):
            u = pltpu.bitcast(late[0:8, :], u32)
            zero = (u >> 31) & (~u >> 31)
            top = pltpu.bitcast(x[0:8], u32) | jnp.concatenate([zero] * (x.shape[1] // D), axis=1)
            return jnp.concatenate([pltpu.bitcast(top, f32), x[8:]], axis=0).astype(bf16)

        def outer(j, mem):
            prev = deferred_rows()

            def partial(i, late):
                x = [after(p[:, i * PP * D:(i + 1) * PP * D], late) for p in prev]
                return out_project(*x, i * PP, (i + 1) * PP)
            acc = None
            for i in range(OUTER):
                mem, late = step(j * OUTER + i, i, mem)
                acc = out_add(acc, partial(i, late))
            finish(jnp.maximum(j - 1, 0), acc)

            @pl.when(j > 0)
            def _():
                out_copy(j - 1).start()
            return mem
        with _scope("b_loop"):
            post_v[...] = jnp.zeros(post_v.shape, f32)
            mem0 = mem_v[0:MEM, :].astype(f32)
            jax.lax.fori_loop(0, NOUTER, outer, jnp.concatenate([mem0, mem0[:, DM - HD:]], axis=1))
            finish(NOUTER - 1, out_add(None, out_project(*[x.astype(bf16) for x in deferred_rows()], 0, HP)))
            out_copy(NOUTER - 1).start()
        with _scope("b_outwait"):
            for j in range(NOUTER):
                out_copy(j).wait()

    pl.run_scoped(
        phase_b,
        pltpu.VMEM((2, OUTER * PRE, HP * D), f32),
    )


@jax.jit
def pallas_concat_heads__compressed_kv_cla__memory_aug_recurrent_mem_tr__prompt_kernel(
    A_x: jax.Array,
    A_c_kv: jax.Array,
    A_w_q: jax.Array,
    A_w_uk: jax.Array,
    A_w_uv: jax.Array,
    A_w_o: jax.Array,
    B_x: jax.Array,
    B_mem0: jax.Array,
    B_Wq: jax.Array,
    B_Wk: jax.Array,
    B_Wv: jax.Array,
    B_Wo: jax.Array,
    B_seg_len=SEG,
):
    def t2(x):
        return jnp.transpose(x, (0, 2, 1)).reshape(DM, S)

    def w3(w):
        return w.reshape(w.shape[0] // 2, 2 * H, D)

    def wo3(w):
        return jnp.transpose(w, (0, 2, 1))

    any_spec = pl.BlockSpec(memory_space=pl.ANY)
    out = pl.pallas_call(
        _kernel,
        out_shape=jax.ShapeDtypeStruct((S, 2 * DM), bf16),
        in_specs=[any_spec] * 12,
        out_specs=any_spec,
        scratch_shapes=[
            pltpu.VMEM((S, 2 * DM), bf16),
            pltpu.VMEM((S, DMP), bf16),
            pltpu.VMEM((NSEG * PRE, DMP), bf16),
            pltpu.VMEM((3, 2, HP, DM // 2, D), u32),
            pltpu.VMEM((2, HP * D // 2, KM + 2 * HD), u32),
            pltpu.VMEM((HP * D // 2, D), u32),
            pltpu.VMEM((8 * MEM, DM), bf16),
            pltpu.VMEM((HP, S // 2, 2 * D), u32),
            pltpu.VMEM((H, S // 2, 2 * D), u32),
            pltpu.SemaphoreType.DMA((NSEM,)),
        ],
        compiler_params=pltpu.CompilerParams(vmem_limit_bytes=126 * 1024 * 1024),
    )(t2(A_x), A_c_kv.reshape(S, DC), w3(A_w_q), w3(A_w_uk), w3(A_w_uv), wo3(A_w_o),
      t2(B_x), B_mem0.reshape(MEM, DM), w3(B_Wq), w3(B_Wk), w3(B_Wv), wo3(B_Wo))
    return out.reshape(1, S, 2 * DM)
```

```python
import contextlib

import jax
import jax.numpy as jnp
import jax.experimental.pallas as pl
import jax.experimental.pallas.tpu as pltpu

S = 2048
DM = 576
DC = 512
H = 32
D = 128
MEM = 8
SEG = 32
L = MEM + SEG
NSEG = S // SEG
HP = H // 2
HD = D // 2
KM = DM - 3 * HD
DMP = DM + HD

LOG2E = 1.4426950408889634
QSCALE = D ** -0.5 * LOG2E
NEG = -1.0e9 * LOG2E

TQ = 128
UH = 4
ANCHOR_LAG = 2000
ANCHOR_MIN = 6
RB = 512
HG = 4
G = H // HG
PRE = 8
T = SEG - PRE
OUTER = 4
NOUTER = NSEG // OUTER

bf16 = jnp.bfloat16
f32 = jnp.float32
u32 = jnp.uint32
NT = (((1,), (1,)), ((), ()))

SEM_CKV = 0
SEM_XAT = 5
SEM_XBT = 6
SEM_MEM = 7
SEM_WOA = 8
SEM_WOB = 9
SEM_OUT = 10
SEM_WALL = SEM_OUT + NOUTER
SEM_W = SEM_WALL + 4
NSEM = SEM_W + 6

_PROFILE = False
I0 = 0
I1 = 30
KS = 4
KU = 2
CL = 16
CR = 8
PVT = 5
PG = 1
QS = 2

def _scope(name):
    return jax.named_scope(name) if _PROFILE else contextlib.nullcontext()


def _unpack(w32):
    return pltpu.bitcast(w32, bf16)


def _pack(x):
    return pltpu.bitcast(x, u32)


def _lo(w):
    return pltpu.bitcast(w << 16, f32)


def _hi(w):
    return pltpu.bitcast(w & u32(0xFFFF0000), f32)


def _words(even, odd):
    return pltpu.bitcast(pltpu.pack_elementwise([even, odd], packed_dtype=bf16), u32)


def _strassen_lhs(a11, a12, a21, a22):
    return [a11 + a22, a21 + a22, a11, a22, a11 + a12, a21 - a11, a12 - a22]


def _strassen_rhs(b11, b12, b21, b22):
    return [b11 + b22, b11, b12 - b22, b21 - b11, b22, b11 + b12, b21 + b22]


def _sum_words(combine, x11, x12, x21, x22, raw_idx, raw):
    lo = combine(_lo(x11), _lo(x12), _lo(x21), _lo(x22))
    hi = combine(_hi(x11), _hi(x12), _hi(x21), _hi(x22))
    words = [pltpu.bitcast(pltpu.pack_elementwise([a, b], packed_dtype=bf16), u32) for a, b in zip(lo, hi)]
    for i, r in zip(raw_idx, raw):
        words[i] = r
    return words


def _strassen(lhs, rhs, dims, done, order=0):
    def m(i):
        acc = None
        for s in range(KS):
            part = jax.lax.dot_general(lhs(i - 1, s), rhs(i - 1, s), dims, preferred_element_type=f32)
            acc = part if acc is None else acc + part
            if i != 7 or s < KS - 1:
                yield
        return acc
    if order == 0:
        m1 = yield from m(1)
        m2 = yield from m(2)
        c22 = m1 - m2
        m4 = yield from m(4)
        c11 = m1 + m4
        c21 = m2 + m4
        c22 = c22 + (yield from m(6))
        m3 = yield from m(3)
        c22 = c22 + m3
        m5 = yield from m(5)
        c11 = c11 - m5
        c12 = m3 + m5
        c11 = c11 + (yield from m(7))
        done(c11, c12, c21, c22)
        yield
        return
    m3 = yield from m(3)
    m4 = yield from m(4)
    m5 = yield from m(5)
    c12 = m3 + m5
    c11 = m4 - m5
    m2 = yield from m(2)
    c21 = m4 + m2
    c22 = m3 - m2
    m1 = yield from m(1)
    c11 = c11 + m1
    c22 = c22 + m1
    c22 = c22 + (yield from m(6))
    c11 = c11 + (yield from m(7))
    done(c11, c12, c21, c22)
    yield


def _rhs_words(s0, s1, z0, z1):
    per = [_strassen_rhs(_lo(s), _hi(s), _lo(z), _hi(z)) for s, z in ((s0, z0), (s1, z1))]
    words = [pltpu.bitcast(pltpu.pack_elementwise([per[0][i], per[1][i]], packed_dtype=bf16), u32)
             for i in range(7)]
    words[1] = (s0 & u32(0xFFFF)) | (s1 << 16)
    words[4] = (z0 >> 16) | (z1 & u32(0xFFFF0000))
    return words


_L233 = (((0, 1, 1), (1, 0, 1)), ((0, 1, 1),), ((0, 0, 1), (1, 0, -1)), ((0, 1, 1), (1, 1, -1)), ((1, 0, 1),),
         ((0, 0, -1), (0, 1, -1)), ((1, 0, 1), (1, 1, 1)), ((0, 0, 1), (0, 2, 1), (1, 0, -1)), ((1, 2, 1),),
         ((0, 2, 1),), ((1, 0, 1), (1, 2, 1), (0, 0, -1), (0, 2, -1)), ((0, 0, -1), (0, 2, -1)),
         ((1, 1, 1), (1, 2, 1), (0, 1, -1)), ((1, 1, -1), (1, 2, -1)),
         ((0, 1, 1), (0, 2, 1), (1, 1, -1), (1, 2, -1)))
_R233 = (((0, 1, 1), (1, 0, 1)), ((1, 1, 1), (1, 2, 1), (0, 1, -1)), ((0, 0, 1), (0, 1, 1), (2, 0, -1)),
         ((2, 1, 1), (1, 0, -1), (1, 1, -1)), ((0, 0, 1), (0, 2, 1), (1, 0, -1)), ((0, 1, 1),), ((1, 0, 1),),
         ((0, 2, 1), (2, 0, 1)), ((2, 0, 1), (2, 2, 1), (1, 2, -1)), ((2, 1, 1), (2, 2, 1), (0, 2, -1)),
         ((2, 0, 1),), ((0, 2, 1),), ((1, 2, 1), (2, 1, 1)), ((1, 2, 1),), ((2, 1, 1),))
_PIECES = ((0, 32, 64), (128, 160, 96), (192, 224, 256))


def _signed_sum(terms, get):
    acc = None
    for a, b, c in terms:
        x = get(a, b)
        if acc is None:
            acc = x if c > 0 else -x
        else:
            acc = acc + x if c > 0 else acc - x
    return acc


def _lhs233(y1, y2, store, extra=()):
    low = jax.lax.broadcasted_iota(jnp.int32, (1, D), 1) < HD
    base = {}
    for i in range(2):
        t1 = [y1[i][:, c * D:(c + 1) * D] for c in range(5)]
        t2 = [y2[i][:, c * D:(c + 1) * D] for c in range(5)]
        r1, r2 = pltpu.roll(t1[1], HD, 1), pltpu.roll(t2[1], HD, 1)
        for k in range(3):
            a1, a2 = t1[(0, 2, 3)[k]], t2[(0, 2, 3)[k]]
            lo1 = (t1[1], r1, t1[4])[k]
            hi1, hi2 = (r1, t1[1], t1[4])[k], (r2, t2[1], t2[4])[k]
            base[i, k] = (jnp.where(low, a1, a1 - a2), jnp.where(low, a2, hi2 - hi1), jnp.where(low, lo1, a2))
    for r, terms in enumerate(_L233 + extra):
        for p in range(3):
            store(r, p, _pack(_signed_sum(terms, lambda i, k: base[i, k][p]).astype(bf16)))


def _rhs233(slabs):
    def chunk(j, par, k):
        s = slabs[j][par]
        a, b, c = _PIECES[k]
        return s[a:a + 96] if k != 1 else jnp.concatenate([s[a:a + 64], s[c:c + 32]], axis=0)

    def words(r):
        terms = _R233[r]
        if len(terms) == 1:
            k, j, _ = terms[0]
            s0, s1 = chunk(j, 0, k), chunk(j, 1, k)
            return (s0 & u32(0xFFFF)) | (s1 << 16), (s0 >> 16) | (s1 & u32(0xFFFF0000))
        half = [[_signed_sum(terms, lambda k, j: f(chunk(j, par, k))) for par in range(2)] for f in (_lo, _hi)]
        return _words(*half[0]), _words(*half[1])
    return words


def _passes(w):
    return (w[0:64], jnp.concatenate([w[0:32], w[64:96]], axis=0), jnp.concatenate([w[64:96], w[32:64]], axis=0))


def _mm233(product):
    def add(a, b):
        return [x + y for x, y in zip(a, b)]

    def sub(a, b):
        return [x - y for x, y in zip(a, b)]
    p13 = product(13)
    s1 = add(product(12), p13)
    s2 = add(s1, product(14))
    p11 = product(11)
    yield (0, 2), sub(sub(product(9), s2), p11)
    s3 = add(product(7), p11)
    s4 = add(s3, product(10))
    yield (1, 2), sub(sub(product(8), s4), p13)
    p4 = product(4)
    p6 = product(6)
    yield (1, 0), add(add(p6, s4), p4)
    c11 = sub(s1, p6)
    p5 = product(5)
    p1 = product(1)
    yield (0, 1), sub(add(p1, s2), p5)
    c11 = add(c11, p1)
    p0 = product(0)
    yield (1, 1), add(add(product(3), c11), p0)
    yield (0, 0), add(add(add(add(product(2), s3), p4), p5), p0)


_A424_TEMPS = ((3, 7, -1), (5, 7, -1), (0, 6, -1), (2, 6, -1), (4, 9, -1))
_A424_ROWS = (((4, 1), (0, -1)), ((1, 1), (5, -1)), ((4, 1), (1, -1)), ((0, 1), (1, -1)), ((4, 1),), ((5, 1), (4, -1)), ((1, 1),), ((12, 1),), ((3, 1), (1, -1)), ((2, 1), (1, -1)), ((1, 1), (10, -1)), ((2, 1), (0, -1)), ((10, 1),), ((2, 1),), ((6, 1),), ((2, 1), (3, -1)), ((6, 1), (12, -1)), ((8, 1), (2, -1)), ((8, 1), (11, -1)), ((8, 1),), ((7, 1),), ((8, 1), (10, -1)), ((9, 1),), ((4, 1), (11, 1)), ((2, 1), (9, 1)), ((5, 1), (8, 1)))
_B424_TEMPS = ((0, 2, 1), (2, 3, -1), (5, 6, -1), (7, 9, -1), (4, 8, 1), (1, 10, 1))
_B424_ROWS = (((0, 1), (1, 1)), ((4, 1), (5, 1)), ((1, 1), (4, -1)), ((1, 1),), ((0, 1), (4, 1)), ((4, 1),), ((1, 1), (5, 1)), ((12, 1),), ((5, 1), (7, -1)), ((1, 1), (7, 1)), ((13, 1),), ((1, 1), (3, -1)), ((2, 1), (13, -1)), ((3, 1), (7, 1)), ((2, 1),), ((7, 1),), ((8, 1),), ((11, 1),), ((9, 1),), ((6, 1), (11, -1)), ((6, 1),), ((9, 1), (10, -1)), ((6, 1), (12, 1)), ((3, 1), (8, 1)), ((7, 1), (8, -1)), ((4, 1), (6, 1), (7, 1)))
_POST424 = ((0,), (0,), (0,), (-1, 2, 0), (-1, 2, 1), (0,), (-1, 3, 5), (0,), (1, 6, 7), (2, 0, 8), (0,), (1, 7, 9), (-1, 4, 9), (2, 8, 10), (0,), (1, 5, 12), (1, 11, 12), (2, 1, 13), (2, 9, 14), (0,), (-1, 15, 7), (1, 9, 15), (0,), (0,), (1, 18, 19), (-1, 5, 19), (1, 12, 20), (0,), (-1, 12, 23), (0,), (1, 21, 25), (-1, 22, 25), (0,), (1, 24, 28), (1, 27, 28), (0,), (1, 26, 31), (2, 3, 32), (0,), (1, 29, 33), (-1, 17, 33), (2, 2, 34), (0,), (-1, 22, 36), (-1, 31, 36), (2, 5, 37), (2, 7, 38), (0,), (1, 35, 39), (2, 12, 40), (0,), (1, 31, 41), (-1, 39, 42), (0,), (1, 36, 44), (-1, 33, 45), (1, 43, 46), (1, 30, 46), (-1, 46, 41), (2, 15, 49), (0,), (1, 42, 50), (-1, 48, 51), (0,), (1, 51, 53), (1, 16, 53), (1, 33, 53), (-1, 36, 54), (2, 6, 54), (2, 14, 56), (0,), (1, 52, 58), (2, 13, 59), (0,), (-1, 57, 60), (1, 55, 60), (2, 10, 62), (0,), (1, 47, 63), (0,), (-1, 61, 65), (1, 64, 65), (2, 11, 67), (0,), (1, 66, 68), (2, 4, 69))


def _plain(rows, r):
    return rows[r][0][0] if len(rows[r]) == 1 and rows[r][0][0] < 8 else None


def _operands(block, temps, rows, which):
    x = {}

    def get(v):
        if v not in x:
            if v < 8:
                x[v] = block(v)
            else:
                a, b, c = temps[v - 8]
                x[v] = get(a) + get(b) if c > 0 else get(a) - get(b)
        return x[v]
    out = {}
    for r in which:
        acc = get(rows[r][0][0])
        for v, c in rows[r][1:]:
            acc = acc + get(v) if c > 0 else acc - get(v)
        out[r] = acc
    return out


def _mm424(product, store):
    val, r = [], 0
    for ins in _POST424:
        if ins[0] == 0:
            val.append(product(r))
            r += 1
        elif ins[0] == 2:
            store(ins[1] // 4, ins[1] % 4, val[ins[2]])
        else:
            val.append(val[ins[1]] + val[ins[2]] if ins[0] > 0 else val[ins[1]] - val[ins[2]])


def _recip(l):
    r = pl.reciprocal(l, approx=True)
    return r * (2.0 - l * r)


def _kernel(xat_hbm, ckv_hbm, wqa_hbm, wuk_hbm, wuv_hbm, woa_hbm,
            xbt_hbm, mem0_hbm, wqb_hbm, wkb_hbm, wvb_hbm, wob_hbm,
            out_hbm,
            out_v, xb_v, xpre_v, wb_v, wob_v, wos_v, mem_v, q_v, kv_v, sem):

    def w_copy(w_hbm, dst, slot, par, hp):
        return pltpu.make_async_copy(w_hbm.bitcast(u32).at[:, par * HP + hp, :], dst.at[par, hp], sem.at[slot])

    def w_start_shared(w_hbm, dst, widx, hps):
        for hp in hps:
            for par in range(2):
                w_copy(w_hbm, dst, SEM_WALL + widx, par, hp).start()

    def w_wait_shared(dst, widx):
        pltpu.make_async_copy(dst, dst, sem.at[SEM_WALL + widx]).wait()

    def w_combine(dst, hp):
        a = dst[0, hp]
        b = dst[1, hp]
        ev = (a & u32(0xFFFF)) | (b << 16)
        od = (a >> 16) | (b & u32(0xFFFF0000))
        return ev, od

    def w_pair(dst, hp):
        return jnp.concatenate(w_combine(dst, hp), axis=1)

    wb_hbm = (wqb_hbm, wkb_hbm, wvb_hbm)

    def pre_ref(j):
        n = NSEG * PRE
        return q_v.at[j // 4], (j % 4 // 2) * n, (j % 2) * D

    def lp_prep(lp_v):
        nr = NSEG * PRE // 4
        x = xpre_v[...].astype(f32)

        def store(r, p, w):
            lp_v.at[r][:, p * D:(p + 1) * D] = w
        _lhs233([x[0:nr], x[2 * nr:3 * nr]], [x[nr:2 * nr], x[3 * nr:]], store)

    def b_pre(lp_v, tick):
        nr = NSEG * PRE // 4
        with _scope("b_pre"):
            for g in range(HP // PG):
                hps = range(g * PG, (g + 1) * PG)
                slabs = {}
                for hp in hps:
                    for t in range(3):
                        s0, s1 = wb_v[t, 0, hp], wb_v[t, 1, hp]
                        slabs[hp, t] = (s0, s1)
                        ev = (s0 & u32(0xFFFF)) | (s1 << 16)
                        od = (s0 >> 16) | (s1 & u32(0xFFFF0000))
                        a, b = (KM + HD) // 2, (KM + 2 * HD) // 2
                        d12 = _words(_lo(s0[a:b]) - _hi(s0[a:b]), _lo(s1[a:b]) - _hi(s1[a:b]))
                        d21 = _words(_hi(s0[b:]) - _lo(s0[b:]), _hi(s1[b:]) - _lo(s1[b:]))
                        wb_v[t, 0, hp] = jnp.concatenate([ev[:a], d12, ev[b:]], axis=0)
                        wb_v[t, 1, hp] = jnp.concatenate([od[:a], d21, od[a:b]], axis=0)
                rhs = [_rhs233([slabs[hp, t] for t in range(3)]) for hp in hps]

                def product(r):
                    ws = [x for f in rhs for x in f(r)]
                    res = []
                    for w in ws:
                        wa, wb, wc = _passes(w)
                        c = jnp.dot(_unpack(lp_v[r, :, 2 * D:3 * D]), _unpack(wc), preferred_element_type=f32)
                        a = jnp.dot(_unpack(lp_v[r, :, 0:D]), _unpack(wa), preferred_element_type=f32)
                        b = jnp.dot(_unpack(lp_v[r, :, D:2 * D]), _unpack(wb), preferred_element_type=f32)
                        res.append((a + c, b + c))
                    tick()
                    return [jnp.concatenate([x[y] for x in res], axis=1) for y in range(2)]
                for (i, t), blk in _mm233(product):
                    for y in range(2):
                        x0 = (2 * i + y) * nr
                        for n, hp in enumerate(hps):
                            two = [blk[y][:, (2 * n + e) * D:(2 * n + e + 1) * D] for e in range(2)]
                            if t == 0:
                                two = [z * QSCALE for z in two]
                            two = [z.reshape(nr // PRE, 1, PRE, D) for z in two]
                            two = jnp.concatenate(two, axis=1).reshape(2 * nr, D)
                            ref, r0, l0 = pre_ref(hp * 3 + t)
                            ref[r0 + x0:r0 + x0 + nr, l0:l0 + D] = _pack(two.astype(bf16))

    def phase_a(woa_v, xbt_v, wobt_v, lp_v):
        woa_cp = pltpu.make_async_copy(woa_hbm.bitcast(u32), woa_v, sem.at[SEM_WOA])
        xbt_cp = pltpu.make_async_copy(xbt_hbm, xbt_v, sem.at[SEM_XBT])
        mem_cp = pltpu.make_async_copy(mem0_hbm, mem_v.at[0:MEM, :], sem.at[SEM_MEM])
        wob_cp = pltpu.make_async_copy(wob_hbm.bitcast(u32), wobt_v, sem.at[SEM_WOB])

        def projections(ckv_v, xat_v, wuk_v, wuv_v, wqa_v, lq_v):
            UR = 2 * D
            NU = S // UR
            QR = UR // 4
            kh = DC // 2
            NG = H // 4

            batches = [(0, 1), (2, 4), (4, 8), (8, 12), (12, 16), (1, 2)]

            def batch_start(n):
                for hp in range(*batches[n]):
                    for w_hbm, dst in ((wuk_hbm, wuk_v), (wuv_hbm, wuv_v)):
                        for par in range(2):
                            w_copy(w_hbm, dst, SEM_W + n, par, hp).start()

            def batch_wait(npairs, slot):
                part = wuk_v.at[:, 0:2 * npairs]
                pltpu.make_async_copy(part, part, sem.at[SEM_W + slot]).wait()

            pieces = [(0, 1), (1, 2), (2, 4), (4, 6), (6, 8)]

            def ckv_cp(j):
                rows = slice(pieces[j][0] * UR, pieces[j][1] * UR)
                return pltpu.make_async_copy(ckv_hbm.at[rows, :], ckv_v.at[rows, :], sem.at[SEM_CKV + j])
            xat_cp = pltpu.make_async_copy(xat_hbm, xat_v, sem.at[SEM_XAT])

            with _scope("a_issue0"):
                ckv_cp(0).start()
                batch_start(0)
                ckv_cp(1).start()
                batch_start(5)
                for j in range(2, 5):
                    ckv_cp(j).start()
                for n in range(1, 5):
                    batch_start(n)

            slot_of = {}
            for r in range(26):
                if _plain(_A424_ROWS, r) is None:
                    slot_of[r] = len(slot_of)

            def la_ref(n):
                return q_v.at[3 + n // 4], (n % 4) * (S // 8)

            def t_ref(n):
                return q_v.at[9 + n // 8], (n % 8) * (kh // 2)

            def t_get(n):
                ref, r0 = t_ref(n)
                return ref[r0:r0 + kh // 2, :]

            def lhs_prep(u):
                for c0 in range(0, QR, CL):
                    def block(v):
                        r0 = u * UR + v // 2 * QR + c0
                        return ckv_v[r0:r0 + CL, v % 2 * kh:(v % 2 + 1) * kh].astype(f32)
                    for r, o in _operands(block, _A424_TEMPS, _A424_ROWS, slot_of).items():
                        ref, r0 = la_ref(slot_of[r])
                        p0 = r0 + (u * QR + c0) // 2
                        ref[p0:p0 + CL // 2, :] = _pack(o.astype(bf16))

            def lhs(r, u0, u1):
                v = _plain(_A424_ROWS, r)
                if v is None:
                    ref, r0 = la_ref(slot_of[r])
                    return _unpack(ref[r0 + u0 * QR // 2:r0 + u1 * QR // 2, :])
                i, k = v // 2, v % 2
                return jnp.concatenate([ckv_v[u * UR + i * QR:u * UR + (i + 1) * QR, k * kh:(k + 1) * kh]
                                        for u in range(u0, u1)], axis=0)

            def put_chunk(g, par, c, m, sub=range(26)):
                zero = None if m is None else (pltpu.bitcast(m[0:8, 0:D], u32) >> 31) >> 1
                n = kh // 2
                for e, w_v in enumerate((wuk_v, wuv_v)):
                    raw = {}

                    def words(p, v):
                        if (p, v // 2) not in raw:
                            w = w_v[p, 2 * g + v // 2 % 2, v // 4 * n + c * CR:v // 4 * n + (c + 1) * CR, :]
                            raw[p, v // 2] = w if zero is None else w | zero
                        return raw[p, v // 2]
                    sums = [r for r in sub if _plain(_B424_ROWS, r) is None]
                    ops = [_operands(lambda v: (_hi if v % 2 else _lo)(words(p, v)), _B424_TEMPS, _B424_ROWS, sums)
                           for p in range(2)]
                    for r in sub:
                        v = _plain(_B424_ROWS, r)
                        if v is None:
                            w = _words(ops[0][r], ops[1][r])
                        elif v % 2 == 0:
                            w = (words(0, v) & u32(0xFFFF)) | (words(1, v) << 16)
                        else:
                            w = (words(0, v) >> 16) | (words(1, v) & u32(0xFFFF0000))
                        ref, r0 = t_ref(26 * par + r)
                        ref[r0 + c * CR:r0 + (c + 1) * CR, e * D:(e + 1) * D] = w

            def project_kv(par, g, u0, u1, hooks=None, pre=None):
                def product(r):
                    if pre and r in pre:
                        pre[r]()
                    m = jnp.dot(lhs(r, u0, u1), _unpack(t_get(26 * par + r)), preferred_element_type=f32)
                    if hooks:
                        for c in hooks[1].get(r, ()):
                            put_chunk(hooks[0], 1 - par, c, m)
                    return m

                def store(i, j, blk):
                    for u in range(u0, u1):
                        p0 = (u * UR + i * QR) // 2
                        kv_v.at[4 * g + j][p0:p0 + QR // 2, :] = _pack(blk[(u - u0) * QR:(u - u0 + 1) * QR, :].astype(bf16))
                _mm424(product, store)

            def put_rhs(g, par, which):
                for c in range(kh // 2 // CR):
                    put_chunk(g, par, c, None, which)

            def hook_plan(npiece):
                nch = kh // 2 // CR
                plan = [{} for _ in range(npiece)]
                for c in range(nch):
                    sl = c * (npiece * 26 - 8) // nch
                    plan[sl // 26].setdefault(sl % 26, []).append(c)
                return plan

            def project_group(par, g, nxt):
                plan = hook_plan(NU // KU)
                for u in range(0, NU, KU):
                    project_kv(par, g, u, u + KU, (nxt, plan[u // KU]))

            def kv_first():
                ckv_cp(0).wait()
                lhs_prep(0)
                batch_wait(1, 0)
                put_rhs(0, 0, range(0, 7))
                ckv_cp(1).wait()
                lhs_prep(1)

                def rest():
                    batch_wait(1, 5)
                    for r in (7, 14, 20):
                        put_rhs(0, 0, range(r, {7: 14, 14: 20, 20: 26}[r]))
                project_kv(0, 0, 0, 2, pre={7: rest})
                ckv_cp(2).wait()
                lhs_prep(2)
                lhs_prep(3)
                ckv_cp(3).wait()
                lhs_prep(4)
                lhs_prep(5)
                project_kv(0, 0, 2, 4)
                ckv_cp(4).wait()
                batch_wait(2, 1)
                lhs_prep(6)
                lhs_prep(7)
                plan = hook_plan(2)
                for u in range(4, 8, 2):
                    project_kv(0, 0, u, u + 2, (1, plan[(u - 4) // 2]))

            def kv_body(j, c):
                @pl.when(j == 0)
                def _():
                    xat_cp.start()
                    w_start_shared(wqa_hbm, wqa_v, 0, range(HP))
                    xbt_cp.start()
                batch_wait(4, 2 + j)
                project_group(1, 2 * j + 1, 2 * j + 2)
                project_group(0, 2 * j + 2, 2 * j + 3)
                return c

            with _scope("a_kvproj"):
                kv_first()
                jax.lax.fori_loop(0, NG // 2 - 1, kv_body, 0)

            woa_cp.start()
            wob_cp.start()
            mem_cp.start()
            w_start_shared(wqb_hbm, wb_v.at[0], 1, range(HP))
            w_start_shared(wkb_hbm, wb_v.at[1], 2, range(HP // 2))

            QB = 4 * D
            plain = {(0, 0): 15, (0, 1): 1, (0, 2): 9, (1, 0): 4, (1, 1): 16, (1, 2): 8}

            def xa_prep(b):
                x = []
                for t in range(4 * b, 4 * b + 4):
                    xt = xat_v[:, t * D:(t + 1) * D]
                    x.append(jnp.concatenate([xt, xt[DM - HD:]], axis=0).astype(f32).T)

                def store(r, p, w):
                    lq_v.at[r][b * HD:(b + 1) * HD, p * D:(p + 1) * D] = w
                _lhs233([x[0], x[2]], [x[1], x[3]], store, extra=(((0, 0, 1),), ((1, 1, 1),)))

            def q_store(blk, hp, x0):
                q_v.at[hp][x0 // 2:(x0 + blk.shape[0]) // 2, :] = _pack((blk * QSCALE).astype(bf16))

            def q_rhs(hp):
                f = _rhs233([(wqa_v[0, hp + n], wqa_v[1, hp + n]) for n in range(3)])
                return [_passes(jnp.concatenate(f(r), axis=1)) for r in range(15)]

            def project_q(t, hp, b):
                nr = D // QS
                for s in range(QS):
                    rows = slice(b * HD + s * nr // 2, b * HD + (s + 1) * nr // 2)

                    def product(r):
                        wa, wb, wc = t[r]
                        c = jnp.dot(_unpack(lq_v[r, rows, 2 * D:3 * D]), _unpack(wc), preferred_element_type=f32)
                        a = jnp.dot(_unpack(lq_v[r, rows, 0 * D:1 * D]), _unpack(wa), preferred_element_type=f32)
                        b = jnp.dot(_unpack(lq_v[r, rows, 1 * D:2 * D]), _unpack(wb), preferred_element_type=f32)
                        return [a + c, b + c]
                    for (i, j), blk in _mm233(product):
                        for y in range(2):
                            q_store(blk[y], hp + j, b * QB + (2 * i + y) * D + s * nr)

            def project_q_last(hp):
                s0, s1 = wqa_v[0, hp], wqa_v[1, hp]
                w = jnp.concatenate([(s0 & u32(0xFFFF)) | (s1 << 16), (s0 >> 16) | (s1 & u32(0xFFFF0000))], axis=1)
                per = [_passes(jnp.concatenate([w[a:a + 64], w[c:c + 32]] if k == 1 else [w[a:a + 96]], axis=0))
                       for k, (a, _, c) in enumerate(_PIECES)]
                wp = [_unpack(jnp.concatenate([per[k][p] for k in range(3)], axis=0)) for p in range(3)]
                for b in range(S // QB):
                    rows = slice(b * HD, (b + 1) * HD)
                    for i in range(2):
                        a, bb, c = [jnp.dot(_unpack(jnp.concatenate([lq_v[plain[i, k], rows, p * D:(p + 1) * D] for k in range(3)], axis=1)),
                                            wp[p], preferred_element_type=f32) for p in range(3)]
                        q_store(a + c, hp, b * QB + 2 * i * D)
                        q_store(bb + c, hp, b * QB + (2 * i + 1) * D)

            def xb_prep(t):
                t0 = pl.multiple_of(t * D, D)
                xt = xbt_v[:, pl.ds(t0, D)]
                xb = jnp.concatenate([xt, xt[DM - HD:]], axis=0).T
                xb_v[pl.ds(t0, D), :] = xb
                for sg in range(D // SEG):
                    p0 = pl.multiple_of((t * (D // SEG) + sg) * PRE, PRE)
                    xpre_v[pl.ds(p0, PRE), :] = xb[sg * SEG:sg * SEG + PRE, :]

            with _scope("a_qproj"):
                xat_cp.wait()
                xbt_cp.wait()
                w_wait_shared(wqa_v, 0)
                t = q_rhs(0)
                for b in range(S // QB):
                    xa_prep(b)
                    for u in range(0, NU, KU):
                        if u // 2 == b:
                            project_kv(1, NG - 1, u, u + KU)
                    project_q(t, 0, b)
                XG = 4

                def q_body(j, c):
                    hp = 3 * j
                    for n in range(XG):
                        xb_prep((j - 1) * XG + n)
                    t = q_rhs(hp)
                    for b in range(S // QB):
                        project_q(t, hp, b)
                    return c
                jax.lax.fori_loop(1, 5, q_body, 0)
                lp_prep(lp_v)
                w_start_shared(wkb_hbm, wb_v.at[1], 2, range(HP // 2, HP))
                w_start_shared(wvb_hbm, wb_v.at[2], 3, range(HP))
                project_q_last(HP - 1)

        pl.run_scoped(
            projections,
            pltpu.VMEM((S, DC), bf16),
            pltpu.VMEM((DM, S), bf16),
            pltpu.VMEM((2, HP, DC // 2, D), u32),
            pltpu.VMEM((2, HP, DC // 2, D), u32),
            pltpu.VMEM((2, HP, DM // 2, D), u32),
            pltpu.VMEM((17, S // 8, 3 * D), u32),
        )

        def attention(c_v, s_v):
            row = jax.lax.broadcasted_iota(jnp.int32, (TQ, TQ), 0)
            col = jax.lax.broadcasted_iota(jnp.int32, (TQ, TQ), 1)
            tri = col <= row
            nb = S // TQ
            hq = TQ // 2
            npiece = 2
            pw = S // npiece

            def q_rows(h, r0, r1):
                return q_v[h[0], r0:r1, h[1] * D:(h[1] + 1) * D]

            def head(h):
                return 2 * h[0] + h[1]

            def qk_piece(h, j):
                q = _unpack(q_rows(h, (nb - 1) * hq, nb * hq))
                k = _unpack(kv_v[head(h), j * pw // 2:(j + 1) * pw // 2, 0:D])
                s_v[:, j * pw:(j + 1) * pw] = jax.lax.dot_general(q, k, NT, preferred_element_type=f32)

            def qk(h, i, j0=0, j1=None):
                j1 = i + 1 if j1 is None else j1
                q = _unpack(q_rows(h, i * hq, (i + 1) * hq))
                k = _unpack(kv_v[head(h), j0 * hq:j1 * hq, 0:D])
                return jax.lax.dot_general(q, k, NT, preferred_element_type=f32)

            def pv_shared(p, hd, i):
                low = jax.lax.broadcasted_iota(jnp.int32, (1, TQ), 1) < HD
                qr = TQ // 4

                def mm(x, w):
                    return jnp.dot(x.astype(bf16), _unpack(w), preferred_element_type=f32)
                pa, pd = p[:, (i - 1) * TQ:i * TQ], p[:, i * TQ:]
                y1a, y2a, y1d, y2d = pa[0:qr], pa[qr:2 * qr], pd[0:qr], pd[qr:2 * qr]
                va = kv_v[hd, (i - 1) * hq:i * hq, D:2 * D]
                vd = kv_v[hd, i * hq:(i + 1) * hq, D:2 * D]
                la = jnp.where(low, y1a, y1a - y2a)
                lb = jnp.where(low, y2a, pltpu.roll(y2d - y1d, HD, 1))
                lc = jnp.where(low, y1d, y2a)
                o = None
                if i > 1:
                    o = mm(p[:, :(i - 1) * TQ], kv_v[hd, 0:(i - 1) * hq, D:2 * D])
                o2 = mm(jnp.concatenate([la, pa[2 * qr:]], axis=0), va)
                o3 = mm(pd[2 * qr:], vd)
                ob = mm(lb, jnp.concatenate([va[0:qr], vd[0:qr]], axis=0))
                oc = mm(lc, jnp.concatenate([vd[0:qr], va[qr:]], axis=0))
                r = jnp.concatenate([o2[0:qr] + oc, ob + oc, o2[qr:] + o3], axis=0)
                return r if o is None else o + r

            def anchor_plan():
                ops = []
                for e in range(UH):
                    for i in range(nb - 1, -1, -1):
                        if i > 0:
                            ops.append(("qk", e, i - 1, 32 * i))
                        if i < npiece:
                            ops.append(("piece", e, i, 32 * nb // npiece))
                        ops.append(("pv", e, i, 32 * (i + 1)))
                t, start, end = 0, [], []
                for op in ops:
                    start.append(t)
                    t += op[3]
                    end.append(t)
                plan = {}
                for a, op in enumerate(ops):
                    if op[0] != "pv" or op[2] < ANCHOR_MIN:
                        continue
                    for b in range(a + 1, len(ops)):
                        if ops[b][0] == "qk" and start[b] >= end[a] + ANCHOR_LAG:
                            plan.setdefault((ops[b][1], ops[b][2]), []).append((op[1], op[2]))
                            break
                return plan

            def heads(j, c):

                plan = anchor_plan()


                def gated_qk(e, i):
                    h = (j * (UH // 2) + e // 2, e % 2)
                    if (e, i) not in plan:
                        return qk(h, i)
                    w = None
                    for ea, ia in plan[e, i]:
                        u = c_v[j * (UH // 2) + ea // 2, ia * hq:(ia + 1) * hq, (ea % 2) * D:(ea % 2 + 1) * D]
                        for r in range(0, hq, 8):
                            w = u[r:r + 8] if w is None else w | u[r:r + 8]
                    zero = (w >> 31) >> 1
                    q = q_rows(h, i * hq, (i + 1) * hq)
                    q = _unpack(jnp.concatenate([q[0:8] | zero, q[8:]], axis=0))
                    k = _unpack(kv_v[head(h), 0:(i + 1) * hq, 0:D])
                    return jax.lax.dot_general(q, k, NT, preferred_element_type=f32)

                s_next = s_v[...]
                for e in range(UH):
                    h = (j * (UH // 2) + e // 2, e % 2)
                    if e == UH - 1:
                        hn = (jnp.minimum(h[0] + 1, HP - 1), 0)
                    else:
                        hn = (j * (UH // 2) + (e + 1) // 2, (e + 1) % 2)
                    pieces = []
                    for i in range(nb - 1, -1, -1):
                        s = s_next
                        if i > 0:
                            s_next = gated_qk(e, i - 1)
                        if i < npiece:
                            if e == UH - 1:
                                qk_piece(hn, npiece - 1 - i)
                            else:
                                jj = npiece - 1 - i
                                pieces.append(qk(hn, nb - 1, jj * nb // npiece, (jj + 1) * nb // npiece))
                        sd = jnp.where(tri, s[:, i * TQ:], NEG)
                        s = jnp.concatenate([s[:, :i * TQ], sd], axis=1) if i > 0 else sd
                        m = jnp.max(s, axis=1, keepdims=True)
                        p = jnp.exp2(s - m)
                        l = jnp.sum(p, axis=1, keepdims=True)
                        if i < PVT:
                            v = _unpack(kv_v[head(h), 0:(i + 1) * hq, D:2 * D])
                            o = jnp.dot(p.astype(bf16), v, preferred_element_type=f32)
                        else:
                            o = pv_shared(p, head(h), i)
                        c_v.at[h[0]][i * hq:(i + 1) * hq, h[1] * D:(h[1] + 1) * D] = _pack((o * _recip(l)).astype(bf16))
                    if e < UH - 1:
                        s_next = jnp.concatenate(pieces, axis=1)
                return c
            with _scope("a_attn"):
                for j in range(npiece):
                    qk_piece((0, 0), j)
                jax.lax.fori_loop(0, H // UH, heads, 0)

            woa_cp.wait()
            wob_cp.wait()
            mem_cp.wait()
            for t in range(3):
                w_wait_shared(wb_v.at[t], 1 + t)
            mh = DM // 4
            slot = {0: 0, 1: 1, 4: 2, 5: 3, 6: 4}

            def wo_prep(hh):
                a11, a21 = woa_v[hh, 0:mh, :], woa_v[hh, mh:2 * mh, :]
                a12, a22 = woa_v[hh + HP, 0:mh, :], woa_v[hh + HP, mh:2 * mh, :]
                for i, w in enumerate(_sum_words(_strassen_lhs, a11, a12, a21, a22, (2, 3), (a11, a22))):
                    if i in slot:
                        kv_v[hh, slot[i] * mh:(slot[i] + 1) * mh, 0:D] = w

            def wob_prep(hp):
                w1, w2 = _unpack(wobt_v[2 * hp]), _unpack(wobt_v[2 * hp + 1])
                a, b = KM + HD, KM + 2 * HD
                d12 = (w1[a:b].astype(f32) - w2[a:b].astype(f32)).astype(bf16)
                d21 = (w2[b:].astype(f32) - w1[b:].astype(f32)).astype(bf16)
                rows = slice(hp * HD, (hp + 1) * HD)
                wob_v[0, rows, :] = _pack(jnp.concatenate([w1[:a], d12], axis=0).T)
                wob_v[1, rows, :] = _pack(jnp.concatenate([w2[:a], d21], axis=0).T)
                wos_v[rows, :] = _pack(jnp.concatenate([w1[b:], w2[a:b]], axis=0).T)

            def oproj(tp):
                w0 = tp * D
                per = []
                for hh in range(HP):
                    def ctx(h, r0):
                        return c_v[h // 2, r0:r0 + D // 2, (h % 2) * D:(h % 2 + 1) * D]
                    b11, b21 = ctx(hh, w0), ctx(hh + HP, w0)
                    b12, b22 = ctx(hh, w0 + D // 2), ctx(hh + HP, w0 + D // 2)
                    per.append(_sum_words(_strassen_rhs, b11, b12, b21, b22, (1, 4), (b11, b22)))

                def lhs(i, s):
                    hhs = range(s * HP // KS, (s + 1) * HP // KS)
                    if i == 2:
                        return _unpack(jnp.concatenate([woa_v[hh, 0:mh, :] for hh in hhs], axis=1))
                    if i == 3:
                        return _unpack(jnp.concatenate([woa_v[hh + HP, mh:2 * mh, :] for hh in hhs], axis=1))
                    return _unpack(jnp.concatenate([kv_v[hh, slot[i] * mh:(slot[i] + 1) * mh, 0:D] for hh in hhs], axis=1))

                def rhs(i, s):
                    return _unpack(jnp.concatenate([per[hh][i] for hh in range(s * HP // KS, (s + 1) * HP // KS)], axis=1))

                def done(c11, c12, c21, c22):
                    t0 = 2 * tp * D
                    out_v[t0:t0 + D, 0:DM] = jnp.concatenate([c11, c21], axis=0).T.astype(bf16)
                    out_v[t0 + D:t0 + 2 * D, 0:DM] = jnp.concatenate([c12, c22], axis=0).T.astype(bf16)
                yield from _strassen(lhs, rhs, NT, done, 1 if tp == 0 else 0)

            def outputs():
                for hh in range(HP):
                    wo_prep(hh)
                for tp in range(S // D // 2):
                    yield from oproj(tp)
                    for hp in range(2 * tp, 2 * tp + 2):
                        wob_prep(hp)

            steps, na, nb_ = outputs(), KS * 7 * (S // D // 2), 15 * HP // PG
            count = [0, 0]

            def tick():
                count[0] += 1
                while count[1] < na and I0 + count[1] * (nb_ - I0 - I1) // na <= count[0]:
                    next(steps)
                    count[1] += 1
            with _scope("post"):
                b_pre(lp_v, tick)
                for _ in steps:
                    pass

        pl.run_scoped(
            attention,
            pltpu.VMEM((HP, S // 2, 2 * D), u32),
            pltpu.VMEM((TQ, S), f32),
        )

    pl.run_scoped(
        phase_a,
        pltpu.VMEM((H, DM // 2, D), u32),
        pltpu.VMEM((DM, S), bf16),
        pltpu.VMEM((H, DM // 2, D), u32),
        pltpu.VMEM((15, NSEG * PRE // 8, 3 * D), u32),
    )

    def out_copy(j):
        rows = pl.ds(pl.multiple_of(j * (OUTER * SEG), OUTER * SEG), OUTER * SEG)
        return pltpu.make_async_copy(out_v.at[rows, :], out_hbm.at[rows, :], sem.at[SEM_OUT + j])

    def phase_b(post_v):
        GP = HG // 2
        GC = GP * 3 * D
        KA = KM + 2 * HD
        lane = jax.lax.broadcasted_iota(jnp.int32, (1, GC), 1)
        colscale = jnp.where(lane % (3 * D) < D, QSCALE, 1.0).astype(f32)
        low = jax.lax.broadcasted_iota(jnp.int32, (1, D), 1) < HD

        def swap(x):
            return pltpu.roll(x, HD, 1)

        def wgroup(g):
            cols = [(hp, t) for hp in range(g * GP, (g + 1) * GP) for t in range(3)]
            own = [_unpack(jnp.concatenate([wb_v[t, e, hp, 0:KA // 2, :] for hp, t in cols], axis=1)) for e in range(2)]
            both = jnp.concatenate([jnp.concatenate([wb_v[t, e, hp, KA // 2:, :] for hp, t in cols], axis=1)
                                    for e in range(2)], axis=0)
            return own[0], own[1], _unpack(both)

        def out_project(even, odd, both, p0, p1):
            rows = slice(p0 * HD, p1 * HD)
            return [jnp.dot(even, _unpack(wob_v[0, rows, :]), preferred_element_type=f32),
                    jnp.dot(odd, _unpack(wob_v[1, rows, :]), preferred_element_type=f32),
                    jnp.dot(both, _unpack(wos_v[rows, :]), preferred_element_type=f32)]

        def out_add(acc, part):
            e, o, b = part
            new = [e[:, :KM] + o[:, :KM], e[:, KM:], o[:, KM:], b]
            return new if acc is None else [x + y for x, y in zip(acc, new)]

        def out_finish(acc):
            main, e, o, b = acc
            mid = e + jnp.where(low, o, b)
            last = jnp.where(low, swap(o) + b, o + swap(b))
            return jnp.concatenate([main, mid, last], axis=1)

        ri = jax.lax.broadcasted_iota(jnp.int32, (2 * L, 2 * L), 0)
        ci = jax.lax.broadcasted_iota(jnp.int32, (2 * L, 2 * L), 1)

        def second(i):
            return jnp.where(i < 2 * SEG, i // SEG, (i - 2 * SEG) // PRE)

        def pos(i):
            j = i % SEG
            return jnp.where(i < 2 * SEG, jnp.where(j < T, j + (MEM + PRE), j - T), MEM + i % PRE)
        same = second(ri) == second(ci)
        mask = same & ((pos(ri) < MEM) | (pos(ri) >= pos(ci)))
        fill = jnp.where(same, NEG, -jnp.inf).astype(f32)

        def step(s, slot, mem):
            xt = xb_v[pl.ds(pl.multiple_of(SEG * s + PRE, 8), T), :]
            l1 = jnp.concatenate([xt.astype(f32), mem], axis=0)
            mid, last = l1[:, KM:KA], l1[:, KA:]
            l_even = l1[:, :KA].astype(bf16)
            l_odd = jnp.concatenate([l1[:, :KM], jnp.where(low, mid, last)], axis=1).astype(bf16)
            l_both = jnp.where(low, last, mid).astype(bf16)
            p0 = pl.multiple_of(PRE * s, 8)
            proj = []
            for g in range(G):
                w_even, w_odd, w_both = wgroup(g)
                both = jnp.dot(l_both, w_both, preferred_element_type=f32)
                even = jnp.dot(l_even, w_even, preferred_element_type=f32)
                odd = jnp.dot(l_odd, w_odd, preferred_element_type=f32)
                proj.append([(x + both) * colscale for x in (even, odd)])

            def rows(hp, t):
                g, c0 = hp // GP, (hp % GP) * 3 * D + t * D
                ref, r0, l0 = pre_ref(hp * 3 + t)
                return jnp.concatenate([proj[g][0][:, c0:c0 + D], proj[g][1][:, c0:c0 + D],
                                        _unpack(ref[pl.ds(r0 + p0, PRE), l0:l0 + D]).astype(f32)], axis=0).astype(bf16)

            scores = [jax.lax.dot_general(rows(hp, 0), rows(hp, 1), NT, preferred_element_type=f32)
                      for hp in range(HP)]
            ctx = {}
            tails = []

            def attend(g):
                for hp in range(g * HG // 2, (g + 1) * HG // 2):
                    sc = jnp.where(mask, scores[hp], fill)
                    m = jnp.max(sc, axis=1, keepdims=True)
                    p = jnp.exp2(sc - m)
                    l = jnp.sum(p, axis=1, keepdims=True)
                    o = jnp.dot(p.astype(bf16), rows(hp, 2), preferred_element_type=f32) * _recip(l)
                    ctx[hp] = [o[0:SEG, :], o[SEG:2 * SEG, :], o[0:SEG, :] + o[SEG:2 * SEG, :]]
                    for e in range(2):
                        post_v[e, slot * PRE:(slot + 1) * PRE, hp * D:(hp + 1) * D] = o[2 * SEG + e * PRE:2 * SEG + (e + 1) * PRE, :]
                        tails.append(o[2 * SEG + e * PRE:2 * SEG + (e + 1) * PRE, :])

            parts = []

            def oproj(g):
                lhs = [jnp.concatenate([ctx[hp][e] for hp in range(g * GP, (g + 1) * GP)], axis=1).astype(bf16)
                       for e in range(3)]
                parts.append(out_project(*lhs, g * GP, (g + 1) * GP))

            for t in range(G + 2):
                if t < G:
                    attend(t)
                if t >= 2:
                    oproj(t - 2)
            acc = None
            for a in parts:
                acc = out_add(acc, a)
            accb = out_finish(acc).astype(bf16)
            out_v[pl.ds(pl.multiple_of(SEG * s + PRE, 8), T), DM:2 * DM] = accb[0:T, 0:DM]
            late = pltpu.bitcast(ctx[HP - 1][1][0:8], u32)
            for x in tails:
                late = late | pltpu.bitcast(x, u32)
            return accb[T:, :].astype(f32), late

        PP = HP // OUTER

        def deferred_rows():
            even, odd = post_v[0], post_v[1]
            return even, odd, even + odd

        def finish(j, acc):
            r = out_finish(acc).astype(bf16)
            for sg in range(OUTER):
                r0 = pl.multiple_of((j * OUTER + sg) * SEG, SEG)
                out_v[pl.ds(r0, PRE), DM:2 * DM] = r[sg * PRE:(sg + 1) * PRE, 0:DM]

        def after(x, late):
            u = late
            zero = (u >> 31) & (~u >> 31)
            top = pltpu.bitcast(x[0:8], u32) | jnp.concatenate([zero] * (x.shape[1] // D), axis=1)
            return jnp.concatenate([pltpu.bitcast(top, f32), x[8:]], axis=0).astype(bf16)

        def outer(j, c):
            mem, done = c
            finish(jnp.maximum(j - 2, 0), done)
            prev = deferred_rows()

            def partial(i, late):
                x = [after(p[:, i * PP * D:(i + 1) * PP * D], late) for p in prev]
                return out_project(*x, i * PP, (i + 1) * PP)
            acc = None
            for i in range(OUTER):
                mem, late = step(j * OUTER + i, i, mem)
                acc = out_add(acc, partial(i, late))

            @pl.when(j >= 2)
            def _():
                out_copy(j - 2).start()
            return mem, acc
        with _scope("b_loop"):
            post_v[...] = jnp.zeros(post_v.shape, f32)
            mem0 = mem_v[0:MEM, :].astype(f32)
            zeros = [jnp.zeros((OUTER * PRE, n), f32) for n in (KM, D, D, D)]
            _, done = jax.lax.fori_loop(0, NOUTER, outer,
                                        (jnp.concatenate([mem0, mem0[:, DM - HD:]], axis=1), zeros))
            finish(NOUTER - 2, done)
            out_copy(NOUTER - 2).start()
            out_copy(0).wait()
            finish(NOUTER - 1, out_add(None, out_project(*[x.astype(bf16) for x in deferred_rows()], 0, HP)))
            out_copy(NOUTER - 1).start()
        with _scope("b_outwait"):
            for j in range(1, NOUTER):
                out_copy(j).wait()

    pl.run_scoped(
        phase_b,
        pltpu.VMEM((2, OUTER * PRE, HP * D), f32),
    )


@jax.jit
def pallas_concat_heads__compressed_kv_cla__memory_aug_recurrent_mem_tr__prompt_kernel(
    A_x: jax.Array,
    A_c_kv: jax.Array,
    A_w_q: jax.Array,
    A_w_uk: jax.Array,
    A_w_uv: jax.Array,
    A_w_o: jax.Array,
    B_x: jax.Array,
    B_mem0: jax.Array,
    B_Wq: jax.Array,
    B_Wk: jax.Array,
    B_Wv: jax.Array,
    B_Wo: jax.Array,
    B_seg_len=SEG,
):
    def t2(x):
        return jnp.transpose(x, (0, 2, 1)).reshape(DM, S)

    def w3(w):
        return w.reshape(w.shape[0] // 2, 2 * H, D)

    def wo3(w):
        return jnp.transpose(w, (0, 2, 1))

    any_spec = pl.BlockSpec(memory_space=pl.ANY)
    out = pl.pallas_call(
        _kernel,
        out_shape=jax.ShapeDtypeStruct((S, 2 * DM), bf16),
        in_specs=[any_spec] * 12,
        out_specs=any_spec,
        scratch_shapes=[
            pltpu.VMEM((S, 2 * DM), bf16),
            pltpu.VMEM((S, DMP), bf16),
            pltpu.VMEM((NSEG * PRE, DMP), bf16),
            pltpu.VMEM((3, 2, HP, DM // 2, D), u32),
            pltpu.VMEM((2, HP * D // 2, KM + 2 * HD), u32),
            pltpu.VMEM((HP * D // 2, D), u32),
            pltpu.VMEM((8 * MEM, DM), bf16),
            pltpu.VMEM((HP, S // 2, 2 * D), u32),
            pltpu.VMEM((H, S // 2, 2 * D), u32),
            pltpu.SemaphoreType.DMA((NSEM,)),
        ],
        compiler_params=pltpu.CompilerParams(vmem_limit_bytes=126 * 1024 * 1024),
    )(t2(A_x), A_c_kv.reshape(S, DC), w3(A_w_q), w3(A_w_uk), w3(A_w_uv), wo3(A_w_o),
      t2(B_x), B_mem0.reshape(MEM, DM), w3(B_Wq), w3(B_Wk), w3(B_Wv), wo3(B_Wo))
    return out.reshape(1, S, 2 * DM)
```

```python
import contextlib

import jax
import jax.numpy as jnp
import jax.experimental.pallas as pl
import jax.experimental.pallas.tpu as pltpu

S = 2048
DM = 576
DC = 512
H = 32
D = 128
MEM = 8
SEG = 32
L = MEM + SEG
NSEG = S // SEG
HP = H // 2
HD = D // 2
KM = DM - 3 * HD
DMP = DM + HD

LOG2E = 1.4426950408889634
QSCALE = D ** -0.5 * LOG2E
NEG = -1.0e9 * LOG2E

TQ = 128
UH = 4
ANCHOR_LAG = 2000
ANCHOR_MIN = 6
RB = 512
HG = 4
G = H // HG
PRE = 8
T = SEG - PRE
OUTER = 4
NOUTER = NSEG // OUTER

bf16 = jnp.bfloat16
f32 = jnp.float32
u32 = jnp.uint32
NT = (((1,), (1,)), ((), ()))

SEM_CKV = 0
SEM_XAT = 5
SEM_XBT = 6
SEM_MEM = 7
SEM_WOA = 8
SEM_WOB = 9
SEM_OUT = 10
SEM_WALL = SEM_OUT + NOUTER
SEM_W = SEM_WALL + 4
NSEM = SEM_W + 6

_PROFILE = False
I0 = 0
I1 = 30
KS = 4
KU = 2
CL = 16
CR = 8
PVT = 5
PG = 1
HT = 14
QS = 2

def _scope(name):
    return jax.named_scope(name) if _PROFILE else contextlib.nullcontext()


def _unpack(w32):
    return pltpu.bitcast(w32, bf16)


def _pack(x):
    return pltpu.bitcast(x, u32)


def _lo(w):
    return pltpu.bitcast(w << 16, f32)


def _hi(w):
    return pltpu.bitcast(w & u32(0xFFFF0000), f32)


def _words(even, odd):
    return pltpu.bitcast(pltpu.pack_elementwise([even, odd], packed_dtype=bf16), u32)


def _strassen_lhs(a11, a12, a21, a22):
    return [a11 + a22, a21 + a22, a11, a22, a11 + a12, a21 - a11, a12 - a22]


def _strassen_rhs(b11, b12, b21, b22):
    return [b11 + b22, b11, b12 - b22, b21 - b11, b22, b11 + b12, b21 + b22]


def _sum_words(combine, x11, x12, x21, x22, raw_idx, raw):
    lo = combine(_lo(x11), _lo(x12), _lo(x21), _lo(x22))
    hi = combine(_hi(x11), _hi(x12), _hi(x21), _hi(x22))
    words = [pltpu.bitcast(pltpu.pack_elementwise([a, b], packed_dtype=bf16), u32) for a, b in zip(lo, hi)]
    for i, r in zip(raw_idx, raw):
        words[i] = r
    return words


def _strassen(lhs, rhs, dims, done, order=0):
    def m(i):
        acc = None
        for s in range(KS):
            part = jax.lax.dot_general(lhs(i - 1, s), rhs(i - 1, s), dims, preferred_element_type=f32)
            acc = part if acc is None else acc + part
            if i != 7 or s < KS - 1:
                yield
        return acc
    if order == 0:
        m1 = yield from m(1)
        m2 = yield from m(2)
        c22 = m1 - m2
        m4 = yield from m(4)
        c11 = m1 + m4
        c21 = m2 + m4
        c22 = c22 + (yield from m(6))
        m3 = yield from m(3)
        c22 = c22 + m3
        m5 = yield from m(5)
        c11 = c11 - m5
        c12 = m3 + m5
        c11 = c11 + (yield from m(7))
        done(c11, c12, c21, c22)
        yield
        return
    m3 = yield from m(3)
    m4 = yield from m(4)
    m5 = yield from m(5)
    c12 = m3 + m5
    c11 = m4 - m5
    m2 = yield from m(2)
    c21 = m4 + m2
    c22 = m3 - m2
    m1 = yield from m(1)
    c11 = c11 + m1
    c22 = c22 + m1
    c22 = c22 + (yield from m(6))
    c11 = c11 + (yield from m(7))
    done(c11, c12, c21, c22)
    yield


def _rhs_words(s0, s1, z0, z1):
    per = [_strassen_rhs(_lo(s), _hi(s), _lo(z), _hi(z)) for s, z in ((s0, z0), (s1, z1))]
    words = [pltpu.bitcast(pltpu.pack_elementwise([per[0][i], per[1][i]], packed_dtype=bf16), u32)
             for i in range(7)]
    words[1] = (s0 & u32(0xFFFF)) | (s1 << 16)
    words[4] = (z0 >> 16) | (z1 & u32(0xFFFF0000))
    return words


_L233 = (((0, 1, 1), (1, 0, 1)), ((0, 1, 1),), ((0, 0, 1), (1, 0, -1)), ((0, 1, 1), (1, 1, -1)), ((1, 0, 1),),
         ((0, 0, -1), (0, 1, -1)), ((1, 0, 1), (1, 1, 1)), ((0, 0, 1), (0, 2, 1), (1, 0, -1)), ((1, 2, 1),),
         ((0, 2, 1),), ((1, 0, 1), (1, 2, 1), (0, 0, -1), (0, 2, -1)), ((0, 0, -1), (0, 2, -1)),
         ((1, 1, 1), (1, 2, 1), (0, 1, -1)), ((1, 1, -1), (1, 2, -1)),
         ((0, 1, 1), (0, 2, 1), (1, 1, -1), (1, 2, -1)))
_R233 = (((0, 1, 1), (1, 0, 1)), ((1, 1, 1), (1, 2, 1), (0, 1, -1)), ((0, 0, 1), (0, 1, 1), (2, 0, -1)),
         ((2, 1, 1), (1, 0, -1), (1, 1, -1)), ((0, 0, 1), (0, 2, 1), (1, 0, -1)), ((0, 1, 1),), ((1, 0, 1),),
         ((0, 2, 1), (2, 0, 1)), ((2, 0, 1), (2, 2, 1), (1, 2, -1)), ((2, 1, 1), (2, 2, 1), (0, 2, -1)),
         ((2, 0, 1),), ((0, 2, 1),), ((1, 2, 1), (2, 1, 1)), ((1, 2, 1),), ((2, 1, 1),))
_PIECES = ((0, 32, 64), (128, 160, 96), (192, 224, 256))


def _signed_sum(terms, get):
    acc = None
    for a, b, c in terms:
        x = get(a, b)
        if acc is None:
            acc = x if c > 0 else -x
        else:
            acc = acc + x if c > 0 else acc - x
    return acc


def _lhs233(y1, y2, store, extra=()):
    low = jax.lax.broadcasted_iota(jnp.int32, (1, D), 1) < HD
    base = {}
    for i in range(2):
        t1 = [y1[i][:, c * D:(c + 1) * D] for c in range(5)]
        t2 = [y2[i][:, c * D:(c + 1) * D] for c in range(5)]
        r1, r2 = pltpu.roll(t1[1], HD, 1), pltpu.roll(t2[1], HD, 1)
        for k in range(3):
            a1, a2 = t1[(0, 2, 3)[k]], t2[(0, 2, 3)[k]]
            lo1 = (t1[1], r1, t1[4])[k]
            hi1, hi2 = (r1, t1[1], t1[4])[k], (r2, t2[1], t2[4])[k]
            base[i, k] = (jnp.where(low, a1, a1 - a2), jnp.where(low, a2, hi2 - hi1), jnp.where(low, lo1, a2))
    for r, terms in enumerate(_L233 + extra):
        for p in range(3):
            store(r, p, _pack(_signed_sum(terms, lambda i, k: base[i, k][p]).astype(bf16)))


def _rhs233(slabs):
    def chunk(j, par, k):
        s = slabs[j][par]
        a, b, c = _PIECES[k]
        return s[a:a + 96] if k != 1 else jnp.concatenate([s[a:a + 64], s[c:c + 32]], axis=0)

    def words(r):
        terms = _R233[r]
        if len(terms) == 1:
            k, j, _ = terms[0]
            s0, s1 = chunk(j, 0, k), chunk(j, 1, k)
            return (s0 & u32(0xFFFF)) | (s1 << 16), (s0 >> 16) | (s1 & u32(0xFFFF0000))
        half = [[_signed_sum(terms, lambda k, j: f(chunk(j, par, k))) for par in range(2)] for f in (_lo, _hi)]
        return _words(*half[0]), _words(*half[1])
    return words


def _passes(w):
    return (w[0:64], jnp.concatenate([w[0:32], w[64:96]], axis=0), jnp.concatenate([w[64:96], w[32:64]], axis=0))


def _mm233(product):
    def add(a, b):
        return [x + y for x, y in zip(a, b)]

    def sub(a, b):
        return [x - y for x, y in zip(a, b)]
    p13 = product(13)
    s1 = add(product(12), p13)
    s2 = add(s1, product(14))
    p11 = product(11)
    yield (0, 2), sub(sub(product(9), s2), p11)
    s3 = add(product(7), p11)
    s4 = add(s3, product(10))
    yield (1, 2), sub(sub(product(8), s4), p13)
    p4 = product(4)
    p6 = product(6)
    yield (1, 0), add(add(p6, s4), p4)
    c11 = sub(s1, p6)
    p5 = product(5)
    p1 = product(1)
    yield (0, 1), sub(add(p1, s2), p5)
    c11 = add(c11, p1)
    p0 = product(0)
    yield (1, 1), add(add(product(3), c11), p0)
    yield (0, 0), add(add(add(add(product(2), s3), p4), p5), p0)


_A424_TEMPS = ((3, 7, -1), (5, 7, -1), (0, 6, -1), (2, 6, -1), (4, 9, -1))
_A424_ROWS = (((4, 1), (0, -1)), ((1, 1), (5, -1)), ((4, 1), (1, -1)), ((0, 1), (1, -1)), ((4, 1),), ((5, 1), (4, -1)), ((1, 1),), ((12, 1),), ((3, 1), (1, -1)), ((2, 1), (1, -1)), ((1, 1), (10, -1)), ((2, 1), (0, -1)), ((10, 1),), ((2, 1),), ((6, 1),), ((2, 1), (3, -1)), ((6, 1), (12, -1)), ((8, 1), (2, -1)), ((8, 1), (11, -1)), ((8, 1),), ((7, 1),), ((8, 1), (10, -1)), ((9, 1),), ((4, 1), (11, 1)), ((2, 1), (9, 1)), ((5, 1), (8, 1)))
_B424_TEMPS = ((0, 2, 1), (2, 3, -1), (5, 6, -1), (7, 9, -1), (4, 8, 1), (1, 10, 1))
_B424_ROWS = (((0, 1), (1, 1)), ((4, 1), (5, 1)), ((1, 1), (4, -1)), ((1, 1),), ((0, 1), (4, 1)), ((4, 1),), ((1, 1), (5, 1)), ((12, 1),), ((5, 1), (7, -1)), ((1, 1), (7, 1)), ((13, 1),), ((1, 1), (3, -1)), ((2, 1), (13, -1)), ((3, 1), (7, 1)), ((2, 1),), ((7, 1),), ((8, 1),), ((11, 1),), ((9, 1),), ((6, 1), (11, -1)), ((6, 1),), ((9, 1), (10, -1)), ((6, 1), (12, 1)), ((3, 1), (8, 1)), ((7, 1), (8, -1)), ((4, 1), (6, 1), (7, 1)))
_POST424 = ((0,), (0,), (0,), (-1, 2, 0), (-1, 2, 1), (0,), (-1, 3, 5), (0,), (1, 6, 7), (2, 0, 8), (0,), (1, 7, 9), (-1, 4, 9), (2, 8, 10), (0,), (1, 5, 12), (1, 11, 12), (2, 1, 13), (2, 9, 14), (0,), (-1, 15, 7), (1, 9, 15), (0,), (0,), (1, 18, 19), (-1, 5, 19), (1, 12, 20), (0,), (-1, 12, 23), (0,), (1, 21, 25), (-1, 22, 25), (0,), (1, 24, 28), (1, 27, 28), (0,), (1, 26, 31), (2, 3, 32), (0,), (1, 29, 33), (-1, 17, 33), (2, 2, 34), (0,), (-1, 22, 36), (-1, 31, 36), (2, 5, 37), (2, 7, 38), (0,), (1, 35, 39), (2, 12, 40), (0,), (1, 31, 41), (-1, 39, 42), (0,), (1, 36, 44), (-1, 33, 45), (1, 43, 46), (1, 30, 46), (-1, 46, 41), (2, 15, 49), (0,), (1, 42, 50), (-1, 48, 51), (0,), (1, 51, 53), (1, 16, 53), (1, 33, 53), (-1, 36, 54), (2, 6, 54), (2, 14, 56), (0,), (1, 52, 58), (2, 13, 59), (0,), (-1, 57, 60), (1, 55, 60), (2, 10, 62), (0,), (1, 47, 63), (0,), (-1, 61, 65), (1, 64, 65), (2, 11, 67), (0,), (1, 66, 68), (2, 4, 69))


def _plain(rows, r):
    return rows[r][0][0] if len(rows[r]) == 1 and rows[r][0][0] < 8 else None


def _operands(block, temps, rows, which):
    x = {}

    def get(v):
        if v not in x:
            if v < 8:
                x[v] = block(v)
            else:
                a, b, c = temps[v - 8]
                x[v] = get(a) + get(b) if c > 0 else get(a) - get(b)
        return x[v]
    out = {}
    for r in which:
        acc = get(rows[r][0][0])
        for v, c in rows[r][1:]:
            acc = acc + get(v) if c > 0 else acc - get(v)
        out[r] = acc
    return out


def _mm424(product, store):
    val, r = [], 0
    for ins in _POST424:
        if ins[0] == 0:
            val.append(product(r))
            r += 1
        elif ins[0] == 2:
            store(ins[1] // 4, ins[1] % 4, val[ins[2]])
        else:
            val.append(val[ins[1]] + val[ins[2]] if ins[0] > 0 else val[ins[1]] - val[ins[2]])


def _gate(m):
    return (pltpu.bitcast(m[0:8, 0:D], u32) >> 31) >> 1


def _gated_rows(x, m):
    zero = jnp.concatenate([_gate(m)] * (x.shape[1] // D), axis=1)
    return _unpack(_pack(x) | zero).astype(f32)


def _recip(l):
    r = pl.reciprocal(l, approx=True)
    return r * (2.0 - l * r)


def _kernel(xat_hbm, ckv_hbm, wqa_hbm, wuk_hbm, wuv_hbm, woa_hbm,
            xbt_hbm, mem0_hbm, wqb_hbm, wkb_hbm, wvb_hbm, wob_hbm,
            out_hbm,
            out_v, xb_v, xpre_v, wb_v, wob_v, wos_v, mem_v, q_v, kv_v, sem):

    def w_copy(w_hbm, dst, slot, par, hp):
        return pltpu.make_async_copy(w_hbm.bitcast(u32).at[:, par * HP + hp, :], dst.at[par, hp], sem.at[slot])

    def w_start_shared(w_hbm, dst, widx, hps):
        for hp in hps:
            for par in range(2):
                w_copy(w_hbm, dst, SEM_WALL + widx, par, hp).start()

    def w_wait_shared(dst, widx):
        pltpu.make_async_copy(dst, dst, sem.at[SEM_WALL + widx]).wait()

    def w_combine(dst, hp):
        a = dst[0, hp]
        b = dst[1, hp]
        ev = (a & u32(0xFFFF)) | (b << 16)
        od = (a >> 16) | (b & u32(0xFFFF0000))
        return ev, od

    def w_pair(dst, hp):
        return jnp.concatenate(w_combine(dst, hp), axis=1)

    wb_hbm = (wqb_hbm, wkb_hbm, wvb_hbm)

    def pre_ref(j):
        n = NSEG * PRE
        return q_v.at[j // 4], (j % 4 // 2) * n, (j % 2) * D

    def lp_chunk(lp_v, c, m):
        nr = NSEG * PRE // 4
        x = [_gated_rows(xpre_v[n * nr + c * 16:n * nr + (c + 1) * 16, :], m) for n in range(4)]

        def store(r, p, w):
            lp_v.at[r][c * 8:(c + 1) * 8, p * D:(p + 1) * D] = w
        _lhs233([x[0], x[2]], [x[1], x[3]], store)

    def b_pre(lp_v, tick):
        nr = NSEG * PRE // 4
        with _scope("b_pre"):
            for g in range(HP // PG):
                hps = range(g * PG, (g + 1) * PG)
                slabs = {}
                for hp in hps:
                    for t in range(3):
                        s0, s1 = wb_v[t, 0, hp], wb_v[t, 1, hp]
                        slabs[hp, t] = (s0, s1)
                        ev = (s0 & u32(0xFFFF)) | (s1 << 16)
                        od = (s0 >> 16) | (s1 & u32(0xFFFF0000))
                        a, b = (KM + HD) // 2, (KM + 2 * HD) // 2
                        d12 = _words(_lo(s0[a:b]) - _hi(s0[a:b]), _lo(s1[a:b]) - _hi(s1[a:b]))
                        d21 = _words(_hi(s0[b:]) - _lo(s0[b:]), _hi(s1[b:]) - _lo(s1[b:]))
                        wb_v[t, 0, hp] = jnp.concatenate([ev[:a], d12, ev[b:]], axis=0)
                        wb_v[t, 1, hp] = jnp.concatenate([od[:a], d21, od[a:b]], axis=0)
                rhs = [_rhs233([slabs[hp, t] for t in range(3)]) for hp in hps]

                def product(r):
                    ws = [x for f in rhs for x in f(r)]
                    res = []
                    for w in ws:
                        wa, wb, wc = _passes(w)
                        c = jnp.dot(_unpack(lp_v[r, :, 2 * D:3 * D]), _unpack(wc), preferred_element_type=f32)
                        a = jnp.dot(_unpack(lp_v[r, :, 0:D]), _unpack(wa), preferred_element_type=f32)
                        b = jnp.dot(_unpack(lp_v[r, :, D:2 * D]), _unpack(wb), preferred_element_type=f32)
                        res.append((a + c, b + c))
                    tick(c)
                    return [jnp.concatenate([x[y] for x in res], axis=1) for y in range(2)]
                for (i, t), blk in _mm233(product):
                    for y in range(2):
                        x0 = (2 * i + y) * nr
                        for n, hp in enumerate(hps):
                            two = [blk[y][:, (2 * n + e) * D:(2 * n + e + 1) * D] for e in range(2)]
                            if t == 0:
                                two = [z * QSCALE for z in two]
                            two = [z.reshape(nr // PRE, 1, PRE, D) for z in two]
                            two = jnp.concatenate(two, axis=1).reshape(2 * nr, D)
                            ref, r0, l0 = pre_ref(hp * 3 + t)
                            ref[r0 + x0:r0 + x0 + nr, l0:l0 + D] = _pack(two.astype(bf16))

    def phase_a(woa_v, xbt_v, wobt_v, lp_v, s_v):
        woa_cp = pltpu.make_async_copy(woa_hbm.bitcast(u32), woa_v, sem.at[SEM_WOA])
        xbt_cp = pltpu.make_async_copy(xbt_hbm, xbt_v, sem.at[SEM_XBT])
        mem_cp = pltpu.make_async_copy(mem0_hbm, mem_v.at[0:MEM, :], sem.at[SEM_MEM])
        wob_cp = pltpu.make_async_copy(wob_hbm.bitcast(u32), wobt_v, sem.at[SEM_WOB])

        def first_scores(j):
            hq, pw = TQ // 2, S // 2
            q = _unpack(q_v[0, S // 2 - hq:S // 2, 0:D])
            k = _unpack(kv_v[0, j * pw // 2:(j + 1) * pw // 2, 0:D])
            s_v[:, j * pw:(j + 1) * pw] = jax.lax.dot_general(q, k, NT, preferred_element_type=f32)

        def projections(ckv_v, xat_v, wuk_v, wuv_v, wqa_v, lq_v, st_v):
            UR = 2 * D
            NU = S // UR
            QR = UR // 4
            kh = DC // 2
            NG = H // 4

            batches = [(0, 1), (2, 4), (4, 8), (8, 12), (12, 16), (1, 2)]

            def batch_start(n):
                for hp in range(*batches[n]):
                    for w_hbm, dst in ((wuk_hbm, wuk_v), (wuv_hbm, wuv_v)):
                        for par in range(2):
                            w_copy(w_hbm, dst, SEM_W + n, par, hp).start()

            def batch_wait(npairs, slot):
                part = wuk_v.at[:, 0:2 * npairs]
                pltpu.make_async_copy(part, part, sem.at[SEM_W + slot]).wait()

            pieces = [(0, 1), (1, 2), (2, 4), (4, 6), (6, 8)]

            def ckv_cp(j):
                rows = slice(pieces[j][0] * UR, pieces[j][1] * UR)
                return pltpu.make_async_copy(ckv_hbm.at[rows, :], ckv_v.at[rows, :], sem.at[SEM_CKV + j])
            xat_cp = pltpu.make_async_copy(xat_hbm, xat_v, sem.at[SEM_XAT])

            with _scope("a_issue0"):
                ckv_cp(0).start()
                batch_start(0)
                ckv_cp(1).start()
                batch_start(5)
                for j in range(2, 5):
                    ckv_cp(j).start()
                for n in range(1, 5):
                    batch_start(n)

            slot_of = {}
            for r in range(26):
                if _plain(_A424_ROWS, r) is None:
                    slot_of[r] = len(slot_of)

            def la_ref(n):
                return q_v.at[3 + n // 4], (n % 4) * (S // 8)

            def t_ref(n):
                return q_v.at[9 + n // 8], (n % 8) * (kh // 2)

            def t_get(n):
                ref, r0 = t_ref(n)
                return ref[r0:r0 + kh // 2, :]

            def lhs_prep(u):
                for c0 in range(0, QR, CL):
                    def block(v):
                        r0 = u * UR + v // 2 * QR + c0
                        return ckv_v[r0:r0 + CL, v % 2 * kh:(v % 2 + 1) * kh].astype(f32)
                    for r, o in _operands(block, _A424_TEMPS, _A424_ROWS, slot_of).items():
                        ref, r0 = la_ref(slot_of[r])
                        p0 = r0 + (u * QR + c0) // 2
                        ref[p0:p0 + CL // 2, :] = _pack(o.astype(bf16))

            def lhs(r, u0, u1):
                v = _plain(_A424_ROWS, r)
                if v is None:
                    ref, r0 = la_ref(slot_of[r])
                    return _unpack(ref[r0 + u0 * QR // 2:r0 + u1 * QR // 2, :])
                i, k = v // 2, v % 2
                return jnp.concatenate([ckv_v[u * UR + i * QR:u * UR + (i + 1) * QR, k * kh:(k + 1) * kh]
                                        for u in range(u0, u1)], axis=0)

            def put_chunk(g, par, c, m, sub=range(26), es=(0, 1)):
                zero = None if m is None else _gate(m)
                n = kh // 2
                for e in es:
                    w_v = (wuk_v, wuv_v)[e]
                    raw = {}

                    def words(p, v):
                        if (p, v // 2) not in raw:
                            w = w_v[p, 2 * g + v // 2 % 2, v // 4 * n + c * CR:v // 4 * n + (c + 1) * CR, :]
                            raw[p, v // 2] = w if zero is None else w | zero
                        return raw[p, v // 2]
                    sums = [r for r in sub if _plain(_B424_ROWS, r) is None]
                    ops = [_operands(lambda v: (_hi if v % 2 else _lo)(words(p, v)), _B424_TEMPS, _B424_ROWS, sums)
                           for p in range(2)]
                    for r in sub:
                        v = _plain(_B424_ROWS, r)
                        if v is None:
                            w = _words(ops[0][r], ops[1][r])
                        elif v % 2 == 0:
                            w = (words(0, v) & u32(0xFFFF)) | (words(1, v) << 16)
                        else:
                            w = (words(0, v) >> 16) | (words(1, v) & u32(0xFFFF0000))
                        ref, r0 = t_ref(26 * par + r)
                        ref[r0 + c * CR:r0 + (c + 1) * CR, e * D:(e + 1) * D] = w

            def project_kv(par, g, u0, u1, hooks=None, pre=None, post=None):
                def product(r):
                    if pre and r in pre:
                        pre[r]()
                    m = jnp.dot(lhs(r, u0, u1), _unpack(t_get(26 * par + r)), preferred_element_type=f32)
                    if post and r in post:
                        post[r](m)
                    if hooks:
                        for c, e in hooks[1].get(r, ()):
                            put_chunk(hooks[0], 1 - par, c, m, es=(e,))
                    return m

                def store(i, j, blk):
                    for u in range(u0, u1):
                        p0 = (u * UR + i * QR) // 2
                        kv_v.at[4 * g + j][p0:p0 + QR // 2, :] = _pack(blk[(u - u0) * QR:(u - u0 + 1) * QR, :].astype(bf16))
                _mm424(product, store)

            def put_rhs(g, par, which):
                for c in range(kh // 2 // CR):
                    put_chunk(g, par, c, None, which)

            def hook_plan(npiece):
                items = [(c, e) for c in range(kh // 2 // CR) for e in range(2)]
                plan = [{} for _ in range(npiece)]
                for n, item in enumerate(items):
                    sl = n * (npiece * 26 - HT) // len(items)
                    plan[sl // 26].setdefault(sl % 26, []).append(item)
                return plan

            def project_group(par, g, nxt):
                plan = hook_plan(NU // KU)
                for u in range(0, NU, KU):
                    project_kv(par, g, u, u + KU, (nxt, plan[u // KU]))

            def kv_first():
                ckv_cp(0).wait()
                lhs_prep(0)
                batch_wait(1, 0)
                put_rhs(0, 0, range(0, 2))
                put_rhs(0, 0, range(2, 7))
                ckv_cp(1).wait()
                lhs_prep(1)

                def rest():
                    batch_wait(1, 5)
                    for a, b in ((7, 9), (9, 14), (14, 20), (20, 26)):
                        put_rhs(0, 0, range(a, b))
                project_kv(0, 0, 0, 2, pre={7: rest})
                ckv_cp(2).wait()
                lhs_prep(2)
                lhs_prep(3)
                ckv_cp(3).wait()
                lhs_prep(4)
                lhs_prep(5)
                project_kv(0, 0, 2, 4)
                ckv_cp(4).wait()
                batch_wait(2, 1)
                lhs_prep(6)
                lhs_prep(7)
                plan = hook_plan(2)
                for u in range(4, 8, 2):
                    project_kv(0, 0, u, u + 2, (1, plan[(u - 4) // 2]))

            def kv_body(j, c):
                @pl.when(j == 0)
                def _():
                    xat_cp.start()
                    w_start_shared(wqa_hbm, wqa_v, 0, range(HP))
                    xbt_cp.start()
                batch_wait(4, 2 + j)
                project_group(1, 2 * j + 1, 2 * j + 2)
                project_group(0, 2 * j + 2, 2 * j + 3)
                return c

            with _scope("a_kvproj"):
                kv_first()
                jax.lax.fori_loop(0, NG // 2 - 1, kv_body, 0)

            woa_cp.start()
            wob_cp.start()
            mem_cp.start()
            w_start_shared(wqb_hbm, wb_v.at[0], 1, range(HP))
            w_start_shared(wkb_hbm, wb_v.at[1], 2, range(HP // 2))

            QB = 4 * D
            plain = {(0, 0): 15, (0, 1): 1, (0, 2): 9, (1, 0): 4, (1, 1): 16, (1, 2): 8}

            def xa_stage(b):
                for n in range(4):
                    xt = xat_v[:, (4 * b + n) * D:(4 * b + n + 1) * D]
                    st_v[n] = jnp.concatenate([xt, xt[DM - HD:]], axis=0).T

            def xa_chunk(b, c, m):
                x = [_gated_rows(st_v[n, c * 16:(c + 1) * 16, :], m) for n in range(4)]

                def store(r, p, w):
                    lq_v.at[r][b * HD + c * 8:b * HD + (c + 1) * 8, p * D:(p + 1) * D] = w
                _lhs233([x[0], x[2]], [x[1], x[3]], store, extra=(((0, 0, 1),), ((1, 1, 1),)))

            def q_store(blk, hp, x0):
                q_v.at[hp][x0 // 2:(x0 + blk.shape[0]) // 2, :] = _pack((blk * QSCALE).astype(bf16))

            def q_rhs(hp):
                f = _rhs233([(wqa_v[0, hp + n], wqa_v[1, hp + n]) for n in range(3)])
                return [_passes(jnp.concatenate(f(r), axis=1)) for r in range(15)]

            def project_q(t, hp, b):
                nr = D // QS
                for s in range(QS):
                    rows = slice(b * HD + s * nr // 2, b * HD + (s + 1) * nr // 2)

                    def product(r):
                        wa, wb, wc = t[r]
                        c = jnp.dot(_unpack(lq_v[r, rows, 2 * D:3 * D]), _unpack(wc), preferred_element_type=f32)
                        a = jnp.dot(_unpack(lq_v[r, rows, 0 * D:1 * D]), _unpack(wa), preferred_element_type=f32)
                        b = jnp.dot(_unpack(lq_v[r, rows, 1 * D:2 * D]), _unpack(wb), preferred_element_type=f32)
                        return [a + c, b + c]
                    for (i, j), blk in _mm233(product):
                        for y in range(2):
                            q_store(blk[y], hp + j, b * QB + (2 * i + y) * D + s * nr)

            def project_q_last(hp):
                s0, s1 = wqa_v[0, hp], wqa_v[1, hp]
                w = jnp.concatenate([(s0 & u32(0xFFFF)) | (s1 << 16), (s0 >> 16) | (s1 & u32(0xFFFF0000))], axis=1)
                per = [_passes(jnp.concatenate([w[a:a + 64], w[c:c + 32]] if k == 1 else [w[a:a + 96]], axis=0))
                       for k, (a, _, c) in enumerate(_PIECES)]
                wp = [_unpack(jnp.concatenate([per[k][p] for k in range(3)], axis=0)) for p in range(3)]
                for b in range(S // QB):
                    rows = slice(b * HD, (b + 1) * HD)
                    for i in range(2):
                        a, bb, c = [jnp.dot(_unpack(jnp.concatenate([lq_v[plain[i, k], rows, p * D:(p + 1) * D] for k in range(3)], axis=1)),
                                            wp[p], preferred_element_type=f32) for p in range(3)]
                        for p, m in enumerate((a, bb, c)):
                            n = (2 * b + i) * 3 + p
                            if n % 2 == 0 and n // 2 < D // 16:
                                lp_chunk(lp_v, n // 2, m)
                        q_store(a + c, hp, b * QB + 2 * i * D)
                        q_store(bb + c, hp, b * QB + (2 * i + 1) * D)

            def xb_prep(t):
                t0 = pl.multiple_of(t * D, D)
                xt = xbt_v[:, pl.ds(t0, D)]
                xb = jnp.concatenate([xt, xt[DM - HD:]], axis=0).T
                xb_v[pl.ds(t0, D), :] = xb
                for sg in range(D // SEG):
                    p0 = pl.multiple_of((t * (D // SEG) + sg) * PRE, PRE)
                    xpre_v[pl.ds(p0, PRE), :] = xb[sg * SEG:sg * SEG + PRE, :]

            with _scope("a_qproj"):
                xat_cp.wait()
                xbt_cp.wait()
                w_wait_shared(wqa_v, 0)
                t = q_rhs(0)
                xa_stage(0)
                for b in range(S // QB):
                    post = {3 * c: (lambda m, c=c: xa_chunk(b, c, m)) for c in range(D // 16)}
                    project_kv(1, NG - 1, KU * b, KU * (b + 1), post=post)
                    if b + 1 < S // QB:
                        xa_stage(b + 1)
                    project_q(t, 0, b)
                XG = 4

                def q_body(j, c):
                    hp = 3 * j
                    for n in range(XG):
                        xb_prep((j - 1) * XG + n)
                    t = q_rhs(hp)
                    for b in range(S // QB):
                        project_q(t, hp, b)
                    return c
                jax.lax.fori_loop(1, 5, q_body, 0)
                w_start_shared(wkb_hbm, wb_v.at[1], 2, range(HP // 2, HP))
                w_start_shared(wvb_hbm, wb_v.at[2], 3, range(HP))
                project_q_last(HP - 1)
                for j in range(2):
                    first_scores(j)

        pl.run_scoped(
            projections,
            pltpu.VMEM((S, DC), bf16),
            pltpu.VMEM((DM, S), bf16),
            pltpu.VMEM((2, HP, DC // 2, D), u32),
            pltpu.VMEM((2, HP, DC // 2, D), u32),
            pltpu.VMEM((2, HP, DM // 2, D), u32),
            pltpu.VMEM((17, S // 8, 3 * D), u32),
            pltpu.VMEM((4, D, DMP), bf16),
        )

        def attention(c_v):
            row = jax.lax.broadcasted_iota(jnp.int32, (TQ, TQ), 0)
            col = jax.lax.broadcasted_iota(jnp.int32, (TQ, TQ), 1)
            tri = col <= row
            nb = S // TQ
            hq = TQ // 2
            npiece = 2
            pw = S // npiece

            def q_rows(h, r0, r1):
                return q_v[h[0], r0:r1, h[1] * D:(h[1] + 1) * D]

            def head(h):
                return 2 * h[0] + h[1]

            def qk_piece(h, j):
                q = _unpack(q_rows(h, (nb - 1) * hq, nb * hq))
                k = _unpack(kv_v[head(h), j * pw // 2:(j + 1) * pw // 2, 0:D])
                s_v[:, j * pw:(j + 1) * pw] = jax.lax.dot_general(q, k, NT, preferred_element_type=f32)

            def qk(h, i, j0=0, j1=None):
                j1 = i + 1 if j1 is None else j1
                q = _unpack(q_rows(h, i * hq, (i + 1) * hq))
                k = _unpack(kv_v[head(h), j0 * hq:j1 * hq, 0:D])
                return jax.lax.dot_general(q, k, NT, preferred_element_type=f32)

            def pv_shared(p, hd, i):
                low = jax.lax.broadcasted_iota(jnp.int32, (1, TQ), 1) < HD
                qr = TQ // 4

                def mm(x, w):
                    return jnp.dot(x.astype(bf16), _unpack(w), preferred_element_type=f32)
                pa, pd = p[:, (i - 1) * TQ:i * TQ], p[:, i * TQ:]
                y1a, y2a, y1d, y2d = pa[0:qr], pa[qr:2 * qr], pd[0:qr], pd[qr:2 * qr]
                va = kv_v[hd, (i - 1) * hq:i * hq, D:2 * D]
                vd = kv_v[hd, i * hq:(i + 1) * hq, D:2 * D]
                la = jnp.where(low, y1a, y1a - y2a)
                lb = jnp.where(low, y2a, pltpu.roll(y2d - y1d, HD, 1))
                lc = jnp.where(low, y1d, y2a)
                o = None
                if i > 1:
                    o = mm(p[:, :(i - 1) * TQ], kv_v[hd, 0:(i - 1) * hq, D:2 * D])
                o2 = mm(jnp.concatenate([la, pa[2 * qr:]], axis=0), va)
                o3 = mm(pd[2 * qr:], vd)
                ob = mm(lb, jnp.concatenate([va[0:qr], vd[0:qr]], axis=0))
                oc = mm(lc, jnp.concatenate([vd[0:qr], va[qr:]], axis=0))
                r = jnp.concatenate([o2[0:qr] + oc, ob + oc, o2[qr:] + o3], axis=0)
                return r if o is None else o + r

            def anchor_plan():
                ops = []
                for e in range(UH):
                    for i in range(nb - 1, -1, -1):
                        if i > 0:
                            ops.append(("qk", e, i - 1, 32 * i))
                        if i < npiece:
                            ops.append(("piece", e, i, 32 * nb // npiece))
                        ops.append(("pv", e, i, 32 * (i + 1)))
                t, start, end = 0, [], []
                for op in ops:
                    start.append(t)
                    t += op[3]
                    end.append(t)
                plan = {}
                for a, op in enumerate(ops):
                    if op[0] != "pv" or op[2] < ANCHOR_MIN:
                        continue
                    for b in range(a + 1, len(ops)):
                        if ops[b][0] == "qk" and start[b] >= end[a] + ANCHOR_LAG:
                            plan.setdefault((ops[b][1], ops[b][2]), []).append((op[1], op[2]))
                            break
                return plan

            def heads(j, c):

                plan = anchor_plan()


                def gated_qk(e, i):
                    h = (j * (UH // 2) + e // 2, e % 2)
                    if (e, i) not in plan:
                        return qk(h, i)
                    w = None
                    for ea, ia in plan[e, i]:
                        u = c_v[j * (UH // 2) + ea // 2, ia * hq:(ia + 1) * hq, (ea % 2) * D:(ea % 2 + 1) * D]
                        for r in range(0, hq, 8):
                            w = u[r:r + 8] if w is None else w | u[r:r + 8]
                    zero = (w >> 31) >> 1
                    q = q_rows(h, i * hq, (i + 1) * hq)
                    q = _unpack(jnp.concatenate([q[0:8] | zero, q[8:]], axis=0))
                    k = _unpack(kv_v[head(h), 0:(i + 1) * hq, 0:D])
                    return jax.lax.dot_general(q, k, NT, preferred_element_type=f32)

                s_next = s_v[...]
                for e in range(UH):
                    h = (j * (UH // 2) + e // 2, e % 2)
                    if e == UH - 1:
                        hn = (jnp.minimum(h[0] + 1, HP - 1), 0)
                    else:
                        hn = (j * (UH // 2) + (e + 1) // 2, (e + 1) % 2)
                    pieces = []
                    for i in range(nb - 1, -1, -1):
                        s = s_next
                        if i > 0:
                            s_next = gated_qk(e, i - 1)
                        if i < npiece:
                            if e == UH - 1:
                                qk_piece(hn, npiece - 1 - i)
                            else:
                                jj = npiece - 1 - i
                                pieces.append(qk(hn, nb - 1, jj * nb // npiece, (jj + 1) * nb // npiece))
                        sd = jnp.where(tri, s[:, i * TQ:], NEG)
                        s = jnp.concatenate([s[:, :i * TQ], sd], axis=1) if i > 0 else sd
                        m = jnp.max(s, axis=1, keepdims=True)
                        p = jnp.exp2(s - m)
                        l = jnp.sum(p, axis=1, keepdims=True)
                        if i < PVT:
                            v = _unpack(kv_v[head(h), 0:(i + 1) * hq, D:2 * D])
                            o = jnp.dot(p.astype(bf16), v, preferred_element_type=f32)
                        else:
                            o = pv_shared(p, head(h), i)
                        c_v.at[h[0]][i * hq:(i + 1) * hq, h[1] * D:(h[1] + 1) * D] = _pack((o * _recip(l)).astype(bf16))
                    if e < UH - 1:
                        s_next = jnp.concatenate(pieces, axis=1)
                return c
            with _scope("a_attn"):
                jax.lax.fori_loop(0, H // UH, heads, 0)

            woa_cp.wait()
            wob_cp.wait()
            mem_cp.wait()
            for t in range(3):
                w_wait_shared(wb_v.at[t], 1 + t)
            mh = DM // 4
            slot = {0: 0, 1: 1, 4: 2, 5: 3, 6: 4}

            def wo_prep(hh):
                a11, a21 = woa_v[hh, 0:mh, :], woa_v[hh, mh:2 * mh, :]
                a12, a22 = woa_v[hh + HP, 0:mh, :], woa_v[hh + HP, mh:2 * mh, :]
                for i, w in enumerate(_sum_words(_strassen_lhs, a11, a12, a21, a22, (2, 3), (a11, a22))):
                    if i in slot:
                        kv_v[hh, slot[i] * mh:(slot[i] + 1) * mh, 0:D] = w

            def wob_prep(hp, m):
                w1, w2 = [_unpack((wobt_v[2 * hp + e].reshape(DM // 16, 8, D) | _gate(m)).reshape(DM // 2, D))
                          for e in range(2)]
                a, b = KM + HD, KM + 2 * HD
                d12 = (w1[a:b].astype(f32) - w2[a:b].astype(f32)).astype(bf16)
                d21 = (w2[b:].astype(f32) - w1[b:].astype(f32)).astype(bf16)
                rows = slice(hp * HD, (hp + 1) * HD)
                wob_v[0, rows, :] = _pack(jnp.concatenate([w1[:a], d12], axis=0).T)
                wob_v[1, rows, :] = _pack(jnp.concatenate([w2[:a], d21], axis=0).T)
                wos_v[rows, :] = _pack(jnp.concatenate([w1[b:], w2[a:b]], axis=0).T)

            def oproj(tp):
                w0 = tp * D
                per = []
                for hh in range(HP):
                    def ctx(h, r0):
                        return c_v[h // 2, r0:r0 + D // 2, (h % 2) * D:(h % 2 + 1) * D]
                    b11, b21 = ctx(hh, w0), ctx(hh + HP, w0)
                    b12, b22 = ctx(hh, w0 + D // 2), ctx(hh + HP, w0 + D // 2)
                    per.append(_sum_words(_strassen_rhs, b11, b12, b21, b22, (1, 4), (b11, b22)))

                def lhs(i, s):
                    hhs = range(s * HP // KS, (s + 1) * HP // KS)
                    if i == 2:
                        return _unpack(jnp.concatenate([woa_v[hh, 0:mh, :] for hh in hhs], axis=1))
                    if i == 3:
                        return _unpack(jnp.concatenate([woa_v[hh + HP, mh:2 * mh, :] for hh in hhs], axis=1))
                    return _unpack(jnp.concatenate([kv_v[hh, slot[i] * mh:(slot[i] + 1) * mh, 0:D] for hh in hhs], axis=1))

                def rhs(i, s):
                    return _unpack(jnp.concatenate([per[hh][i] for hh in range(s * HP // KS, (s + 1) * HP // KS)], axis=1))

                def done(c11, c12, c21, c22):
                    t0 = 2 * tp * D
                    out_v[t0:t0 + D, 0:DM] = jnp.concatenate([c11, c21], axis=0).T.astype(bf16)
                    out_v[t0 + D:t0 + 2 * D, 0:DM] = jnp.concatenate([c12, c22], axis=0).T.astype(bf16)
                yield from _strassen(lhs, rhs, NT, done, 1 if tp == 0 else 0)

            def outputs():
                for hh in range(HP):
                    wo_prep(hh)
                for tp in range(S // D // 2):
                    yield from oproj(tp)

            steps, na, nb_ = outputs(), KS * 7 * (S // D // 2), 15 * HP // PG
            count = [0, 0]

            def tick(m):
                count[0] += 1
                if count[0] % 15 == 1:
                    wob_prep(count[0] // 15, m)
                while count[1] < na and I0 + count[1] * (nb_ - I0 - I1) // na <= count[0]:
                    next(steps)
                    count[1] += 1
            with _scope("post"):
                b_pre(lp_v, tick)
                for _ in steps:
                    pass

        pl.run_scoped(
            attention,
            pltpu.VMEM((HP, S // 2, 2 * D), u32),
        )

    pl.run_scoped(
        phase_a,
        pltpu.VMEM((H, DM // 2, D), u32),
        pltpu.VMEM((DM, S), bf16),
        pltpu.VMEM((H, DM // 2, D), u32),
        pltpu.VMEM((15, NSEG * PRE // 8, 3 * D), u32),
        pltpu.VMEM((TQ, S), f32),
    )

    def out_copy(j):
        rows = pl.ds(pl.multiple_of(j * (OUTER * SEG), OUTER * SEG), OUTER * SEG)
        return pltpu.make_async_copy(out_v.at[rows, :], out_hbm.at[rows, :], sem.at[SEM_OUT + j])

    def phase_b(post_v):
        GP = HG // 2
        GC = GP * 3 * D
        KA = KM + 2 * HD
        lane = jax.lax.broadcasted_iota(jnp.int32, (1, GC), 1)
        colscale = jnp.where(lane % (3 * D) < D, QSCALE, 1.0).astype(f32)
        low = jax.lax.broadcasted_iota(jnp.int32, (1, D), 1) < HD

        def swap(x):
            return pltpu.roll(x, HD, 1)

        def wgroup(g):
            cols = [(hp, t) for hp in range(g * GP, (g + 1) * GP) for t in range(3)]
            own = [_unpack(jnp.concatenate([wb_v[t, e, hp, 0:KA // 2, :] for hp, t in cols], axis=1)) for e in range(2)]
            both = jnp.concatenate([jnp.concatenate([wb_v[t, e, hp, KA // 2:, :] for hp, t in cols], axis=1)
                                    for e in range(2)], axis=0)
            return own[0], own[1], _unpack(both)

        def out_project(even, odd, both, p0, p1):
            rows = slice(p0 * HD, p1 * HD)
            return [jnp.dot(even, _unpack(wob_v[0, rows, :]), preferred_element_type=f32),
                    jnp.dot(odd, _unpack(wob_v[1, rows, :]), preferred_element_type=f32),
                    jnp.dot(both, _unpack(wos_v[rows, :]), preferred_element_type=f32)]

        def out_add(acc, part):
            e, o, b = part
            new = [e[:, :KM] + o[:, :KM], e[:, KM:], o[:, KM:], b]
            return new if acc is None else [x + y for x, y in zip(acc, new)]

        def out_finish(acc):
            main, e, o, b = acc
            mid = e + jnp.where(low, o, b)
            last = jnp.where(low, swap(o) + b, o + swap(b))
            return jnp.concatenate([main, mid, last], axis=1)

        ri = jax.lax.broadcasted_iota(jnp.int32, (2 * L, 2 * L), 0)
        ci = jax.lax.broadcasted_iota(jnp.int32, (2 * L, 2 * L), 1)

        def second(i):
            return jnp.where(i < 2 * SEG, i // SEG, (i - 2 * SEG) // PRE)

        def pos(i):
            j = i % SEG
            return jnp.where(i < 2 * SEG, jnp.where(j < T, j + (MEM + PRE), j - T), MEM + i % PRE)
        same = second(ri) == second(ci)
        mask = same & ((pos(ri) < MEM) | (pos(ri) >= pos(ci)))
        fill = jnp.where(same, NEG, -jnp.inf).astype(f32)

        def step(s, slot, mem):
            xt = xb_v[pl.ds(pl.multiple_of(SEG * s + PRE, 8), T), :]
            l1 = jnp.concatenate([xt.astype(f32), mem], axis=0)
            mid, last = l1[:, KM:KA], l1[:, KA:]
            l_even = l1[:, :KA].astype(bf16)
            l_odd = jnp.concatenate([l1[:, :KM], jnp.where(low, mid, last)], axis=1).astype(bf16)
            l_both = jnp.where(low, last, mid).astype(bf16)
            p0 = pl.multiple_of(PRE * s, 8)
            proj = []
            for g in range(G):
                w_even, w_odd, w_both = wgroup(g)
                both = jnp.dot(l_both, w_both, preferred_element_type=f32)
                even = jnp.dot(l_even, w_even, preferred_element_type=f32)
                odd = jnp.dot(l_odd, w_odd, preferred_element_type=f32)
                proj.append([(x + both) * colscale for x in (even, odd)])

            def rows(hp, t):
                g, c0 = hp // GP, (hp % GP) * 3 * D + t * D
                ref, r0, l0 = pre_ref(hp * 3 + t)
                return jnp.concatenate([proj[g][0][:, c0:c0 + D], proj[g][1][:, c0:c0 + D],
                                        _unpack(ref[pl.ds(r0 + p0, PRE), l0:l0 + D]).astype(f32)], axis=0).astype(bf16)

            scores = [jax.lax.dot_general(rows(hp, 0), rows(hp, 1), NT, preferred_element_type=f32)
                      for hp in range(HP)]
            ctx = {}
            tails = []

            def attend(g):
                for hp in range(g * HG // 2, (g + 1) * HG // 2):
                    sc = jnp.where(mask, scores[hp], fill)
                    m = jnp.max(sc, axis=1, keepdims=True)
                    p = jnp.exp2(sc - m)
                    l = jnp.sum(p, axis=1, keepdims=True)
                    o = jnp.dot(p.astype(bf16), rows(hp, 2), preferred_element_type=f32) * _recip(l)
                    ctx[hp] = [o[0:SEG, :], o[SEG:2 * SEG, :], o[0:SEG, :] + o[SEG:2 * SEG, :]]
                    for e in range(2):
                        post_v[e, slot * PRE:(slot + 1) * PRE, hp * D:(hp + 1) * D] = o[2 * SEG + e * PRE:2 * SEG + (e + 1) * PRE, :]
                        tails.append(o[2 * SEG + e * PRE:2 * SEG + (e + 1) * PRE, :])

            parts = []

            def oproj(g):
                lhs = [jnp.concatenate([ctx[hp][e] for hp in range(g * GP, (g + 1) * GP)], axis=1).astype(bf16)
                       for e in range(3)]
                parts.append(out_project(*lhs, g * GP, (g + 1) * GP))

            for t in range(G + 2):
                if t < G:
                    attend(t)
                if t >= 2:
                    oproj(t - 2)
            acc = None
            for a in parts:
                acc = out_add(acc, a)
            accb = out_finish(acc).astype(bf16)
            out_v[pl.ds(pl.multiple_of(SEG * s + PRE, 8), T), DM:2 * DM] = accb[0:T, 0:DM]
            late = pltpu.bitcast(ctx[HP - 1][1][0:8], u32)
            for x in tails:
                late = late | pltpu.bitcast(x, u32)
            return accb[T:, :].astype(f32), late

        PP = HP // OUTER

        def deferred_rows():
            even, odd = post_v[0], post_v[1]
            return even, odd, even + odd

        def finish(j, acc):
            r = out_finish(acc).astype(bf16)
            for sg in range(OUTER):
                r0 = pl.multiple_of((j * OUTER + sg) * SEG, SEG)
                out_v[pl.ds(r0, PRE), DM:2 * DM] = r[sg * PRE:(sg + 1) * PRE, 0:DM]

        def after(x, late):
            u = late
            zero = (u >> 31) & (~u >> 31)
            top = pltpu.bitcast(x[0:8], u32) | jnp.concatenate([zero] * (x.shape[1] // D), axis=1)
            return jnp.concatenate([pltpu.bitcast(top, f32), x[8:]], axis=0).astype(bf16)

        def outer(j, c):
            mem, done = c
            finish(jnp.maximum(j - 2, 0), done)
            prev = deferred_rows()

            def partial(i, late):
                x = [after(p[:, i * PP * D:(i + 1) * PP * D], late) for p in prev]
                return out_project(*x, i * PP, (i + 1) * PP)
            acc = None
            for i in range(OUTER):
                mem, late = step(j * OUTER + i, i, mem)
                acc = out_add(acc, partial(i, late))

            @pl.when(j >= 2)
            def _():
                out_copy(j - 2).start()
            return mem, acc
        with _scope("b_loop"):
            post_v[...] = jnp.zeros(post_v.shape, f32)
            mem0 = mem_v[0:MEM, :].astype(f32)
            zeros = [jnp.zeros((OUTER * PRE, n), f32) for n in (KM, D, D, D)]
            _, done = jax.lax.fori_loop(0, NOUTER, outer,
                                        (jnp.concatenate([mem0, mem0[:, DM - HD:]], axis=1), zeros))
            finish(NOUTER - 2, done)
            out_copy(NOUTER - 2).start()
            out_copy(0).wait()
            finish(NOUTER - 1, out_add(None, out_project(*[x.astype(bf16) for x in deferred_rows()], 0, HP)))
            out_copy(NOUTER - 1).start()
        with _scope("b_outwait"):
            for j in range(1, NOUTER):
                out_copy(j).wait()

    pl.run_scoped(
        phase_b,
        pltpu.VMEM((2, OUTER * PRE, HP * D), f32),
    )


@jax.jit
def pallas_concat_heads__compressed_kv_cla__memory_aug_recurrent_mem_tr__prompt_kernel(
    A_x: jax.Array,
    A_c_kv: jax.Array,
    A_w_q: jax.Array,
    A_w_uk: jax.Array,
    A_w_uv: jax.Array,
    A_w_o: jax.Array,
    B_x: jax.Array,
    B_mem0: jax.Array,
    B_Wq: jax.Array,
    B_Wk: jax.Array,
    B_Wv: jax.Array,
    B_Wo: jax.Array,
    B_seg_len=SEG,
):
    def t2(x):
        return jnp.transpose(x, (0, 2, 1)).reshape(DM, S)

    def w3(w):
        return w.reshape(w.shape[0] // 2, 2 * H, D)

    def wo3(w):
        return jnp.transpose(w, (0, 2, 1))

    any_spec = pl.BlockSpec(memory_space=pl.ANY)
    out = pl.pallas_call(
        _kernel,
        out_shape=jax.ShapeDtypeStruct((S, 2 * DM), bf16),
        in_specs=[any_spec] * 12,
        out_specs=any_spec,
        scratch_shapes=[
            pltpu.VMEM((S, 2 * DM), bf16),
            pltpu.VMEM((S, DMP), bf16),
            pltpu.VMEM((NSEG * PRE, DMP), bf16),
            pltpu.VMEM((3, 2, HP, DM // 2, D), u32),
            pltpu.VMEM((2, HP * D // 2, KM + 2 * HD), u32),
            pltpu.VMEM((HP * D // 2, D), u32),
            pltpu.VMEM((8 * MEM, DM), bf16),
            pltpu.VMEM((HP, S // 2, 2 * D), u32),
            pltpu.VMEM((H, S // 2, 2 * D), u32),
            pltpu.SemaphoreType.DMA((NSEM,)),
        ],
        compiler_params=pltpu.CompilerParams(vmem_limit_bytes=126 * 1024 * 1024),
    )(t2(A_x), A_c_kv.reshape(S, DC), w3(A_w_q), w3(A_w_uk), w3(A_w_uv), wo3(A_w_o),
      t2(B_x), B_mem0.reshape(MEM, DM), w3(B_Wq), w3(B_Wk), w3(B_Wv), wo3(B_Wo))
    return out.reshape(1, S, 2 * DM)
```
